```python
import jax
import jax.numpy as jnp

def _softmax(x, axis=-1):
    return jax.nn.softmax(x, axis=axis)

def _gelu(x):
    return jax.nn.gelu(x, approximate=True)

def _silu(x):
    return jax.nn.silu(x)

def _sigmoid(x):
    return jax.nn.sigmoid(x)

def _layernorm(x, axis=-1, eps=1e-05):
    m = jnp.mean(x, axis=axis, keepdims=True)
    v = jnp.var(x, axis=axis, keepdims=True)
    return (x - m) / jnp.sqrt(v + eps)

def _scatter_add(tgt, idx, src, axis=0):
    return tgt.at[idx].add(src)

def _segment_sum(src, seg, n):
    return jax.ops.segment_sum(src, seg, n)

class _Rng:

    def __init__(self, key):
        self._k = key

    def _next(self):
        self._k, sub = jax.random.split(self._k)
        return sub

    def normal(self, shape):
        return jax.random.normal(self._next(), shape, dtype=jnp.bfloat16)

    def randint(self, lo, hi, shape):
        return jax.random.randint(self._next(), shape, lo, hi, dtype=jnp.int32)

    def uniform(self, shape, lo=0.0, hi=1.0):
        return jax.random.uniform(self._next(), shape, jnp.bfloat16, lo, hi)

    def permutation(self, n):
        return jax.random.permutation(self._next(), n)
kernel_name = 'adaLN_cond__memory_aug_recurrent_mem_tr__glu_gated_swiglu__prompt'

def setup_inputs():
    _rng = _Rng(jax.random.key(int.from_bytes(__import__("os").urandom(4), "little")))
    _w = lambda a: (lambda t: t.astype(jnp.bfloat16) if jnp.issubdtype(t.dtype, jnp.floating) else t)(jnp.asarray(a))

    def _A_setup():
        B, S, Dm = (1, 2048, 1024)
        H, Dh = (32, 128)
        M, seg = (8, 32)
        seg = min(seg, S)
        S = S // seg * seg
        return {'x': _w((lambda *s: _rng.normal(s) * 0.05)(B, S, Dm)), 'mem0': _w((lambda *s: _rng.normal(s) * 0.05)(B, M, Dm)), 'Wq': _w((lambda *s: _rng.normal(s) * 0.05)(Dm, H, Dh) * Dm ** (-0.5)), 'Wk': _w((lambda *s: _rng.normal(s) * 0.05)(Dm, H, Dh) * Dm ** (-0.5)), 'Wv': _w((lambda *s: _rng.normal(s) * 0.05)(Dm, H, Dh) * Dm ** (-0.5)), 'Wo': _w((lambda *s: _rng.normal(s) * 0.05)(H, Dh, Dm) * (H * Dh) ** (-0.5)), 'seg_len': seg}
    _A_in = _A_setup()

    def _B_setup():
        B, S, D, F = (1, 2048, 1024, 3584)
        return {'x': _w((lambda *s: _rng.normal(s) * 0.05)(B, S, D)), 'w1': _w((lambda *s: _rng.normal(s) * 0.05)(D, F) * (2.0 / D) ** 0.5), 'w3': _w((lambda *s: _rng.normal(s) * 0.05)(D, F) * (2.0 / D) ** 0.5), 'w2': _w((lambda *s: _rng.normal(s) * 0.05)(F, D) * (2.0 / F) ** 0.5)}
    _B_in = _B_setup()
    return {'A_x': _A_in['x'], 'A_mem0': _A_in['mem0'], 'A_Wq': _A_in['Wq'], 'A_Wk': _A_in['Wk'], 'A_Wv': _A_in['Wv'], 'A_Wo': _A_in['Wo'], 'A_seg_len': _A_in['seg_len'], 'B_x': _B_in['x'], 'B_w1': _B_in['w1'], 'B_w3': _B_in['w3'], 'B_w2': _B_in['w2'], 'c': _w((lambda *s: _rng.normal(s) * 0.05)(1, 1024)), 'w_mod': _w((lambda *s: _rng.normal(s) * 0.05)(1024, 6 * 1024) * 1024 ** (-0.5))}

def reference(A_x, A_mem0, A_Wq, A_Wk, A_Wv, A_Wo, A_seg_len, B_x, B_w1, B_w3, B_w2, c, w_mod):

    def _A_ref(x, mem0, Wq, Wk, Wv, Wo, seg_len):
        B, S, Dm = x.shape
        H, Dh = (Wq.shape[1], Wq.shape[2])
        M = mem0.shape[1]
        scale = Dh ** (-0.5)
        n_seg = S // seg_len
        L = M + seg_len
        idx = jnp.arange(L)
        mask = (idx[:, None] < M) | (idx[:, None] >= idx[None, :])
        mem = mem0
        outs = []
        for s in range(n_seg):
            xs = x[:, s * seg_len:(s + 1) * seg_len, :].copy()
            h = jnp.concatenate([mem, xs], axis=1)
            q = jnp.einsum('btd,dhe->bhte', h, Wq)
            k = jnp.einsum('btd,dhe->bhte', h, Wk)
            v = jnp.einsum('btd,dhe->bhte', h, Wv)
            scores = jnp.einsum('bhqe,bhke->bhqk', q, k) * scale
            scores = jnp.where(mask[None, None], scores, -1000000000.0)
            p = _softmax(scores, axis=-1)
            o = jnp.einsum('bhqk,bhke->bhqe', p, v)
            o = jnp.einsum('bhte,hed->btd', o, Wo)
            mem = o[:, :M, :].copy()
            outs.append(o[:, M:, :])
        return jnp.concatenate(outs, axis=1)

    def _B_ref(x, w1, w3, w2):
        gate = jnp.einsum('bsd,df->bsf', x, w1)
        up = jnp.einsum('bsd,df->bsf', x, w3)
        h = _silu(gate) * up
        out = jnp.einsum('bsf,fd->bsd', h, w2)
        return out
    x = A_x
    mod = (_silu(c) @ w_mod).reshape(c.shape[0], 6, 1, -1)
    sa, ca, ga, sb, cb, gb = (mod[:, 0].copy(), mod[:, 1].copy(), mod[:, 2].copy(), mod[:, 3].copy(), mod[:, 4].copy(), mod[:, 5].copy())
    h = _layernorm(x, axis=-1) * (1 + ca) + sa
    x = x + ga * _A_ref(h, A_mem0, A_Wq, A_Wk, A_Wv, A_Wo, A_seg_len)
    h = _layernorm(x, axis=-1) * (1 + cb) + sb
    x = x + gb * _B_ref(h, B_w1, B_w3, B_w2)
    return x
```

```python
import functools
import math

import jax
import jax.numpy as jnp
from jax import lax
import jax.experimental.pallas as pl
import jax.experimental.pallas.tpu as pltpu

S, D, H, DH, MEM, SEG, F = 2048, 1024, 32, 128, 8, 32, 3584
NSEG = S // SEG
NP = H // 2
HD = H * DH
EARLY = 8
NEARLY = NSEG * EARLY
L2 = 2 * (MEM + SEG)
CH = 8
NCH = 3 * H // CH
TM = 128
NBLK = S // TM
SPB = TM // SEG
FC = 256
EPS = 1e-5
SCALE = DH ** -0.5
MASK_FILL = -1000000000.0

BF16, F32, U32 = jnp.bfloat16, jnp.float32, jnp.uint32


def _bf(x_u32):
    return pltpu.bitcast(x_u32, BF16)


def _pk(x_f32):
    return pltpu.bitcast(x_f32.astype(BF16), U32)


def _dot(a, b):
    return jnp.dot(a, b, preferred_element_type=F32)


def _ln_mod(x, shift, scale1):
    m = jnp.mean(x, axis=-1, keepdims=True)
    xc = x - m
    v = jnp.mean(xc * xc, axis=-1, keepdims=True)
    return xc * lax.rsqrt(v + EPS) * scale1 + shift


def _attn_mask():
    def meta(i):
        head = jnp.where(i < 2 * SEG, i // SEG, (i - 2 * SEG) // EARLY)
        j = i % SEG
        pos = jnp.where(i < 2 * SEG, jnp.where(j < MEM, j, j + EARLY), MEM + (i - 2 * SEG) % EARLY)
        return head, pos
    r = lax.broadcasted_iota(jnp.int32, (L2, L2), 0)
    c = lax.broadcasted_iota(jnp.int32, (L2, L2), 1)
    rh, rp = meta(r)
    chd, cp = meta(c)
    same = rh == chd
    keep = same & ((rp < MEM) | (rp >= cp))
    fill = jnp.where(same, MASK_FILL / SCALE, -jnp.inf).astype(F32)
    return keep, fill


def _kernel(x_hbm, m0_hbm, wq_hbm, wk_hbm, wv_hbm, wo_hbm, w1_hbm, w3_hbm, w2_hbm, c_hbm, wm_hbm,
            out_hbm,
            wqkv, wo, w1, w3, w2, wm, xb, cb, m0, mod, p32, pre, l32, ob, odef, a32,
            h2, act, ost, keep_s, fill_s, sem, wsem, osem):
    w_hbm = [r.bitcast(U32) for r in (wq_hbm, wk_hbm, wv_hbm)]
    wm_u = wm_hbm.bitcast(U32)

    def chunk_copies(t):
        m, c0 = divmod(t, H // CH)
        cps = []
        for jj in range(CH // 2):
            j = c0 * (CH // 2) + jj
            for par in range(2):
                cps.append(pltpu.make_async_copy(
                    w_hbm[m].at[:, par * NP + j, :], wqkv.at[m * H + 2 * j + par], wsem.at[t]))
        return cps

    def wait_chunk(t):
        blk = wqkv.at[pl.ds(t * CH, CH)]
        pltpu.make_async_copy(blk, blk, wsem.at[t]).wait()

    def unzip(slot):
        for r in range(0, D // 2, 32):
            e, o = wqkv[slot, r:r + 32, :], wqkv[slot + 1, r:r + 32, :]
            wqkv[slot, r:r + 32, :] = (e & 0xFFFF) | (o << 16)
            wqkv[slot + 1, r:r + 32, :] = (e >> 16) | (o & jnp.uint32(0xFFFF0000))

    cp_c = pltpu.make_async_copy(c_hbm, cb, sem.at[0])
    cp_wm0 = pltpu.make_async_copy(wm_u.at[:, 0:2 * D], wm.at[:, 0:2 * D], sem.at[1])
    cp_xe = pltpu.make_async_copy(x_hbm.at[:, 0:EARLY, :], xb.at[:, 0:EARLY, :], sem.at[2])
    cp_m0 = pltpu.make_async_copy(m0_hbm, m0, sem.at[3])
    cp_xr = pltpu.make_async_copy(x_hbm.at[:, EARLY:SEG, :], xb.at[:, EARLY:SEG, :], sem.at[4])
    cp_wo = pltpu.make_async_copy(wo_hbm.bitcast(U32), wo, sem.at[5])
    cp_wm1 = pltpu.make_async_copy(wm_u.at[:, 2 * D:6 * D], wm.at[:, 2 * D:6 * D], sem.at[6])
    cp_w1 = pltpu.make_async_copy(w1_hbm.bitcast(U32), w1, sem.at[7])
    cp_w3 = pltpu.make_async_copy(w3_hbm.bitcast(U32), w3, sem.at[8])
    cp_w2 = pltpu.make_async_copy(w2_hbm.bitcast(U32), w2, sem.at[9])

    cp_c.start()
    cp_wm0.start()
    cp_xe.start()
    for cp in chunk_copies(0):
        cp.start()
    cp_m0.start()
    for cp in chunk_copies(1):
        cp.start()

    keep, fill = _attn_mask()
    keep_s[...] = keep.astype(jnp.int32)
    fill_s[...] = fill

    cp_c.wait()
    cf = cb[...].astype(F32)
    sc = jnp.broadcast_to(cf * jax.nn.sigmoid(cf), (16, D)).astype(BF16)

    def mod_cols(lo, hi):
        for n in range(lo, hi, 512):
            mod[:, n:n + 512] = _dot(sc, _bf(wm[:, n:n + 512]))[0:8]

    cp_wm0.wait()
    mod_cols(0, 2 * D)

    def ln1(xf):
        return _ln_mod(xf, mod[0:1, 0:D], 1.0 + mod[0:1, D:2 * D])

    cp_xe.wait()
    for g in range(NSEG // 8):
        xe = xb[8 * g:8 * g + 8, 0:EARLY, :].astype(F32).reshape(8 * EARLY, D)
        p32[32 * g:32 * g + 32, :] = _pk(ln1(xe))

    wait_chunk(0)
    for jj in range(CH // 2):
        unzip(2 * jj)

    def prologue(t, carry):
        for tt in range(2, NCH):
            @pl.when(t + 2 == tt)
            def _():
                for cp in chunk_copies(tt):
                    cp.start()

        @pl.when(t == 2)
        def _():
            cp_xr.start()

        @pl.when(t == NCH - 2)
        def _():
            cp_wo.start()

        @pl.when(t + 1 < NCH)
        def _():
            wait_chunk(t + 1)

        for jj in range(CH // 2):
            slot = t * CH + 2 * jj
            wa, wb = _bf(wqkv[slot]), _bf(wqkv[slot + 1])
            for c in range(NEARLY // 128):
                lhs = _bf(p32[64 * c:64 * c + 64, :])
                a = _dot(lhs, wa).reshape(16, EARLY, DH)
                b = _dot(lhs, wb).reshape(16, EARLY, DH)
                pre[t * (CH // 2) + jj, 16 * c:16 * c + 16] = _pk(jnp.concatenate([a, b], axis=1))
            unzip(slot + CH)
        return carry

    lax.fori_loop(0, NCH, prologue, 0)

    cp_wm1.start()
    cp_w1.start()
    cp_w3.start()
    cp_w2.start()
    cp_m0.wait()
    cp_xr.wait()
    cp_wo.wait()

    def next_lhs(mem_f32, s):
        hx = ln1(xb[s, EARLY:SEG, :].astype(F32))
        l32[...] = _pk(jnp.concatenate([mem_f32, hx], axis=0))

    next_lhs(m0[...].astype(F32), 0)

    c_exp = SCALE * math.log2(math.e)

    def step(s, carry):
        lhs = _bf(l32[...])
        qkv = {}
        prob = {}

        def project(j):
            out = []
            for m in range(3):
                a = _dot(lhs, _bf(wqkv[m * H + 2 * j])).astype(BF16)
                b = _dot(lhs, _bf(wqkv[m * H + 2 * j + 1])).astype(BF16)
                out.append(jnp.concatenate([a, b, _bf(pre[m * NP + j, s])], axis=0))
            qkv[j] = out

        def scores(j):
            q, k, _ = qkv[j]
            sc_ = lax.dot_general(q, k, (((1,), (1,)), ((), ())), preferred_element_type=F32)
            sc_ = jnp.where(keep_s[...] != 0, sc_, fill_s[...])
            e = jnp.exp2((sc_ - jnp.max(sc_, axis=1, keepdims=True)) * c_exp)
            den = jnp.sum(e, axis=1, keepdims=True)
            r = pl.reciprocal(den, approx=True)
            r = r * (2.0 - den * r)
            prob[j] = (e * r).astype(BF16)

        def values(j):
            o = _dot(prob.pop(j), qkv.pop(j)[2])
            c0 = 2 * j * DH
            ob[:, c0:c0 + DH] = _pk(o[0:SEG])
            ob[:, c0 + DH:c0 + 2 * DH] = _pk(o[SEG:2 * SEG])
            odef[s, :, c0:c0 + DH] = o[2 * SEG:2 * SEG + EARLY]
            odef[s, :, c0 + DH:c0 + 2 * DH] = o[2 * SEG + EARLY:L2]

        nb = 256

        def wo_part(n, j0, j1):
            k0, k1 = j0 * 2 * DH, j1 * 2 * DH
            return _dot(_bf(ob[:, k0:k1]), _bf(wo[k0 // 2:k1 // 2, n * nb:(n + 1) * nb]))

        for j in range(NP):
            project(j)
            if j >= 1:
                scores(j - 1)
            if j >= 2:
                values(j - 2)
        y0 = wo_part(0, 0, 6)
        scores(NP - 1)
        y0 = y0 + wo_part(0, 6, 13)
        values(NP - 2)
        y1 = wo_part(1, 0, 13)
        values(NP - 1)
        y2 = wo_part(2, 0, 14)
        y0 = y0 + wo_part(0, 13, NP)
        y1 = y1 + wo_part(1, 13, NP)
        y2 = y2 + wo_part(2, 14, NP)
        ys = [y0, y1, y2, wo_part(3, 0, NP)]
        y = jnp.concatenate(ys, axis=1)
        a32[s] = _pk(y)
        next_lhs(y[0:MEM], jnp.minimum(s + 1, NSEG - 1))
        return carry

    lax.fori_loop(0, NSEG, step, 0)

    def early_wo(c, carry):
        s0 = pl.multiple_of(c * 16, 16)
        lhs = odef[pl.ds(s0, 16)].reshape(16 * EARLY, HD).astype(BF16)
        for n in range(0, D, 256):
            y = _dot(lhs, _bf(wo[:, n:n + 256])).reshape(16, EARLY, 256)
            a32[pl.ds(s0, 16), 0:EARLY // 2, n:n + 256] = _pk(y)
        return carry

    lax.fori_loop(0, NSEG // 16, early_wo, 0)

    cp_wm1.wait()
    mod_cols(2 * D, 6 * D)
    cp_w1.wait()
    cp_w3.wait()
    cp_w2.wait()

    def resid1(i):
        s0 = pl.multiple_of(i * SPB, SPB)
        xf = xb[pl.ds(s0, SPB)].astype(F32).reshape(TM, D)
        af = _bf(a32[pl.ds(s0, SPB)]).astype(F32).reshape(TM, D)
        return xf + mod[0:1, 2 * D:3 * D] * af

    def ln2(i, slot):
        h2[slot] = _pk(_ln_mod(resid1(i), mod[0:1, 3 * D:4 * D], 1.0 + mod[0:1, 4 * D:5 * D]))

    def out_copy(i, slot):
        return pltpu.make_async_copy(ost.at[slot], out_hbm.at[pl.ds(i * SPB, SPB)], osem.at[slot])

    ln2(0, 0)

    def ffn(i, carry):
        slot = i % 2

        @pl.when(i >= 2)
        def _():
            out_copy(i - 2, slot).wait()

        hh = _bf(h2[slot])
        for f0 in range(0, F, FC):
            g = _dot(hh, _bf(w1[:, f0:f0 + FC]))
            u = _dot(hh, _bf(w3[:, f0:f0 + FC]))
            act[:, f0:f0 + FC] = _pk(g * jax.nn.sigmoid(g) * u)
        ln2(jnp.minimum(i + 1, NBLK - 1), 1 - slot)
        x1 = resid1(i)
        aa = _bf(act[...])
        for n in range(0, D, 256):
            y = _dot(aa, _bf(w2[:, n:n + 256]))
            res = x1[:, n:n + 256] + mod[0:1, 5 * D + n:5 * D + n + 256] * y
            ost[slot, :, :, n:n + 256] = res.astype(BF16).reshape(SPB, SEG, 256)
        out_copy(i, slot).start()
        return carry

    lax.fori_loop(0, NBLK, ffn, 0)
    out_copy(NBLK - 2, 0).wait()
    out_copy(NBLK - 1, 1).wait()


@functools.partial(jax.jit, static_argnames=("A_seg_len",))
def pallas_adaLN_cond__memory_aug_recurrent_mem_tr__glu_gated_swiglu__prompt_kernel(
    A_x, A_mem0, A_Wq, A_Wk, A_Wv, A_Wo, A_seg_len, B_x, B_w1, B_w3, B_w2, c, w_mod,
):
    assert int(A_seg_len) == SEG and A_x.shape == (1, S, D) and A_mem0.shape == (1, MEM, D)
    del B_x
    vm = pltpu.VMEM
    scratch = [
        vm((3 * H + CH, D // 2, DH), U32),
        vm((HD // 2, D), U32),
        vm((D // 2, F), U32),
        vm((D // 2, F), U32),
        vm((F // 2, D), U32),
        vm((D // 2, 6 * D), U32),
        vm((NSEG, SEG, D), BF16),
        vm((1, D), BF16),
        vm((MEM, D), BF16),
        vm((8, 6 * D), F32),
        vm((NEARLY // 2, D), U32),
        vm((3 * NP, NSEG, EARLY, DH), U32),
        vm((SEG // 2, D), U32),
        vm((SEG // 2, HD), U32),
        vm((NSEG, EARLY, HD), F32),
        vm((NSEG, SEG // 2, D), U32),
        vm((2, TM // 2, D), U32),
        vm((TM // 2, F), U32),
        vm((2, SPB, SEG, D), BF16),
        vm((L2, L2), jnp.int32),
        vm((L2, L2), F32),
        pltpu.SemaphoreType.DMA((10,)),
        pltpu.SemaphoreType.DMA((NCH,)),
        pltpu.SemaphoreType.DMA((2,)),
    ]
    out = pl.pallas_call(
        _kernel,
        out_shape=jax.ShapeDtypeStruct((NSEG, SEG, D), BF16),
        in_specs=[pl.BlockSpec(memory_space=pl.ANY)] * 11,
        out_specs=pl.BlockSpec(memory_space=pl.ANY),
        scratch_shapes=scratch,
        compiler_params=pltpu.CompilerParams(vmem_limit_bytes=120 * 1024 * 1024),
    )(
        A_x.reshape(NSEG, SEG, D),
        A_mem0.reshape(MEM, D),
        A_Wq.reshape(D // 2, 2 * H, DH),
        A_Wk.reshape(D // 2, 2 * H, DH),
        A_Wv.reshape(D // 2, 2 * H, DH),
        A_Wo.reshape(HD, D),
        B_w1, B_w3, B_w2, c, w_mod,
    )
    return out.reshape(1, S, D)
```

```python
import functools
import math

import jax
import jax.numpy as jnp
from jax import lax
import jax.experimental.pallas as pl
import jax.experimental.pallas.tpu as pltpu

S, D, H, DH, MEM, SEG, F = 2048, 1024, 32, 128, 8, 32, 3584
NSEG = S // SEG
NP = H // 2
HD = H * DH
EARLY = 8
NEARLY = NSEG * EARLY
L2 = 2 * (MEM + SEG)
CH = 8
NCH = 3 * H // CH
NPAIR = NSEG // 2
PR = 2 * SEG
LAG = 2
NRING = 4
EPS = 1e-5
SCALE = DH ** -0.5
MASK_FILL = -1000000000.0

BF16, F32, U32 = jnp.bfloat16, jnp.float32, jnp.uint32


def _bf(x_u32):
    return pltpu.bitcast(x_u32, BF16)


def _pk(x_f32):
    return pltpu.bitcast(x_f32.astype(BF16), U32)


def _dot(a, b):
    return jnp.dot(a, b, preferred_element_type=F32)


def _ln_mod(x, shift, scale1):
    m = jnp.mean(x, axis=-1, keepdims=True)
    xc = x - m
    v = jnp.mean(xc * xc, axis=-1, keepdims=True)
    return xc * lax.rsqrt(v + EPS) * scale1 + shift


def _attn_mask():
    def meta(i):
        head = jnp.where(i < 2 * SEG, i // SEG, (i - 2 * SEG) // EARLY)
        j = i % SEG
        pos = jnp.where(i < 2 * SEG, jnp.where(j < MEM, j, j + EARLY), MEM + (i - 2 * SEG) % EARLY)
        return head, pos
    r = lax.broadcasted_iota(jnp.int32, (L2, L2), 0)
    c = lax.broadcasted_iota(jnp.int32, (L2, L2), 1)
    rh, rp = meta(r)
    chd, cp = meta(c)
    same = rh == chd
    keep = same & ((rp < MEM) | (rp >= cp))
    fill = jnp.where(same, MASK_FILL / SCALE, -jnp.inf).astype(F32)
    return keep, fill


def _kernel(x_hbm, m0_hbm, wq_hbm, wk_hbm, wv_hbm, wo_hbm, w1_hbm, w3_hbm, w2_hbm, c_hbm, wm_hbm,
            out_hbm,
            wqkv, wo, w1, w3, w2, wm, xb, cb, m0, mod, p32, pre, l32, ob, oda, abuf,
            x1s, h2, act, ost, keep_s, fill_s, sem, wsem, osem):
    w_hbm = [r.bitcast(U32) for r in (wq_hbm, wk_hbm, wv_hbm)]
    wm_u = wm_hbm.bitcast(U32)

    def chunk_copies(t):
        m, c0 = divmod(t, H // CH)
        cps = []
        for jj in range(CH // 2):
            j = c0 * (CH // 2) + jj
            for par in range(2):
                cps.append(pltpu.make_async_copy(
                    w_hbm[m].at[:, par * NP + j, :], wqkv.at[m * H + 2 * j + par], wsem.at[t]))
        return cps

    def wait_chunk(t):
        blk = wqkv.at[pl.ds(t * CH, CH)]
        pltpu.make_async_copy(blk, blk, wsem.at[t]).wait()

    def unzip(slot):
        for r in range(0, D // 2, 32):
            e, o = wqkv[slot, r:r + 32, :], wqkv[slot + 1, r:r + 32, :]
            wqkv[slot, r:r + 32, :] = (e & 0xFFFF) | (o << 16)
            wqkv[slot + 1, r:r + 32, :] = (e >> 16) | (o & jnp.uint32(0xFFFF0000))

    cp_c = pltpu.make_async_copy(c_hbm, cb, sem.at[0])
    cp_wm = [pltpu.make_async_copy(wm_u.at[:, k * D:(k + 1) * D], wm.at[k], sem.at[10 + k])
             for k in range(6)]
    cp_xe = pltpu.make_async_copy(x_hbm.at[:, 0:EARLY, :], xb.at[:, 0:EARLY, :], sem.at[2])
    cp_m0 = pltpu.make_async_copy(m0_hbm, m0, sem.at[3])
    cp_xr = pltpu.make_async_copy(x_hbm.at[:, EARLY:SEG, :], xb.at[:, EARLY:SEG, :], sem.at[4])
    cp_wo = pltpu.make_async_copy(wo_hbm.bitcast(U32), wo, sem.at[5])
    cp_w1 = pltpu.make_async_copy(w1_hbm.bitcast(U32), w1, sem.at[7])
    cp_w3 = pltpu.make_async_copy(w3_hbm.bitcast(U32), w3, sem.at[8])
    cp_w2 = pltpu.make_async_copy(w2_hbm.bitcast(U32), w2, sem.at[9])

    cp_c.start()
    cp_wm[0].start()
    cp_wm[1].start()
    cp_xe.start()
    for cp in chunk_copies(0):
        cp.start()
    cp_m0.start()
    for cp in chunk_copies(1):
        cp.start()

    keep, fill = _attn_mask()
    keep_s[...] = keep.astype(jnp.int32)
    fill_s[...] = fill

    cp_c.wait()
    cf = cb[...].astype(F32)
    sc = jnp.broadcast_to(cf * jax.nn.sigmoid(cf), (16, D)).astype(BF16)

    def mod_unit(k, n):
        mod[k, :, n:n + 512] = _dot(sc, _bf(wm[k, :, n:n + 512]))[0:8]

    for k in range(2):
        cp_wm[k].wait()
        mod_unit(k, 0)
        mod_unit(k, 512)

    def ln1(xf):
        return _ln_mod(xf, mod[0, 0:1, :], 1.0 + mod[1, 0:1, :])

    cp_xe.wait()
    for g in range(NSEG // 8):
        xe = xb[8 * g:8 * g + 8, 0:EARLY, :].astype(F32).reshape(8 * EARLY, D)
        p32[32 * g:32 * g + 32, :] = _pk(ln1(xe))

    wait_chunk(0)
    for jj in range(CH // 2):
        unzip(2 * jj)

    dma_plan = [chunk_copies(2 * tt + 2) + chunk_copies(2 * tt + 3) for tt in range(NCH // 2 - 1)]
    dma_plan += [[cp_xr, cp_wo], cp_wm[2:6] + [cp_w1], [cp_w3, cp_w2]]

    def prologue(t, carry):
        for tt, cps in enumerate(dma_plan):
            @pl.when(t == tt)
            def _():
                for cp in cps:
                    cp.start()

        @pl.when(t + 1 < NCH)
        def _():
            wait_chunk(t + 1)

        for jj in range(CH // 2):
            slot = t * CH + 2 * jj
            wa, wb = _bf(wqkv[slot]), _bf(wqkv[slot + 1])
            for c in range(NEARLY // 128):
                lhs = _bf(p32[64 * c:64 * c + 64, :])
                a = _dot(lhs, wa).reshape(16, EARLY, DH)
                b = _dot(lhs, wb).reshape(16, EARLY, DH)
                pre[t * (CH // 2) + jj, 16 * c:16 * c + 16] = _pk(jnp.concatenate([a, b], axis=1))
            unzip(slot + CH)
        return carry

    with jax.named_scope('prologue'):
        lax.fori_loop(0, NCH, prologue, 0)

    with jax.named_scope('wait1'):
        cp_m0.wait()
        cp_xr.wait()
        cp_wo.wait()
        for k in range(2, 6):
            cp_wm[k].wait()

    def next_lhs(mem_f32, s):
        hx = ln1(xb[s, EARLY:SEG, :].astype(F32))
        l32[...] = _pk(jnp.concatenate([mem_f32, hx], axis=0))

    next_lhs(m0[...].astype(F32), 0)

    def out_copy(p, npairs, slot):
        return pltpu.make_async_copy(ost.at[slot, 0:2 * npairs], out_hbm.at[pl.ds(2 * p, 2 * npairs)],
                                     osem.at[slot])

    def ffn_units(p, npairs, slot):
        rows = npairs * PR
        for q in range(npairs):
            xf = xb[pl.ds(2 * (p + q), 2)].astype(F32).reshape(PR, D)
            x1 = xf + mod[2, 0:1, :] * abuf[(p + q) % NRING]
            x1s[q * PR:(q + 1) * PR, :] = x1
            h2[q * SEG:(q + 1) * SEG, :] = _pk(_ln_mod(x1, mod[3, 0:1, :], 1.0 + mod[4, 0:1, :]))

        def gate_up(f0):
            hh = _bf(h2[0:rows // 2, :])
            t = 0.5 * _dot(hh, _bf(w1[:, f0:f0 + 128]))
            u = _dot(hh, _bf(w3[:, f0:f0 + 128]))
            act[0:rows // 2, f0:f0 + 128] = _pk((t + t * jnp.tanh(t)) * u)

        def down(n0):
            y = _dot(_bf(act[0:rows // 2, :]), _bf(w2[:, n0:n0 + 128]))
            res = x1s[0:rows, n0:n0 + 128] + mod[5, 0:1, n0:n0 + 128] * y
            ost[slot, 0:2 * npairs, :, n0:n0 + 128] = res.astype(BF16).reshape(2 * npairs, SEG, 128)

        return ([functools.partial(gate_up, f0) for f0 in range(0, F, 128)],
                [functools.partial(down, n0) for n0 in range(0, D, 128)])

    c_exp = SCALE * math.log2(math.e)
    nb = 256

    def step(s, second, fill):
        rows = SEG + 2 * EARLY if second else SEG
        lhs = _bf(l32[...])
        qkv, prob = {}, {}

        def project(j):
            out = []
            for m in range(3):
                a = _dot(lhs, _bf(wqkv[m * H + 2 * j])).astype(BF16)
                b = _dot(lhs, _bf(wqkv[m * H + 2 * j + 1])).astype(BF16)
                out.append(jnp.concatenate([a, b, _bf(pre[m * NP + j, s])], axis=0))
            qkv[j] = out

        def scores(j):
            q, k, _ = qkv[j]
            sc_ = lax.dot_general(q, k, (((1,), (1,)), ((), ())), preferred_element_type=F32)
            sc_ = jnp.where(keep_s[...] != 0, sc_, fill_s[...])
            e = jnp.exp2((sc_ - jnp.max(sc_, axis=1, keepdims=True)) * c_exp)
            den = jnp.sum(e, axis=1, keepdims=True)
            r = pl.reciprocal(den, approx=True)
            r = r * (2.0 - den * r)
            prob[j] = (e * r).astype(BF16)

        def values(j):
            o = _dot(prob.pop(j), qkv.pop(j)[2])
            for hh in range(2):
                c0 = (2 * j + hh) * DH
                main = o[hh * SEG:(hh + 1) * SEG]
                early = o[2 * SEG + hh * EARLY:2 * SEG + (hh + 1) * EARLY]
                if second:
                    ob[:, c0:c0 + DH] = _pk(jnp.concatenate([main, oda[:, c0:c0 + DH], early], axis=0))
                else:
                    ob[0:SEG // 2, c0:c0 + DH] = _pk(main)
                    oda[:, c0:c0 + DH] = early

        def wo_part(n, j0, j1):
            k0, k1 = j0 * 2 * DH, j1 * 2 * DH
            return _dot(_bf(ob[0:rows // 2, k0:k1]), _bf(wo[k0 // 2:k1 // 2, n * nb:(n + 1) * nb]))

        for j in range(NP):
            project(j)
            if j >= 1:
                scores(j - 1)
            if j >= 3:
                values(j - 3)
            fill(j)
        y0 = wo_part(0, 0, 6)
        scores(NP - 1)
        values(NP - 3)
        y0 = y0 + wo_part(0, 6, 12)
        values(NP - 2)
        fill(NP)
        y1 = wo_part(1, 0, 8)
        values(NP - 1)
        y1 = y1 + wo_part(1, 8, 13)
        y2 = wo_part(2, 0, 14)
        y0 = y0 + wo_part(0, 12, NP)
        y1 = y1 + wo_part(1, 13, NP)
        y2 = y2 + wo_part(2, 14, NP)
        y = jnp.concatenate([y0, y1, y2, wo_part(3, 0, NP)], axis=1)
        next_lhs(y[0:MEM], jnp.minimum(s + 1, NSEG - 1))
        fill(NP + 1)
        return y

    def pair(i, plan):
        def filler(second):
            def fill(point):
                for unit in plan.get((second, point), ()):
                    unit()
            return fill

        slot = i % NRING
        ya = step(2 * i, False, filler(False))
        abuf[slot, EARLY:SEG, :] = ya[MEM:SEG]
        yb = step(2 * i + 1, True, filler(True))
        abuf[slot, 0:EARLY, :] = yb[SEG:SEG + EARLY]
        abuf[slot, SEG:SEG + EARLY, :] = yb[SEG + EARLY:SEG + 2 * EARLY]
        abuf[slot, SEG + EARLY:PR, :] = yb[MEM:SEG]

    def head_pairs(i, carry):
        units = [functools.partial(mod_unit, 2 + 2 * i + kk, n) for kk in range(2) for n in (0, 512)]
        pair(i, {(False, NP): units[0:1], (False, NP + 1): units[1:3], (True, NP): units[3:4]})
        return carry

    with jax.named_scope('head'):
        lax.fori_loop(0, LAG, head_pairs, 0)
    with jax.named_scope('wait2'):
        cp_w1.wait()
        cp_w3.wait()
        cp_w2.wait()

    def main_pairs(i, carry):
        p = i - LAG
        slot = p % 2

        @pl.when(p >= 2)
        def _():
            out_copy(p - 2, 1, slot).wait()

        gu, dn = ffn_units(p, 1, slot)
        plan = {}
        it = iter(gu)
        for j in range(2, NP):
            plan[(False, j)] = [next(it) for _ in range(2 if j % 2 == 0 else 1)]
        plan[(False, NP)] = [next(it)]
        plan[(False, NP + 1)] = [next(it), next(it)]
        for j in range(4):
            plan[(True, j)] = [next(it)]
        for k, j in enumerate((6, 8, 10, 12, 14)):
            plan[(True, j)] = [dn[k]]
        plan[(True, NP)] = [dn[5]]
        plan[(True, NP + 1)] = dn[6:8]
        pair(i, plan)
        out_copy(p, 1, slot).start()
        return carry

    with jax.named_scope('main'):
        lax.fori_loop(LAG, NPAIR, main_pairs, 0)

    p0 = NPAIR - LAG
    out_copy(p0 - 2, 1, 0).wait()
    gu, dn = ffn_units(p0, LAG, 0)
    for unit in gu + dn:
        unit()
    out_copy(p0, LAG, 0).start()
    out_copy(p0 - 1, 1, 1).wait()
    out_copy(p0, LAG, 0).wait()


@functools.partial(jax.jit, static_argnames=("A_seg_len",))
def pallas_adaLN_cond__memory_aug_recurrent_mem_tr__glu_gated_swiglu__prompt_kernel(
    A_x, A_mem0, A_Wq, A_Wk, A_Wv, A_Wo, A_seg_len, B_x, B_w1, B_w3, B_w2, c, w_mod,
):
    assert int(A_seg_len) == SEG and A_x.shape == (1, S, D) and A_mem0.shape == (1, MEM, D)
    del B_x
    vm = pltpu.VMEM
    scratch = [
        vm((3 * H + CH, D // 2, DH), U32),
        vm((HD // 2, D), U32),
        vm((D // 2, F), U32),
        vm((D // 2, F), U32),
        vm((F // 2, D), U32),
        vm((6, D // 2, D), U32),
        vm((NSEG, SEG, D), BF16),
        vm((1, D), BF16),
        vm((MEM, D), BF16),
        vm((6, 8, D), F32),
        vm((NEARLY // 2, D), U32),
        vm((3 * NP, NSEG, EARLY, DH), U32),
        vm((SEG // 2, D), U32),
        vm((SEG // 2 + EARLY, HD), U32),
        vm((EARLY, HD), F32),
        vm((NRING, PR, D), F32),
        vm((LAG * PR, D), F32),
        vm((LAG * SEG, D), U32),
        vm((LAG * SEG, F), U32),
        vm((2, 2 * LAG, SEG, D), BF16),
        vm((L2, L2), jnp.int32),
        vm((L2, L2), F32),
        pltpu.SemaphoreType.DMA((16,)),
        pltpu.SemaphoreType.DMA((NCH,)),
        pltpu.SemaphoreType.DMA((2,)),
    ]
    out = pl.pallas_call(
        _kernel,
        out_shape=jax.ShapeDtypeStruct((NSEG, SEG, D), BF16),
        in_specs=[pl.BlockSpec(memory_space=pl.ANY)] * 11,
        out_specs=pl.BlockSpec(memory_space=pl.ANY),
        scratch_shapes=scratch,
        compiler_params=pltpu.CompilerParams(vmem_limit_bytes=120 * 1024 * 1024),
    )(
        A_x.reshape(NSEG, SEG, D),
        A_mem0.reshape(MEM, D),
        A_Wq.reshape(D // 2, 2 * H, DH),
        A_Wk.reshape(D // 2, 2 * H, DH),
        A_Wv.reshape(D // 2, 2 * H, DH),
        A_Wo.reshape(HD, D),
        B_w1, B_w3, B_w2, c, w_mod,
    )
    return out.reshape(1, S, D)
```

```python
import functools
import math

import jax
import jax.numpy as jnp
from jax import lax
import jax.experimental.pallas as pl
import jax.experimental.pallas.tpu as pltpu

S, D, H, DH, MEM, SEG, F = 2048, 1024, 32, 128, 8, 32, 3584
NSEG = S // SEG
NP = H // 2
HD = H * DH
EARLY = 8
NEARLY = NSEG * EARLY
L2 = 2 * (MEM + SEG)
CH = 8
NCH = 3 * H // CH
NPAIR = NSEG // 2
PR = 2 * SEG
LAG = 2
NRING = 4
EPS = 1e-5
SCALE = DH ** -0.5
MASK_FILL = -1000000000.0

BF16, F32, U32 = jnp.bfloat16, jnp.float32, jnp.uint32


def _bf(x_u32):
    return pltpu.bitcast(x_u32, BF16)


def _pk(x_f32):
    return pltpu.bitcast(x_f32.astype(BF16), U32)


def _dot(a, b):
    return jnp.dot(a, b, preferred_element_type=F32)


def _norm(x):
    m = jnp.mean(x, axis=-1, keepdims=True)
    xc = x - m
    v = jnp.mean(xc * xc, axis=-1, keepdims=True)
    return xc * lax.rsqrt(v + EPS)


def _attn_mask():
    def meta(i):
        head = jnp.where(i < 2 * SEG, i // SEG, (i - 2 * SEG) // EARLY)
        j = i % SEG
        pos = jnp.where(i < 2 * SEG, jnp.where(j < MEM, j, j + EARLY), MEM + (i - 2 * SEG) % EARLY)
        return head, pos
    r = lax.broadcasted_iota(jnp.int32, (L2, L2), 0)
    c = lax.broadcasted_iota(jnp.int32, (L2, L2), 1)
    rh, rp = meta(r)
    chd, cp = meta(c)
    same = rh == chd
    keep = same & ((rp < MEM) | (rp >= cp))
    fill = jnp.where(same, MASK_FILL / SCALE, -jnp.inf).astype(F32)
    return keep, fill


def _kernel(x_hbm, m0_hbm, wq_hbm, wk_hbm, wv_hbm, wo_hbm, w1_hbm, w3_hbm, w2_hbm, c_hbm, wm_hbm,
            out_hbm,
            wqkv, wo, w1, w3, w2, wm, xb, cb, m0, mod, nrm, p32, pre, l32, ob, oda, abuf,
            x1s, h2, act, ost, keep_s, fill_s, sem, wsem, osem):
    w_hbm = [r.bitcast(U32) for r in (wq_hbm, wk_hbm, wv_hbm)]
    wm_u = wm_hbm.bitcast(U32)

    def pair_copies(m, j, dsem):
        return [pltpu.make_async_copy(w_hbm[m].at[:, par * NP + j, :], wqkv.at[m * H + 2 * j + par], dsem)
                for par in range(2)]

    def chunk_copies(t):
        m, c0 = divmod(t, H // CH)
        return [cp for jj in range(CH // 2)
                for cp in pair_copies(m, c0 * (CH // 2) + jj, wsem.at[t])]

    def wait_chunk(t):
        blk = wqkv.at[pl.ds(t * CH, CH)]
        pltpu.make_async_copy(blk, blk, wsem.at[t]).wait()

    def unzip(slot):
        for r in range(0, D // 2, 32):
            e, o = wqkv[slot, r:r + 32, :], wqkv[slot + 1, r:r + 32, :]
            wqkv[slot, r:r + 32, :] = (e & 0xFFFF) | (o << 16)
            wqkv[slot + 1, r:r + 32, :] = (e >> 16) | (o & jnp.uint32(0xFFFF0000))

    cp_c = pltpu.make_async_copy(c_hbm, cb, sem.at[0])
    cp_wm = [pltpu.make_async_copy(wm_u.at[:, k * D:(k + 1) * D], wm.at[k], sem.at[10 + k])
             for k in range(6)]
    cp_wm1 = [pltpu.make_async_copy(wm_u.at[:, D + n:D + n + 512], wm.at[1, :, n:n + 512], sem.at[16 + n // 512])
              for n in (0, 512)]
    cp_p0 = [pair_copies(0, jj, sem.at[18 + jj]) for jj in range(CH // 2)]
    cp_xe = pltpu.make_async_copy(x_hbm.at[:, 0:EARLY, :], xb.at[:, 0:EARLY, :], sem.at[2])
    cp_m0 = pltpu.make_async_copy(m0_hbm, m0, sem.at[3])
    cp_xr = pltpu.make_async_copy(x_hbm.at[:, EARLY:SEG, :], xb.at[:, EARLY:SEG, :], sem.at[4])
    cp_wo = pltpu.make_async_copy(wo_hbm.bitcast(U32), wo, sem.at[5])
    cp_w1 = pltpu.make_async_copy(w1_hbm.bitcast(U32), w1, sem.at[7])
    cp_w3 = pltpu.make_async_copy(w3_hbm.bitcast(U32), w3, sem.at[8])
    cp_w2 = pltpu.make_async_copy(w2_hbm.bitcast(U32), w2, sem.at[9])

    cp_c.start()
    cp_xe.start()
    keep, fill = _attn_mask()
    keep_s[...] = keep.astype(jnp.int32)
    fill_s[...] = fill
    cp_c.wait()
    cp_wm[0].start()
    cf = cb[...].astype(F32)
    sc = jnp.broadcast_to(cf * jax.nn.sigmoid(cf), (16, D)).astype(BF16)
    cp_xe.wait()
    cp_wm1[0].start()
    for g in range(NSEG // 8):
        nrm[64 * g:64 * g + 64, :] = _norm(xb[8 * g:8 * g + 8, 0:EARLY, :].astype(F32).reshape(8 * EARLY, D))

    def mod_unit(k, n):
        mod[k, :, n:n + 512] = _dot(sc, _bf(wm[k, :, n:n + 512]))[0:8]

    def start_all(cps):
        for cp in cps:
            cp.start()

    def wait_all(cps):
        for cp in cps:
            cp.wait()

    cp_wm[0].wait()
    cp_wm1[1].start()
    mod_unit(0, 0)
    mod_unit(0, 512)
    cp_wm1[0].wait()
    start_all(cp_p0[0])
    mod_unit(1, 0)
    cp_wm1[1].wait()
    start_all(cp_p0[1])
    mod_unit(1, 512)

    def ln1_mod(n):
        return n * (1.0 + mod[1, 0:1, :]) + mod[0, 0:1, :]

    for g in range(NSEG // 8):
        p32[32 * g:32 * g + 32, :] = _pk(ln1_mod(nrm[64 * g:64 * g + 64, :]))

    def early_qkv(slot):
        wa, wb = _bf(wqkv[slot]), _bf(wqkv[slot + 1])
        for c in range(NEARLY // 128):
            lhs = _bf(p32[64 * c:64 * c + 64, :])
            a = _dot(lhs, wa).reshape(16, EARLY, DH)
            b = _dot(lhs, wb).reshape(16, EARLY, DH)
            pre[slot // 2, 16 * c:16 * c + 16] = _pk(jnp.concatenate([a, b], axis=1))

    wait_all(cp_p0[0])
    start_all(cp_p0[2] + cp_p0[3])
    unzip(0)
    early_qkv(0)
    wait_all(cp_p0[1])
    start_all(chunk_copies(1))
    unzip(2)
    early_qkv(2)
    wait_all(cp_p0[2] + cp_p0[3])
    start_all(chunk_copies(2) + [cp_m0])
    unzip(4)
    unzip(6)
    early_qkv(4)

    def early_run(slot0, npairs):
        unzip(slot0)
        for g in range(npairs):
            if g + 1 < npairs:
                unzip(slot0 + 2 * g + 2)
            early_qkv(slot0 + 2 * g)

    wait_chunk(1)
    start_all([cp for t in range(3, 8) for cp in chunk_copies(t)])
    early_qkv(6)
    early_run(CH, CH // 2)

    def prologue(r, carry):
        wait_chunk(2 * r)
        wait_chunk(2 * r + 1)

        @pl.when(r == 1)
        def _():
            start_all([cp for t in range(8, NCH) for cp in chunk_copies(t)])

        @pl.when(r == 2)
        def _():
            start_all([cp_xr, cp_wo] + cp_wm[2:6] + [cp_w1, cp_w3, cp_w2])

        early_run(2 * r * CH, CH)
        return carry

    with jax.named_scope('prologue'):
        lax.fori_loop(1, NCH // 2, prologue, 0)

    with jax.named_scope('wait1'):
        cp_m0.wait()
        cp_xr.wait()
        cp_wo.wait()
        for k in range(2, 6):
            cp_wm[k].wait()

    def next_lhs(mem_f32, s):
        hx = ln1_mod(_norm(xb[s, EARLY:SEG, :].astype(F32)))
        l32[...] = _pk(jnp.concatenate([mem_f32, hx], axis=0))

    next_lhs(m0[...].astype(F32), 0)

    def out_copy(p, npairs, slot):
        return pltpu.make_async_copy(ost.at[slot, 0:2 * npairs], out_hbm.at[pl.ds(2 * p, 2 * npairs)],
                                     osem.at[slot])

    def ffn_units(p, npairs, slot):
        rows = npairs * PR
        for q in range(npairs):
            xf = xb[pl.ds(2 * (p + q), 2)].astype(F32).reshape(PR, D)
            x1 = xf + mod[2, 0:1, :] * abuf[(p + q) % NRING]
            x1s[q * PR:(q + 1) * PR, :] = x1
            h2[q * SEG:(q + 1) * SEG, :] = _pk(_norm(x1) * (1.0 + mod[4, 0:1, :]) + mod[3, 0:1, :])

        def gate_up(f0):
            hh = _bf(h2[0:rows // 2, :])
            t = 0.5 * _dot(hh, _bf(w1[:, f0:f0 + 128]))
            u = _dot(hh, _bf(w3[:, f0:f0 + 128]))
            act[0:rows // 2, f0:f0 + 128] = _pk((t + t * jnp.tanh(t)) * u)

        def down(n0):
            y = _dot(_bf(act[0:rows // 2, :]), _bf(w2[:, n0:n0 + 128]))
            res = x1s[0:rows, n0:n0 + 128] + mod[5, 0:1, n0:n0 + 128] * y
            ost[slot, 0:2 * npairs, :, n0:n0 + 128] = res.astype(BF16).reshape(2 * npairs, SEG, 128)

        return ([functools.partial(gate_up, f0) for f0 in range(0, F, 128)],
                [functools.partial(down, n0) for n0 in range(0, D, 128)])

    c_exp = SCALE * math.log2(math.e)
    nb = 256

    def step(s, second, fill):
        rows = SEG + 2 * EARLY if second else SEG
        lhs = _bf(l32[...])
        qkv, prob = {}, {}

        def project(j):
            out = []
            for m in range(3):
                a = _dot(lhs, _bf(wqkv[m * H + 2 * j])).astype(BF16)
                b = _dot(lhs, _bf(wqkv[m * H + 2 * j + 1])).astype(BF16)
                out.append(jnp.concatenate([a, b, _bf(pre[m * NP + j, s])], axis=0))
            qkv[j] = out

        def scores(j):
            q, k, _ = qkv[j]
            sc_ = lax.dot_general(q, k, (((1,), (1,)), ((), ())), preferred_element_type=F32)
            sc_ = jnp.where(keep_s[...] != 0, sc_, fill_s[...])
            e = jnp.exp2((sc_ - jnp.max(sc_, axis=1, keepdims=True)) * c_exp)
            den = jnp.sum(e, axis=1, keepdims=True)
            r = pl.reciprocal(den, approx=True)
            r = r * (2.0 - den * r)
            prob[j] = (e * r).astype(BF16)

        def values(j):
            o = _dot(prob.pop(j), qkv.pop(j)[2])
            for hh in range(2):
                c0 = (2 * j + hh) * DH
                main = o[hh * SEG:(hh + 1) * SEG]
                early = o[2 * SEG + hh * EARLY:2 * SEG + (hh + 1) * EARLY]
                if second:
                    ob[:, c0:c0 + DH] = _pk(jnp.concatenate([main, oda[:, c0:c0 + DH], early], axis=0))
                else:
                    ob[0:SEG // 2, c0:c0 + DH] = _pk(main)
                    oda[:, c0:c0 + DH] = early

        def wo_part(n, j0, j1):
            k0, k1 = j0 * 2 * DH, j1 * 2 * DH
            return _dot(_bf(ob[0:rows // 2, k0:k1]), _bf(wo[k0 // 2:k1 // 2, n * nb:(n + 1) * nb]))

        for j in range(NP):
            project(j)
            if j >= 1:
                scores(j - 1)
            if j >= 3:
                values(j - 3)
            fill(j)
        y0 = wo_part(0, 0, 6)
        scores(NP - 1)
        values(NP - 3)
        y0 = y0 + wo_part(0, 6, 12)
        values(NP - 2)
        fill(NP)
        y1 = wo_part(1, 0, 8)
        values(NP - 1)
        y1 = y1 + wo_part(1, 8, 13)
        y2 = wo_part(2, 0, 14)
        y0 = y0 + wo_part(0, 12, NP)
        y1 = y1 + wo_part(1, 13, NP)
        y2 = y2 + wo_part(2, 14, NP)
        y = jnp.concatenate([y0, y1, y2, wo_part(3, 0, NP)], axis=1)
        next_lhs(y[0:MEM], jnp.minimum(s + 1, NSEG - 1))
        fill(NP + 1)
        return y

    def pair(i, plan):
        def filler(second):
            def fill(point):
                for unit in plan.get((second, point), ()):
                    unit()
            return fill

        slot = i % NRING
        ya = step(2 * i, False, filler(False))
        abuf[slot, EARLY:SEG, :] = ya[MEM:SEG]
        yb = step(2 * i + 1, True, filler(True))
        abuf[slot, 0:EARLY, :] = yb[SEG:SEG + EARLY]
        abuf[slot, SEG:SEG + EARLY, :] = yb[SEG + EARLY:SEG + 2 * EARLY]
        abuf[slot, SEG + EARLY:PR, :] = yb[MEM:SEG]

    def head_pairs(i, carry):
        units = [functools.partial(mod_unit, 2 + 2 * i + kk, n) for kk in range(2) for n in (0, 512)]
        pair(i, {(False, NP): units[0:1], (False, NP + 1): units[1:3], (True, NP): units[3:4]})
        return carry

    with jax.named_scope('head'):
        lax.fori_loop(0, LAG, head_pairs, 0)
    with jax.named_scope('wait2'):
        cp_w1.wait()
        cp_w3.wait()
        cp_w2.wait()

    def main_pairs(i, carry):
        p = i - LAG
        slot = p % 2

        @pl.when(p >= 2)
        def _():
            out_copy(p - 2, 1, slot).wait()

        gu, dn = ffn_units(p, 1, slot)
        plan = {}
        it = iter(gu)
        for j in range(2, NP):
            plan[(False, j)] = [next(it) for _ in range(2 if j % 2 == 0 else 1)]
        plan[(False, NP)] = [next(it)]
        plan[(False, NP + 1)] = [next(it), next(it)]
        for j in range(4):
            plan[(True, j)] = [next(it)]
        for k, j in enumerate((6, 8, 10, 12, 14)):
            plan[(True, j)] = [dn[k]]
        plan[(True, NP)] = [dn[5]]
        plan[(True, NP + 1)] = dn[6:8]
        pair(i, plan)
        out_copy(p, 1, slot).start()
        return carry

    with jax.named_scope('main'):
        lax.fori_loop(LAG, NPAIR, main_pairs, 0)

    p0 = NPAIR - LAG
    out_copy(p0 - 2, 1, 0).wait()
    gu, dn = ffn_units(p0, LAG, 0)
    for unit in gu + dn:
        unit()
    out_copy(p0, LAG, 0).start()
    out_copy(p0 - 1, 1, 1).wait()
    out_copy(p0, LAG, 0).wait()


@functools.partial(jax.jit, static_argnames=("A_seg_len",))
def pallas_adaLN_cond__memory_aug_recurrent_mem_tr__glu_gated_swiglu__prompt_kernel(
    A_x, A_mem0, A_Wq, A_Wk, A_Wv, A_Wo, A_seg_len, B_x, B_w1, B_w3, B_w2, c, w_mod,
):
    assert int(A_seg_len) == SEG and A_x.shape == (1, S, D) and A_mem0.shape == (1, MEM, D)
    del B_x
    vm = pltpu.VMEM
    scratch = [
        vm((3 * H, D // 2, DH), U32),
        vm((HD // 2, D), U32),
        vm((D // 2, F), U32),
        vm((D // 2, F), U32),
        vm((F // 2, D), U32),
        vm((6, D // 2, D), U32),
        vm((NSEG, SEG, D), BF16),
        vm((1, D), BF16),
        vm((MEM, D), BF16),
        vm((6, 8, D), F32),
        vm((NEARLY, D), F32),
        vm((NEARLY // 2, D), U32),
        vm((3 * NP, NSEG, EARLY, DH), U32),
        vm((SEG // 2, D), U32),
        vm((SEG // 2 + EARLY, HD), U32),
        vm((EARLY, HD), F32),
        vm((NRING, PR, D), F32),
        vm((LAG * PR, D), F32),
        vm((LAG * SEG, D), U32),
        vm((LAG * SEG, F), U32),
        vm((2, 2 * LAG, SEG, D), BF16),
        vm((L2, L2), jnp.int32),
        vm((L2, L2), F32),
        pltpu.SemaphoreType.DMA((22,)),
        pltpu.SemaphoreType.DMA((NCH,)),
        pltpu.SemaphoreType.DMA((2,)),
    ]
    out = pl.pallas_call(
        _kernel,
        out_shape=jax.ShapeDtypeStruct((NSEG, SEG, D), BF16),
        in_specs=[pl.BlockSpec(memory_space=pl.ANY)] * 11,
        out_specs=pl.BlockSpec(memory_space=pl.ANY),
        scratch_shapes=scratch,
        compiler_params=pltpu.CompilerParams(vmem_limit_bytes=120 * 1024 * 1024),
    )(
        A_x.reshape(NSEG, SEG, D),
        A_mem0.reshape(MEM, D),
        A_Wq.reshape(D // 2, 2 * H, DH),
        A_Wk.reshape(D // 2, 2 * H, DH),
        A_Wv.reshape(D // 2, 2 * H, DH),
        A_Wo.reshape(HD, D),
        B_w1, B_w3, B_w2, c, w_mod,
    )
    return out.reshape(1, S, D)
```

```python
import functools
import math

import jax
import jax.numpy as jnp
from jax import lax
import jax.experimental.pallas as pl
import jax.experimental.pallas.tpu as pltpu

S, D, H, DH, MEM, SEG, F = 2048, 1024, 32, 128, 8, 32, 3584
NSEG = S // SEG
NP = H // 2
HD = H * DH
EARLY = 8
NEARLY = NSEG * EARLY
L2 = 2 * (MEM + SEG)
CH = 8
NCH = 3 * H // CH
NPAIR = NSEG // 2
PR = 2 * SEG
LAG = 2
NRING = 4
UNROLL = 1
EPS = 1e-5
SCALE = DH ** -0.5
MASK_FILL = -1000000000.0

BF16, F32, U32 = jnp.bfloat16, jnp.float32, jnp.uint32


def _bf(x_u32):
    return pltpu.bitcast(x_u32, BF16)


def _pk(x_f32):
    return pltpu.bitcast(x_f32.astype(BF16), U32)


def _dot(a, b):
    return jnp.dot(a, b, preferred_element_type=F32)


def _norm(x):
    m = jnp.mean(x, axis=-1, keepdims=True)
    xc = x - m
    v = jnp.mean(xc * xc, axis=-1, keepdims=True)
    return xc * lax.rsqrt(v + EPS)


def _attn_mask():
    def meta(i):
        head = jnp.where(i < 2 * SEG, i // SEG, (i - 2 * SEG) // EARLY)
        j = i % SEG
        pos = jnp.where(i < 2 * SEG, jnp.where(j < MEM, j, j + EARLY), MEM + (i - 2 * SEG) % EARLY)
        return head, pos
    r = lax.broadcasted_iota(jnp.int32, (L2, L2), 0)
    c = lax.broadcasted_iota(jnp.int32, (L2, L2), 1)
    rh, rp = meta(r)
    chd, cp = meta(c)
    same = rh == chd
    keep = same & ((rp < MEM) | (rp >= cp))
    fill = jnp.where(same, MASK_FILL / SCALE, -jnp.inf).astype(F32)
    return keep, fill


def _kernel(x_hbm, m0_hbm, wq_hbm, wk_hbm, wv_hbm, wo_hbm, w1_hbm, w3_hbm, w2_hbm, c_hbm, wm_hbm,
            out_hbm,
            wqkv, wo, w1, w3, w2, wm, xb, cb, m0, mod, nrm, p32, pre, l32, ob, oda, abuf,
            h2, act, ost, keep_s, fill_s, sem, wsem, osem):
    w_hbm = [r.bitcast(U32) for r in (wq_hbm, wk_hbm, wv_hbm)]
    wm_u = wm_hbm.bitcast(U32)

    def pair_copies(m, j, dsem):
        return [pltpu.make_async_copy(w_hbm[m].at[:, par * NP + j, :], wqkv.at[m * H + 2 * j + par], dsem)
                for par in range(2)]

    def chunk_copies(t):
        m, c0 = divmod(t, H // CH)
        return [cp for jj in range(CH // 2)
                for cp in pair_copies(m, c0 * (CH // 2) + jj, wsem.at[t])]

    def wait_chunk(t):
        blk = wqkv.at[pl.ds(t * CH, CH)]
        pltpu.make_async_copy(blk, blk, wsem.at[t]).wait()

    def unzip(slot):
        for r in range(0, D // 2, 32):
            e, o = wqkv[slot, r:r + 32, :], wqkv[slot + 1, r:r + 32, :]
            wqkv[slot, r:r + 32, :] = (e & 0xFFFF) | (o << 16)
            wqkv[slot + 1, r:r + 32, :] = (e >> 16) | (o & jnp.uint32(0xFFFF0000))

    cp_c = pltpu.make_async_copy(c_hbm, cb, sem.at[0])
    cp_wm = {k: pltpu.make_async_copy(wm_u.at[:, k * D:(k + 1) * D], wm.at[k], sem.at[10 + k])
             for k in (0, 2, 3, 4, 5)}
    cp_wm1 = [pltpu.make_async_copy(wm_u.at[:, D + n:D + n + 512], wm.at[1, :, n:n + 512], sem.at[16 + n // 512])
              for n in (0, 512)]
    cp_p0 = [pair_copies(0, jj, sem.at[18 + jj]) for jj in range(CH // 2)]
    cp_xe = pltpu.make_async_copy(x_hbm.at[:, 0:EARLY, :], xb.at[:, 0:EARLY, :], sem.at[2])
    cp_m0 = pltpu.make_async_copy(m0_hbm, m0, sem.at[3])
    cp_xr = pltpu.make_async_copy(x_hbm.at[:, EARLY:SEG, :], xb.at[:, EARLY:SEG, :], sem.at[4])
    cp_wo = pltpu.make_async_copy(wo_hbm.bitcast(U32), wo, sem.at[5])
    cp_w1 = pltpu.make_async_copy(w1_hbm.bitcast(U32), w1, sem.at[7])
    cp_w3 = pltpu.make_async_copy(w3_hbm.bitcast(U32), w3, sem.at[8])
    cp_w2 = pltpu.make_async_copy(w2_hbm.bitcast(U32), w2, sem.at[9])

    cp_c.start()
    cp_xe.start()
    keep, fill = _attn_mask()
    keep_s[...] = keep.astype(jnp.int32)
    fill_s[...] = fill
    cp_c.wait()
    cp_wm[0].start()
    cf = cb[...].astype(F32)
    sc = jnp.broadcast_to(cf * jax.nn.sigmoid(cf), (16, D)).astype(BF16)
    cp_xe.wait()
    cp_wm1[0].start()
    for g in range(NSEG // 8):
        nrm[64 * g:64 * g + 64, :] = _norm(xb[8 * g:8 * g + 8, 0:EARLY, :].astype(F32).reshape(8 * EARLY, D))

    def mod_unit(k, n):
        mod[k, :, n:n + 512] = _dot(sc, _bf(wm[k, :, n:n + 512]))[0:8]

    def start_all(cps):
        for cp in cps:
            cp.start()

    def wait_all(cps):
        for cp in cps:
            cp.wait()

    cp_wm[0].wait()
    cp_wm1[1].start()
    mod_unit(0, 0)
    mod_unit(0, 512)
    cp_wm1[0].wait()
    start_all(cp_p0[0])
    mod_unit(1, 0)
    cp_wm1[1].wait()
    start_all(cp_p0[1])
    mod_unit(1, 512)

    def ln1_mod(n):
        return n * (1.0 + mod[1, 0:1, :]) + mod[0, 0:1, :]

    for g in range(NSEG // 8):
        p32[32 * g:32 * g + 32, :] = _pk(ln1_mod(nrm[64 * g:64 * g + 64, :]))

    def early_qkv(slot):
        wa, wb = _bf(wqkv[slot]), _bf(wqkv[slot + 1])
        for c in range(NEARLY // 128):
            lhs = _bf(p32[64 * c:64 * c + 64, :])
            a = _dot(lhs, wa).reshape(16, EARLY, DH)
            b = _dot(lhs, wb).reshape(16, EARLY, DH)
            pre[slot // 2, 16 * c:16 * c + 16] = _pk(jnp.concatenate([a, b], axis=1))

    wait_all(cp_p0[0])
    start_all(cp_p0[2] + cp_p0[3])
    unzip(0)
    early_qkv(0)
    wait_all(cp_p0[1])
    start_all(chunk_copies(1))
    unzip(2)
    early_qkv(2)
    wait_all(cp_p0[2] + cp_p0[3])
    start_all(chunk_copies(2) + [cp_m0])
    unzip(4)
    unzip(6)
    early_qkv(4)

    def early_run(slot0, npairs):
        unzip(slot0)
        for g in range(npairs):
            if g + 1 < npairs:
                unzip(slot0 + 2 * g + 2)
            early_qkv(slot0 + 2 * g)

    wait_chunk(1)
    start_all([cp for t in range(3, 8) for cp in chunk_copies(t)])
    early_qkv(6)
    early_run(CH, CH // 2)

    def prologue(r, carry):
        wait_chunk(2 * r)
        wait_chunk(2 * r + 1)

        @pl.when(r == 1)
        def _():
            start_all([cp for t in range(8, NCH) for cp in chunk_copies(t)])

        @pl.when(r == 2)
        def _():
            start_all([cp_xr, cp_wo] + [cp_wm[k] for k in range(2, 6)] + [cp_w1, cp_w3, cp_w2])

        early_run(2 * r * CH, CH)
        return carry

    with jax.named_scope('prologue'):
        lax.fori_loop(1, NCH // 2, prologue, 0)

    with jax.named_scope('wait1'):
        cp_m0.wait()
        cp_xr.wait()
        cp_wo.wait()
        for k in range(2, 6):
            cp_wm[k].wait()

    def next_lhs(mem_f32, s):
        hx = ln1_mod(_norm(xb[s, EARLY:SEG, :].astype(F32)))
        l32[...] = _pk(jnp.concatenate([mem_f32, hx], axis=0))

    next_lhs(m0[...].astype(F32), 0)

    def resid1(p, c0, c1):
        xf = xb[pl.ds(2 * p, 2), :, c0:c1].astype(F32).reshape(PR, c1 - c0)
        return xf + mod[2, 0:1, c0:c1] * abuf[p & (NRING - 1), :, c0:c1]

    def ln2(p, q):
        h2[q * SEG:(q + 1) * SEG, :] = _pk(_norm(resid1(p, 0, D)) * (1.0 + mod[4, 0:1, :]) + mod[3, 0:1, :])

    def gate_up_units(q0, q1, chunks):
        r0, r1 = q0 * SEG, q1 * SEG
        half = {}

        def gate(f0):
            half[f0] = 0.5 * _dot(_bf(h2[r0:r1, :]), _bf(w1[:, f0:f0 + 128]))

        def up(f0):
            t = half.pop(f0)
            u = _dot(_bf(h2[r0:r1, :]), _bf(w3[:, f0:f0 + 128]))
            act[r0:r1, f0:f0 + 128] = _pk((t + t * jnp.tanh(t)) * u)

        return [functools.partial(fn, 128 * ck) for ck in chunks for fn in (gate, up)]

    def down_units(p, npairs, dst, nsplit):
        kq = F // nsplit
        acc = {}

        def down(n0, k):
            y = _dot(_bf(act[0:npairs * SEG, k * kq:(k + 1) * kq]),
                     _bf(w2[k * kq // 2:(k + 1) * kq // 2, n0:n0 + 128]))
            if k > 0:
                y = y + acc.pop(n0)
            if k + 1 < nsplit:
                acc[n0] = y
                return
            for q in range(npairs):
                res = resid1(p + q, n0, n0 + 128) + mod[5, 0:1, n0:n0 + 128] * y[q * PR:(q + 1) * PR]
                dst[2 * q:2 * q + 2, :, n0:n0 + 128] = res.astype(BF16).reshape(2, SEG, 128)

        return [functools.partial(down, n0, k) for n0 in range(0, D, 128) for k in range(nsplit)]

    def out_copy(p, npairs, slot):
        return pltpu.make_async_copy(ost.at[slot, 0:2 * npairs], out_hbm.at[pl.ds(2 * p, 2 * npairs)],
                                     osem.at[slot])

    c_exp = SCALE * math.log2(math.e)
    nb = 256

    def step(s, second, fill):
        rows = SEG + 2 * EARLY if second else SEG
        lhs = _bf(l32[...])
        qkv, prob = {}, {}

        def project(j):
            out = []
            for m in range(3):
                a = _dot(lhs, _bf(wqkv[m * H + 2 * j])).astype(BF16)
                b = _dot(lhs, _bf(wqkv[m * H + 2 * j + 1])).astype(BF16)
                out.append(jnp.concatenate([a, b, _bf(pre[m * NP + j, s])], axis=0))
                fill(3 * j + m)
            qkv[j] = out

        def scores(j):
            q, k, _ = qkv[j]
            sc_ = lax.dot_general(q, k, (((1,), (1,)), ((), ())), preferred_element_type=F32)
            sc_ = jnp.where(keep_s[...] != 0, sc_, fill_s[...])
            e = jnp.exp2((sc_ - jnp.max(sc_, axis=1, keepdims=True)) * c_exp)
            den = jnp.sum(e, axis=1, keepdims=True)
            r = pl.reciprocal(den, approx=True)
            r = r * (2.0 - den * r)
            prob[j] = (e * r).astype(BF16)

        def values(j):
            o = _dot(prob.pop(j), qkv.pop(j)[2])
            for hh in range(2):
                c0 = (2 * j + hh) * DH
                main = o[hh * SEG:(hh + 1) * SEG]
                early = o[2 * SEG + hh * EARLY:2 * SEG + (hh + 1) * EARLY]
                if second:
                    ob[:, c0:c0 + DH] = _pk(jnp.concatenate([main, oda[:, c0:c0 + DH], early], axis=0))
                else:
                    ob[0:SEG // 2, c0:c0 + DH] = _pk(main)
                    oda[:, c0:c0 + DH] = early

        def wo_part(n, j0, j1):
            k0, k1 = j0 * 2 * DH, j1 * 2 * DH
            return _dot(_bf(ob[0:rows // 2, k0:k1]), _bf(wo[k0 // 2:k1 // 2, n * nb:(n + 1) * nb]))

        for j in range(NP):
            project(j)
            if j >= 1:
                scores(j - 1)
            if j >= 3:
                values(j - 3)
        y0 = wo_part(0, 0, 6)
        scores(NP - 1)
        values(NP - 3)
        y0 = y0 + wo_part(0, 6, 12)
        values(NP - 2)
        fill('mid')
        y1 = wo_part(1, 0, 8)
        values(NP - 1)
        y1 = y1 + wo_part(1, 8, 13)
        y2 = wo_part(2, 0, 14)
        y0 = y0 + wo_part(0, 12, NP)
        y1 = y1 + wo_part(1, 13, NP)
        y2 = y2 + wo_part(2, 14, NP)
        y = jnp.concatenate([y0, y1, y2, wo_part(3, 0, NP)], axis=1)
        next_lhs(y[0:MEM], jnp.minimum(s + 1, NSEG - 1))
        fill('end')
        return y

    def pair(i, units, counts):
        units = list(units)

        def filler(second):
            def fill(point):
                for _ in range(counts.get((second, point), 0)):
                    units.pop(0)()
            return fill

        slot = i & (NRING - 1)
        ya = step(2 * i, False, filler(False))
        abuf[slot, EARLY:SEG, :] = ya[MEM:SEG]
        yb = step(2 * i + 1, True, filler(True))
        abuf[slot, 0:EARLY, :] = yb[SEG:SEG + EARLY]
        abuf[slot, SEG:SEG + EARLY, :] = yb[SEG + EARLY:SEG + 2 * EARLY]
        abuf[slot, SEG + EARLY:PR, :] = yb[MEM:SEG]
        assert not units

    def head_pairs(i, carry):
        units = [functools.partial(mod_unit, 2 + 2 * i + kk, n) for kk in range(2) for n in (0, 512)]
        pair(i, units, {(False, 'mid'): 1, (False, 'end'): 2, (True, 'mid'): 1})
        return carry

    with jax.named_scope('head'):
        lax.fori_loop(0, LAG, head_pairs, 0)
    with jax.named_scope('wait2'):
        cp_w1.wait()
        cp_w3.wait()
        cp_w2.wait()
    ln2(0, 0)

    nf = F // 128
    counts = {(False, 'mid'): 2, (False, 'end'): 4, (True, 'mid'): 2, (True, 'end'): 5}
    n_inner = 2 * nf + 1 + 32 - sum(counts.values())
    for k in range(6 * NP):
        counts[(k >= 3 * NP, k % (3 * NP))] = (k + 1) * n_inner // (6 * NP) - k * n_inner // (6 * NP)

    def main_pairs(b, carry):
        p0 = b * UNROLL
        slot = b & 1

        @pl.when(b >= 2)
        def _():
            out_copy(p0 - 2 * UNROLL, UNROLL, slot).wait()

        for u in range(UNROLL):
            p = p0 + u
            units = gate_up_units(0, 1, range(nf))
            units.append(functools.partial(ln2, p + 1, 0))
            units += down_units(p, 1, ost.at[slot, 2 * u:2 * u + 2], 4)
            pair(p + LAG, units, counts)
        out_copy(p0, UNROLL, slot).start()
        return carry

    nbody = (NPAIR - LAG) // UNROLL
    with jax.named_scope('main'):
        lax.fori_loop(0, nbody, main_pairs, 0)

    p0 = NPAIR - LAG
    slot = nbody & 1
    out_copy(p0 - 2 * UNROLL, UNROLL, slot).wait()
    ln2(p0 + 1, 1)
    units = gate_up_units(0, 1, range(2)) + gate_up_units(1, 2, range(2)) + gate_up_units(0, 2, range(2, nf))
    for unit in units + down_units(p0, LAG, ost.at[slot], 1):
        unit()
    out_copy(p0, LAG, slot).start()
    out_copy(p0 - UNROLL, UNROLL, 1 - slot).wait()
    out_copy(p0, LAG, slot).wait()


@functools.partial(jax.jit, static_argnames=("A_seg_len",))
def pallas_adaLN_cond__memory_aug_recurrent_mem_tr__glu_gated_swiglu__prompt_kernel(
    A_x, A_mem0, A_Wq, A_Wk, A_Wv, A_Wo, A_seg_len, B_x, B_w1, B_w3, B_w2, c, w_mod,
):
    assert int(A_seg_len) == SEG and A_x.shape == (1, S, D) and A_mem0.shape == (1, MEM, D)
    del B_x
    vm = pltpu.VMEM
    scratch = [
        vm((3 * H, D // 2, DH), U32),
        vm((HD // 2, D), U32),
        vm((D // 2, F), U32),
        vm((D // 2, F), U32),
        vm((F // 2, D), U32),
        vm((6, D // 2, D), U32),
        vm((NSEG, SEG, D), BF16),
        vm((1, D), BF16),
        vm((MEM, D), BF16),
        vm((6, 8, D), F32),
        vm((NEARLY, D), F32),
        vm((NEARLY // 2, D), U32),
        vm((3 * NP, NSEG, EARLY, DH), U32),
        vm((SEG // 2, D), U32),
        vm((SEG // 2 + EARLY, HD), U32),
        vm((EARLY, HD), F32),
        vm((NRING, PR, D), F32),
        vm((LAG * SEG, D), U32),
        vm((LAG * SEG, F), U32),
        vm((2, 2 * max(LAG, UNROLL), SEG, D), BF16),
        vm((L2, L2), jnp.int32),
        vm((L2, L2), F32),
        pltpu.SemaphoreType.DMA((22,)),
        pltpu.SemaphoreType.DMA((NCH,)),
        pltpu.SemaphoreType.DMA((2,)),
    ]
    out = pl.pallas_call(
        _kernel,
        out_shape=jax.ShapeDtypeStruct((NSEG, SEG, D), BF16),
        in_specs=[pl.BlockSpec(memory_space=pl.ANY)] * 11,
        out_specs=pl.BlockSpec(memory_space=pl.ANY),
        scratch_shapes=scratch,
        compiler_params=pltpu.CompilerParams(vmem_limit_bytes=120 * 1024 * 1024,
                                             disable_bounds_checks=True),
    )(
        A_x.reshape(NSEG, SEG, D),
        A_mem0.reshape(MEM, D),
        A_Wq.reshape(D // 2, 2 * H, DH),
        A_Wk.reshape(D // 2, 2 * H, DH),
        A_Wv.reshape(D // 2, 2 * H, DH),
        A_Wo.reshape(HD, D),
        B_w1, B_w3, B_w2, c, w_mod,
    )
    return out.reshape(1, S, D)
```

```python
import functools
import math

import jax
import jax.numpy as jnp
from jax import lax
import jax.experimental.pallas as pl
import jax.experimental.pallas.tpu as pltpu

S, D, H, DH, MEM, SEG, F = 2048, 1024, 32, 128, 8, 32, 3584
NSEG = S // SEG
NP = H // 2
HD = H * DH
EARLY = 8
NEARLY = NSEG * EARLY
L2 = 2 * (MEM + SEG)
CH = 8
NCH = 3 * H // CH
NPAIR = NSEG // 2
PR = 2 * SEG
LAG = 2
NRING = 4
EPS = 1e-5
SCALE = DH ** -0.5
MASK_FILL = -1000000000.0

BF16, F32, U32 = jnp.bfloat16, jnp.float32, jnp.uint32


def _bf(x_u32):
    return pltpu.bitcast(x_u32, BF16)


def _pk(x_f32):
    return pltpu.bitcast(x_f32.astype(BF16), U32)


def _dot(a, b):
    return jnp.dot(a, b, preferred_element_type=F32)


def _norm(x):
    m = jnp.mean(x, axis=-1, keepdims=True)
    xc = x - m
    v = jnp.mean(xc * xc, axis=-1, keepdims=True)
    return xc * lax.rsqrt(v + EPS)


def _attn_mask():
    def meta(i):
        head = jnp.where(i < 2 * SEG, i // SEG, (i - 2 * SEG) // EARLY)
        j = i % SEG
        pos = jnp.where(i < 2 * SEG, jnp.where(j < MEM, j, j + EARLY), MEM + (i - 2 * SEG) % EARLY)
        return head, pos
    r = lax.broadcasted_iota(jnp.int32, (L2, L2), 0)
    c = lax.broadcasted_iota(jnp.int32, (L2, L2), 1)
    rh, rp = meta(r)
    chd, cp = meta(c)
    same = rh == chd
    keep = same & ((rp < MEM) | (rp >= cp))
    fill = jnp.where(same, MASK_FILL / SCALE, -jnp.inf).astype(F32)
    return keep, fill


def _kernel(x_hbm, m0_hbm, wq_hbm, wk_hbm, wv_hbm, wo_hbm, w1_hbm, w3_hbm, w2_hbm, c_hbm, wm_hbm,
            out_hbm,
            wqkv, wo, w1, w3, w2, wm, xb, cb, m0, mod, nrm, p32, pre, l32, ob, oda, abuf,
            h2, act, ost, keep_s, fill_s, sem, wsem, osem):
    w_hbm = [r.bitcast(U32) for r in (wq_hbm, wk_hbm, wv_hbm)]
    wm_u = wm_hbm.bitcast(U32)

    def pair_copies(m, j, dsem):
        return [pltpu.make_async_copy(w_hbm[m].at[:, par * NP + j, :], wqkv.at[m * H + 2 * j + par], dsem)
                for par in range(2)]

    def chunk_copies(t):
        m, c0 = divmod(t, H // CH)
        return [cp for jj in range(CH // 2)
                for cp in pair_copies(m, c0 * (CH // 2) + jj, wsem.at[t])]

    def wait_chunk(t):
        blk = wqkv.at[pl.ds(t * CH, CH)]
        pltpu.make_async_copy(blk, blk, wsem.at[t]).wait()

    def unzip(slot):
        for r in range(0, D // 2, 32):
            e, o = wqkv[slot, r:r + 32, :], wqkv[slot + 1, r:r + 32, :]
            wqkv[slot, r:r + 32, :] = (e & 0xFFFF) | (o << 16)
            wqkv[slot + 1, r:r + 32, :] = (e >> 16) | (o & jnp.uint32(0xFFFF0000))

    cp_c = pltpu.make_async_copy(c_hbm, cb, sem.at[0])
    cp_wm = {k: pltpu.make_async_copy(wm_u.at[:, k * D:(k + 1) * D], wm.at[k], sem.at[10 + k])
             for k in (0, 2, 3, 4, 5)}
    cp_wm1 = [pltpu.make_async_copy(wm_u.at[:, D + n:D + n + 512], wm.at[1, :, n:n + 512], sem.at[16 + n // 512])
              for n in (0, 512)]
    cp_p0 = [pair_copies(0, jj, sem.at[18 + jj]) for jj in range(CH // 2)]
    cp_xe = pltpu.make_async_copy(x_hbm.at[:, 0:EARLY, :], xb.at[:, 0:EARLY, :], sem.at[2])
    cp_m0 = pltpu.make_async_copy(m0_hbm, m0, sem.at[3])
    cp_xr = pltpu.make_async_copy(x_hbm.at[:, EARLY:SEG, :], xb.at[:, EARLY:SEG, :], sem.at[4])
    cp_wo = pltpu.make_async_copy(wo_hbm.bitcast(U32), wo, sem.at[5])
    cp_w1 = pltpu.make_async_copy(w1_hbm.bitcast(U32), w1, sem.at[7])
    cp_w3 = pltpu.make_async_copy(w3_hbm.bitcast(U32), w3, sem.at[8])
    cp_w2 = pltpu.make_async_copy(w2_hbm.bitcast(U32), w2, sem.at[9])

    cp_c.start()
    cp_xe.start()
    keep, fill = _attn_mask()
    keep_s[...] = keep.astype(jnp.int32)
    fill_s[...] = fill
    cp_c.wait()
    cp_wm[0].start()
    cf = cb[...].astype(F32)
    sc = jnp.broadcast_to(cf * jax.nn.sigmoid(cf), (16, D)).astype(BF16)
    cp_xe.wait()
    cp_wm1[0].start()
    for g in range(NSEG // 8):
        nrm[64 * g:64 * g + 64, :] = _norm(xb[8 * g:8 * g + 8, 0:EARLY, :].astype(F32).reshape(8 * EARLY, D))

    def mod_unit(k, n):
        mod[k, :, n:n + 512] = _dot(sc, _bf(wm[k, :, n:n + 512]))[0:8]

    def start_all(cps):
        for cp in cps:
            cp.start()

    def wait_all(cps):
        for cp in cps:
            cp.wait()

    cp_wm[0].wait()
    cp_wm1[1].start()
    mod_unit(0, 0)
    mod_unit(0, 512)
    cp_wm1[0].wait()
    start_all(cp_p0[0])
    mod_unit(1, 0)
    cp_wm1[1].wait()
    start_all(cp_p0[1])
    mod_unit(1, 512)

    def ln1_mod(n):
        return n * (1.0 + mod[1, 0:1, :]) + mod[0, 0:1, :]

    for g in range(NSEG // 8):
        p32[32 * g:32 * g + 32, :] = _pk(ln1_mod(nrm[64 * g:64 * g + 64, :]))

    def early_qkv(slot):
        wa, wb = _bf(wqkv[slot]), _bf(wqkv[slot + 1])
        for c in range(NEARLY // 128):
            lhs = _bf(p32[64 * c:64 * c + 64, :])
            a = _dot(lhs, wa).reshape(16, EARLY, DH)
            b = _dot(lhs, wb).reshape(16, EARLY, DH)
            pre[slot // 2, 16 * c:16 * c + 16] = _pk(jnp.concatenate([a, b], axis=1))

    wait_all(cp_p0[0])
    start_all(cp_p0[2] + cp_p0[3])
    unzip(0)
    early_qkv(0)
    wait_all(cp_p0[1])
    start_all(chunk_copies(1))
    unzip(2)
    early_qkv(2)
    wait_all(cp_p0[2] + cp_p0[3])
    start_all(chunk_copies(2) + [cp_m0])
    unzip(4)
    unzip(6)
    early_qkv(4)

    def early_run(slot0, npairs):
        unzip(slot0)
        for g in range(npairs):
            if g + 1 < npairs:
                unzip(slot0 + 2 * g + 2)
            early_qkv(slot0 + 2 * g)

    wait_chunk(1)
    start_all([cp for t in range(3, 8) for cp in chunk_copies(t)])
    early_qkv(6)
    early_run(CH, CH // 2)

    def prologue(r, carry):
        wait_chunk(2 * r)
        wait_chunk(2 * r + 1)

        @pl.when(r == 1)
        def _():
            start_all([cp for t in range(8, NCH) for cp in chunk_copies(t)])

        @pl.when(r == 2)
        def _():
            start_all([cp_xr, cp_wo] + [cp_wm[k] for k in range(2, 6)] + [cp_w1, cp_w3, cp_w2])

        early_run(2 * r * CH, CH)
        return carry

    with jax.named_scope('prologue'):
        lax.fori_loop(1, NCH // 2, prologue, 0)

    with jax.named_scope('wait1'):
        cp_m0.wait()
        cp_xr.wait()
        cp_wo.wait()
        for k in range(2, 6):
            cp_wm[k].wait()

    def next_lhs(mem_f32, s):
        hx = ln1_mod(_norm(xb[s, EARLY:SEG, :].astype(F32)))
        l32[...] = _pk(jnp.concatenate([mem_f32, hx], axis=0))

    next_lhs(m0[...].astype(F32), 0)

    def resid1(p, c0, c1):
        xf = xb[pl.ds(2 * p, 2), :, c0:c1].astype(F32).reshape(PR, c1 - c0)
        return xf + mod[2, 0:1, c0:c1] * abuf[p & (NRING - 1), :, c0:c1]

    def ln2(p, q):
        h2[q * SEG:(q + 1) * SEG, :] = _pk(_norm(resid1(p, 0, D)) * (1.0 + mod[4, 0:1, :]) + mod[3, 0:1, :])

    def gate_up_units(q0, q1, chunks):
        r0, r1 = q0 * SEG, q1 * SEG
        half = {}

        def gate(f0):
            half[f0] = 0.5 * _dot(_bf(h2[r0:r1, :]), _bf(w1[:, f0:f0 + 128]))

        def up(f0):
            t = half.pop(f0)
            u = _dot(_bf(h2[r0:r1, :]), _bf(w3[:, f0:f0 + 128]))
            act[r0:r1, f0:f0 + 128] = _pk((t + t * jnp.tanh(t)) * u)

        return [functools.partial(fn, 128 * ck) for ck in chunks for fn in (gate, up)]

    def down_units(p, npairs, nsplit):
        kq = F // nsplit
        acc = {}

        def down(n0, k):
            y = _dot(_bf(act[0:npairs * SEG, k * kq:(k + 1) * kq]),
                     _bf(w2[k * kq // 2:(k + 1) * kq // 2, n0:n0 + 128]))
            if k > 0:
                y = y + acc.pop(n0)
            if k + 1 < nsplit:
                acc[n0] = y
                return
            for q in range(npairs):
                res = resid1(p + q, n0, n0 + 128) + mod[5, 0:1, n0:n0 + 128] * y[q * PR:(q + 1) * PR]
                ost[pl.ds(2 * (p + q), 2), :, n0:n0 + 128] = res.astype(BF16).reshape(2, SEG, 128)

        return [functools.partial(down, n0, k) for n0 in range(0, D, 128) for k in range(nsplit)]

    def out_copy(p, npairs):
        rows = pl.ds(2 * p, 2 * npairs)
        return pltpu.make_async_copy(ost.at[rows], out_hbm.at[rows], osem)

    c_exp = SCALE * math.log2(math.e)
    nb = 256

    def step(s, second, fill):
        rows = SEG + 2 * EARLY if second else SEG
        lhs = _bf(l32[...])
        qkv, prob = {}, {}

        def project(j):
            out = []
            for m in range(3):
                a = _dot(lhs, _bf(wqkv[m * H + 2 * j])).astype(BF16)
                b = _dot(lhs, _bf(wqkv[m * H + 2 * j + 1])).astype(BF16)
                out.append(jnp.concatenate([a, b, _bf(pre[m * NP + j, s])], axis=0))
                fill(3 * j + m)
            qkv[j] = out

        def scores(j):
            q, k, _ = qkv[j]
            sc_ = lax.dot_general(q, k, (((1,), (1,)), ((), ())), preferred_element_type=F32)
            sc_ = jnp.where(keep_s[...] != 0, sc_, fill_s[...])
            e = jnp.exp2((sc_ - jnp.max(sc_, axis=1, keepdims=True)) * c_exp)
            den = jnp.sum(e, axis=1, keepdims=True)
            r = pl.reciprocal(den, approx=True)
            r = r * (2.0 - den * r)
            prob[j] = (e * r).astype(BF16)

        def values(j):
            o = _dot(prob.pop(j), qkv.pop(j)[2])
            for hh in range(2):
                c0 = (2 * j + hh) * DH
                main = o[hh * SEG:(hh + 1) * SEG]
                early = o[2 * SEG + hh * EARLY:2 * SEG + (hh + 1) * EARLY]
                if second:
                    ob[:, c0:c0 + DH] = _pk(jnp.concatenate([main, oda[:, c0:c0 + DH], early], axis=0))
                else:
                    ob[0:SEG // 2, c0:c0 + DH] = _pk(main)
                    oda[:, c0:c0 + DH] = early

        def wo_part(n, j0, j1):
            k0, k1 = j0 * 2 * DH, j1 * 2 * DH
            return _dot(_bf(ob[0:rows // 2, k0:k1]), _bf(wo[k0 // 2:k1 // 2, n * nb:(n + 1) * nb]))

        for j in range(NP):
            project(j)
            if j >= 1:
                scores(j - 1)
            if j >= 3:
                values(j - 3)
        y0 = wo_part(0, 0, 6)
        scores(NP - 1)
        values(NP - 3)
        y0 = y0 + wo_part(0, 6, 12)
        values(NP - 2)
        fill('mid')
        y1 = wo_part(1, 0, 8)
        values(NP - 1)
        y1 = y1 + wo_part(1, 8, 13)
        y2 = wo_part(2, 0, 14)
        y0 = y0 + wo_part(0, 12, NP)
        y1 = y1 + wo_part(1, 13, NP)
        y2 = y2 + wo_part(2, 14, NP)
        y = jnp.concatenate([y0, y1, y2, wo_part(3, 0, NP)], axis=1)
        next_lhs(y[0:MEM], jnp.minimum(s + 1, NSEG - 1))
        fill('end')
        return y

    def pair(i, units, counts):
        units = list(units)

        def filler(second):
            def fill(point):
                for _ in range(counts.get((second, point), 0)):
                    units.pop(0)()
            return fill

        slot = i & (NRING - 1)
        ya = step(2 * i, False, filler(False))
        abuf[slot, EARLY:SEG, :] = ya[MEM:SEG]
        yb = step(2 * i + 1, True, filler(True))
        abuf[slot, 0:EARLY, :] = yb[SEG:SEG + EARLY]
        abuf[slot, SEG:SEG + EARLY, :] = yb[SEG + EARLY:SEG + 2 * EARLY]
        abuf[slot, SEG + EARLY:PR, :] = yb[MEM:SEG]
        assert not units

    def head_pairs(i, carry):
        units = [functools.partial(mod_unit, 2 + 2 * i + kk, n) for kk in range(2) for n in (0, 512)]
        pair(i, units, {(False, 'mid'): 1, (False, 'end'): 2, (True, 'mid'): 1})
        return carry

    with jax.named_scope('head'):
        lax.fori_loop(0, LAG, head_pairs, 0)
    with jax.named_scope('wait2'):
        cp_w1.wait()
        cp_w3.wait()
        cp_w2.wait()
    ln2(0, 0)

    nf = F // 128
    counts = {(False, 'mid'): 2, (False, 'end'): 4, (True, 'mid'): 2, (True, 'end'): 5}
    n_inner = 2 * nf + 1 + 32 - sum(counts.values())
    for k in range(6 * NP):
        counts[(k >= 3 * NP, k % (3 * NP))] = (k + 1) * n_inner // (6 * NP) - k * n_inner // (6 * NP)

    def main_pairs(p, carry):
        @pl.when(p >= 1)
        def _():
            out_copy(p - 1, 1).start()

        units = gate_up_units(0, 1, range(nf))
        units.append(functools.partial(ln2, p + 1, 0))
        units += down_units(p, 1, 4)
        pair(p + LAG, units, counts)
        return carry

    with jax.named_scope('main'):
        lax.fori_loop(0, NPAIR - LAG, main_pairs, 0)

    p0 = NPAIR - LAG
    out_copy(p0 - 1, 1).start()
    ln2(p0 + 1, 1)
    units = gate_up_units(0, 1, range(2)) + gate_up_units(1, 2, range(2)) + gate_up_units(0, 2, range(2, nf))
    for unit in units + down_units(p0, LAG, 1):
        unit()
    out_copy(p0, LAG).start()
    out_copy(0, NPAIR).wait()


@functools.partial(jax.jit, static_argnames=("A_seg_len",))
def pallas_adaLN_cond__memory_aug_recurrent_mem_tr__glu_gated_swiglu__prompt_kernel(
    A_x, A_mem0, A_Wq, A_Wk, A_Wv, A_Wo, A_seg_len, B_x, B_w1, B_w3, B_w2, c, w_mod,
):
    assert int(A_seg_len) == SEG and A_x.shape == (1, S, D) and A_mem0.shape == (1, MEM, D)
    del B_x
    vm = pltpu.VMEM
    scratch = [
        vm((3 * H, D // 2, DH), U32),
        vm((HD // 2, D), U32),
        vm((D // 2, F), U32),
        vm((D // 2, F), U32),
        vm((F // 2, D), U32),
        vm((6, D // 2, D), U32),
        vm((NSEG, SEG, D), BF16),
        vm((1, D), BF16),
        vm((MEM, D), BF16),
        vm((6, 8, D), F32),
        vm((NEARLY, D), F32),
        vm((NEARLY // 2, D), U32),
        vm((3 * NP, NSEG, EARLY, DH), U32),
        vm((SEG // 2, D), U32),
        vm((SEG // 2 + EARLY, HD), U32),
        vm((EARLY, HD), F32),
        vm((NRING, PR, D), F32),
        vm((LAG * SEG, D), U32),
        vm((LAG * SEG, F), U32),
        vm((NSEG, SEG, D), BF16),
        vm((L2, L2), jnp.int32),
        vm((L2, L2), F32),
        pltpu.SemaphoreType.DMA((22,)),
        pltpu.SemaphoreType.DMA((NCH,)),
        pltpu.SemaphoreType.DMA(()),
    ]
    out = pl.pallas_call(
        _kernel,
        out_shape=jax.ShapeDtypeStruct((NSEG, SEG, D), BF16),
        in_specs=[pl.BlockSpec(memory_space=pl.ANY)] * 11,
        out_specs=pl.BlockSpec(memory_space=pl.ANY),
        scratch_shapes=scratch,
        compiler_params=pltpu.CompilerParams(vmem_limit_bytes=120 * 1024 * 1024,
                                             disable_bounds_checks=True,
                                             disable_semaphore_checks=True),
    )(
        A_x.reshape(NSEG, SEG, D),
        A_mem0.reshape(MEM, D),
        A_Wq.reshape(D // 2, 2 * H, DH),
        A_Wk.reshape(D // 2, 2 * H, DH),
        A_Wv.reshape(D // 2, 2 * H, DH),
        A_Wo.reshape(HD, D),
        B_w1, B_w3, B_w2, c, w_mod,
    )
    return out.reshape(1, S, D)
```

```python
import functools
import math

import jax
import jax.numpy as jnp
from jax import lax
import jax.experimental.pallas as pl
import jax.experimental.pallas.tpu as pltpu

S, D, H, DH, MEM, SEG, F = 2048, 1024, 32, 128, 8, 32, 3584
NSEG = S // SEG
NP = H // 2
HD = H * DH
EARLY = 8
NEARLY = NSEG * EARLY
L2 = 2 * (MEM + SEG)
CH = 8
NCH = 3 * H // CH
KS = CH
NPAIR = NSEG // 2
PR = 2 * SEG
LAG = 2
NRING = 4
EPS = 1e-5
SCALE = DH ** -0.5
MASK_FILL = -1000000000.0

BF16, F32, U32 = jnp.bfloat16, jnp.float32, jnp.uint32


def _bf(x_u32):
    return pltpu.bitcast(x_u32, BF16)


def _pk(x_f32):
    return pltpu.bitcast(x_f32.astype(BF16), U32)


def _dot(a, b):
    return jnp.dot(a, b, preferred_element_type=F32)


def _norm(x):
    m = jnp.mean(x, axis=-1, keepdims=True)
    xc = x - m
    v = jnp.mean(xc * xc, axis=-1, keepdims=True)
    return xc * lax.rsqrt(v + EPS)


def _attn_mask():
    def meta(i):
        head = jnp.where(i < 2 * SEG, i // SEG, (i - 2 * SEG) // EARLY)
        j = i % SEG
        pos = jnp.where(i < 2 * SEG, jnp.where(j < MEM, j, j + EARLY), MEM + (i - 2 * SEG) % EARLY)
        return head, pos
    r = lax.broadcasted_iota(jnp.int32, (L2, L2), 0)
    c = lax.broadcasted_iota(jnp.int32, (L2, L2), 1)
    rh, rp = meta(r)
    chd, cp = meta(c)
    same = rh == chd
    keep = same & ((rp < MEM) | (rp >= cp))
    fill = jnp.where(same, MASK_FILL / SCALE, -jnp.inf).astype(F32)
    return keep, fill


def _kernel(x_hbm, m0_hbm, wq_hbm, wk_hbm, wv_hbm, wo_hbm, w1_hbm, w3_hbm, w2_hbm, c_hbm, wm_hbm,
            out_hbm,
            wqkv, wo, w1, w3, w2, wm, xb, cb, m0, mod, nrm, p32, part, pre, l32, ob, oda, abuf,
            h2, act, ost, keep_s, fill_s, sem, wsem, osem):
    w_hbm = [r.bitcast(U32) for r in (wq_hbm, wk_hbm, wv_hbm)]
    wm_u = wm_hbm.bitcast(U32)

    def pair_copies(m, j, dsem, r0=0, r1=D // 2):
        return [pltpu.make_async_copy(w_hbm[m].at[r0:r1, par * NP + j, :],
                                      wqkv.at[m * H + 2 * j + par, r0:r1, :], dsem) for par in range(2)]

    def chunk_copies(t):
        m, c0 = divmod(t, H // CH)
        return [cp for jj in range(CH // 2)
                for cp in pair_copies(m, c0 * (CH // 2) + jj, wsem.at[t])]

    def wait_chunk(t):
        blk = wqkv.at[pl.ds(t * CH, CH)]
        pltpu.make_async_copy(blk, blk, wsem.at[t]).wait()

    def unzip(slot, r0=0, r1=D // 2):
        for r in range(r0, r1, 32):
            e, o = wqkv[slot, r:r + 32, :], wqkv[slot + 1, r:r + 32, :]
            wqkv[slot, r:r + 32, :] = (e & 0xFFFF) | (o << 16)
            wqkv[slot + 1, r:r + 32, :] = (e >> 16) | (o & jnp.uint32(0xFFFF0000))

    def start_all(cps):
        for cp in cps:
            cp.start()

    def wait_all(cps):
        for cp in cps:
            cp.wait()

    HK = D // 2
    cp_c = pltpu.make_async_copy(c_hbm, cb, sem.at[0])
    cp_xe = pltpu.make_async_copy(x_hbm.at[:, 0:EARLY, :], xb.at[:, 0:EARLY, :], sem.at[1])
    cp_x0 = pltpu.make_async_copy(x_hbm.at[0, EARLY:SEG, :], xb.at[0, EARLY:SEG, :], sem.at[2])
    cp_m0 = pltpu.make_async_copy(m0_hbm, m0, sem.at[3])
    cp_xr = pltpu.make_async_copy(x_hbm.at[1:NSEG, EARLY:SEG, :], xb.at[1:NSEG, EARLY:SEG, :], sem.at[4])
    cp_wo = pltpu.make_async_copy(wo_hbm.bitcast(U32), wo, sem.at[5])
    cp_w1 = pltpu.make_async_copy(w1_hbm.bitcast(U32), w1, sem.at[6])
    cp_w3 = pltpu.make_async_copy(w3_hbm.bitcast(U32), w3, sem.at[7])
    cp_w2 = pltpu.make_async_copy(w2_hbm.bitcast(U32), w2, sem.at[8])
    cp_wm = [pltpu.make_async_copy(wm_u.at[:, k * D:(k + 1) * D], wm.at[k], sem.at[7 + k])
             for k in range(2, 6)]
    cp_wa = [[pltpu.make_async_copy(wm_u.at[:, k * D + hf * HK:k * D + (hf + 1) * HK],
                                    wm.at[k, :, hf * HK:(hf + 1) * HK], sem.at[13 + 2 * hf + k])
              for k in range(2)] for hf in range(2)]
    cp_ks = [[[cp for j in (2 * g, 2 * g + 1)
               for cp in pair_copies(0, j, sem.at[17 + hf * (KS // 2) + g], hf * HK // 2, (hf + 1) * HK // 2)]
              for g in range(KS // 2)] for hf in range(2)]

    start_all([cp_xe, cp_c, cp_x0, cp_m0] + cp_wa[0])
    keep, fill = _attn_mask()
    keep_s[...] = keep.astype(jnp.int32)
    fill_s[...] = fill
    wait_all([cp_xe, cp_c, cp_x0, cp_m0])
    start_all(cp_ks[0][0] + cp_ks[0][1])
    cf = cb[...].astype(F32)
    sc16 = jnp.broadcast_to(cf * jax.nn.sigmoid(cf), (16, D)).astype(BF16)
    for g in range(NSEG // 8):
        nrm[64 * g:64 * g + 64, :] = _norm(xb[8 * g:8 * g + 8, 0:EARLY, :].astype(F32).reshape(8 * EARLY, D))

    def mod_unit(k, c0, c1):
        mod[k, :, c0:c1] = _dot(sc16, _bf(wm[k, :, c0:c1]))[0:8]

    def ln1_mod(n, c0=0, c1=D):
        return n * (1.0 + mod[1, 0:1, c0:c1]) + mod[0, 0:1, c0:c1]

    def next_lhs(mem_f32, s):
        hx = ln1_mod(_norm(xb[s, EARLY:SEG, :].astype(F32)))
        l32[...] = _pk(jnp.concatenate([mem_f32, hx], axis=0))

    def ln1_half(hf, issue):
        c0, c1 = hf * HK, (hf + 1) * HK
        for k in range(2):
            cp_wa[hf][k].wait()
            start_all(issue[k])
            mod_unit(k, c0, c1)
        for g in range(NSEG // 8):
            p32[32 * g:32 * g + 32, c0:c1] = _pk(ln1_mod(nrm[64 * g:64 * g + 64, c0:c1], c0, c1))

    def early_dot(head, c, hf=None):
        c0, c1 = (0, D) if hf is None else (hf * HK, (hf + 1) * HK)
        return _dot(_bf(p32[64 * c:64 * c + 64, c0:c1]), _bf(wqkv[head, c0 // 2:c1 // 2, :]))

    def early_store(slot, c, ab):
        pre[slot // 2, 16 * c:16 * c + 16] = _pk(
            jnp.concatenate([v.reshape(16, EARLY, DH) for v in ab], axis=1))

    def early_block(slot, c, hf=None):
        ab = [early_dot(slot + hh, c, hf) for hh in range(2)]
        if hf == 0:
            for hh in range(2):
                part[slot + hh, 128 * c:128 * c + 128, :] = ab[hh]
            return
        if hf == 1:
            ab = [ab[hh] + part[slot + hh, 128 * c:128 * c + 128, :] for hh in range(2)]
        early_store(slot, c, ab)

    def early_run(slot0, npairs, hf=None, blocks=range(NEARLY // 128)):
        rows = (0, D // 2) if hf is None else (hf * HK // 2, (hf + 1) * HK // 2)
        unzip(slot0, *rows)
        for g in range(npairs):
            if g + 1 < npairs:
                unzip(slot0 + 2 * g + 2, *rows)
            for c in blocks:
                early_block(slot0 + 2 * g, c, hf)

    ln1_half(0, [cp_ks[0][2] + cp_ks[0][3], cp_wa[1]])
    for g0, g1, issue in ((0, 1, cp_ks[1][0] + cp_ks[1][1]), (1, 2, cp_ks[1][2] + cp_ks[1][3]),
                          (2, 4, chunk_copies(2))):
        wait_all([cp for g in range(g0, g1) for cp in cp_ks[0][g]])
        start_all(issue)
        early_run(4 * g0, 2 * (g1 - g0), 0)
    ln1_half(1, [chunk_copies(3), chunk_copies(4)])
    next_lhs(m0[...].astype(F32), 0)
    for g0, g1, issue in ((0, 1, chunk_copies(5) + chunk_copies(6)), (1, 4, [])):
        wait_all([cp for g in range(g0, g1) for cp in cp_ks[1][g]])
        start_all(issue)
        early_run(4 * g0, 2 * (g1 - g0), 1)
    wait_chunk(2)
    start_all([cp for t in range(7, NCH) for cp in chunk_copies(t)])
    early_run(2 * CH, CH // 2)

    def prologue(r, carry):
        wait_chunk(2 * r + 1)
        wait_chunk(2 * r + 2)

        @pl.when(r == 1)
        def _():
            start_all([cp_xr, cp_wo] + cp_wm + [cp_w1, cp_w3, cp_w2])

        early_run((2 * r + 1) * CH, CH)
        return carry

    with jax.named_scope('prologue'):
        lax.fori_loop(1, NCH // 2 - 1, prologue, 0)

    wait_chunk(NCH - 1)
    wait_all([cp_xr, cp_wo])
    early_run((NCH - 1) * CH, CH // 2, blocks=(0,))

    def resid1(p, c0, c1):
        xf = xb[pl.ds(2 * p, 2), :, c0:c1].astype(F32).reshape(PR, c1 - c0)
        return xf + mod[2, 0:1, c0:c1] * abuf[p & (NRING - 1), :, c0:c1]

    def ln2(p, q):
        h2[q * SEG:(q + 1) * SEG, :] = _pk(_norm(resid1(p, 0, D)) * (1.0 + mod[4, 0:1, :]) + mod[3, 0:1, :])

    def gate_up_units(q0, q1, chunks):
        r0, r1 = q0 * SEG, q1 * SEG
        half = {}

        def gate(f0):
            half[f0] = 0.5 * _dot(_bf(h2[r0:r1, :]), _bf(w1[:, f0:f0 + 128]))

        def up(f0):
            t = half.pop(f0)
            u = _dot(_bf(h2[r0:r1, :]), _bf(w3[:, f0:f0 + 128]))
            act[r0:r1, f0:f0 + 128] = _pk((t + t * jnp.tanh(t)) * u)

        return [functools.partial(fn, 128 * ck) for ck in chunks for fn in (gate, up)]

    def down_units(p, npairs, nsplit):
        kq = F // nsplit
        acc = {}

        def down(n0, k):
            y = _dot(_bf(act[0:npairs * SEG, k * kq:(k + 1) * kq]),
                     _bf(w2[k * kq // 2:(k + 1) * kq // 2, n0:n0 + 128]))
            if k > 0:
                y = y + acc.pop(n0)
            if k + 1 < nsplit:
                acc[n0] = y
                return
            for q in range(npairs):
                res = resid1(p + q, n0, n0 + 128) + mod[5, 0:1, n0:n0 + 128] * y[q * PR:(q + 1) * PR]
                ost[pl.ds(2 * (p + q), 2), :, n0:n0 + 128] = res.astype(BF16).reshape(2, SEG, 128)

        return [functools.partial(down, n0, k) for n0 in range(0, D, 128) for k in range(nsplit)]

    def out_copy(p, npairs):
        rows = pl.ds(2 * p, 2 * npairs)
        return pltpu.make_async_copy(ost.at[rows], out_hbm.at[rows], osem)

    c_exp = SCALE * math.log2(math.e)
    nb = 256

    def step(s, second, fill):
        rows = SEG + 2 * EARLY if second else SEG
        lhs = _bf(l32[...])
        qkv, prob = {}, {}

        def project(j):
            out = []
            for m in range(3):
                a = _dot(lhs, _bf(wqkv[m * H + 2 * j])).astype(BF16)
                b = _dot(lhs, _bf(wqkv[m * H + 2 * j + 1])).astype(BF16)
                out.append(jnp.concatenate([a, b, _bf(pre[m * NP + j, s])], axis=0))
                fill(3 * j + m)
            qkv[j] = out

        def scores(j):
            q, k, _ = qkv[j]
            sc_ = lax.dot_general(q, k, (((1,), (1,)), ((), ())), preferred_element_type=F32)
            sc_ = jnp.where(keep_s[...] != 0, sc_, fill_s[...])
            e = jnp.exp2((sc_ - jnp.max(sc_, axis=1, keepdims=True)) * c_exp)
            den = jnp.sum(e, axis=1, keepdims=True)
            r = pl.reciprocal(den, approx=True)
            r = r * (2.0 - den * r)
            prob[j] = (e * r).astype(BF16)

        def values(j):
            o = _dot(prob.pop(j), qkv.pop(j)[2])
            for hh in range(2):
                c0 = (2 * j + hh) * DH
                main = o[hh * SEG:(hh + 1) * SEG]
                early = o[2 * SEG + hh * EARLY:2 * SEG + (hh + 1) * EARLY]
                if second:
                    ob[:, c0:c0 + DH] = _pk(jnp.concatenate([main, oda[:, c0:c0 + DH], early], axis=0))
                else:
                    ob[0:SEG // 2, c0:c0 + DH] = _pk(main)
                    oda[:, c0:c0 + DH] = early

        def wo_part(n, j0, j1):
            k0, k1 = j0 * 2 * DH, j1 * 2 * DH
            return _dot(_bf(ob[0:rows // 2, k0:k1]), _bf(wo[k0 // 2:k1 // 2, n * nb:(n + 1) * nb]))

        for j in range(NP):
            project(j)
            if j >= 1:
                scores(j - 1)
            if j >= 3:
                values(j - 3)
        y0 = wo_part(0, 0, 6)
        scores(NP - 1)
        values(NP - 3)
        y0 = y0 + wo_part(0, 6, 12)
        values(NP - 2)
        fill('mid')
        y1 = wo_part(1, 0, 8)
        values(NP - 1)
        y1 = y1 + wo_part(1, 8, 13)
        y2 = wo_part(2, 0, 14)
        y0 = y0 + wo_part(0, 12, NP)
        y1 = y1 + wo_part(1, 13, NP)
        y2 = y2 + wo_part(2, 14, NP)
        y = jnp.concatenate([y0, y1, y2, wo_part(3, 0, NP)], axis=1)
        next_lhs(y[0:MEM], jnp.minimum(s + 1, NSEG - 1))
        fill('end')
        return y

    def pair(i, units, counts):
        units = list(units)

        def filler(second):
            def fill(point):
                for _ in range(counts.get((second, point), 0)):
                    units.pop(0)()
            return fill

        slot = i & (NRING - 1)
        ya = step(2 * i, False, filler(False))
        abuf[slot, EARLY:SEG, :] = ya[MEM:SEG]
        yb = step(2 * i + 1, True, filler(True))
        abuf[slot, 0:EARLY, :] = yb[SEG:SEG + EARLY]
        abuf[slot, SEG:SEG + EARLY, :] = yb[SEG + EARLY:SEG + 2 * EARLY]
        abuf[slot, SEG + EARLY:PR, :] = yb[MEM:SEG]
        assert not units

    def head_pairs(i, carry):
        for kk in range(2):
            k = 2 + 2 * i + kk
            pltpu.make_async_copy(wm.at[k], wm.at[k], sem.at[7 + k]).wait()
        mods = [functools.partial(mod_unit, 2 + 2 * i + kk, n0, n0 + 128)
                for kk in range(2) for n0 in range(0, D, 128)]
        slot0 = (NCH - 1) * CH + 4 * i
        units = []
        for g in range(2):
            for c in range(1, 4):
                held = []
                units += [lambda g=g, c=c, held=held: held.append(early_dot(slot0 + 2 * g, c)), mods.pop(),
                          lambda g=g, c=c, held=held: held.append(early_dot(slot0 + 2 * g + 1, c)), mods.pop(),
                          lambda g=g, c=c, held=held: early_store(slot0 + 2 * g, c, held)]
            if g == 0:
                units += [mods.pop() for _ in range(4)]
        units.append(functools.partial(ln2, 0, 0))
        pair(i, units, {(False, 6): 2, (False, 13): 3, (False, 20): 2, (False, 27): 3, (False, 34): 2,
                        (False, 41): 3, (False, 'end'): 4,
                        (True, 6): 2, (True, 13): 3, (True, 20): 2, (True, 27): 3, (True, 34): 2,
                        (True, 41): 4})
        return carry

    with jax.named_scope('head'):
        lax.fori_loop(0, LAG, head_pairs, 0)
    with jax.named_scope('wait2'):
        wait_all([cp_w1, cp_w3, cp_w2])

    nf = F // 128
    counts = {(False, 'mid'): 2, (False, 'end'): 4, (True, 'mid'): 2, (True, 'end'): 5}
    n_inner = 2 * nf + 1 + 32 - sum(counts.values())
    for k in range(6 * NP):
        counts[(k >= 3 * NP, k % (3 * NP))] = (k + 1) * n_inner // (6 * NP) - k * n_inner // (6 * NP)

    def main_pairs(p, carry):
        @pl.when(p >= 1)
        def _():
            out_copy(p - 1, 1).start()

        units = gate_up_units(0, 1, range(nf))
        units.append(functools.partial(ln2, p + 1, 0))
        units += down_units(p, 1, 4)
        pair(p + LAG, units, counts)
        return carry

    with jax.named_scope('main'):
        lax.fori_loop(0, NPAIR - LAG, main_pairs, 0)

    p0 = NPAIR - LAG
    out_copy(p0 - 1, 1).start()
    ln2(p0 + 1, 1)
    units = gate_up_units(0, 1, range(2)) + gate_up_units(1, 2, range(2)) + gate_up_units(0, 2, range(2, nf))
    for unit in units + down_units(p0, LAG, 1):
        unit()
    out_copy(p0, LAG).start()
    out_copy(0, NPAIR).wait()


@jax.jit
def pallas_adaLN_cond__memory_aug_recurrent_mem_tr__glu_gated_swiglu__prompt_kernel(
    A_x, A_mem0, A_Wq, A_Wk, A_Wv, A_Wo, A_seg_len, B_x, B_w1, B_w3, B_w2, c, w_mod,
):
    assert A_x.shape == (1, S, D) and A_mem0.shape == (1, MEM, D)
    del A_seg_len
    del B_x
    vm = pltpu.VMEM
    scratch = [
        vm((3 * H, D // 2, DH), U32),
        vm((HD // 2, D), U32),
        vm((D // 2, F), U32),
        vm((D // 2, F), U32),
        vm((F // 2, D), U32),
        vm((6, D // 2, D), U32),
        vm((NSEG, SEG, D), BF16),
        vm((1, D), BF16),
        vm((MEM, D), BF16),
        vm((6, 8, D), F32),
        vm((NEARLY, D), F32),
        vm((NEARLY // 2, D), U32),
        vm((2 * KS, NEARLY, DH), F32),
        vm((3 * NP, NSEG, EARLY, DH), U32),
        vm((SEG // 2, D), U32),
        vm((SEG // 2 + EARLY, HD), U32),
        vm((EARLY, HD), F32),
        vm((NRING, PR, D), F32),
        vm((LAG * SEG, D), U32),
        vm((LAG * SEG, F), U32),
        vm((NSEG, SEG, D), BF16),
        vm((L2, L2), jnp.int32),
        vm((L2, L2), F32),
        pltpu.SemaphoreType.DMA((17 + KS,)),
        pltpu.SemaphoreType.DMA((NCH,)),
        pltpu.SemaphoreType.DMA(()),
    ]
    out = pl.pallas_call(
        _kernel,
        out_shape=jax.ShapeDtypeStruct((NSEG, SEG, D), BF16),
        in_specs=[pl.BlockSpec(memory_space=pl.ANY)] * 11,
        out_specs=pl.BlockSpec(memory_space=pl.ANY),
        scratch_shapes=scratch,
        compiler_params=pltpu.CompilerParams(vmem_limit_bytes=120 * 1024 * 1024,
                                             disable_bounds_checks=True,
                                             disable_semaphore_checks=True),
    )(
        A_x.reshape(NSEG, SEG, D),
        A_mem0.reshape(MEM, D),
        A_Wq.reshape(D // 2, 2 * H, DH),
        A_Wk.reshape(D // 2, 2 * H, DH),
        A_Wv.reshape(D // 2, 2 * H, DH),
        A_Wo.reshape(HD, D),
        B_w1, B_w3, B_w2, c, w_mod,
    )
    return out.reshape(1, S, D)
```

```python
import functools
import math

import jax
import jax.numpy as jnp
from jax import lax
import jax.experimental.pallas as pl
import jax.experimental.pallas.tpu as pltpu

S, D, H, DH, MEM, SEG, F = 2048, 1024, 32, 128, 8, 32, 3584
NSEG = S // SEG
NP = H // 2
HD = H * DH
EARLY = 8
NEARLY = NSEG * EARLY
L2 = 2 * (MEM + SEG)
CH = 8
NCH = 3 * H // CH
KS = CH
NPAIR = NSEG // 2
PR = 2 * SEG
LAG = 2
EPS = 1e-5
SCALE = DH ** -0.5
MASK_FILL = -1000000000.0

BF16, F32, U32 = jnp.bfloat16, jnp.float32, jnp.uint32


def _bf(x_u32):
    return pltpu.bitcast(x_u32, BF16)


def _pk(x_f32):
    return pltpu.bitcast(x_f32.astype(BF16), U32)


def _dot(a, b):
    return jnp.dot(a, b, preferred_element_type=F32)


def _affine(x, scale8, shift8=None):
    y = x.reshape(-1, 8, x.shape[-1]) * scale8[None]
    if shift8 is not None:
        y = y + shift8[None]
    return y.reshape(x.shape)


def _norm(x):
    m = jnp.mean(x, axis=-1, keepdims=True)
    xc = x - m
    v = jnp.mean(xc * xc, axis=-1, keepdims=True)
    return xc * lax.rsqrt(v + EPS)


def _attn_mask():
    def meta(i):
        head = jnp.where(i < 2 * SEG, i // SEG, (i - 2 * SEG) // EARLY)
        j = i % SEG
        pos = jnp.where(i < 2 * SEG, jnp.where(j < MEM, j, j + EARLY), MEM + (i - 2 * SEG) % EARLY)
        return head, pos
    r = lax.broadcasted_iota(jnp.int32, (L2, L2), 0)
    c = lax.broadcasted_iota(jnp.int32, (L2, L2), 1)
    rh, rp = meta(r)
    chd, cp = meta(c)
    same = rh == chd
    keep = same & ((rp < MEM) | (rp >= cp))
    fill = jnp.where(same, MASK_FILL / SCALE, -jnp.inf).astype(F32)
    return keep, fill


def _kernel(x_hbm, m0_hbm, wq_hbm, wk_hbm, wv_hbm, wo_hbm, w1_hbm, w3_hbm, w2_hbm, c_hbm, wm_hbm,
            out_hbm,
            wqkv, wo, w1, w3, w2, wm, xb, cb, m0, mod, nrm, p32, part, pre, l32, ob, oda, abuf,
            x1n, x1c, h2, act, ost, keep_s, fill_s, sem, wsem, osem):
    w_hbm = [r.bitcast(U32) for r in (wq_hbm, wk_hbm, wv_hbm)]
    wm_u = wm_hbm.bitcast(U32)

    def pair_copies(m, j, dsem, r0=0, r1=D // 2):
        return [pltpu.make_async_copy(w_hbm[m].at[r0:r1, par * NP + j, :],
                                      wqkv.at[m * H + 2 * j + par, r0:r1, :], dsem) for par in range(2)]

    def chunk_copies(t):
        m, c0 = divmod(t, H // CH)
        return [cp for jj in range(CH // 2)
                for cp in pair_copies(m, c0 * (CH // 2) + jj, wsem.at[t])]

    def wait_chunk(t):
        blk = wqkv.at[pl.ds(t * CH, CH)]
        pltpu.make_async_copy(blk, blk, wsem.at[t]).wait()

    def unzip(slot, r0=0, r1=D // 2):
        for r in range(r0, r1, 32):
            e, o = wqkv[slot, r:r + 32, :], wqkv[slot + 1, r:r + 32, :]
            wqkv[slot, r:r + 32, :] = (e & 0xFFFF) | (o << 16)
            wqkv[slot + 1, r:r + 32, :] = (e >> 16) | (o & jnp.uint32(0xFFFF0000))

    def start_all(cps):
        for cp in cps:
            cp.start()

    def wait_all(cps):
        for cp in cps:
            cp.wait()

    HK = D // 2
    cp_c = pltpu.make_async_copy(c_hbm, cb, sem.at[0])
    cp_xe = pltpu.make_async_copy(x_hbm.at[:, 0:EARLY, :], xb.at[:, 0:EARLY, :], sem.at[1])
    cp_x0 = pltpu.make_async_copy(x_hbm.at[0, EARLY:SEG, :], xb.at[0, EARLY:SEG, :], sem.at[2])
    cp_m0 = pltpu.make_async_copy(m0_hbm, m0, sem.at[3])
    cp_xr = pltpu.make_async_copy(x_hbm.at[1:NSEG, EARLY:SEG, :], xb.at[1:NSEG, EARLY:SEG, :], sem.at[4])
    cp_wo = pltpu.make_async_copy(wo_hbm.bitcast(U32), wo, sem.at[5])
    cp_w1 = pltpu.make_async_copy(w1_hbm.bitcast(U32), w1, sem.at[6])
    cp_w3 = pltpu.make_async_copy(w3_hbm.bitcast(U32), w3, sem.at[7])
    cp_w2 = pltpu.make_async_copy(w2_hbm.bitcast(U32), w2, sem.at[8])
    cp_wm = [pltpu.make_async_copy(wm_u.at[:, k * D:(k + 1) * D], wm.at[k], sem.at[7 + k])
             for k in range(2, 6)]
    cp_wa = [[pltpu.make_async_copy(wm_u.at[:, k * D + hf * HK:k * D + (hf + 1) * HK],
                                    wm.at[k, :, hf * HK:(hf + 1) * HK], sem.at[13 + 2 * hf + k])
              for k in range(2)] for hf in range(2)]
    cp_ks = [[[cp for j in (2 * g, 2 * g + 1)
               for cp in pair_copies(0, j, sem.at[17 + hf * (KS // 2) + g], hf * HK // 2, (hf + 1) * HK // 2)]
              for g in range(KS // 2)] for hf in range(2)]

    start_all([cp_xe, cp_c, cp_x0, cp_m0] + cp_wa[0])
    keep, fill = _attn_mask()
    keep_s[...] = keep.astype(jnp.int32)
    fill_s[...] = fill
    wait_all([cp_xe, cp_c, cp_x0, cp_m0])
    start_all(cp_ks[0][0])
    cf = cb[...].astype(F32)
    sc16 = jnp.broadcast_to(cf * jax.nn.sigmoid(cf), (16, D)).astype(BF16)
    for g in range(NSEG // 8):
        nrm[64 * g:64 * g + 64, :] = _norm(xb[8 * g:8 * g + 8, 0:EARLY, :].astype(F32).reshape(8 * EARLY, D))

    def mod_unit(k, c0, c1):
        mod[k, :, c0:c1] = _dot(sc16, _bf(wm[k, :, c0:c1]))[0:8]

    def ln1_mod(n, c0=0, c1=D):
        return _affine(n, 1.0 + mod[1, :, c0:c1], mod[0, :, c0:c1])

    def next_lhs(mem_f32, s):
        hx = ln1_mod(_norm(xb[s, EARLY:SEG, :].astype(F32)))
        l32[...] = _pk(jnp.concatenate([mem_f32, hx], axis=0))

    def ln1_early(hf):
        c0, c1 = hf * HK, (hf + 1) * HK
        for n in range(c0, c1, 128):
            for g in range(NEARLY // 128):
                p32[64 * g:64 * g + 64, n:n + 128] = _pk(ln1_mod(nrm[128 * g:128 * g + 128, n:n + 128], n, n + 128))

    def early_dot(head, c, hf=None):
        c0, c1 = (0, D) if hf is None else (hf * HK, (hf + 1) * HK)
        return _dot(_bf(p32[64 * c:64 * c + 64, c0:c1]), _bf(wqkv[head, c0 // 2:c1 // 2, :]))

    def early_store(slot, c, ab):
        pre[slot // 2, 16 * c:16 * c + 16] = _pk(
            jnp.concatenate([v.reshape(16, EARLY, DH) for v in ab], axis=1))

    def early_block(slot, c, hf=None):
        ab = [early_dot(slot + hh, c, hf) for hh in range(2)]
        if hf == 0:
            for hh in range(2):
                part[slot + hh, 128 * c:128 * c + 128, :] = ab[hh]
            return
        if hf == 1:
            ab = [ab[hh] + part[slot + hh, 128 * c:128 * c + 128, :] for hh in range(2)]
        early_store(slot, c, ab)

    def early_run(slot0, npairs, hf=None, blocks=range(NEARLY // 128)):
        rows = (0, D // 2) if hf is None else (hf * HK // 2, (hf + 1) * HK // 2)
        unzip(slot0, *rows)
        for g in range(npairs):
            if g + 1 < npairs:
                unzip(slot0 + 2 * g + 2, *rows)
            for c in blocks:
                early_block(slot0 + 2 * g, c, hf)

    for k, issue in enumerate((cp_ks[0][1], cp_ks[0][2] + cp_wa[1])):
        cp_wa[0][k].wait()
        start_all(issue)
        mod_unit(k, 0, HK)
    ln1_early(0)
    for g, issue in enumerate((cp_ks[0][3], cp_ks[1][0] + cp_ks[1][1], cp_ks[1][2] + cp_ks[1][3])):
        wait_all(cp_ks[0][g])
        start_all(issue)
        early_run(4 * g, 2, 0)
    wait_all(cp_ks[0][3] + cp_wa[1])
    start_all(chunk_copies(2) + chunk_copies(3))
    unzip(12, 0, HK // 2)
    unzip(14, 0, HK // 2)
    for u in range(8):
        early_block(12 + 2 * (u // 4), u % 4, 0)
        if u < 4:
            for k in range(2):
                mod_unit(k, HK + 128 * u, HK + 128 * (u + 1))
    ln1_early(1)
    next_lhs(m0[...].astype(F32), 0)
    wait_all(cp_ks[1][0] + cp_ks[1][1])
    start_all(chunk_copies(4) + chunk_copies(5) + chunk_copies(6))
    early_run(0, 4, 1)
    wait_all(cp_ks[1][2] + cp_ks[1][3])
    early_run(8, 4, 1)
    wait_chunk(2)
    start_all([cp for t in range(7, NCH) for cp in chunk_copies(t)])
    early_run(2 * CH, CH // 2)

    def prologue(r, carry):
        wait_chunk(2 * r + 1)
        wait_chunk(2 * r + 2)

        @pl.when(r == 1)
        def _():
            start_all([cp_xr, cp_wo] + cp_wm + [cp_w1, cp_w3, cp_w2])

        early_run((2 * r + 1) * CH, CH)
        return carry

    with jax.named_scope('prologue'):
        lax.fori_loop(1, NCH // 2 - 1, prologue, 0)

    wait_chunk(NCH - 1)
    wait_all([cp_xr, cp_wo])
    early_run((NCH - 1) * CH, CH // 2, blocks=(0,))

    def resid1(p, dst):
        for n in range(0, D, 256):
            xf = xb[pl.ds(2 * p, 2), :, n:n + 256].astype(F32).reshape(PR, 256)
            dst[:, n:n + 256] = xf + _affine(abuf[:, n:n + 256], mod[2, :, n:n + 256])

    def advance(p):
        x1c[...] = x1n[...]
        resid1(p, x1n)

    def ln2(src, q):
        h2[q * SEG:(q + 1) * SEG, :] = _pk(_affine(_norm(src[...]), 1.0 + mod[4], mod[3]))

    def gate_up_units(q0, q1, chunks):
        r0, r1 = q0 * SEG, q1 * SEG
        half = {}

        def gate(f0):
            half[f0] = 0.5 * _dot(_bf(h2[r0:r1, :]), _bf(w1[:, f0:f0 + 128]))

        def up(f0):
            t = half.pop(f0)
            u = _dot(_bf(h2[r0:r1, :]), _bf(w3[:, f0:f0 + 128]))
            act[r0:r1, f0:f0 + 128] = _pk((t + t * jnp.tanh(t)) * u)

        return [functools.partial(fn, 128 * ck) for ck in chunks for fn in (gate, up)]

    def down_units(p, q, x1, nsplit):
        kq = F // nsplit
        acc = {}

        def down(n0, k):
            y = _dot(_bf(act[q * SEG:(q + 1) * SEG, k * kq:(k + 1) * kq]),
                     _bf(w2[k * kq // 2:(k + 1) * kq // 2, n0:n0 + 128]))
            if k > 0:
                y = y + acc.pop(n0)
            if k + 1 < nsplit:
                acc[n0] = y
                return
            res = x1[:, n0:n0 + 128] + _affine(y, mod[5, :, n0:n0 + 128])
            ost[pl.ds(2 * p, 2), :, n0:n0 + 128] = res.astype(BF16).reshape(2, SEG, 128)

        return [functools.partial(down, n0, k) for n0 in range(0, D, 128) for k in range(nsplit)]

    def out_copy(p, npairs):
        rows = pl.ds(2 * p, 2 * npairs)
        return pltpu.make_async_copy(ost.at[rows], out_hbm.at[rows], osem)

    c_exp = SCALE * math.log2(math.e)
    nb = 256

    def step(s, second, fill):
        rows = SEG + 2 * EARLY if second else SEG
        lhs = _bf(l32[...])
        qkv, prob = {}, {}

        def project(j):
            out = []
            for m in range(3):
                a = _dot(lhs, _bf(wqkv[m * H + 2 * j])).astype(BF16)
                b = _dot(lhs, _bf(wqkv[m * H + 2 * j + 1])).astype(BF16)
                out.append(jnp.concatenate([a, b, _bf(pre[m * NP + j, s])], axis=0))
                fill(3 * j + m)
            qkv[j] = out

        def scores(j):
            q, k, _ = qkv[j]
            sc_ = lax.dot_general(q, k, (((1,), (1,)), ((), ())), preferred_element_type=F32)
            sc_ = jnp.where(keep_s[...] != 0, sc_, fill_s[...])
            e = jnp.exp2((sc_ - jnp.max(sc_, axis=1, keepdims=True)) * c_exp)
            den = jnp.sum(e, axis=1, keepdims=True)
            r = pl.reciprocal(den, approx=True)
            r = r * (2.0 - den * r)
            prob[j] = (e * r).astype(BF16)

        def values(j):
            o = _dot(prob.pop(j), qkv.pop(j)[2])
            for hh in range(2):
                c0 = (2 * j + hh) * DH
                main = o[hh * SEG:(hh + 1) * SEG]
                early = o[2 * SEG + hh * EARLY:2 * SEG + (hh + 1) * EARLY]
                if second:
                    ob[:, c0:c0 + DH] = _pk(jnp.concatenate([main, oda[:, c0:c0 + DH], early], axis=0))
                else:
                    ob[0:SEG // 2, c0:c0 + DH] = _pk(main)
                    oda[:, c0:c0 + DH] = early

        def wo_part(n, j0, j1):
            k0, k1 = j0 * 2 * DH, j1 * 2 * DH
            return _dot(_bf(ob[0:rows // 2, k0:k1]), _bf(wo[k0 // 2:k1 // 2, n * nb:(n + 1) * nb]))

        for j in range(NP):
            project(j)
            if j >= 1:
                scores(j - 1)
            if j >= 3:
                values(j - 3)
        y0 = wo_part(0, 0, 6)
        scores(NP - 1)
        values(NP - 3)
        y0 = y0 + wo_part(0, 6, 12)
        values(NP - 2)
        fill('mid')
        y1 = wo_part(1, 0, 8)
        values(NP - 1)
        y1 = y1 + wo_part(1, 8, 13)
        y2 = wo_part(2, 0, 14)
        y0 = y0 + wo_part(0, 12, NP)
        y1 = y1 + wo_part(1, 13, NP)
        y2 = y2 + wo_part(2, 14, NP)
        y = jnp.concatenate([y0, y1, y2, wo_part(3, 0, NP)], axis=1)
        next_lhs(y[0:MEM], jnp.minimum(s + 1, NSEG - 1))
        fill('end')
        return y

    def pair(i, units, counts):
        units = list(units)

        def filler(second):
            def fill(point):
                for _ in range(counts.get((second, point), 0)):
                    units.pop(0)()
            return fill

        advance(jnp.maximum(i - 1, 0))
        ya = step(2 * i, False, filler(False))
        abuf[EARLY:SEG, :] = ya[MEM:SEG]
        yb = step(2 * i + 1, True, filler(True))
        abuf[0:EARLY, :] = yb[SEG:SEG + EARLY]
        abuf[SEG:SEG + EARLY, :] = yb[SEG + EARLY:SEG + 2 * EARLY]
        abuf[SEG + EARLY:PR, :] = yb[MEM:SEG]
        assert not units

    def head_pairs(i, carry):
        for kk in range(2):
            k = 2 + 2 * i + kk
            pltpu.make_async_copy(wm.at[k], wm.at[k], sem.at[7 + k]).wait()
        mods = [functools.partial(mod_unit, 2 + 2 * i + kk, n0, n0 + 128)
                for kk in range(2) for n0 in range(0, D, 128)]
        slot0 = (NCH - 1) * CH + 4 * i
        held = {}

        def piece(slot, c, hh, hf):
            v = early_dot(slot + hh, c, hf)
            held[hh] = v if hf == 0 else v + held[hh]
            if hh == 1 and hf == 1:
                early_store(slot, c, [held.pop(0), held.pop(1)])

        units, counts = [], {}
        for g in range(2):
            for q in range(12):
                units.append(functools.partial(piece, slot0 + 2 * g, 1 + q // 4, q % 4 // 2, q % 2))
                counts[(g == 1, 4 * q + 2)] = 1
                if q % 2 == 1:
                    units.append(mods.pop())
                    counts[(g == 1, 4 * q + 2)] = 2
            if g == 0:
                units += [mods.pop() for _ in range(4)]
                counts[(False, 'end')] = 4
        units.append(functools.partial(ln2, x1n, 0))
        counts[(True, 'mid')] = 1
        pair(i, units, counts)
        return carry

    with jax.named_scope('head'):
        lax.fori_loop(0, LAG, head_pairs, 0)
    with jax.named_scope('wait2'):
        wait_all([cp_w1, cp_w3, cp_w2])

    nf = F // 128
    counts = {(False, 'mid'): 2, (False, 'end'): 4, (True, 'mid'): 2, (True, 'end'): 5}
    n_inner = 2 * nf + 1 + 32 - sum(counts.values())
    for k in range(6 * NP):
        counts[(k >= 3 * NP, k % (3 * NP))] = (k + 1) * n_inner // (6 * NP) - k * n_inner // (6 * NP)

    def main_pairs(p, carry):
        @pl.when(p >= 1)
        def _():
            out_copy(p - 1, 1).start()

        units = gate_up_units(0, 1, range(nf))
        units.append(functools.partial(ln2, x1n, 0))
        units += down_units(p, 0, x1c, 4)
        pair(p + LAG, units, counts)
        return carry

    with jax.named_scope('main'):
        lax.fori_loop(0, NPAIR - LAG, main_pairs, 0)

    p0 = NPAIR - LAG
    out_copy(p0 - 1, 1).start()
    resid1(p0 + 1, x1c)
    ln2(x1c, 1)
    units = gate_up_units(0, 1, range(2)) + gate_up_units(1, 2, range(2)) + gate_up_units(0, 2, range(2, nf))
    for q in range(LAG):
        units += down_units(p0 + q, q, (x1n, x1c)[q], 1) + [out_copy(p0 + q, 1).start]
    for unit in units:
        unit()
    out_copy(0, NPAIR).wait()


@jax.jit
def pallas_adaLN_cond__memory_aug_recurrent_mem_tr__glu_gated_swiglu__prompt_kernel(
    A_x, A_mem0, A_Wq, A_Wk, A_Wv, A_Wo, A_seg_len, B_x, B_w1, B_w3, B_w2, c, w_mod,
):
    assert A_x.shape == (1, S, D) and A_mem0.shape == (1, MEM, D)
    del A_seg_len
    del B_x
    vm = pltpu.VMEM
    scratch = [
        vm((3 * H, D // 2, DH), U32),
        vm((HD // 2, D), U32),
        vm((D // 2, F), U32),
        vm((D // 2, F), U32),
        vm((F // 2, D), U32),
        vm((6, D // 2, D), U32),
        vm((NSEG, SEG, D), BF16),
        vm((1, D), BF16),
        vm((MEM, D), BF16),
        vm((6, 8, D), F32),
        vm((NEARLY, D), F32),
        vm((NEARLY // 2, D), U32),
        vm((2 * KS, NEARLY, DH), F32),
        vm((3 * NP, NSEG, EARLY, DH), U32),
        vm((SEG // 2, D), U32),
        vm((SEG // 2 + EARLY, HD), U32),
        vm((EARLY, HD), F32),
        vm((PR, D), F32),
        vm((PR, D), F32),
        vm((PR, D), F32),
        vm((LAG * SEG, D), U32),
        vm((LAG * SEG, F), U32),
        vm((NSEG, SEG, D), BF16),
        vm((L2, L2), jnp.int32),
        vm((L2, L2), F32),
        pltpu.SemaphoreType.DMA((17 + KS,)),
        pltpu.SemaphoreType.DMA((NCH,)),
        pltpu.SemaphoreType.DMA(()),
    ]
    out = pl.pallas_call(
        _kernel,
        out_shape=jax.ShapeDtypeStruct((NSEG, SEG, D), BF16),
        in_specs=[pl.BlockSpec(memory_space=pl.ANY)] * 11,
        out_specs=pl.BlockSpec(memory_space=pl.ANY),
        scratch_shapes=scratch,
        compiler_params=pltpu.CompilerParams(vmem_limit_bytes=120 * 1024 * 1024,
                                             disable_bounds_checks=True,
                                             disable_semaphore_checks=True),
    )(
        A_x.reshape(NSEG, SEG, D),
        A_mem0.reshape(MEM, D),
        A_Wq.reshape(D // 2, 2 * H, DH),
        A_Wk.reshape(D // 2, 2 * H, DH),
        A_Wv.reshape(D // 2, 2 * H, DH),
        A_Wo.reshape(HD, D),
        B_w1, B_w3, B_w2, c, w_mod,
    )
    return out.reshape(1, S, D)
```

```python
import functools
import math

import jax
import jax.numpy as jnp
from jax import lax
import jax.experimental.pallas as pl
import jax.experimental.pallas.tpu as pltpu

S, D, H, DH, MEM, SEG, F = 2048, 1024, 32, 128, 8, 32, 3584
NSEG = S // SEG
NP = H // 2
HD = H * DH
EARLY = 8
NEARLY = NSEG * EARLY
L2 = 2 * (MEM + SEG)
CH = 8
NCH = 3 * H // CH
KS = CH
XS = 8
NDEF = 2
NPAIR = NSEG // 2
PR = 2 * SEG
LAG = 2
EPS = 1e-5
SCALE = DH ** -0.5
MASK_FILL = -1000000000.0

BF16, F32, U32 = jnp.bfloat16, jnp.float32, jnp.uint32


def _bf(x_u32):
    return pltpu.bitcast(x_u32, BF16)


def _pk(x_f32):
    return pltpu.bitcast(x_f32.astype(BF16), U32)


def _dot(a, b):
    return jnp.dot(a, b, preferred_element_type=F32)


def _affine(x, scale8, shift8=None):
    y = x.reshape(-1, 8, x.shape[-1]) * scale8[None]
    if shift8 is not None:
        y = y + shift8[None]
    return y.reshape(x.shape)


def _norm(x):
    m = jnp.mean(x, axis=-1, keepdims=True)
    xc = x - m
    v = jnp.mean(xc * xc, axis=-1, keepdims=True)
    return xc * lax.rsqrt(v + EPS)


def _attn_mask():
    def meta(i):
        head = jnp.where(i < 2 * SEG, i // SEG, (i - 2 * SEG) // EARLY)
        j = i % SEG
        pos = jnp.where(i < 2 * SEG, jnp.where(j < MEM, j, j + EARLY), MEM + (i - 2 * SEG) % EARLY)
        return head, pos
    r = lax.broadcasted_iota(jnp.int32, (L2, L2), 0)
    c = lax.broadcasted_iota(jnp.int32, (L2, L2), 1)
    rh, rp = meta(r)
    chd, cp = meta(c)
    same = rh == chd
    keep = same & ((rp < MEM) | (rp >= cp))
    fill = jnp.where(same, MASK_FILL / SCALE, -jnp.inf).astype(F32)
    return keep, fill


def _kernel(x_hbm, m0_hbm, wq_hbm, wk_hbm, wv_hbm, wo_hbm, w1_hbm, w3_hbm, w2_hbm, c_hbm, wm_hbm,
            out_hbm,
            wqkv, wo, w1, w3, w2, wm, xb, cb, m0, mod, nrm, p32, part, pre, l32, ob, oda, abuf,
            x1n, x1c, h2, act, ost, keep_s, fill_s, sem, wsem, osem):
    w_hbm = [r.bitcast(U32) for r in (wq_hbm, wk_hbm, wv_hbm)]
    wm_u = wm_hbm.bitcast(U32)

    def pair_copies(m, j, dsem, r0=0, r1=D // 2):
        return [pltpu.make_async_copy(w_hbm[m].at[r0:r1, par * NP + j, :],
                                      wqkv.at[m * H + 2 * j + par, r0:r1, :], dsem) for par in range(2)]

    def chunk_copies(t):
        m, c0 = divmod(t, H // CH)
        return [cp for jj in range(CH // 2)
                for cp in pair_copies(m, c0 * (CH // 2) + jj, wsem.at[t])]

    def wait_chunk(t):
        blk = wqkv.at[pl.ds(t * CH, CH)]
        pltpu.make_async_copy(blk, blk, wsem.at[t]).wait()

    def unzip(slot, r0=0, r1=D // 2):
        for r in range(r0, r1, 32):
            e, o = wqkv[slot, r:r + 32, :], wqkv[slot + 1, r:r + 32, :]
            wqkv[slot, r:r + 32, :] = (e & 0xFFFF) | (o << 16)
            wqkv[slot + 1, r:r + 32, :] = (e >> 16) | (o & jnp.uint32(0xFFFF0000))

    def start_all(cps):
        for cp in cps:
            cp.start()

    def wait_all(cps):
        for cp in cps:
            cp.wait()

    HK = D // 2
    cp_c = pltpu.make_async_copy(c_hbm, cb, sem.at[0])
    cp_xe = pltpu.make_async_copy(x_hbm.at[:, 0:EARLY, :], xb.at[:, 0:EARLY, :], sem.at[1])
    cp_x0 = pltpu.make_async_copy(x_hbm.at[0, EARLY:SEG, :], xb.at[0, EARLY:SEG, :], sem.at[2])
    cp_m0 = pltpu.make_async_copy(m0_hbm, m0, sem.at[3])
    cp_xr = pltpu.make_async_copy(x_hbm.at[1:XS, EARLY:SEG, :], xb.at[1:XS, EARLY:SEG, :], sem.at[4])
    cp_xl = pltpu.make_async_copy(x_hbm.at[XS:NSEG, EARLY:SEG, :], xb.at[XS:NSEG, EARLY:SEG, :], sem.at[17 + KS])
    cp_wo = pltpu.make_async_copy(wo_hbm.bitcast(U32), wo, sem.at[5])
    cp_w1 = pltpu.make_async_copy(w1_hbm.bitcast(U32), w1, sem.at[6])
    cp_w3 = pltpu.make_async_copy(w3_hbm.bitcast(U32), w3, sem.at[7])
    cp_w2 = pltpu.make_async_copy(w2_hbm.bitcast(U32), w2, sem.at[8])
    cp_wm = [pltpu.make_async_copy(wm_u.at[:, k * D:(k + 1) * D], wm.at[k], sem.at[7 + k])
             for k in range(2, 6)]
    cp_wa = [[pltpu.make_async_copy(wm_u.at[:, k * D + hf * HK:k * D + (hf + 1) * HK],
                                    wm.at[k, :, hf * HK:(hf + 1) * HK], sem.at[13 + 2 * hf + k])
              for k in range(2)] for hf in range(2)]
    cp_ks = [[[cp for j in (2 * g, 2 * g + 1)
               for cp in pair_copies(0, j, sem.at[17 + hf * (KS // 2) + g], hf * HK // 2, (hf + 1) * HK // 2)]
              for g in range(KS // 2)] for hf in range(2)]

    start_all([cp_xe, cp_c, cp_x0, cp_m0] + cp_wa[0])
    keep, fill = _attn_mask()
    keep_s[...] = keep.astype(jnp.int32)
    fill_s[...] = fill
    wait_all([cp_xe, cp_c, cp_x0, cp_m0])
    start_all(cp_ks[0][0])
    cf = cb[...].astype(F32)
    sc16 = jnp.broadcast_to(cf * jax.nn.sigmoid(cf), (16, D)).astype(BF16)
    for g in range(NSEG // 8):
        nrm[64 * g:64 * g + 64, :] = _norm(xb[8 * g:8 * g + 8, 0:EARLY, :].astype(F32).reshape(8 * EARLY, D))

    def mod_unit(k, c0, c1):
        mod[k, :, c0:c1] = _dot(sc16, _bf(wm[k, :, c0:c1]))[0:8]

    def ln1_mod(n, c0=0, c1=D):
        return _affine(n, 1.0 + mod[1, :, c0:c1], mod[0, :, c0:c1])

    def next_lhs(mem_f32, s):
        hx = ln1_mod(_norm(xb[s, EARLY:SEG, :].astype(F32)))
        l32[...] = _pk(jnp.concatenate([mem_f32, hx], axis=0))

    def ln1_early(hf):
        c0, c1 = hf * HK, (hf + 1) * HK
        for n in range(c0, c1, 128):
            for g in range(NEARLY // 128):
                p32[64 * g:64 * g + 64, n:n + 128] = _pk(ln1_mod(nrm[128 * g:128 * g + 128, n:n + 128], n, n + 128))

    def early_dot(head, c, hf=None):
        c0, c1 = (0, D) if hf is None else (hf * HK, (hf + 1) * HK)
        return _dot(_bf(p32[64 * c:64 * c + 64, c0:c1]), _bf(wqkv[head, c0 // 2:c1 // 2, :]))

    def early_store(slot, c, ab):
        pre[slot // 2, 16 * c:16 * c + 16] = _pk(
            jnp.concatenate([v.reshape(16, EARLY, DH) for v in ab], axis=1))

    def early_block(slot, c, hf=None):
        ab = [early_dot(slot + hh, c, hf) for hh in range(2)]
        if hf == 0:
            for hh in range(2):
                part[slot + hh, 128 * c:128 * c + 128, :] = ab[hh]
            return
        if hf == 1:
            ab = [ab[hh] + part[slot + hh, 128 * c:128 * c + 128, :] for hh in range(2)]
        early_store(slot, c, ab)

    def early_run(slot0, npairs, hf=None, blocks=range(NEARLY // 128)):
        rows = (0, D // 2) if hf is None else (hf * HK // 2, (hf + 1) * HK // 2)
        unzip(slot0, *rows)
        for g in range(npairs):
            if g + 1 < npairs:
                unzip(slot0 + 2 * g + 2, *rows)
            for c in blocks:
                early_block(slot0 + 2 * g, c, hf)

    for k, issue in enumerate((cp_ks[0][1], cp_ks[0][2] + cp_wa[1])):
        cp_wa[0][k].wait()
        start_all(issue)
        mod_unit(k, 0, HK)
    ln1_early(0)
    wait_all(cp_ks[0][0])
    start_all(cp_ks[0][3])
    early_run(0, 2, 0)
    wait_all(cp_ks[0][1] + cp_ks[0][2])
    start_all([cp for g in range(KS // 2) for cp in cp_ks[1][g]])
    early_run(4, 4, 0)
    wait_all(cp_ks[0][3] + cp_wa[1])
    start_all(chunk_copies(2) + chunk_copies(3))
    unzip(12, 0, HK // 2)
    unzip(14, 0, HK // 2)
    for u in range(8):
        early_block(12 + 2 * (u // 4), u % 4, 0)
        if u < 4:
            for k in range(2):
                mod_unit(k, HK + 128 * u, HK + 128 * (u + 1))
    ln1_early(1)
    next_lhs(m0[...].astype(F32), 0)
    wait_all(cp_ks[1][0] + cp_ks[1][1])
    start_all(chunk_copies(4) + chunk_copies(5) + chunk_copies(6))
    early_run(0, 4, 1)
    wait_all(cp_ks[1][2] + cp_ks[1][3])
    start_all([cp for t in range(7, NCH) for cp in chunk_copies(t)])
    early_run(8, 4, 1)

    def prologue(r, carry):
        wait_chunk(2 * r)
        wait_chunk(2 * r + 1)

        @pl.when(r == 1)
        def _():
            start_all([cp_xr, cp_wo] + cp_wm + [cp_w1, cp_w3, cp_w2, cp_xl])

        early_run(2 * r * CH, CH)
        return carry

    with jax.named_scope('prologue'):
        lax.fori_loop(1, (NCH - NDEF) // 2, prologue, 0)

    for t in range(NCH - NDEF, NCH):
        wait_chunk(t)
    wait_all([cp_xr, cp_wo])
    early_run((NCH - NDEF) * CH, NDEF * CH // 2, blocks=(0,))

    def resid1(p, dst):
        for n in range(0, D, 256):
            xf = xb[pl.ds(2 * p, 2), :, n:n + 256].astype(F32).reshape(PR, 256)
            dst[:, n:n + 256] = xf + _affine(abuf[:, n:n + 256], mod[2, :, n:n + 256])

    def advance(p):
        x1c[...] = x1n[...]
        resid1(p, x1n)

    def ln2(src, q):
        h2[q * SEG:(q + 1) * SEG, :] = _pk(_affine(_norm(src[...]), 1.0 + mod[4], mod[3]))

    def gate_up_units(q0, q1, chunks):
        r0, r1 = q0 * SEG, q1 * SEG
        half = {}

        def gate(f0):
            half[f0] = 0.5 * _dot(_bf(h2[r0:r1, :]), _bf(w1[:, f0:f0 + 128]))

        def up(f0):
            t = half.pop(f0)
            u = _dot(_bf(h2[r0:r1, :]), _bf(w3[:, f0:f0 + 128]))
            act[r0:r1, f0:f0 + 128] = _pk((t + t * jnp.tanh(t)) * u)

        return [functools.partial(fn, 128 * ck) for ck in chunks for fn in (gate, up)]

    def down_units(p, q, x1, nsplit):
        kq = F // nsplit
        acc = {}

        def down(n0, k):
            y = _dot(_bf(act[q * SEG:(q + 1) * SEG, k * kq:(k + 1) * kq]),
                     _bf(w2[k * kq // 2:(k + 1) * kq // 2, n0:n0 + 128]))
            if k > 0:
                y = y + acc.pop(n0)
            if k + 1 < nsplit:
                acc[n0] = y
                return
            res = x1[:, n0:n0 + 128] + _affine(y, mod[5, :, n0:n0 + 128])
            ost[pl.ds(2 * p, 2), :, n0:n0 + 128] = res.astype(BF16).reshape(2, SEG, 128)

        return [functools.partial(down, n0, k) for n0 in range(0, D, 128) for k in range(nsplit)]

    def out_copy(p, npairs):
        rows = pl.ds(2 * p, 2 * npairs)
        return pltpu.make_async_copy(ost.at[rows], out_hbm.at[rows], osem)

    c_exp = SCALE * math.log2(math.e)
    nb = 256

    def step(s, second, fill):
        rows = SEG + 2 * EARLY if second else SEG
        lhs = _bf(l32[...])
        qkv, prob = {}, {}

        def project(j):
            out = []
            for m in range(3):
                a = _dot(lhs, _bf(wqkv[m * H + 2 * j])).astype(BF16)
                b = _dot(lhs, _bf(wqkv[m * H + 2 * j + 1])).astype(BF16)
                out.append(jnp.concatenate([a, b, _bf(pre[m * NP + j, s])], axis=0))
                fill(3 * j + m)
            qkv[j] = out

        def scores(j):
            q, k, _ = qkv[j]
            sc_ = lax.dot_general(q, k, (((1,), (1,)), ((), ())), preferred_element_type=F32)
            sc_ = jnp.where(keep_s[...] != 0, sc_, fill_s[...])
            e = jnp.exp2((sc_ - jnp.max(sc_, axis=1, keepdims=True)) * c_exp)
            den = jnp.sum(e, axis=1, keepdims=True)
            r = pl.reciprocal(den, approx=True)
            r = r * (2.0 - den * r)
            prob[j] = (e * r).astype(BF16)

        def values(j):
            o = _dot(prob.pop(j), qkv.pop(j)[2])
            for hh in range(2):
                c0 = (2 * j + hh) * DH
                main = o[hh * SEG:(hh + 1) * SEG]
                early = o[2 * SEG + hh * EARLY:2 * SEG + (hh + 1) * EARLY]
                if second:
                    ob[:, c0:c0 + DH] = _pk(jnp.concatenate([main, oda[:, c0:c0 + DH], early], axis=0))
                else:
                    ob[0:SEG // 2, c0:c0 + DH] = _pk(main)
                    oda[:, c0:c0 + DH] = early

        def wo_part(n, j0, j1):
            k0, k1 = j0 * 2 * DH, j1 * 2 * DH
            return _dot(_bf(ob[0:rows // 2, k0:k1]), _bf(wo[k0 // 2:k1 // 2, n * nb:(n + 1) * nb]))

        for j in range(NP):
            project(j)
            if j >= 1:
                scores(j - 1)
            if j >= 3:
                values(j - 3)
        y0 = wo_part(0, 0, 6)
        scores(NP - 1)
        values(NP - 3)
        y0 = y0 + wo_part(0, 6, 12)
        values(NP - 2)
        fill('mid')
        y1 = wo_part(1, 0, 8)
        values(NP - 1)
        y1 = y1 + wo_part(1, 8, 13)
        y2 = wo_part(2, 0, 14)
        y0 = y0 + wo_part(0, 12, NP)
        y1 = y1 + wo_part(1, 13, NP)
        y2 = y2 + wo_part(2, 14, NP)
        y = jnp.concatenate([y0, y1, y2, wo_part(3, 0, NP)], axis=1)
        next_lhs(y[0:MEM], jnp.minimum(s + 1, NSEG - 1))
        fill('end')
        return y

    def pair(i, units, counts):
        units = list(units)

        def filler(second):
            def fill(point):
                for _ in range(counts.get((second, point), 0)):
                    units.pop(0)()
            return fill

        advance(jnp.maximum(i - 1, 0))
        ya = step(2 * i, False, filler(False))
        abuf[EARLY:SEG, :] = ya[MEM:SEG]
        yb = step(2 * i + 1, True, filler(True))
        abuf[0:EARLY, :] = yb[SEG:SEG + EARLY]
        abuf[SEG:SEG + EARLY, :] = yb[SEG + EARLY:SEG + 2 * EARLY]
        abuf[SEG + EARLY:PR, :] = yb[MEM:SEG]
        assert not units

    def head_pairs(i, carry):
        for kk in range(2):
            k = 2 + 2 * i + kk
            pltpu.make_async_copy(wm.at[k], wm.at[k], sem.at[7 + k]).wait()
        mods = [functools.partial(mod_unit, 2 + 2 * i + kk, n0, n0 + 128)
                for kk in range(2) for n0 in range(0, D, 128)]
        npr = NDEF * CH // 2 // LAG
        slot0 = (NCH - NDEF) * CH + 2 * npr * i
        held = {}

        def piece(slot, c, hh, hf):
            v = early_dot(slot + hh, c, hf)
            held[hh] = v if hf == 0 else v + held[hh]
            if hh == 1 and hf == 1:
                early_store(slot, c, [held.pop(0), held.pop(1)])

        pieces = [functools.partial(piece, slot0 + 2 * g, c, hh, hf)
                  for g in range(npr) for c in range(1, 4) for hh in range(2) for hf in range(2)]
        units, counts = [], {}
        tail = {(False, 'mid'): 2, (False, 'end'): 3, (True, 'mid'): 2, (True, 'end'): 3}
        inner = len(pieces) - sum(tail.values())
        for second in (False, True):
            for pt in list(range(3 * NP)) + ['mid', 'end']:
                if pt in ('mid', 'end'):
                    n = tail[(second, pt)]
                else:
                    k = second * 3 * NP + pt
                    n = (k + 1) * inner // (6 * NP) - k * inner // (6 * NP)
                here = []
                for _ in range(n):
                    here.append(pieces.pop(0))
                    if mods and len(pieces) % 2 == 0:
                        here.append(mods.pop(0))
                if second and pt == 'mid':
                    assert not mods
                    here.append(functools.partial(ln2, x1n, 0))
                units += here
                counts[(second, pt)] = len(here)
        pair(i, units, counts)
        return carry

    with jax.named_scope('head'):
        lax.fori_loop(0, LAG, head_pairs, 0)
    with jax.named_scope('wait2'):
        wait_all([cp_w1, cp_w3, cp_w2])

    nf = F // 128
    counts = {(False, 'mid'): 2, (False, 'end'): 4, (True, 'mid'): 2, (True, 'end'): 5}
    n_inner = 2 * nf + 1 + 32 - sum(counts.values())
    for k in range(6 * NP):
        counts[(k >= 3 * NP, k % (3 * NP))] = (k + 1) * n_inner // (6 * NP) - k * n_inner // (6 * NP)

    def main_pairs(p, carry):
        @pl.when(p == 1)
        def _():
            cp_xl.wait()

        @pl.when(p >= 1)
        def _():
            out_copy(p - 1, 1).start()

        units = gate_up_units(0, 1, range(nf))
        units.append(functools.partial(ln2, x1n, 0))
        units += down_units(p, 0, x1c, 4)
        pair(p + LAG, units, counts)
        return carry

    with jax.named_scope('main'):
        lax.fori_loop(0, NPAIR - LAG, main_pairs, 0)

    p0 = NPAIR - LAG
    out_copy(p0 - 1, 1).start()
    resid1(p0 + 1, x1c)
    ln2(x1c, 1)
    units = gate_up_units(0, 1, range(2)) + gate_up_units(1, 2, range(2)) + gate_up_units(0, 2, range(2, nf))
    for q in range(LAG):
        units += down_units(p0 + q, q, (x1n, x1c)[q], 1) + [out_copy(p0 + q, 1).start]
    for unit in units:
        unit()
    out_copy(0, NPAIR).wait()


@jax.jit
def pallas_adaLN_cond__memory_aug_recurrent_mem_tr__glu_gated_swiglu__prompt_kernel(
    A_x, A_mem0, A_Wq, A_Wk, A_Wv, A_Wo, A_seg_len, B_x, B_w1, B_w3, B_w2, c, w_mod,
):
    assert A_x.shape == (1, S, D) and A_mem0.shape == (1, MEM, D)
    del A_seg_len
    del B_x
    vm = pltpu.VMEM
    scratch = [
        vm((3 * H, D // 2, DH), U32),
        vm((HD // 2, D), U32),
        vm((D // 2, F), U32),
        vm((D // 2, F), U32),
        vm((F // 2, D), U32),
        vm((6, D // 2, D), U32),
        vm((NSEG, SEG, D), BF16),
        vm((1, D), BF16),
        vm((MEM, D), BF16),
        vm((6, 8, D), F32),
        vm((NEARLY, D), F32),
        vm((NEARLY // 2, D), U32),
        vm((2 * KS, NEARLY, DH), F32),
        vm((3 * NP, NSEG, EARLY, DH), U32),
        vm((SEG // 2, D), U32),
        vm((SEG // 2 + EARLY, HD), U32),
        vm((EARLY, HD), F32),
        vm((PR, D), F32),
        vm((PR, D), F32),
        vm((PR, D), F32),
        vm((LAG * SEG, D), U32),
        vm((LAG * SEG, F), U32),
        vm((NSEG, SEG, D), BF16),
        vm((L2, L2), jnp.int32),
        vm((L2, L2), F32),
        pltpu.SemaphoreType.DMA((18 + KS,)),
        pltpu.SemaphoreType.DMA((NCH,)),
        pltpu.SemaphoreType.DMA(()),
    ]
    out = pl.pallas_call(
        _kernel,
        out_shape=jax.ShapeDtypeStruct((NSEG, SEG, D), BF16),
        in_specs=[pl.BlockSpec(memory_space=pl.ANY)] * 11,
        out_specs=pl.BlockSpec(memory_space=pl.ANY),
        scratch_shapes=scratch,
        compiler_params=pltpu.CompilerParams(vmem_limit_bytes=120 * 1024 * 1024,
                                             disable_bounds_checks=True,
                                             disable_semaphore_checks=True),
    )(
        A_x.reshape(NSEG, SEG, D),
        A_mem0.reshape(MEM, D),
        A_Wq.reshape(D // 2, 2 * H, DH),
        A_Wk.reshape(D // 2, 2 * H, DH),
        A_Wv.reshape(D // 2, 2 * H, DH),
        A_Wo.reshape(HD, D),
        B_w1, B_w3, B_w2, c, w_mod,
    )
    return out.reshape(1, S, D)
```

```python
import functools
import math

import jax
import jax.numpy as jnp
from jax import lax
import jax.experimental.pallas as pl
import jax.experimental.pallas.tpu as pltpu

S, D, H, DH, MEM, SEG, F = 2048, 1024, 32, 128, 8, 32, 3584
NSEG = S // SEG
NP = H // 2
HD = H * DH
EARLY = 8
NEARLY = NSEG * EARLY
L2 = 2 * (MEM + SEG)
CH = 8
NCH = 3 * H // CH
KS = CH
XS = 8
NDEF = 2
NPAIR = NSEG // 2
PR = 2 * SEG
LAG = 2
EPS = 1e-5
SCALE = DH ** -0.5
MASK_FILL = -1000000000.0

BF16, F32, U32 = jnp.bfloat16, jnp.float32, jnp.uint32


def _bf(x_u32):
    return pltpu.bitcast(x_u32, BF16)


def _pk(x_f32):
    return pltpu.bitcast(x_f32.astype(BF16), U32)


def _dot(a, b):
    return jnp.dot(a, b, preferred_element_type=F32)


def _affine(x, scale8, shift8=None):
    y = x.reshape(-1, 8, x.shape[-1]) * scale8[None]
    if shift8 is not None:
        y = y + shift8[None]
    return y.reshape(x.shape)


def _norm(x):
    m = jnp.mean(x, axis=-1, keepdims=True)
    xc = x - m
    v = jnp.mean(xc * xc, axis=-1, keepdims=True)
    return xc * lax.rsqrt(v + EPS)


def _attn_mask():
    def meta(i):
        head = jnp.where(i < 2 * SEG, i // SEG, (i - 2 * SEG) // EARLY)
        j = i % SEG
        pos = jnp.where(i < 2 * SEG, jnp.where(j < MEM, j, j + EARLY), MEM + (i - 2 * SEG) % EARLY)
        return head, pos
    r = lax.broadcasted_iota(jnp.int32, (L2, L2), 0)
    c = lax.broadcasted_iota(jnp.int32, (L2, L2), 1)
    rh, rp = meta(r)
    chd, cp = meta(c)
    same = rh == chd
    keep = same & ((rp < MEM) | (rp >= cp))
    fill = jnp.where(same, MASK_FILL / SCALE, -jnp.inf).astype(F32)
    return keep, fill


def _kernel(x_hbm, m0_hbm, wq_hbm, wk_hbm, wv_hbm, wo_hbm, w1_hbm, w3_hbm, w2_hbm, c_hbm, wm_hbm,
            out_hbm,
            wqkv, wo, w1, w3, w2, wm, xb, xe, cb, m0, mod, nrm, p32, part, pre, l32, ob, oda, abuf,
            x1n, x1c, h2, act, ost, keep_s, fill_s, sem, wsem, osem):
    w_hbm = [r.bitcast(U32) for r in (wq_hbm, wk_hbm, wv_hbm)]
    wm_u = wm_hbm.bitcast(U32)

    def pair_copies(m, j, dsem, r0=0, r1=D // 2):
        return [pltpu.make_async_copy(w_hbm[m].at[r0:r1, par * NP + j, :],
                                      wqkv.at[m * H + 2 * j + par, r0:r1, :], dsem) for par in range(2)]

    def chunk_copies(t):
        m, c0 = divmod(t, H // CH)
        return [cp for jj in range(CH // 2)
                for cp in pair_copies(m, c0 * (CH // 2) + jj, wsem.at[t])]

    def wait_chunk(t):
        blk = wqkv.at[pl.ds(t * CH, CH)]
        pltpu.make_async_copy(blk, blk, wsem.at[t]).wait()

    def unzip(slot, r0=0, r1=D // 2):
        for r in range(r0, r1, 32):
            e, o = wqkv[slot, r:r + 32, :], wqkv[slot + 1, r:r + 32, :]
            wqkv[slot, r:r + 32, :] = (e & 0xFFFF) | (o << 16)
            wqkv[slot + 1, r:r + 32, :] = (e >> 16) | (o & jnp.uint32(0xFFFF0000))

    def start_all(cps):
        for cp in cps:
            cp.start()

    def wait_all(cps):
        for cp in cps:
            cp.wait()

    HK = D // 2
    cp_c = pltpu.make_async_copy(c_hbm, cb, sem.at[0])
    x_u = x_hbm.bitcast(U32)
    cp_xe = pltpu.make_async_copy(x_hbm.at[:, 0:EARLY, :], xe, sem.at[1])
    cp_x0 = pltpu.make_async_copy(x_u.at[0], xb.at[0], sem.at[2])
    cp_m0 = pltpu.make_async_copy(m0_hbm, m0, sem.at[3])
    cp_xr = pltpu.make_async_copy(x_u.at[1:XS], xb.at[1:XS], sem.at[4])
    cp_xl = pltpu.make_async_copy(x_u.at[XS:NSEG], xb.at[XS:NSEG], sem.at[17 + KS])
    cp_wo = pltpu.make_async_copy(wo_hbm.bitcast(U32), wo, sem.at[5])
    cp_w1 = pltpu.make_async_copy(w1_hbm.bitcast(U32), w1, sem.at[6])
    cp_w3 = pltpu.make_async_copy(w3_hbm.bitcast(U32), w3, sem.at[7])
    cp_w2 = pltpu.make_async_copy(w2_hbm.bitcast(U32), w2, sem.at[8])
    cp_wm = [pltpu.make_async_copy(wm_u.at[:, k * D:(k + 1) * D], wm.at[k], sem.at[7 + k])
             for k in range(2, 6)]
    cp_wa = [[pltpu.make_async_copy(wm_u.at[:, k * D + hf * HK:k * D + (hf + 1) * HK],
                                    wm.at[k, :, hf * HK:(hf + 1) * HK], sem.at[13 + 2 * hf + k])
              for k in range(2)] for hf in range(2)]
    cp_ks = [[[cp for j in (2 * g, 2 * g + 1)
               for cp in pair_copies(0, j, sem.at[17 + hf * (KS // 2) + g], hf * HK // 2, (hf + 1) * HK // 2)]
              for g in range(KS // 2)] for hf in range(2)]

    start_all([cp_xe, cp_c, cp_x0, cp_m0] + cp_wa[0])
    keep, fill = _attn_mask()
    keep_s[...] = keep.astype(jnp.int32)
    fill_s[...] = fill
    wait_all([cp_xe, cp_c, cp_x0, cp_m0])
    start_all(cp_ks[0][0])
    cf = cb[...].astype(F32)
    sc16 = jnp.broadcast_to(cf * jax.nn.sigmoid(cf), (16, D)).astype(BF16)
    for g in range(NSEG // 8):
        nrm[64 * g:64 * g + 64, :] = _norm(xe[8 * g:8 * g + 8].astype(F32).reshape(8 * EARLY, D))

    def mod_unit(k, c0, c1):
        mod[k, :, c0:c1] = _dot(sc16, _bf(wm[k, :, c0:c1]))[0:8]

    def ln1_mod(n, c0=0, c1=D):
        return _affine(n, 1.0 + mod[1, :, c0:c1], mod[0, :, c0:c1])

    def next_lhs(mem_f32, s):
        hx = ln1_mod(_norm(_bf(xb[s]).astype(F32)[EARLY:SEG]))
        l32[...] = _pk(jnp.concatenate([mem_f32, hx], axis=0))

    def ln1_early(hf):
        c0, c1 = hf * HK, (hf + 1) * HK
        for n in range(c0, c1, 128):
            for g in range(NEARLY // 128):
                p32[64 * g:64 * g + 64, n:n + 128] = _pk(ln1_mod(nrm[128 * g:128 * g + 128, n:n + 128], n, n + 128))

    def early_dot(head, c, hf=None):
        c0, c1 = (0, D) if hf is None else (hf * HK, (hf + 1) * HK)
        return _dot(_bf(p32[64 * c:64 * c + 64, c0:c1]), _bf(wqkv[head, c0 // 2:c1 // 2, :]))

    def early_store(slot, c, ab):
        pre[slot // 2, 16 * c:16 * c + 16] = _pk(
            jnp.concatenate([v.reshape(16, EARLY, DH) for v in ab], axis=1))

    def early_block(slot, c, hf=None):
        ab = [early_dot(slot + hh, c, hf) for hh in range(2)]
        if hf == 0:
            for hh in range(2):
                part[slot + hh, 128 * c:128 * c + 128, :] = ab[hh]
            return
        if hf == 1:
            ab = [ab[hh] + part[slot + hh, 128 * c:128 * c + 128, :] for hh in range(2)]
        early_store(slot, c, ab)

    def early_run(slot0, npairs, hf=None, blocks=range(NEARLY // 128)):
        rows = (0, D // 2) if hf is None else (hf * HK // 2, (hf + 1) * HK // 2)
        unzip(slot0, *rows)
        for g in range(npairs):
            if g + 1 < npairs:
                unzip(slot0 + 2 * g + 2, *rows)
            for c in blocks:
                early_block(slot0 + 2 * g, c, hf)

    for k, issue in enumerate((cp_ks[0][1], cp_ks[0][2] + cp_wa[1])):
        cp_wa[0][k].wait()
        start_all(issue)
        mod_unit(k, 0, HK)
    ln1_early(0)
    wait_all(cp_ks[0][0])
    start_all(cp_ks[0][3])
    early_run(0, 2, 0)
    wait_all(cp_ks[0][1] + cp_ks[0][2])
    start_all([cp for g in range(KS // 2) for cp in cp_ks[1][g]])
    early_run(4, 4, 0)
    wait_all(cp_ks[0][3] + cp_wa[1])
    start_all(chunk_copies(2) + chunk_copies(3))
    unzip(12, 0, HK // 2)
    unzip(14, 0, HK // 2)
    for u in range(8):
        early_block(12 + 2 * (u // 4), u % 4, 0)
        if u < 4:
            for k in range(2):
                mod_unit(k, HK + 128 * u, HK + 128 * (u + 1))
    ln1_early(1)
    next_lhs(m0[...].astype(F32), 0)
    wait_all(cp_ks[1][0] + cp_ks[1][1])
    start_all(chunk_copies(4) + chunk_copies(5) + chunk_copies(6))
    early_run(0, 4, 1)
    wait_all(cp_ks[1][2] + cp_ks[1][3])
    start_all([cp for t in range(7, NCH) for cp in chunk_copies(t)])
    early_run(8, 4, 1)

    def prologue(r, carry):
        wait_chunk(2 * r)
        wait_chunk(2 * r + 1)

        @pl.when(r == 1)
        def _():
            start_all([cp_xr, cp_wo] + cp_wm + [cp_w1, cp_w3, cp_w2, cp_xl])

        early_run(2 * r * CH, CH)
        return carry

    with jax.named_scope('prologue'):
        lax.fori_loop(1, (NCH - NDEF) // 2, prologue, 0)

    for t in range(NCH - NDEF, NCH):
        wait_chunk(t)
    wait_all([cp_xr, cp_wo])
    early_run((NCH - NDEF) * CH, NDEF * CH // 2, blocks=(0,))

    def resid1(p, dst):
        for n in range(0, D, 256):
            xf = _bf(xb[pl.ds(2 * p, 2), :, n:n + 256]).astype(F32).reshape(PR, 256)
            dst[:, n:n + 256] = xf + _affine(abuf[:, n:n + 256], mod[2, :, n:n + 256])

    def advance(p):
        x1c[...] = x1n[...]
        resid1(p, x1n)

    def ln2(src, q):
        h2[q * SEG:(q + 1) * SEG, :] = _pk(_affine(_norm(src[...]), 1.0 + mod[4], mod[3]))

    def gate_up_units(q0, q1, chunks):
        r0, r1 = q0 * SEG, q1 * SEG
        half = {}

        def gate(f0):
            half[f0] = 0.5 * _dot(_bf(h2[r0:r1, :]), _bf(w1[:, f0:f0 + 128]))

        def up(f0):
            t = half.pop(f0)
            u = _dot(_bf(h2[r0:r1, :]), _bf(w3[:, f0:f0 + 128]))
            act[r0:r1, f0:f0 + 128] = _pk((t + t * jnp.tanh(t)) * u)

        return [functools.partial(fn, 128 * ck) for ck in chunks for fn in (gate, up)]

    def down_units(p, q, x1, nsplit):
        kq = F // nsplit
        acc = {}

        def down(n0, k):
            y = _dot(_bf(act[q * SEG:(q + 1) * SEG, k * kq:(k + 1) * kq]),
                     _bf(w2[k * kq // 2:(k + 1) * kq // 2, n0:n0 + 128]))
            if k > 0:
                y = y + acc.pop(n0)
            if k + 1 < nsplit:
                acc[n0] = y
                return
            res = x1[:, n0:n0 + 128] + _affine(y, mod[5, :, n0:n0 + 128])
            ost[pl.ds(2 * p, 2), :, n0:n0 + 128] = res.astype(BF16).reshape(2, SEG, 128)

        return [functools.partial(down, n0, k) for n0 in range(0, D, 128) for k in range(nsplit)]

    def out_copy(p, npairs):
        rows = pl.ds(2 * p, 2 * npairs)
        return pltpu.make_async_copy(ost.at[rows], out_hbm.at[rows], osem)

    c_exp = SCALE * math.log2(math.e)
    nb = 256

    def step(s, second, fill):
        rows = SEG + 2 * EARLY if second else SEG
        lhs = _bf(l32[...])
        qkv, prob = {}, {}

        def project(j):
            out = []
            for m in range(3):
                a = _dot(lhs, _bf(wqkv[m * H + 2 * j])).astype(BF16)
                b = _dot(lhs, _bf(wqkv[m * H + 2 * j + 1])).astype(BF16)
                out.append(jnp.concatenate([a, b, _bf(pre[m * NP + j, s])], axis=0))
                fill(3 * j + m)
            qkv[j] = out

        def scores(j):
            q, k, _ = qkv[j]
            sc_ = lax.dot_general(q, k, (((1,), (1,)), ((), ())), preferred_element_type=F32)
            sc_ = jnp.where(keep_s[...] != 0, sc_, fill_s[...])
            e = jnp.exp2((sc_ - jnp.max(sc_, axis=1, keepdims=True)) * c_exp)
            den = jnp.sum(e, axis=1, keepdims=True)
            r = pl.reciprocal(den, approx=True)
            r = r * (2.0 - den * r)
            prob[j] = (e * r).astype(BF16)

        def values(j):
            o = _dot(prob.pop(j), qkv.pop(j)[2])
            for hh in range(2):
                c0 = (2 * j + hh) * DH
                main = o[hh * SEG:(hh + 1) * SEG]
                early = o[2 * SEG + hh * EARLY:2 * SEG + (hh + 1) * EARLY]
                if second:
                    ob[:, c0:c0 + DH] = _pk(jnp.concatenate([main, oda[:, c0:c0 + DH], early], axis=0))
                else:
                    ob[0:SEG // 2, c0:c0 + DH] = _pk(main)
                    oda[:, c0:c0 + DH] = early

        def wo_part(n, j0, j1):
            k0, k1 = j0 * 2 * DH, j1 * 2 * DH
            return _dot(_bf(ob[0:rows // 2, k0:k1]), _bf(wo[k0 // 2:k1 // 2, n * nb:(n + 1) * nb]))

        for j in range(NP):
            project(j)
            if j >= 1:
                scores(j - 1)
            if j >= 3:
                values(j - 3)
        y0 = wo_part(0, 0, 6)
        scores(NP - 1)
        values(NP - 3)
        y0 = y0 + wo_part(0, 6, 12)
        values(NP - 2)
        fill('mid')
        y1 = wo_part(1, 0, 8)
        values(NP - 1)
        y1 = y1 + wo_part(1, 8, 13)
        y2 = wo_part(2, 0, 14)
        y0 = y0 + wo_part(0, 12, NP)
        y1 = y1 + wo_part(1, 13, NP)
        y2 = y2 + wo_part(2, 14, NP)
        y = jnp.concatenate([y0, y1, y2, wo_part(3, 0, NP)], axis=1)
        next_lhs(y[0:MEM], jnp.minimum(s + 1, NSEG - 1))
        fill('end')
        return y

    def pair(i, units, counts):
        units = list(units)

        def filler(second):
            def fill(point):
                for _ in range(counts.get((second, point), 0)):
                    units.pop(0)()
            return fill

        advance(jnp.maximum(i - 1, 0))
        ya = step(2 * i, False, filler(False))
        abuf[EARLY:SEG, :] = ya[MEM:SEG]
        yb = step(2 * i + 1, True, filler(True))
        abuf[0:EARLY, :] = yb[SEG:SEG + EARLY]
        abuf[SEG:SEG + EARLY, :] = yb[SEG + EARLY:SEG + 2 * EARLY]
        abuf[SEG + EARLY:PR, :] = yb[MEM:SEG]
        assert not units

    def head_pairs(i, carry):
        for kk in range(2):
            k = 2 + 2 * i + kk
            pltpu.make_async_copy(wm.at[k], wm.at[k], sem.at[7 + k]).wait()
        mods = [functools.partial(mod_unit, 2 + 2 * i + kk, n0, n0 + 128)
                for kk in range(2) for n0 in range(0, D, 128)]
        npr = NDEF * CH // 2 // LAG
        slot0 = (NCH - NDEF) * CH + 2 * npr * i
        held = {}

        def piece(slot, c, hh, hf):
            v = early_dot(slot + hh, c, hf)
            held[hh] = v if hf == 0 else v + held[hh]
            if hh == 1 and hf == 1:
                early_store(slot, c, [held.pop(0), held.pop(1)])

        pieces = [functools.partial(piece, slot0 + 2 * g, c, hh, hf)
                  for g in range(npr) for c in range(1, 4) for hh in range(2) for hf in range(2)]
        units, counts = [], {}
        tail = {(False, 'mid'): 2, (False, 'end'): 3, (True, 'mid'): 2, (True, 'end'): 3}
        inner = len(pieces) - sum(tail.values())
        for second in (False, True):
            for pt in list(range(3 * NP)) + ['mid', 'end']:
                if pt in ('mid', 'end'):
                    n = tail[(second, pt)]
                else:
                    k = second * 3 * NP + pt
                    n = (k + 1) * inner // (6 * NP) - k * inner // (6 * NP)
                here = []
                for _ in range(n):
                    here.append(pieces.pop(0))
                    if mods and len(pieces) % 2 == 0:
                        here.append(mods.pop(0))
                if second and pt == 'mid':
                    assert not mods
                    here.append(functools.partial(ln2, x1n, 0))
                units += here
                counts[(second, pt)] = len(here)
        pair(i, units, counts)
        return carry

    with jax.named_scope('head'):
        lax.fori_loop(0, LAG, head_pairs, 0)
    with jax.named_scope('wait2'):
        wait_all([cp_w1, cp_w3, cp_w2])

    nf = F // 128
    counts = {(False, 'mid'): 2, (False, 'end'): 4, (True, 'mid'): 2, (True, 'end'): 5}
    n_inner = 2 * nf + 1 + 32 - sum(counts.values())
    for k in range(6 * NP):
        counts[(k >= 3 * NP, k % (3 * NP))] = (k + 1) * n_inner // (6 * NP) - k * n_inner // (6 * NP)

    def main_pairs(p, carry):
        @pl.when(p == 1)
        def _():
            cp_xl.wait()

        @pl.when(p >= 1)
        def _():
            out_copy(p - 1, 1).start()

        units = gate_up_units(0, 1, range(nf))
        units.append(functools.partial(ln2, x1n, 0))
        units += down_units(p, 0, x1c, 4)
        pair(p + LAG, units, counts)
        return carry

    with jax.named_scope('main'):
        lax.fori_loop(0, NPAIR - LAG, main_pairs, 0)

    p0 = NPAIR - LAG
    out_copy(p0 - 1, 1).start()
    resid1(p0 + 1, x1c)
    ln2(x1c, 1)
    units = gate_up_units(0, 1, range(2)) + gate_up_units(1, 2, range(2)) + gate_up_units(0, 2, range(2, nf))
    for q in range(LAG):
        units += down_units(p0 + q, q, (x1n, x1c)[q], 1) + [out_copy(p0 + q, 1).start]
    for unit in units:
        unit()
    out_copy(0, NPAIR).wait()


@jax.jit
def pallas_adaLN_cond__memory_aug_recurrent_mem_tr__glu_gated_swiglu__prompt_kernel(
    A_x, A_mem0, A_Wq, A_Wk, A_Wv, A_Wo, A_seg_len, B_x, B_w1, B_w3, B_w2, c, w_mod,
):
    assert A_x.shape == (1, S, D) and A_mem0.shape == (1, MEM, D)
    del A_seg_len
    del B_x
    vm = pltpu.VMEM
    scratch = [
        vm((3 * H, D // 2, DH), U32),
        vm((HD // 2, D), U32),
        vm((D // 2, F), U32),
        vm((D // 2, F), U32),
        vm((F // 2, D), U32),
        vm((6, D // 2, D), U32),
        vm((NSEG, SEG // 2, D), U32),
        vm((NSEG, EARLY, D), BF16),
        vm((1, D), BF16),
        vm((MEM, D), BF16),
        vm((6, 8, D), F32),
        vm((NEARLY, D), F32),
        vm((NEARLY // 2, D), U32),
        vm((2 * KS, NEARLY, DH), F32),
        vm((3 * NP, NSEG, EARLY, DH), U32),
        vm((SEG // 2, D), U32),
        vm((SEG // 2 + EARLY, HD), U32),
        vm((EARLY, HD), F32),
        vm((PR, D), F32),
        vm((PR, D), F32),
        vm((PR, D), F32),
        vm((LAG * SEG, D), U32),
        vm((LAG * SEG, F), U32),
        vm((NSEG, SEG, D), BF16),
        vm((L2, L2), jnp.int32),
        vm((L2, L2), F32),
        pltpu.SemaphoreType.DMA((18 + KS,)),
        pltpu.SemaphoreType.DMA((NCH,)),
        pltpu.SemaphoreType.DMA(()),
    ]
    out = pl.pallas_call(
        _kernel,
        out_shape=jax.ShapeDtypeStruct((NSEG, SEG, D), BF16),
        in_specs=[pl.BlockSpec(memory_space=pl.ANY)] * 11,
        out_specs=pl.BlockSpec(memory_space=pl.ANY),
        scratch_shapes=scratch,
        compiler_params=pltpu.CompilerParams(vmem_limit_bytes=120 * 1024 * 1024,
                                             disable_bounds_checks=True,
                                             disable_semaphore_checks=True),
    )(
        A_x.reshape(NSEG, SEG, D),
        A_mem0.reshape(MEM, D),
        A_Wq.reshape(D // 2, 2 * H, DH),
        A_Wk.reshape(D // 2, 2 * H, DH),
        A_Wv.reshape(D // 2, 2 * H, DH),
        A_Wo.reshape(HD, D),
        B_w1, B_w3, B_w2, c, w_mod,
    )
    return out.reshape(1, S, D)
```

```python
import functools
import math

import jax
import jax.numpy as jnp
from jax import lax
import jax.experimental.pallas as pl
import jax.experimental.pallas.tpu as pltpu

S, D, H, DH, MEM, SEG, F = 2048, 1024, 32, 128, 8, 32, 3584
NSEG = S // SEG
NP = H // 2
HD = H * DH
EARLY = 8
NEARLY = NSEG * EARLY
L2 = 2 * (MEM + SEG)
CH = 8
NCH = 3 * H // CH
NS = 4
SW = D // NS
XS = 8
NDEF = 1
NPAIR = NSEG // 2
PR = 2 * SEG
LAG = 2
EPS = 1e-5
SCALE = DH ** -0.5
MASK_FILL = -1000000000.0

BF16, F32, U32 = jnp.bfloat16, jnp.float32, jnp.uint32


def _bf(x_u32):
    return pltpu.bitcast(x_u32, BF16)


def _pk(x_f32):
    return pltpu.bitcast(x_f32.astype(BF16), U32)


def _dot(a, b):
    return jnp.dot(a, b, preferred_element_type=F32)


def _affine(x, scale8, shift8=None):
    y = x.reshape(-1, 8, x.shape[-1]) * scale8[None]
    if shift8 is not None:
        y = y + shift8[None]
    return y.reshape(x.shape)


def _norm(x):
    m = jnp.mean(x, axis=-1, keepdims=True)
    xc = x - m
    v = jnp.mean(xc * xc, axis=-1, keepdims=True)
    return xc * lax.rsqrt(v + EPS)


def _attn_mask():
    def meta(i):
        head = jnp.where(i < 2 * SEG, i // SEG, (i - 2 * SEG) // EARLY)
        j = i % SEG
        pos = jnp.where(i < 2 * SEG, jnp.where(j < MEM, j, j + EARLY), MEM + (i - 2 * SEG) % EARLY)
        return head, pos
    r = lax.broadcasted_iota(jnp.int32, (L2, L2), 0)
    c = lax.broadcasted_iota(jnp.int32, (L2, L2), 1)
    rh, rp = meta(r)
    chd, cp = meta(c)
    same = rh == chd
    keep = same & ((rp < MEM) | (rp >= cp))
    fill = jnp.where(same, MASK_FILL / SCALE, -jnp.inf).astype(F32)
    return keep, fill


def _kernel(x_hbm, m0_hbm, wq_hbm, wk_hbm, wv_hbm, wo_hbm, w1_hbm, w3_hbm, w2_hbm, c_hbm, wm_hbm,
            out_hbm,
            wqkv, wo, w1, w3, w2, wm, xb, xe, cb, m0, mod, nrm, p32, part, pre, l32, ob, oda, abuf,
            x1n, x1c, h2, act, ost, keep_s, fill_s, sem, wsem, osem):
    w_hbm = [r.bitcast(U32) for r in (wq_hbm, wk_hbm, wv_hbm)]
    wm_u = wm_hbm.bitcast(U32)

    def pair_copies(m, j, dsem, r0=0, r1=D // 2):
        return [pltpu.make_async_copy(w_hbm[m].at[r0:r1, par * NP + j, :],
                                      wqkv.at[m * H + 2 * j + par, r0:r1, :], dsem) for par in range(2)]

    def chunk_copies(t):
        m, c0 = divmod(t, H // CH)
        return [cp for jj in range(CH // 2)
                for cp in pair_copies(m, c0 * (CH // 2) + jj, wsem.at[t])]

    def wait_chunk(t):
        blk = wqkv.at[pl.ds(t * CH, CH)]
        pltpu.make_async_copy(blk, blk, wsem.at[t]).wait()

    def unzip(slot, r0=0, r1=D // 2):
        for r in range(r0, r1, 32):
            e, o = wqkv[slot, r:r + 32, :], wqkv[slot + 1, r:r + 32, :]
            wqkv[slot, r:r + 32, :] = (e & 0xFFFF) | (o << 16)
            wqkv[slot + 1, r:r + 32, :] = (e >> 16) | (o & jnp.uint32(0xFFFF0000))

    def start_all(cps):
        for cp in cps:
            cp.start()

    def wait_all(cps):
        for cp in cps:
            cp.wait()

    cp_c = pltpu.make_async_copy(c_hbm, cb, sem.at[0])
    x_u = x_hbm.bitcast(U32)
    cp_xe = pltpu.make_async_copy(x_hbm.at[:, 0:EARLY, :], xe, sem.at[1])
    cp_x0 = pltpu.make_async_copy(x_u.at[0], xb.at[0], sem.at[2])
    cp_m0 = pltpu.make_async_copy(m0_hbm, m0, sem.at[3])
    cp_xr = pltpu.make_async_copy(x_u.at[1:XS], xb.at[1:XS], sem.at[4])
    cp_wo = pltpu.make_async_copy(wo_hbm.bitcast(U32), wo, sem.at[5])
    cp_w1 = pltpu.make_async_copy(w1_hbm.bitcast(U32), w1, sem.at[6])
    cp_w3 = pltpu.make_async_copy(w3_hbm.bitcast(U32), w3, sem.at[7])
    cp_w2 = pltpu.make_async_copy(w2_hbm.bitcast(U32), w2, sem.at[8])
    cp_wm = [pltpu.make_async_copy(wm_u.at[:, k * D:(k + 1) * D], wm.at[k], sem.at[7 + k])
             for k in range(2, 6)]
    cp_xl = pltpu.make_async_copy(x_u.at[XS:NSEG], xb.at[XS:NSEG], sem.at[13])
    cp_wa = [[pltpu.make_async_copy(wm_u.at[:, k * D + q * SW:k * D + (q + 1) * SW],
                                    wm.at[k, :, q * SW:(q + 1) * SW], sem.at[14 + 3 * q])
              for k in range(2)] for q in range(NS)]
    cp_ks = [[[cp for j in range(4 * t, 4 * t + 4)
               for cp in pair_copies(0, j, sem.at[15 + 3 * q + t], q * SW // 2, (q + 1) * SW // 2)]
              for t in range(2)] for q in range(NS)]

    start_all([cp_xe, cp_c, cp_x0, cp_m0] + cp_wa[0])
    keep, fill = _attn_mask()
    keep_s[...] = keep.astype(jnp.int32)
    fill_s[...] = fill
    wait_all([cp_xe, cp_c, cp_x0, cp_m0])
    start_all(cp_ks[0][0] + cp_ks[0][1])
    cf = cb[...].astype(F32)
    sc16 = jnp.broadcast_to(cf * jax.nn.sigmoid(cf), (16, D)).astype(BF16)
    for g in range(NSEG // 8):
        nrm[64 * g:64 * g + 64, :] = _norm(xe[8 * g:8 * g + 8].astype(F32).reshape(8 * EARLY, D))

    def mod_unit(k, c0, c1):
        mod[k, :, c0:c1] = _dot(sc16, _bf(wm[k, :, c0:c1]))[0:8]

    def ln1_mod(n, c0=0, c1=D):
        return _affine(n, 1.0 + mod[1, :, c0:c1], mod[0, :, c0:c1])

    def next_lhs(mem_f32, s):
        hx = ln1_mod(_norm(_bf(xb[s]).astype(F32)[EARLY:SEG]))
        l32[...] = _pk(jnp.concatenate([mem_f32, hx], axis=0))

    def early_dot(head, c, c0=0, c1=D):
        return _dot(_bf(p32[64 * c:64 * c + 64, c0:c1]), _bf(wqkv[head, c0 // 2:c1 // 2, :]))

    def early_store(slot, c, ab):
        pre[slot // 2, 16 * c:16 * c + 16] = _pk(
            jnp.concatenate([v.reshape(16, EARLY, DH) for v in ab], axis=1))

    def early_run(slot0, npairs, c0=0, c1=D, blocks=range(NEARLY // 128)):
        unzip(slot0, c0 // 2, c1 // 2)
        for slot in range(0, 2 * npairs, 2):
            if slot + 2 < 2 * npairs:
                unzip(slot0 + slot + 2, c0 // 2, c1 // 2)
            for c in blocks:
                ab = [early_dot(slot0 + slot + hh, c, c0, c1) for hh in range(2)]
                rows = slice(128 * c, 128 * c + 128)
                if c0 > 0:
                    ab = [ab[hh] + part[slot0 + slot + hh, rows, :] for hh in range(2)]
                if c1 < D:
                    for hh in range(2):
                        part[slot0 + slot + hh, rows, :] = ab[hh]
                else:
                    early_store(slot0 + slot, c, ab)

    later = [cp_wa[q] + cp_ks[q][0] + cp_ks[q][1] for q in range(1, NS)]
    later += [chunk_copies(2) + chunk_copies(3) + chunk_copies(4)]
    for q in range(NS):
        c0, c1 = q * SW, (q + 1) * SW
        wait_all(cp_wa[q])
        start_all(later[q])
        for k in range(2):
            mod_unit(k, c0, c1)
        for n in range(c0, c1, 128):
            for g in range(NEARLY // 128):
                p32[64 * g:64 * g + 64, n:n + 128] = _pk(ln1_mod(nrm[128 * g:128 * g + 128, n:n + 128], n, n + 128))
        if q + 2 < NS:
            for t in range(2):
                wait_all(cp_ks[q][t])
                early_run(t * CH, CH // 2, c0, c1)
        else:
            wait_all(cp_ks[q][0] + cp_ks[q][1])
            early_run(0, CH, c0, c1)
    next_lhs(m0[...].astype(F32), 0)
    wait_chunk(2)
    start_all([cp for t in range(5, 9) for cp in chunk_copies(t)])
    early_run(2 * CH, CH // 2)

    def prologue(r, carry):
        wait_chunk(2 * r + 1)
        wait_chunk(2 * r + 2)

        @pl.when(r == 1)
        def _():
            start_all([cp for t in range(9, NCH) for cp in chunk_copies(t)])

        @pl.when(r == 2)
        def _():
            start_all([cp_xr, cp_wo] + cp_wm + [cp_w1, cp_w3, cp_w2, cp_xl])

        early_run((2 * r + 1) * CH, CH)
        return carry

    with jax.named_scope('prologue'):
        lax.fori_loop(1, (NCH - NDEF - 1) // 2, prologue, 0)

    for t in range(NCH - NDEF, NCH):
        wait_chunk(t)
    wait_all([cp_xr, cp_wo])
    early_run((NCH - NDEF) * CH, NDEF * CH // 2, blocks=(0,))

    def resid1(p, dst):
        for n in range(0, D, 256):
            xf = _bf(xb[pl.ds(2 * p, 2), :, n:n + 256]).astype(F32).reshape(PR, 256)
            dst[:, n:n + 256] = xf + _affine(abuf[:, n:n + 256], mod[2, :, n:n + 256])

    def advance(p):
        x1c[...] = x1n[...]
        resid1(p, x1n)

    def ln2(src, q):
        h2[q * SEG:(q + 1) * SEG, :] = _pk(_affine(_norm(src[...]), 1.0 + mod[4], mod[3]))

    def gate_up_units(q0, q1, chunks):
        r0, r1 = q0 * SEG, q1 * SEG
        half = {}

        def gate(f0):
            half[f0] = 0.5 * _dot(_bf(h2[r0:r1, :]), _bf(w1[:, f0:f0 + 128]))

        def up(f0):
            t = half.pop(f0)
            u = _dot(_bf(h2[r0:r1, :]), _bf(w3[:, f0:f0 + 128]))
            act[r0:r1, f0:f0 + 128] = _pk((t + t * jnp.tanh(t)) * u)

        return [functools.partial(fn, 128 * ck) for ck in chunks for fn in (gate, up)]

    def down_units(p, q, x1, nsplit):
        kq = F // nsplit
        acc = {}

        def down(n0, k):
            y = _dot(_bf(act[q * SEG:(q + 1) * SEG, k * kq:(k + 1) * kq]),
                     _bf(w2[k * kq // 2:(k + 1) * kq // 2, n0:n0 + 128]))
            if k > 0:
                y = y + acc.pop(n0)
            if k + 1 < nsplit:
                acc[n0] = y
                return
            res = x1[:, n0:n0 + 128] + _affine(y, mod[5, :, n0:n0 + 128])
            ost[pl.ds(2 * p, 2), :, n0:n0 + 128] = res.astype(BF16).reshape(2, SEG, 128)

        return [functools.partial(down, n0, k) for n0 in range(0, D, 128) for k in range(nsplit)]

    def out_copy(p, npairs):
        rows = pl.ds(2 * p, 2 * npairs)
        return pltpu.make_async_copy(ost.at[rows], out_hbm.at[rows], osem)

    c_exp = SCALE * math.log2(math.e)
    nb = 256

    def step(s, second, fill):
        rows = SEG + 2 * EARLY if second else SEG
        lhs = _bf(l32[...])
        qkv, prob = {}, {}

        def project(j):
            out = []
            for m in range(3):
                a = _dot(lhs, _bf(wqkv[m * H + 2 * j])).astype(BF16)
                b = _dot(lhs, _bf(wqkv[m * H + 2 * j + 1])).astype(BF16)
                out.append(jnp.concatenate([a, b, _bf(pre[m * NP + j, s])], axis=0))
                fill(3 * j + m)
            qkv[j] = out

        def scores(j):
            q, k, _ = qkv[j]
            sc_ = lax.dot_general(q, k, (((1,), (1,)), ((), ())), preferred_element_type=F32)
            sc_ = jnp.where(keep_s[...] != 0, sc_, fill_s[...])
            e = jnp.exp2((sc_ - jnp.max(sc_, axis=1, keepdims=True)) * c_exp)
            den = jnp.sum(e, axis=1, keepdims=True)
            r = pl.reciprocal(den, approx=True)
            r = r * (2.0 - den * r)
            prob[j] = (e * r).astype(BF16)

        def values(j):
            o = _dot(prob.pop(j), qkv.pop(j)[2])
            for hh in range(2):
                c0 = (2 * j + hh) * DH
                main = o[hh * SEG:(hh + 1) * SEG]
                early = o[2 * SEG + hh * EARLY:2 * SEG + (hh + 1) * EARLY]
                if second:
                    ob[:, c0:c0 + DH] = _pk(jnp.concatenate([main, oda[:, c0:c0 + DH], early], axis=0))
                else:
                    ob[0:SEG // 2, c0:c0 + DH] = _pk(main)
                    oda[:, c0:c0 + DH] = early

        def wo_part(n, j0, j1):
            k0, k1 = j0 * 2 * DH, j1 * 2 * DH
            return _dot(_bf(ob[0:rows // 2, k0:k1]), _bf(wo[k0 // 2:k1 // 2, n * nb:(n + 1) * nb]))

        for j in range(NP):
            project(j)
            if j >= 1:
                scores(j - 1)
            if j >= 3:
                values(j - 3)
        y0 = wo_part(0, 0, 6)
        scores(NP - 1)
        values(NP - 3)
        y0 = y0 + wo_part(0, 6, 12)
        values(NP - 2)
        fill('mid')
        y1 = wo_part(1, 0, 8)
        values(NP - 1)
        y1 = y1 + wo_part(1, 8, 13)
        y2 = wo_part(2, 0, 14)
        y0 = y0 + wo_part(0, 12, NP)
        y1 = y1 + wo_part(1, 13, NP)
        y2 = y2 + wo_part(2, 14, NP)
        y = jnp.concatenate([y0, y1, y2, wo_part(3, 0, NP)], axis=1)
        next_lhs(y[0:MEM], jnp.minimum(s + 1, NSEG - 1))
        fill('end')
        return y

    def pair(i, units, counts):
        units = list(units)

        def filler(second):
            def fill(point):
                for _ in range(counts.get((second, point), 0)):
                    units.pop(0)()
            return fill

        advance(jnp.maximum(i - 1, 0))
        ya = step(2 * i, False, filler(False))
        abuf[EARLY:SEG, :] = ya[MEM:SEG]
        yb = step(2 * i + 1, True, filler(True))
        abuf[0:EARLY, :] = yb[SEG:SEG + EARLY]
        abuf[SEG:SEG + EARLY, :] = yb[SEG + EARLY:SEG + 2 * EARLY]
        abuf[SEG + EARLY:PR, :] = yb[MEM:SEG]
        assert not units

    def head_pairs(i, carry):
        for kk in range(2):
            k = 2 + 2 * i + kk
            pltpu.make_async_copy(wm.at[k], wm.at[k], sem.at[7 + k]).wait()
        mods = [functools.partial(mod_unit, 2 + 2 * i + kk, n0, n0 + 128)
                for kk in range(2) for n0 in range(0, D, 128)]
        npr = NDEF * CH // 2 // LAG
        slot0 = (NCH - NDEF) * CH + 2 * npr * i
        held = {}

        def piece(slot, c, hh, hf):
            v = early_dot(slot + hh, c, hf * D // 2, (hf + 1) * D // 2)
            held[hh] = v if hf == 0 else v + held[hh]
            if hh == 1 and hf == 1:
                early_store(slot, c, [held.pop(0), held.pop(1)])

        pieces = [functools.partial(piece, slot0 + 2 * g, c, hh, hf)
                  for g in range(npr) for c in range(1, 4) for hh in range(2) for hf in range(2)]
        units, counts = [], {}
        tail = {(False, 'mid'): 1, (False, 'end'): 3, (True, 'mid'): 1, (True, 'end'): 2}
        inner = len(pieces) - sum(tail.values())
        for second in (False, True):
            for pt in list(range(3 * NP)) + ['mid', 'end']:
                if pt in ('mid', 'end'):
                    n = tail[(second, pt)]
                else:
                    k = second * 3 * NP + pt
                    n = (k + 1) * inner // (6 * NP) - k * inner // (6 * NP)
                here = []
                for _ in range(n):
                    here.append(pieces.pop(0))
                    if mods:
                        here.append(mods.pop(0))
                if second and pt == 'mid':
                    assert not mods
                    here.append(functools.partial(ln2, x1n, 0))
                units += here
                counts[(second, pt)] = len(here)
        pair(i, units, counts)
        return carry

    with jax.named_scope('head'):
        lax.fori_loop(0, LAG, head_pairs, 0)
    with jax.named_scope('wait2'):
        wait_all([cp_w1, cp_w3, cp_w2])

    nf = F // 128
    counts = {(False, 'mid'): 2, (False, 'end'): 4, (True, 'mid'): 2, (True, 'end'): 5}
    n_inner = 2 * nf + 1 + 32 - sum(counts.values())
    for k in range(6 * NP):
        counts[(k >= 3 * NP, k % (3 * NP))] = (k + 1) * n_inner // (6 * NP) - k * n_inner // (6 * NP)

    def main_pairs(p, carry):
        @pl.when(p == 1)
        def _():
            cp_xl.wait()

        @pl.when(p >= 1)
        def _():
            out_copy(p - 1, 1).start()

        units = gate_up_units(0, 1, range(nf))
        units.append(functools.partial(ln2, x1n, 0))
        units += down_units(p, 0, x1c, 4)
        pair(p + LAG, units, counts)
        return carry

    with jax.named_scope('main'):
        lax.fori_loop(0, NPAIR - LAG, main_pairs, 0)

    p0 = NPAIR - LAG
    out_copy(p0 - 1, 1).start()
    resid1(p0 + 1, x1c)
    ln2(x1c, 1)
    units = gate_up_units(0, 1, range(2)) + gate_up_units(1, 2, range(2)) + gate_up_units(0, 2, range(2, nf))
    for q in range(LAG):
        units += down_units(p0 + q, q, (x1n, x1c)[q], 1) + [out_copy(p0 + q, 1).start]
    for unit in units:
        unit()
    out_copy(0, NPAIR).wait()


@jax.jit
def pallas_adaLN_cond__memory_aug_recurrent_mem_tr__glu_gated_swiglu__prompt_kernel(
    A_x, A_mem0, A_Wq, A_Wk, A_Wv, A_Wo, A_seg_len, B_x, B_w1, B_w3, B_w2, c, w_mod,
):
    assert A_x.shape == (1, S, D) and A_mem0.shape == (1, MEM, D)
    del A_seg_len
    del B_x
    vm = pltpu.VMEM
    scratch = [
        vm((3 * H, D // 2, DH), U32),
        vm((HD // 2, D), U32),
        vm((D // 2, F), U32),
        vm((D // 2, F), U32),
        vm((F // 2, D), U32),
        vm((6, D // 2, D), U32),
        vm((NSEG, SEG // 2, D), U32),
        vm((NSEG, EARLY, D), BF16),
        vm((1, D), BF16),
        vm((MEM, D), BF16),
        vm((6, 8, D), F32),
        vm((NEARLY, D), F32),
        vm((NEARLY // 2, D), U32),
        vm((2 * CH, NEARLY, DH), F32),
        vm((3 * NP, NSEG, EARLY, DH), U32),
        vm((SEG // 2, D), U32),
        vm((SEG // 2 + EARLY, HD), U32),
        vm((EARLY, HD), F32),
        vm((PR, D), F32),
        vm((PR, D), F32),
        vm((PR, D), F32),
        vm((LAG * SEG, D), U32),
        vm((LAG * SEG, F), U32),
        vm((NSEG, SEG, D), BF16),
        vm((L2, L2), jnp.int32),
        vm((L2, L2), F32),
        pltpu.SemaphoreType.DMA((14 + 3 * NS,)),
        pltpu.SemaphoreType.DMA((NCH,)),
        pltpu.SemaphoreType.DMA(()),
    ]
    out = pl.pallas_call(
        _kernel,
        out_shape=jax.ShapeDtypeStruct((NSEG, SEG, D), BF16),
        in_specs=[pl.BlockSpec(memory_space=pl.ANY)] * 11,
        out_specs=pl.BlockSpec(memory_space=pl.ANY),
        scratch_shapes=scratch,
        compiler_params=pltpu.CompilerParams(vmem_limit_bytes=120 * 1024 * 1024,
                                             disable_bounds_checks=True,
                                             disable_semaphore_checks=True),
    )(
        A_x.reshape(NSEG, SEG, D),
        A_mem0.reshape(MEM, D),
        A_Wq.reshape(D // 2, 2 * H, DH),
        A_Wk.reshape(D // 2, 2 * H, DH),
        A_Wv.reshape(D // 2, 2 * H, DH),
        A_Wo.reshape(HD, D),
        B_w1, B_w3, B_w2, c, w_mod,
    )
    return out.reshape(1, S, D)
```

```python
import functools
import math

import jax
import jax.numpy as jnp
from jax import lax
import jax.experimental.pallas as pl
import jax.experimental.pallas.tpu as pltpu

S, D, H, DH, MEM, SEG, F = 2048, 1024, 32, 128, 8, 32, 3584
NSEG = S // SEG
NP = H // 2
HD = H * DH
EARLY = 8
NEARLY = NSEG * EARLY
L2 = 2 * (MEM + SEG)
CH = 8
NCH = 3 * H // CH
NS = 4
SW = D // NS
XS = 8
NDEF = 1
NPAIR = NSEG // 2
PR = 2 * SEG
LAG = 2
EPS = 1e-5
SCALE = DH ** -0.5
MASK_FILL = -1000000000.0

BF16, F32, U32 = jnp.bfloat16, jnp.float32, jnp.uint32


def _bf(x_u32):
    return pltpu.bitcast(x_u32, BF16)


def _pk(x_f32):
    return pltpu.bitcast(x_f32.astype(BF16), U32)


def _dot(a, b):
    return jnp.dot(a, b, preferred_element_type=F32)


def _affine(x, scale8, shift8=None):
    y = x.reshape(-1, 8, x.shape[-1]) * scale8[None]
    if shift8 is not None:
        y = y + shift8[None]
    return y.reshape(x.shape)


def _norm(x):
    m = jnp.mean(x, axis=-1, keepdims=True)
    xc = x - m
    v = jnp.mean(xc * xc, axis=-1, keepdims=True)
    return xc * lax.rsqrt(v + EPS)


def _attn_mask():
    def meta(i):
        head = jnp.where(i < 2 * SEG, i // SEG, (i - 2 * SEG) // EARLY)
        j = i % SEG
        pos = jnp.where(i < 2 * SEG, jnp.where(j < MEM, j, j + EARLY), MEM + (i - 2 * SEG) % EARLY)
        return head, pos
    r = lax.broadcasted_iota(jnp.int32, (L2, L2), 0)
    c = lax.broadcasted_iota(jnp.int32, (L2, L2), 1)
    rh, rp = meta(r)
    chd, cp = meta(c)
    same = rh == chd
    keep = same & ((rp < MEM) | (rp >= cp))
    fill = jnp.where(same, MASK_FILL / SCALE, -jnp.inf).astype(F32)
    return keep, fill


def _kernel(x_hbm, m0_hbm, wq_hbm, wk_hbm, wv_hbm, wo_hbm, w1_hbm, w3_hbm, w2_hbm, c_hbm, wm_hbm,
            out_hbm,
            wqkv, wo, w1, w3, w2, wm, xb, xe, cb, m0, mod, nrm, p32, part, pre, l32, ob, oda, abuf,
            x1n, x1c, h2, act, ost, keep_s, fill_s, sem, wsem, osem):
    w_hbm = [r.bitcast(U32) for r in (wq_hbm, wk_hbm, wv_hbm)]
    wm_u = wm_hbm.bitcast(U32)

    def pair_copies(m, j, dsem, r0=0, r1=D // 2):
        return [pltpu.make_async_copy(w_hbm[m].at[r0:r1, par * NP + j, :],
                                      wqkv.at[m * H + 2 * j + par, r0:r1, :], dsem) for par in range(2)]

    def chunk_copies(t):
        m, c0 = divmod(t, H // CH)
        return [cp for jj in range(CH // 2)
                for cp in pair_copies(m, c0 * (CH // 2) + jj, wsem.at[t])]

    def wait_chunk(t):
        blk = wqkv.at[pl.ds(t * CH, CH)]
        pltpu.make_async_copy(blk, blk, wsem.at[t]).wait()

    def unzip(slot, r0=0, r1=D // 2):
        for r in range(r0, r1, 32):
            e, o = wqkv[slot, r:r + 32, :], wqkv[slot + 1, r:r + 32, :]
            wqkv[slot, r:r + 32, :] = (e & 0xFFFF) | (o << 16)
            wqkv[slot + 1, r:r + 32, :] = (e >> 16) | (o & jnp.uint32(0xFFFF0000))

    def start_all(cps):
        for cp in cps:
            cp.start()

    def wait_all(cps):
        for cp in cps:
            cp.wait()

    cp_c = pltpu.make_async_copy(c_hbm, cb, sem.at[0])
    x_u = x_hbm.bitcast(U32)
    cp_xe = pltpu.make_async_copy(x_hbm.at[:, 0:EARLY, :], xe, sem.at[1])
    cp_x0 = pltpu.make_async_copy(x_u.at[0], xb.at[0], sem.at[2])
    cp_m0 = pltpu.make_async_copy(m0_hbm, m0, sem.at[3])
    cp_xr = pltpu.make_async_copy(x_u.at[1:XS], xb.at[1:XS], sem.at[4])
    cp_wo = pltpu.make_async_copy(wo_hbm.bitcast(U32), wo, sem.at[5])
    cp_w1 = pltpu.make_async_copy(w1_hbm.bitcast(U32), w1, sem.at[6])
    cp_w3 = pltpu.make_async_copy(w3_hbm.bitcast(U32), w3, sem.at[7])
    cp_w2 = pltpu.make_async_copy(w2_hbm.bitcast(U32), w2, sem.at[8])
    cp_wm = [pltpu.make_async_copy(wm_u.at[:, k * D:(k + 1) * D], wm.at[k], sem.at[7 + k])
             for k in range(2, 6)]
    cp_xl = pltpu.make_async_copy(x_u.at[XS:NSEG], xb.at[XS:NSEG], sem.at[13])
    cp_wa = [[pltpu.make_async_copy(wm_u.at[:, k * D + q * SW:k * D + (q + 1) * SW],
                                    wm.at[k, :, q * SW:(q + 1) * SW], sem.at[14 + 3 * q])
              for k in range(2)] for q in range(NS)]
    cp_ks = [[[cp for j in range(4 * t, 4 * t + 4)
               for cp in pair_copies(0, j, sem.at[15 + 3 * q + t], q * SW // 2, (q + 1) * SW // 2)]
              for t in range(2)] for q in range(NS)]

    start_all([cp_xe, cp_c, cp_x0, cp_m0] + cp_wa[0])
    keep, fill = _attn_mask()
    keep_s[...] = keep.astype(jnp.int32)
    fill_s[...] = fill
    wait_all([cp_xe, cp_c, cp_x0, cp_m0])
    start_all(cp_ks[0][0] + cp_ks[0][1])
    cf = cb[...].astype(F32)
    sc16 = jnp.broadcast_to(cf * jax.nn.sigmoid(cf), (16, D)).astype(BF16)
    for g in range(NSEG // 8):
        nrm[64 * g:64 * g + 64, :] = _norm(xe[8 * g:8 * g + 8].astype(F32).reshape(8 * EARLY, D))

    def mod_unit(k, c0, c1):
        mod[k, :, c0:c1] = _dot(sc16, _bf(wm[k, :, c0:c1]))[0:8]

    def ln1_mod(n, c0=0, c1=D):
        return _affine(n, 1.0 + mod[1, :, c0:c1], mod[0, :, c0:c1])

    def next_lhs(mem_f32, s):
        hx = ln1_mod(_norm(_bf(xb[s]).astype(F32)[EARLY:SEG]))
        l32[...] = _pk(jnp.concatenate([mem_f32, hx], axis=0))

    def early_dot(head, c, c0=0, c1=D):
        return _dot(_bf(p32[64 * c:64 * c + 64, c0:c1]), _bf(wqkv[head, c0 // 2:c1 // 2, :]))

    def early_store(slot, c, ab):
        pre[slot // 2, 16 * c:16 * c + 16] = _pk(
            jnp.concatenate([v.reshape(16, EARLY, DH) for v in ab], axis=1))

    def early_run(slot0, npairs, c0=0, c1=D, blocks=range(NEARLY // 128)):
        unzip(slot0, c0 // 2, c1 // 2)
        for slot in range(0, 2 * npairs, 2):
            if slot + 2 < 2 * npairs:
                unzip(slot0 + slot + 2, c0 // 2, c1 // 2)
            for c in blocks:
                ab = [early_dot(slot0 + slot + hh, c, c0, c1) for hh in range(2)]
                rows = slice(128 * c, 128 * c + 128)
                if c0 > 0:
                    ab = [ab[hh] + part[slot0 + slot + hh, rows, :] for hh in range(2)]
                if c1 < D:
                    for hh in range(2):
                        part[slot0 + slot + hh, rows, :] = ab[hh]
                else:
                    early_store(slot0 + slot, c, ab)

    later = [cp_wa[q] + cp_ks[q][0] + cp_ks[q][1] for q in range(1, NS)]
    later += [chunk_copies(2) + chunk_copies(3) + chunk_copies(4)]
    for q in range(NS):
        c0, c1 = q * SW, (q + 1) * SW
        wait_all(cp_wa[q])
        start_all(later[q])
        for k in range(2):
            mod_unit(k, c0, c1)
        for n in range(c0, c1, 128):
            for g in range(NEARLY // 128):
                p32[64 * g:64 * g + 64, n:n + 128] = _pk(ln1_mod(nrm[128 * g:128 * g + 128, n:n + 128], n, n + 128))
        if q + 2 < NS:
            for t in range(2):
                wait_all(cp_ks[q][t])
                early_run(t * CH, CH // 2, c0, c1)
        else:
            wait_all(cp_ks[q][0] + cp_ks[q][1])
            early_run(0, CH, c0, c1)
    next_lhs(m0[...].astype(F32), 0)
    wait_chunk(2)
    start_all([cp for t in range(5, 9) for cp in chunk_copies(t)])
    early_run(2 * CH, CH // 2)

    def prologue(r, carry):
        wait_chunk(2 * r + 1)
        wait_chunk(2 * r + 2)

        @pl.when(r == 1)
        def _():
            start_all([cp for t in range(9, NCH) for cp in chunk_copies(t)])

        @pl.when(r == 2)
        def _():
            start_all([cp_xr, cp_wo] + cp_wm + [cp_w1, cp_w3, cp_w2, cp_xl])

        early_run((2 * r + 1) * CH, CH)
        return carry

    lax.fori_loop(1, (NCH - NDEF - 1) // 2, prologue, 0)

    for t in range(NCH - NDEF, NCH):
        wait_chunk(t)
    wait_all([cp_xr, cp_wo])
    early_run((NCH - NDEF) * CH, NDEF * CH // 2, blocks=(0,))

    def resid1(p, dst):
        for n in range(0, D, 256):
            xf = _bf(xb[pl.ds(2 * p, 2), :, n:n + 256]).astype(F32).reshape(PR, 256)
            dst[:, n:n + 256] = xf + _affine(abuf[:, n:n + 256], mod[2, :, n:n + 256])

    def advance(p):
        x1c[...] = x1n[...]
        resid1(p, x1n)

    def ln2(src, q):
        h2[q * SEG:(q + 1) * SEG, :] = _pk(_affine(_norm(src[...]), 1.0 + mod[4], mod[3]))

    def gate_up_units(q0, q1, chunks):
        r0, r1 = q0 * SEG, q1 * SEG
        half = {}

        def gate(f0):
            half[f0] = 0.5 * _dot(_bf(h2[r0:r1, :]), _bf(w1[:, f0:f0 + 128]))

        def up(f0):
            t = half.pop(f0)
            u = _dot(_bf(h2[r0:r1, :]), _bf(w3[:, f0:f0 + 128]))
            act[r0:r1, f0:f0 + 128] = _pk((t + t * jnp.tanh(t)) * u)

        return [functools.partial(fn, 128 * ck) for ck in chunks for fn in (gate, up)]

    def down_units(p, q, x1, nsplit):
        kq = F // nsplit
        acc = {}

        def down(n0, k):
            y = _dot(_bf(act[q * SEG:(q + 1) * SEG, k * kq:(k + 1) * kq]),
                     _bf(w2[k * kq // 2:(k + 1) * kq // 2, n0:n0 + 128]))
            if k > 0:
                y = y + acc.pop(n0)
            if k + 1 < nsplit:
                acc[n0] = y
                return
            res = x1[:, n0:n0 + 128] + _affine(y, mod[5, :, n0:n0 + 128])
            ost[pl.ds(2 * p, 2), :, n0:n0 + 128] = res.astype(BF16).reshape(2, SEG, 128)

        return [functools.partial(down, n0, k) for n0 in range(0, D, 128) for k in range(nsplit)]

    def out_copy(p, npairs):
        rows = pl.ds(2 * p, 2 * npairs)
        return pltpu.make_async_copy(ost.at[rows], out_hbm.at[rows], osem)

    c_exp = SCALE * math.log2(math.e)
    nb = 256

    def step(s, second, fill):
        rows = SEG + 2 * EARLY if second else SEG
        lhs = _bf(l32[...])
        qkv, prob = {}, {}

        def project(j):
            out = []
            for m in range(3):
                a = _dot(lhs, _bf(wqkv[m * H + 2 * j])).astype(BF16)
                b = _dot(lhs, _bf(wqkv[m * H + 2 * j + 1])).astype(BF16)
                out.append(jnp.concatenate([a, b, _bf(pre[m * NP + j, s])], axis=0))
                fill(3 * j + m)
            qkv[j] = out

        def scores(j):
            q, k, _ = qkv[j]
            sc_ = lax.dot_general(q, k, (((1,), (1,)), ((), ())), preferred_element_type=F32)
            sc_ = jnp.where(keep_s[...] != 0, sc_, fill_s[...])
            e = jnp.exp2((sc_ - jnp.max(sc_, axis=1, keepdims=True)) * c_exp)
            den = jnp.sum(e, axis=1, keepdims=True)
            r = pl.reciprocal(den, approx=True)
            r = r * (2.0 - den * r)
            prob[j] = (e * r).astype(BF16)

        def values(j):
            o = _dot(prob.pop(j), qkv.pop(j)[2])
            for hh in range(2):
                c0 = (2 * j + hh) * DH
                main = o[hh * SEG:(hh + 1) * SEG]
                early = o[2 * SEG + hh * EARLY:2 * SEG + (hh + 1) * EARLY]
                if second:
                    ob[:, c0:c0 + DH] = _pk(jnp.concatenate([main, oda[:, c0:c0 + DH], early], axis=0))
                else:
                    ob[0:SEG // 2, c0:c0 + DH] = _pk(main)
                    oda[:, c0:c0 + DH] = early

        def wo_part(n, j0, j1):
            k0, k1 = j0 * 2 * DH, j1 * 2 * DH
            return _dot(_bf(ob[0:rows // 2, k0:k1]), _bf(wo[k0 // 2:k1 // 2, n * nb:(n + 1) * nb]))

        for j in range(NP):
            project(j)
            if j >= 1:
                scores(j - 1)
            if j >= 3:
                values(j - 3)
        y0 = wo_part(0, 0, 6)
        scores(NP - 1)
        values(NP - 3)
        y0 = y0 + wo_part(0, 6, 12)
        values(NP - 2)
        fill('mid')
        y1 = wo_part(1, 0, 8)
        values(NP - 1)
        y1 = y1 + wo_part(1, 8, 13)
        y2 = wo_part(2, 0, 14)
        y0 = y0 + wo_part(0, 12, NP)
        y1 = y1 + wo_part(1, 13, NP)
        y2 = y2 + wo_part(2, 14, NP)
        y = jnp.concatenate([y0, y1, y2, wo_part(3, 0, NP)], axis=1)
        next_lhs(y[0:MEM], jnp.minimum(s + 1, NSEG - 1))
        fill('end')
        return y

    def pair(i, units, counts):
        units = list(units)

        def filler(second):
            def fill(point):
                for _ in range(counts.get((second, point), 0)):
                    units.pop(0)()
            return fill

        advance(jnp.maximum(i - 1, 0))
        ya = step(2 * i, False, filler(False))
        abuf[EARLY:SEG, :] = ya[MEM:SEG]
        yb = step(2 * i + 1, True, filler(True))
        abuf[0:EARLY, :] = yb[SEG:SEG + EARLY]
        abuf[SEG:SEG + EARLY, :] = yb[SEG + EARLY:SEG + 2 * EARLY]
        abuf[SEG + EARLY:PR, :] = yb[MEM:SEG]
        assert not units

    def head_pairs(i, carry):
        for kk in range(2):
            k = 2 + 2 * i + kk
            pltpu.make_async_copy(wm.at[k], wm.at[k], sem.at[7 + k]).wait()
        mods = [functools.partial(mod_unit, 2 + 2 * i + kk, n0, n0 + 128)
                for kk in range(2) for n0 in range(0, D, 128)]
        npr = NDEF * CH // 2 // LAG
        slot0 = (NCH - NDEF) * CH + 2 * npr * i
        held = {}

        def piece(slot, c, hh, hf):
            v = early_dot(slot + hh, c, hf * D // 2, (hf + 1) * D // 2)
            held[hh] = v if hf == 0 else v + held[hh]
            if hh == 1 and hf == 1:
                early_store(slot, c, [held.pop(0), held.pop(1)])

        pieces = [functools.partial(piece, slot0 + 2 * g, c, hh, hf)
                  for g in range(npr) for c in range(1, 4) for hh in range(2) for hf in range(2)]
        units, counts = [], {}
        tail = {(False, 'mid'): 1, (False, 'end'): 3, (True, 'mid'): 1, (True, 'end'): 2}
        inner = len(pieces) - sum(tail.values())
        for second in (False, True):
            for pt in list(range(3 * NP)) + ['mid', 'end']:
                if pt in ('mid', 'end'):
                    n = tail[(second, pt)]
                else:
                    k = second * 3 * NP + pt
                    n = (k + 1) * inner // (6 * NP) - k * inner // (6 * NP)
                here = []
                for _ in range(n):
                    here.append(pieces.pop(0))
                    if mods:
                        here.append(mods.pop(0))
                if second and pt == 'mid':
                    assert not mods
                    here.append(functools.partial(ln2, x1n, 0))
                units += here
                counts[(second, pt)] = len(here)
        pair(i, units, counts)
        return carry

    lax.fori_loop(0, LAG, head_pairs, 0)
    wait_all([cp_w1, cp_w3, cp_w2])

    nf = F // 128
    counts = {(False, 'mid'): 2, (False, 'end'): 4, (True, 'mid'): 2, (True, 'end'): 5}
    n_inner = 2 * nf + 1 + 32 - sum(counts.values())
    for k in range(6 * NP):
        counts[(k >= 3 * NP, k % (3 * NP))] = (k + 1) * n_inner // (6 * NP) - k * n_inner // (6 * NP)

    def main_pairs(p, carry):
        @pl.when(p == 1)
        def _():
            cp_xl.wait()

        @pl.when(p >= 1)
        def _():
            out_copy(p - 1, 1).start()

        units = gate_up_units(0, 1, range(nf))
        units.append(functools.partial(ln2, x1n, 0))
        units += down_units(p, 0, x1c, 4)
        pair(p + LAG, units, counts)
        return carry

    lax.fori_loop(0, NPAIR - LAG, main_pairs, 0)

    p0 = NPAIR - LAG
    out_copy(p0 - 1, 1).start()
    resid1(p0 + 1, x1c)
    ln2(x1c, 1)
    units = gate_up_units(0, 1, range(2)) + gate_up_units(1, 2, range(2)) + gate_up_units(0, 2, range(2, nf))
    for q in range(LAG):
        units += down_units(p0 + q, q, (x1n, x1c)[q], 1) + [out_copy(p0 + q, 1).start]
    for unit in units:
        unit()
    out_copy(0, NPAIR).wait()


@jax.jit
def pallas_adaLN_cond__memory_aug_recurrent_mem_tr__glu_gated_swiglu__prompt_kernel(
    A_x, A_mem0, A_Wq, A_Wk, A_Wv, A_Wo, A_seg_len, B_x, B_w1, B_w3, B_w2, c, w_mod,
):
    assert A_x.shape == (1, S, D) and A_mem0.shape == (1, MEM, D)
    del A_seg_len
    del B_x
    vm = pltpu.VMEM
    scratch = [
        vm((3 * H, D // 2, DH), U32),
        vm((HD // 2, D), U32),
        vm((D // 2, F), U32),
        vm((D // 2, F), U32),
        vm((F // 2, D), U32),
        vm((6, D // 2, D), U32),
        vm((NSEG, SEG // 2, D), U32),
        vm((NSEG, EARLY, D), BF16),
        vm((1, D), BF16),
        vm((MEM, D), BF16),
        vm((6, 8, D), F32),
        vm((NEARLY, D), F32),
        vm((NEARLY // 2, D), U32),
        vm((2 * CH, NEARLY, DH), F32),
        vm((3 * NP, NSEG, EARLY, DH), U32),
        vm((SEG // 2, D), U32),
        vm((SEG // 2 + EARLY, HD), U32),
        vm((EARLY, HD), F32),
        vm((PR, D), F32),
        vm((PR, D), F32),
        vm((PR, D), F32),
        vm((LAG * SEG, D), U32),
        vm((LAG * SEG, F), U32),
        vm((NSEG, SEG, D), BF16),
        vm((L2, L2), jnp.int32),
        vm((L2, L2), F32),
        pltpu.SemaphoreType.DMA((14 + 3 * NS,)),
        pltpu.SemaphoreType.DMA((NCH,)),
        pltpu.SemaphoreType.DMA(()),
    ]
    out = pl.pallas_call(
        _kernel,
        out_shape=jax.ShapeDtypeStruct((NSEG, SEG, D), BF16),
        in_specs=[pl.BlockSpec(memory_space=pl.ANY)] * 11,
        out_specs=pl.BlockSpec(memory_space=pl.ANY),
        scratch_shapes=scratch,
        compiler_params=pltpu.CompilerParams(vmem_limit_bytes=120 * 1024 * 1024,
                                             disable_bounds_checks=True,
                                             disable_semaphore_checks=True),
    )(
        A_x.reshape(NSEG, SEG, D),
        A_mem0.reshape(MEM, D),
        A_Wq.reshape(D // 2, 2 * H, DH),
        A_Wk.reshape(D // 2, 2 * H, DH),
        A_Wv.reshape(D // 2, 2 * H, DH),
        A_Wo.reshape(HD, D),
        B_w1, B_w3, B_w2, c, w_mod,
    )
    return out.reshape(1, S, D)
```

```python
import functools
import math

import jax
import jax.numpy as jnp
from jax import lax
import jax.experimental.pallas as pl
import jax.experimental.pallas.tpu as pltpu

S, D, H, DH, MEM, SEG, F = 2048, 1024, 32, 128, 8, 32, 3584
NSEG = S // SEG
NP = H // 2
HD = H * DH
EARLY = 8
NEARLY = NSEG * EARLY
L2 = 2 * (MEM + SEG)
CH = 8
NCH = 3 * H // CH
NS = 4
SW = D // NS
NKS = 3
XS = 8
NDEF = 1
NPAIR = NSEG // 2
PR = 2 * SEG
LAG = 2
EPS = 1e-5
SCALE = DH ** -0.5
MASK_FILL = -1000000000.0

BF16, F32, U32 = jnp.bfloat16, jnp.float32, jnp.uint32


def _bf(x_u32):
    return pltpu.bitcast(x_u32, BF16)


def _pk(x_f32):
    return pltpu.bitcast(x_f32.astype(BF16), U32)


def _dot(a, b):
    return jnp.dot(a, b, preferred_element_type=F32)


def _affine(x, scale8, shift8=None):
    y = x.reshape(-1, 8, x.shape[-1]) * scale8[None]
    if shift8 is not None:
        y = y + shift8[None]
    return y.reshape(x.shape)


def _norm(x):
    m = jnp.mean(x, axis=-1, keepdims=True)
    xc = x - m
    v = jnp.mean(xc * xc, axis=-1, keepdims=True)
    return xc * lax.rsqrt(v + EPS)


def _attn_mask():
    def meta(i):
        head = jnp.where(i < 2 * SEG, i // SEG, (i - 2 * SEG) // EARLY)
        j = i % SEG
        pos = jnp.where(i < 2 * SEG, jnp.where(j < MEM, j, j + EARLY), MEM + (i - 2 * SEG) % EARLY)
        return head, pos
    r = lax.broadcasted_iota(jnp.int32, (L2, L2), 0)
    c = lax.broadcasted_iota(jnp.int32, (L2, L2), 1)
    rh, rp = meta(r)
    chd, cp = meta(c)
    same = rh == chd
    keep = same & ((rp < MEM) | (rp >= cp))
    fill = jnp.where(same, MASK_FILL / SCALE, -jnp.inf).astype(F32)
    return keep, fill


def _kernel(x_hbm, m0_hbm, wq_hbm, wk_hbm, wv_hbm, wo_hbm, w1_hbm, w3_hbm, w2_hbm, c_hbm, wm_hbm,
            out_hbm,
            wqkv, wo, w1, w3, w2, wm, xb, xe, cb, m0, mod, nrm, p32, part, pre, l32, ob, oda, abuf,
            x1n, x1c, h2, act, ost, keep_s, fill_s, sem, wsem, osem):
    w_hbm = [r.bitcast(U32) for r in (wq_hbm, wk_hbm, wv_hbm)]
    wm_u = wm_hbm.bitcast(U32)

    def pair_copies(m, j, dsem, r0=0, r1=D // 2):
        return [pltpu.make_async_copy(w_hbm[m].at[r0:r1, par * NP + j, :],
                                      wqkv.at[m * H + 2 * j + par, r0:r1, :], dsem) for par in range(2)]

    def chunk_copies(t):
        m, c0 = divmod(t, H // CH)
        return [cp for jj in range(CH // 2)
                for cp in pair_copies(m, c0 * (CH // 2) + jj, wsem.at[t])]

    def wait_chunk(t):
        blk = wqkv.at[pl.ds(t * CH, CH)]
        pltpu.make_async_copy(blk, blk, wsem.at[t]).wait()

    def unzip(slot, r0=0, r1=D // 2):
        for r in range(r0, r1, 32):
            e, o = wqkv[slot, r:r + 32, :], wqkv[slot + 1, r:r + 32, :]
            wqkv[slot, r:r + 32, :] = (e & 0xFFFF) | (o << 16)
            wqkv[slot + 1, r:r + 32, :] = (e >> 16) | (o & jnp.uint32(0xFFFF0000))

    def start_all(cps):
        for cp in cps:
            cp.start()

    def wait_all(cps):
        for cp in cps:
            cp.wait()

    cp_c = pltpu.make_async_copy(c_hbm, cb, sem.at[0])
    x_u = x_hbm.bitcast(U32)
    cp_xe = pltpu.make_async_copy(x_hbm.at[:, 0:EARLY, :], xe, sem.at[1])
    cp_x0 = pltpu.make_async_copy(x_u.at[0], xb.at[0], sem.at[2])
    cp_m0 = pltpu.make_async_copy(m0_hbm, m0, sem.at[3])
    cp_xr = pltpu.make_async_copy(x_u.at[1:XS], xb.at[1:XS], sem.at[4])
    cp_wo = pltpu.make_async_copy(wo_hbm.bitcast(U32), wo, sem.at[5])
    cp_w1 = pltpu.make_async_copy(w1_hbm.bitcast(U32), w1, sem.at[6])
    cp_w3 = pltpu.make_async_copy(w3_hbm.bitcast(U32), w3, sem.at[7])
    cp_w2 = pltpu.make_async_copy(w2_hbm.bitcast(U32), w2, sem.at[8])
    cp_wm = [pltpu.make_async_copy(wm_u.at[:, k * D:(k + 1) * D], wm.at[k], sem.at[7 + k])
             for k in range(2, 6)]
    cp_xl = pltpu.make_async_copy(x_u.at[XS:NSEG], xb.at[XS:NSEG], sem.at[13])
    cp_wa = [[pltpu.make_async_copy(wm_u.at[:, k * D + q * SW:k * D + (q + 1) * SW],
                                    wm.at[k, :, q * SW:(q + 1) * SW], sem.at[14 + (NKS + 1) * q])
              for k in range(2)] for q in range(NS)]
    cp_ks = [[[cp for j in range(4 * t, 4 * t + 4)
               for cp in pair_copies(0, j, sem.at[15 + (NKS + 1) * q + t], q * SW // 2, (q + 1) * SW // 2)]
              for t in range(NKS)] for q in range(NS)]

    start_all([cp_xe, cp_c, cp_x0, cp_m0] + cp_wa[0])
    keep, fill = _attn_mask()
    keep_s[...] = keep.astype(jnp.int32)
    fill_s[...] = fill
    wait_all([cp_xe, cp_c, cp_x0, cp_m0])
    start_all(cp_ks[0][0])
    cf = cb[...].astype(F32)
    sc16 = jnp.broadcast_to(cf * jax.nn.sigmoid(cf), (16, D)).astype(BF16)
    for g in range(NSEG // 8):
        nrm[64 * g:64 * g + 64, :] = _norm(xe[8 * g:8 * g + 8].astype(F32).reshape(8 * EARLY, D))

    def mod_unit(k, c0, c1):
        mod[k, :, c0:c1] = _dot(sc16, _bf(wm[k, :, c0:c1]))[0:8]

    def ln1_mod(n, c0=0, c1=D):
        return _affine(n, 1.0 + mod[1, :, c0:c1], mod[0, :, c0:c1])

    def next_lhs(mem_f32, s):
        hx = ln1_mod(_norm(_bf(xb[s]).astype(F32)[EARLY:SEG]))
        l32[...] = _pk(jnp.concatenate([mem_f32, hx], axis=0))

    def early_dot(head, c, c0=0, c1=D):
        return _dot(_bf(p32[64 * c:64 * c + 64, c0:c1]), _bf(wqkv[head, c0 // 2:c1 // 2, :]))

    def early_store(slot, c, ab):
        pre[slot // 2, 16 * c:16 * c + 16] = _pk(
            jnp.concatenate([v.reshape(16, EARLY, DH) for v in ab], axis=1))

    def early_run(slot0, npairs, c0=0, c1=D, blocks=range(NEARLY // 128)):
        unzip(slot0, c0 // 2, c1 // 2)
        for slot in range(0, 2 * npairs, 2):
            if slot + 2 < 2 * npairs:
                unzip(slot0 + slot + 2, c0 // 2, c1 // 2)
            for c in blocks:
                ab = [early_dot(slot0 + slot + hh, c, c0, c1) for hh in range(2)]
                rows = slice(128 * c, 128 * c + 128)
                if c0 > 0:
                    ab = [ab[hh] + part[slot0 + slot + hh, rows, :] for hh in range(2)]
                if c1 < D:
                    for hh in range(2):
                        part[slot0 + slot + hh, rows, :] = ab[hh]
                else:
                    early_store(slot0 + slot, c, ab)

    def sl(q):
        return cp_wa[q] + [cp for t in range(NKS) for cp in cp_ks[q][t]]

    def ch(*ts):
        return [cp for t in ts for cp in chunk_copies(t)]

    stages = [[((), cp_ks[0][1]), ((0,), cp_ks[0][2]), ((1,), sl(1)), ((2,), [])],
              [((), sl(2)), ((0,), []), ((1, 2), sl(3))],
              [((), []), ((0, 1, 2), ch(3, 4))],
              [((), []), ((0, 1, 2), ch(5, 6, 7, 8))]]
    for q in range(NS):
        c0, c1 = q * SW, (q + 1) * SW
        for ts, issue in stages[q]:
            wait_all([cp for t in ts for cp in cp_ks[q][t]] if ts else cp_wa[q])
            start_all(issue)
            if ts:
                early_run(ts[0] * CH, len(ts) * CH // 2, c0, c1)
                continue
            for k in range(2):
                mod_unit(k, c0, c1)
            for n in range(c0, c1, 128):
                for g in range(NEARLY // 128):
                    p32[64 * g:64 * g + 64, n:n + 128] = _pk(
                        ln1_mod(nrm[128 * g:128 * g + 128, n:n + 128], n, n + 128))
    next_lhs(m0[...].astype(F32), 0)

    def prologue(r, carry):
        wait_chunk(2 * r + 1)
        wait_chunk(2 * r + 2)

        @pl.when(r == 1)
        def _():
            start_all(ch(*range(9, NCH)))

        @pl.when(r == 2)
        def _():
            start_all([cp_xr, cp_wo] + cp_wm + [cp_w1, cp_w3, cp_w2, cp_xl])

        early_run((2 * r + 1) * CH, CH)
        return carry

    lax.fori_loop(1, (NCH - NDEF - 1) // 2, prologue, 0)

    for t in range(NCH - NDEF, NCH):
        wait_chunk(t)
    wait_all([cp_xr, cp_wo])
    early_run((NCH - NDEF) * CH, NDEF * CH // 2, blocks=(0,))

    def resid1(p, dst):
        for n in range(0, D, 256):
            xf = _bf(xb[pl.ds(2 * p, 2), :, n:n + 256]).astype(F32).reshape(PR, 256)
            dst[:, n:n + 256] = xf + _affine(abuf[:, n:n + 256], mod[2, :, n:n + 256])

    def advance(p):
        x1c[...] = x1n[...]
        resid1(p, x1n)

    def ln2(src, q):
        h2[q * SEG:(q + 1) * SEG, :] = _pk(_affine(_norm(src[...]), 1.0 + mod[4], mod[3]))

    def gate_up_units(q0, q1, chunks):
        r0, r1 = q0 * SEG, q1 * SEG
        half = {}

        def gate(f0):
            half[f0] = 0.5 * _dot(_bf(h2[r0:r1, :]), _bf(w1[:, f0:f0 + 128]))

        def up(f0):
            t = half.pop(f0)
            u = _dot(_bf(h2[r0:r1, :]), _bf(w3[:, f0:f0 + 128]))
            act[r0:r1, f0:f0 + 128] = _pk((t + t * jnp.tanh(t)) * u)

        return [functools.partial(fn, 128 * ck) for ck in chunks for fn in (gate, up)]

    def down_units(p, q, x1, nsplit):
        kq = F // nsplit
        acc = {}

        def down(n0, k):
            y = _dot(_bf(act[q * SEG:(q + 1) * SEG, k * kq:(k + 1) * kq]),
                     _bf(w2[k * kq // 2:(k + 1) * kq // 2, n0:n0 + 128]))
            if k > 0:
                y = y + acc.pop(n0)
            if k + 1 < nsplit:
                acc[n0] = y
                return
            res = x1[:, n0:n0 + 128] + _affine(y, mod[5, :, n0:n0 + 128])
            ost[pl.ds(2 * p, 2), :, n0:n0 + 128] = res.astype(BF16).reshape(2, SEG, 128)

        return [functools.partial(down, n0, k) for n0 in range(0, D, 128) for k in range(nsplit)]

    def out_copy(p, npairs):
        rows = pl.ds(2 * p, 2 * npairs)
        return pltpu.make_async_copy(ost.at[rows], out_hbm.at[rows], osem)

    c_exp = SCALE * math.log2(math.e)
    nb = 256

    def step(s, second, fill):
        rows = SEG + 2 * EARLY if second else SEG
        lhs = _bf(l32[...])
        qkv, prob = {}, {}

        def project(j):
            out = []
            for m in range(3):
                a = _dot(lhs, _bf(wqkv[m * H + 2 * j])).astype(BF16)
                b = _dot(lhs, _bf(wqkv[m * H + 2 * j + 1])).astype(BF16)
                out.append(jnp.concatenate([a, b, _bf(pre[m * NP + j, s])], axis=0))
                fill(3 * j + m)
            qkv[j] = out

        def scores(j):
            q, k, _ = qkv[j]
            sc_ = lax.dot_general(q, k, (((1,), (1,)), ((), ())), preferred_element_type=F32)
            sc_ = jnp.where(keep_s[...] != 0, sc_, fill_s[...])
            e = jnp.exp2((sc_ - jnp.max(sc_, axis=1, keepdims=True)) * c_exp)
            den = jnp.sum(e, axis=1, keepdims=True)
            r = pl.reciprocal(den, approx=True)
            r = r * (2.0 - den * r)
            prob[j] = (e * r).astype(BF16)

        def values(j):
            o = _dot(prob.pop(j), qkv.pop(j)[2])
            for hh in range(2):
                c0 = (2 * j + hh) * DH
                main = o[hh * SEG:(hh + 1) * SEG]
                early = o[2 * SEG + hh * EARLY:2 * SEG + (hh + 1) * EARLY]
                if second:
                    ob[:, c0:c0 + DH] = _pk(jnp.concatenate([main, oda[:, c0:c0 + DH], early], axis=0))
                else:
                    ob[0:SEG // 2, c0:c0 + DH] = _pk(main)
                    oda[:, c0:c0 + DH] = early

        def wo_part(n, j0, j1):
            k0, k1 = j0 * 2 * DH, j1 * 2 * DH
            return _dot(_bf(ob[0:rows // 2, k0:k1]), _bf(wo[k0 // 2:k1 // 2, n * nb:(n + 1) * nb]))

        for j in range(NP):
            project(j)
            if j >= 1:
                scores(j - 1)
            if j >= 3:
                values(j - 3)
        y0 = wo_part(0, 0, 6)
        scores(NP - 1)
        values(NP - 3)
        y0 = y0 + wo_part(0, 6, 12)
        values(NP - 2)
        fill('mid')
        y1 = wo_part(1, 0, 8)
        values(NP - 1)
        y1 = y1 + wo_part(1, 8, 13)
        y2 = wo_part(2, 0, 14)
        y0 = y0 + wo_part(0, 12, NP)
        y1 = y1 + wo_part(1, 13, NP)
        y2 = y2 + wo_part(2, 14, NP)
        y = jnp.concatenate([y0, y1, y2, wo_part(3, 0, NP)], axis=1)
        next_lhs(y[0:MEM], jnp.minimum(s + 1, NSEG - 1))
        fill('end')
        return y

    def pair(i, units, counts):
        units = list(units)

        def filler(second):
            def fill(point):
                for _ in range(counts.get((second, point), 0)):
                    units.pop(0)()
            return fill

        advance(jnp.maximum(i - 1, 0))
        ya = step(2 * i, False, filler(False))
        abuf[EARLY:SEG, :] = ya[MEM:SEG]
        yb = step(2 * i + 1, True, filler(True))
        abuf[0:EARLY, :] = yb[SEG:SEG + EARLY]
        abuf[SEG:SEG + EARLY, :] = yb[SEG + EARLY:SEG + 2 * EARLY]
        abuf[SEG + EARLY:PR, :] = yb[MEM:SEG]
        assert not units

    def head_pairs(i, carry):
        for kk in range(2):
            k = 2 + 2 * i + kk
            pltpu.make_async_copy(wm.at[k], wm.at[k], sem.at[7 + k]).wait()
        mods = [functools.partial(mod_unit, 2 + 2 * i + kk, n0, n0 + 128)
                for kk in range(2) for n0 in range(0, D, 128)]
        npr = NDEF * CH // 2 // LAG
        slot0 = (NCH - NDEF) * CH + 2 * npr * i
        held = {}

        def piece(slot, c, hh, hf):
            v = early_dot(slot + hh, c, hf * D // 2, (hf + 1) * D // 2)
            held[hh] = v if hf == 0 else v + held[hh]
            if hh == 1 and hf == 1:
                early_store(slot, c, [held.pop(0), held.pop(1)])

        pieces = [functools.partial(piece, slot0 + 2 * g, c, hh, hf)
                  for g in range(npr) for c in range(1, 4) for hh in range(2) for hf in range(2)]
        units, counts = [], {}
        tail = {(False, 'mid'): 1, (False, 'end'): 3, (True, 'mid'): 1, (True, 'end'): 2}
        inner = len(pieces) - sum(tail.values())
        for second in (False, True):
            for pt in list(range(3 * NP)) + ['mid', 'end']:
                if pt in ('mid', 'end'):
                    n = tail[(second, pt)]
                else:
                    k = second * 3 * NP + pt
                    n = (k + 1) * inner // (6 * NP) - k * inner // (6 * NP)
                here = []
                for _ in range(n):
                    here.append(pieces.pop(0))
                    if mods:
                        here.append(mods.pop(0))
                if second and pt == 'mid':
                    assert not mods
                    here.append(functools.partial(ln2, x1n, 0))
                units += here
                counts[(second, pt)] = len(here)
        pair(i, units, counts)
        return carry

    lax.fori_loop(0, LAG, head_pairs, 0)
    wait_all([cp_w1, cp_w3, cp_w2])

    nf = F // 128
    counts = {(False, 'mid'): 2, (False, 'end'): 4, (True, 'mid'): 2, (True, 'end'): 5}
    n_inner = 2 * nf + 1 + 32 - sum(counts.values())
    for k in range(6 * NP):
        counts[(k >= 3 * NP, k % (3 * NP))] = (k + 1) * n_inner // (6 * NP) - k * n_inner // (6 * NP)

    def main_pairs(p, carry):
        @pl.when(p == 1)
        def _():
            cp_xl.wait()

        @pl.when(p >= 1)
        def _():
            out_copy(p - 1, 1).start()

        units = gate_up_units(0, 1, range(nf))
        units.append(functools.partial(ln2, x1n, 0))
        units += down_units(p, 0, x1c, 4)
        pair(p + LAG, units, counts)
        return carry

    lax.fori_loop(0, NPAIR - LAG, main_pairs, 0)

    p0 = NPAIR - LAG
    out_copy(p0 - 1, 1).start()
    resid1(p0 + 1, x1c)
    ln2(x1c, 1)
    units = gate_up_units(0, 1, range(2)) + gate_up_units(1, 2, range(2)) + gate_up_units(0, 2, range(2, nf))
    for q in range(LAG):
        units += down_units(p0 + q, q, (x1n, x1c)[q], 1) + [out_copy(p0 + q, 1).start]
    for unit in units:
        unit()
    out_copy(0, NPAIR).wait()


@jax.jit
def pallas_adaLN_cond__memory_aug_recurrent_mem_tr__glu_gated_swiglu__prompt_kernel(
    A_x, A_mem0, A_Wq, A_Wk, A_Wv, A_Wo, A_seg_len, B_x, B_w1, B_w3, B_w2, c, w_mod,
):
    assert A_x.shape == (1, S, D) and A_mem0.shape == (1, MEM, D)
    del A_seg_len
    del B_x
    vm = pltpu.VMEM
    scratch = [
        vm((3 * H, D // 2, DH), U32),
        vm((HD // 2, D), U32),
        vm((D // 2, F), U32),
        vm((D // 2, F), U32),
        vm((F // 2, D), U32),
        vm((6, D // 2, D), U32),
        vm((NSEG, SEG // 2, D), U32),
        vm((NSEG, EARLY, D), BF16),
        vm((1, D), BF16),
        vm((MEM, D), BF16),
        vm((6, 8, D), F32),
        vm((NEARLY, D), F32),
        vm((NEARLY // 2, D), U32),
        vm((NKS * CH, NEARLY, DH), F32),
        vm((3 * NP, NSEG, EARLY, DH), U32),
        vm((SEG // 2, D), U32),
        vm((SEG // 2 + EARLY, HD), U32),
        vm((EARLY, HD), F32),
        vm((PR, D), F32),
        vm((PR, D), F32),
        vm((PR, D), F32),
        vm((LAG * SEG, D), U32),
        vm((LAG * SEG, F), U32),
        vm((NSEG, SEG, D), BF16),
        vm((L2, L2), jnp.int32),
        vm((L2, L2), F32),
        pltpu.SemaphoreType.DMA((14 + (NKS + 1) * NS,)),
        pltpu.SemaphoreType.DMA((NCH,)),
        pltpu.SemaphoreType.DMA(()),
    ]
    out = pl.pallas_call(
        _kernel,
        out_shape=jax.ShapeDtypeStruct((NSEG, SEG, D), BF16),
        in_specs=[pl.BlockSpec(memory_space=pl.ANY)] * 11,
        out_specs=pl.BlockSpec(memory_space=pl.ANY),
        scratch_shapes=scratch,
        compiler_params=pltpu.CompilerParams(vmem_limit_bytes=120 * 1024 * 1024,
                                             disable_bounds_checks=True,
                                             disable_semaphore_checks=True),
    )(
        A_x.reshape(NSEG, SEG, D),
        A_mem0.reshape(MEM, D),
        A_Wq.reshape(D // 2, 2 * H, DH),
        A_Wk.reshape(D // 2, 2 * H, DH),
        A_Wv.reshape(D // 2, 2 * H, DH),
        A_Wo.reshape(HD, D),
        B_w1, B_w3, B_w2, c, w_mod,
    )
    return out.reshape(1, S, D)
```

```python
import functools
import math

import jax
import jax.numpy as jnp
from jax import lax
import jax.experimental.pallas as pl
import jax.experimental.pallas.tpu as pltpu

S, D, H, DH, MEM, SEG, F = 2048, 1024, 32, 128, 8, 32, 3584
NSEG = S // SEG
NP = H // 2
HD = H * DH
EARLY = 8
NEARLY = NSEG * EARLY
L2 = 2 * (MEM + SEG)
CH = 8
NCH = 3 * H // CH
SL = (0, 256, 512, D)
NS = len(SL) - 1
NKS = 3
XS = 8
NDEF = 1
NPAIR = NSEG // 2
PR = 2 * SEG
LAG = 2
EPS = 1e-5
SCALE = DH ** -0.5
MASK_FILL = -1000000000.0

BF16, F32, U32 = jnp.bfloat16, jnp.float32, jnp.uint32


def _bf(x_u32):
    return pltpu.bitcast(x_u32, BF16)


def _pk(x_f32):
    return pltpu.bitcast(x_f32.astype(BF16), U32)


def _dot(a, b):
    return jnp.dot(a, b, preferred_element_type=F32)


def _affine(x, scale8, shift8=None):
    y = x.reshape(-1, 8, x.shape[-1]) * scale8[None]
    if shift8 is not None:
        y = y + shift8[None]
    return y.reshape(x.shape)


def _norm(x):
    m = jnp.mean(x, axis=-1, keepdims=True)
    xc = x - m
    v = jnp.mean(xc * xc, axis=-1, keepdims=True)
    return xc * lax.rsqrt(v + EPS)


def _attn_mask():
    def meta(i):
        head = jnp.where(i < 2 * SEG, i // SEG, (i - 2 * SEG) // EARLY)
        j = i % SEG
        pos = jnp.where(i < 2 * SEG, jnp.where(j < MEM, j, j + EARLY), MEM + (i - 2 * SEG) % EARLY)
        return head, pos
    r = lax.broadcasted_iota(jnp.int32, (L2, L2), 0)
    c = lax.broadcasted_iota(jnp.int32, (L2, L2), 1)
    rh, rp = meta(r)
    chd, cp = meta(c)
    same = rh == chd
    keep = same & ((rp < MEM) | (rp >= cp))
    fill = jnp.where(same, MASK_FILL / SCALE, -jnp.inf).astype(F32)
    return keep, fill


def _kernel(x_hbm, m0_hbm, wq_hbm, wk_hbm, wv_hbm, wo_hbm, w1_hbm, w3_hbm, w2_hbm, c_hbm, wm_hbm,
            out_hbm,
            wqkv, wo, w1, w3, w2, wm, xb, xe, cb, m0, mod, nrm, p32, part, pre, l32, ob, oda, abuf,
            x1n, x1c, h2, act, ost, keep_s, fill_s, sem, wsem, osem):
    w_hbm = [r.bitcast(U32) for r in (wq_hbm, wk_hbm, wv_hbm)]
    wm_u = wm_hbm.bitcast(U32)

    def pair_copies(m, j, dsem, r0=0, r1=D // 2):
        return [pltpu.make_async_copy(w_hbm[m].at[r0:r1, par * NP + j, :],
                                      wqkv.at[m * H + 2 * j + par, r0:r1, :], dsem) for par in range(2)]

    def chunk_copies(t):
        m, c0 = divmod(t, H // CH)
        return [cp for jj in range(CH // 2)
                for cp in pair_copies(m, c0 * (CH // 2) + jj, wsem.at[t])]

    def wait_chunk(t):
        blk = wqkv.at[pl.ds(t * CH, CH)]
        pltpu.make_async_copy(blk, blk, wsem.at[t]).wait()

    def unzip(slot, r0=0, r1=D // 2):
        for r in range(r0, r1, 32):
            e, o = wqkv[slot, r:r + 32, :], wqkv[slot + 1, r:r + 32, :]
            wqkv[slot, r:r + 32, :] = (e & 0xFFFF) | (o << 16)
            wqkv[slot + 1, r:r + 32, :] = (e >> 16) | (o & jnp.uint32(0xFFFF0000))

    def start_all(cps):
        for cp in cps:
            cp.start()

    def wait_all(cps):
        for cp in cps:
            cp.wait()

    cp_c = pltpu.make_async_copy(c_hbm, cb, sem.at[0])
    x_u = x_hbm.bitcast(U32)
    cp_xe = pltpu.make_async_copy(x_hbm.at[:, 0:EARLY, :], xe, sem.at[1])
    cp_x0 = pltpu.make_async_copy(x_u.at[0], xb.at[0], sem.at[2])
    cp_m0 = pltpu.make_async_copy(m0_hbm, m0, sem.at[3])
    cp_xr = pltpu.make_async_copy(x_u.at[1:XS], xb.at[1:XS], sem.at[4])
    cp_wo = pltpu.make_async_copy(wo_hbm.bitcast(U32), wo, sem.at[5])
    cp_w1 = pltpu.make_async_copy(w1_hbm.bitcast(U32), w1, sem.at[6])
    cp_w3 = pltpu.make_async_copy(w3_hbm.bitcast(U32), w3, sem.at[7])
    cp_w2 = pltpu.make_async_copy(w2_hbm.bitcast(U32), w2, sem.at[8])
    cp_wm = [pltpu.make_async_copy(wm_u.at[:, k * D:(k + 1) * D], wm.at[k], sem.at[7 + k])
             for k in range(2, 6)]
    cp_xl = pltpu.make_async_copy(x_u.at[XS:NSEG], xb.at[XS:NSEG], sem.at[13])
    cp_wa = [[pltpu.make_async_copy(wm_u.at[:, k * D + SL[q]:k * D + SL[q + 1]],
                                    wm.at[k, :, SL[q]:SL[q + 1]], sem.at[14 + (NKS + 1) * q])
              for k in range(2)] for q in range(NS)]
    cp_ks = [[[cp for j in range(4 * t, 4 * t + 4)
               for cp in pair_copies(0, j, sem.at[15 + (NKS + 1) * q + t], SL[q] // 2, SL[q + 1] // 2)]
              for t in range(NKS)] for q in range(NS)]

    start_all([cp_xe, cp_c, cp_x0, cp_m0] + cp_wa[0])
    keep, fill = _attn_mask()
    keep_s[...] = keep.astype(jnp.int32)
    fill_s[...] = fill
    abuf[...] = jnp.zeros((PR, D), F32)
    x1n[...] = jnp.zeros((PR, D), F32)
    mod[2:6] = jnp.zeros((4, 8, D), F32)
    wait_all([cp_xe, cp_c, cp_x0, cp_m0])
    start_all(cp_ks[0][0])
    cf = cb[...].astype(F32)
    sc16 = jnp.broadcast_to(cf * jax.nn.sigmoid(cf), (16, D)).astype(BF16)
    for g in range(NSEG // 8):
        nrm[64 * g:64 * g + 64, :] = _norm(xe[8 * g:8 * g + 8].astype(F32).reshape(8 * EARLY, D))

    def mod_unit(k, c0, c1):
        mod[k, :, c0:c1] = _dot(sc16, _bf(wm[k, :, c0:c1]))[0:8]

    def ln1_mod(n, c0=0, c1=D):
        return _affine(n, 1.0 + mod[1, :, c0:c1], mod[0, :, c0:c1])

    def next_lhs(mem_f32, s):
        hx = ln1_mod(_norm(_bf(xb[s]).astype(F32)[EARLY:SEG]))
        l32[...] = _pk(jnp.concatenate([mem_f32, hx], axis=0))

    def early_dot(head, c, c0=0, c1=D):
        return _dot(_bf(p32[64 * c:64 * c + 64, c0:c1]), _bf(wqkv[head, c0 // 2:c1 // 2, :]))

    def early_store(slot, c, ab):
        pre[slot // 2, 16 * c:16 * c + 16] = _pk(
            jnp.concatenate([v.reshape(16, EARLY, DH) for v in ab], axis=1))

    def early_run(slot0, npairs, c0=0, c1=D, blocks=range(NEARLY // 128)):
        unzip(slot0, c0 // 2, c1 // 2)
        for slot in range(0, 2 * npairs, 2):
            if slot + 2 < 2 * npairs:
                unzip(slot0 + slot + 2, c0 // 2, c1 // 2)
            for c in blocks:
                ab = [early_dot(slot0 + slot + hh, c, c0, c1) for hh in range(2)]
                rows = slice(128 * c, 128 * c + 128)
                if c0 > 0:
                    ab = [ab[hh] + part[slot0 + slot + hh, rows, :] for hh in range(2)]
                if c1 < D:
                    for hh in range(2):
                        part[slot0 + slot + hh, rows, :] = ab[hh]
                else:
                    early_store(slot0 + slot, c, ab)

    def sl(q):
        return cp_wa[q] + [cp for t in range(NKS) for cp in cp_ks[q][t]]

    def ch(*ts):
        return [cp for t in ts for cp in chunk_copies(t)]

    stages = [[((), cp_ks[0][1]), ((0,), cp_ks[0][2]), ((1,), sl(1)), ((2,), [])],
              [((), cp_wa[2] + cp_ks[2][0]), ((0,), cp_ks[2][1] + cp_ks[2][2]), ((1, 2), ch(3, 4))],
              [((), []), ((0,), []), ((1, 2), ch(5, 6, 7, 8))]]
    for q in range(NS):
        c0, c1 = SL[q], SL[q + 1]
        for ts, issue in stages[q]:
            wait_all([cp for t in ts for cp in cp_ks[q][t]] if ts else cp_wa[q])
            start_all(issue)
            if ts:
                early_run(ts[0] * CH, len(ts) * CH // 2, c0, c1)
                continue
            for k in range(2):
                mod_unit(k, c0, c1)
            for n in range(c0, c1, 128):
                for g in range(NEARLY // 128):
                    p32[64 * g:64 * g + 64, n:n + 128] = _pk(
                        ln1_mod(nrm[128 * g:128 * g + 128, n:n + 128], n, n + 128))
    next_lhs(m0[...].astype(F32), 0)

    def prologue(r, carry):
        wait_chunk(2 * r + 1)
        wait_chunk(2 * r + 2)

        @pl.when(r == 1)
        def _():
            start_all(ch(*range(9, NCH)))

        @pl.when(r == 2)
        def _():
            start_all([cp_xr, cp_wo] + cp_wm + [cp_w1, cp_w3, cp_w2, cp_xl])

        early_run((2 * r + 1) * CH, CH)
        return carry

    lax.fori_loop(1, (NCH - NDEF - 1) // 2, prologue, 0)

    for t in range(NCH - NDEF, NCH):
        wait_chunk(t)
    wait_all([cp_xr, cp_wo])
    early_run((NCH - NDEF) * CH, NDEF * CH // 2, blocks=(0,))

    def resid1(p, dst):
        for n in range(0, D, 256):
            xf = _bf(xb[pl.ds(2 * p, 2), :, n:n + 256]).astype(F32).reshape(PR, 256)
            dst[:, n:n + 256] = xf + _affine(abuf[:, n:n + 256], mod[2, :, n:n + 256])

    def advance(p):
        x1c[...] = x1n[...]
        resid1(p, x1n)

    def ln2(src, q):
        h2[q * SEG:(q + 1) * SEG, :] = _pk(_affine(_norm(src[...]), 1.0 + mod[4], mod[3]))

    def gate_up_units(q0, q1, chunks):
        r0, r1 = q0 * SEG, q1 * SEG
        half = {}

        def gate(f0):
            half[f0] = 0.5 * _dot(_bf(h2[r0:r1, :]), _bf(w1[:, f0:f0 + 128]))

        def up(f0):
            t = half.pop(f0)
            u = _dot(_bf(h2[r0:r1, :]), _bf(w3[:, f0:f0 + 128]))
            act[r0:r1, f0:f0 + 128] = _pk((t + t * jnp.tanh(t)) * u)

        return [functools.partial(fn, 128 * ck) for ck in chunks for fn in (gate, up)]

    def down_units(p, q, x1, nsplit):
        kq = F // nsplit
        acc = {}

        def down(n0, k):
            y = _dot(_bf(act[q * SEG:(q + 1) * SEG, k * kq:(k + 1) * kq]),
                     _bf(w2[k * kq // 2:(k + 1) * kq // 2, n0:n0 + 128]))
            if k > 0:
                y = y + acc.pop(n0)
            if k + 1 < nsplit:
                acc[n0] = y
                return
            res = x1[:, n0:n0 + 128] + _affine(y, mod[5, :, n0:n0 + 128])
            ost[pl.ds(2 * p, 2), :, n0:n0 + 128] = res.astype(BF16).reshape(2, SEG, 128)

        return [functools.partial(down, n0, k) for n0 in range(0, D, 128) for k in range(nsplit)]

    def out_copy(p, npairs):
        rows = pl.ds(2 * p, 2 * npairs)
        return pltpu.make_async_copy(ost.at[rows], out_hbm.at[rows], osem)

    c_exp = SCALE * math.log2(math.e)
    nb = 256

    def step(s, second, fill):
        rows = SEG + 2 * EARLY if second else SEG
        lhs = _bf(l32[...])
        qkv, prob = {}, {}

        def project(j):
            out = []
            for m in range(3):
                a = _dot(lhs, _bf(wqkv[m * H + 2 * j])).astype(BF16)
                b = _dot(lhs, _bf(wqkv[m * H + 2 * j + 1])).astype(BF16)
                out.append(jnp.concatenate([a, b, _bf(pre[m * NP + j, s])], axis=0))
                fill(3 * j + m)
            qkv[j] = out

        def scores(j):
            q, k, _ = qkv[j]
            sc_ = lax.dot_general(q, k, (((1,), (1,)), ((), ())), preferred_element_type=F32)
            sc_ = jnp.where(keep_s[...] != 0, sc_, fill_s[...])
            e = jnp.exp2((sc_ - jnp.max(sc_, axis=1, keepdims=True)) * c_exp)
            den = jnp.sum(e, axis=1, keepdims=True)
            r = pl.reciprocal(den, approx=True)
            r = r * (2.0 - den * r)
            prob[j] = (e * r).astype(BF16)

        def values(j):
            o = _dot(prob.pop(j), qkv.pop(j)[2])
            for hh in range(2):
                c0 = (2 * j + hh) * DH
                main = o[hh * SEG:(hh + 1) * SEG]
                early = o[2 * SEG + hh * EARLY:2 * SEG + (hh + 1) * EARLY]
                if second:
                    ob[:, c0:c0 + DH] = _pk(jnp.concatenate([main, oda[:, c0:c0 + DH], early], axis=0))
                else:
                    ob[0:SEG // 2, c0:c0 + DH] = _pk(main)
                    oda[:, c0:c0 + DH] = early

        def wo_part(n, j0, j1):
            k0, k1 = j0 * 2 * DH, j1 * 2 * DH
            return _dot(_bf(ob[0:rows // 2, k0:k1]), _bf(wo[k0 // 2:k1 // 2, n * nb:(n + 1) * nb]))

        for j in range(NP):
            project(j)
            if j >= 1:
                scores(j - 1)
            if j >= 3:
                values(j - 3)
        y0 = wo_part(0, 0, 6)
        scores(NP - 1)
        values(NP - 3)
        y0 = y0 + wo_part(0, 6, 12)
        values(NP - 2)
        fill('mid')
        y1 = wo_part(1, 0, 8)
        values(NP - 1)
        y1 = y1 + wo_part(1, 8, 13)
        y2 = wo_part(2, 0, 14)
        y0 = y0 + wo_part(0, 12, NP)
        y1 = y1 + wo_part(1, 13, NP)
        y2 = y2 + wo_part(2, 14, NP)
        y = jnp.concatenate([y0, y1, y2, wo_part(3, 0, NP)], axis=1)
        next_lhs(y[0:MEM], jnp.minimum(s + 1, NSEG - 1))
        fill('end')
        return y

    def pair(i, units, counts):
        units = list(units)

        def filler(second):
            def fill(point):
                for _ in range(counts.get((second, point), 0)):
                    units.pop(0)()
            return fill

        advance(jnp.maximum(i - 1, 0))
        ya = step(2 * i, False, filler(False))
        abuf[EARLY:SEG, :] = ya[MEM:SEG]
        yb = step(2 * i + 1, True, filler(True))
        abuf[0:EARLY, :] = yb[SEG:SEG + EARLY]
        abuf[SEG:SEG + EARLY, :] = yb[SEG + EARLY:SEG + 2 * EARLY]
        abuf[SEG + EARLY:PR, :] = yb[MEM:SEG]
        assert not units

    def head_pairs(i, carry):
        for kk in range(2):
            k = 2 + 2 * i + kk
            pltpu.make_async_copy(wm.at[k], wm.at[k], sem.at[7 + k]).wait()
        mods = [functools.partial(mod_unit, 2 + 2 * i + kk, n0, n0 + 128)
                for kk in range(2) for n0 in range(0, D, 128)]
        npr = NDEF * CH // 2 // LAG
        slot0 = (NCH - NDEF) * CH + 2 * npr * i
        held = {}

        def piece(slot, c, hh, hf):
            v = early_dot(slot + hh, c, hf * D // 2, (hf + 1) * D // 2)
            held[hh] = v if hf == 0 else v + held[hh]
            if hh == 1 and hf == 1:
                early_store(slot, c, [held.pop(0), held.pop(1)])

        pieces = [functools.partial(piece, slot0 + 2 * g, c, hh, hf)
                  for g in range(npr) for c in range(1, 4) for hh in range(2) for hf in range(2)]
        units, counts = [], {}
        tail = {(False, 'mid'): 1, (False, 'end'): 3, (True, 'mid'): 1, (True, 'end'): 2}
        inner = len(pieces) - sum(tail.values())
        for second in (False, True):
            for pt in list(range(3 * NP)) + ['mid', 'end']:
                if pt in ('mid', 'end'):
                    n = tail[(second, pt)]
                else:
                    k = second * 3 * NP + pt
                    n = (k + 1) * inner // (6 * NP) - k * inner // (6 * NP)
                here = []
                for _ in range(n):
                    here.append(pieces.pop(0))
                    if mods:
                        here.append(mods.pop(0))
                if second and pt == 'mid':
                    assert not mods
                    here.append(functools.partial(ln2, x1n, 0))
                units += here
                counts[(second, pt)] = len(here)
        pair(i, units, counts)
        return carry

    lax.fori_loop(0, LAG, head_pairs, 0)
    wait_all([cp_w1, cp_w3, cp_w2])

    nf = F // 128
    counts = {(False, 'mid'): 2, (False, 'end'): 4, (True, 'mid'): 2, (True, 'end'): 5}
    n_inner = 2 * nf + 1 + 32 - sum(counts.values())
    for k in range(6 * NP):
        counts[(k >= 3 * NP, k % (3 * NP))] = (k + 1) * n_inner // (6 * NP) - k * n_inner // (6 * NP)

    def main_pairs(p, carry):
        @pl.when(p == 1)
        def _():
            cp_xl.wait()

        @pl.when(p >= 1)
        def _():
            out_copy(p - 1, 1).start()

        units = gate_up_units(0, 1, range(nf))
        units.append(functools.partial(ln2, x1n, 0))
        units += down_units(p, 0, x1c, 4)
        pair(p + LAG, units, counts)
        return carry

    lax.fori_loop(0, NPAIR - LAG, main_pairs, 0)

    p0 = NPAIR - LAG
    out_copy(p0 - 1, 1).start()
    resid1(p0 + 1, x1c)
    ln2(x1c, 1)
    units = gate_up_units(0, 1, range(2)) + gate_up_units(1, 2, range(2)) + gate_up_units(0, 2, range(2, nf))
    for q in range(LAG):
        units += down_units(p0 + q, q, (x1n, x1c)[q], 1) + [out_copy(p0 + q, 1).start]
    for unit in units:
        unit()
    out_copy(0, NPAIR).wait()


@jax.jit
def pallas_adaLN_cond__memory_aug_recurrent_mem_tr__glu_gated_swiglu__prompt_kernel(
    A_x, A_mem0, A_Wq, A_Wk, A_Wv, A_Wo, A_seg_len, B_x, B_w1, B_w3, B_w2, c, w_mod,
):
    assert A_x.shape == (1, S, D) and A_mem0.shape == (1, MEM, D)
    del A_seg_len
    del B_x
    vm = pltpu.VMEM
    scratch = [
        vm((3 * H, D // 2, DH), U32),
        vm((HD // 2, D), U32),
        vm((D // 2, F), U32),
        vm((D // 2, F), U32),
        vm((F // 2, D), U32),
        vm((6, D // 2, D), U32),
        vm((NSEG, SEG // 2, D), U32),
        vm((NSEG, EARLY, D), BF16),
        vm((1, D), BF16),
        vm((MEM, D), BF16),
        vm((6, 8, D), F32),
        vm((NEARLY, D), F32),
        vm((NEARLY // 2, D), U32),
        vm((NKS * CH, NEARLY, DH), F32),
        vm((3 * NP, NSEG, EARLY, DH), U32),
        vm((SEG // 2, D), U32),
        vm((SEG // 2 + EARLY, HD), U32),
        vm((EARLY, HD), F32),
        vm((PR, D), F32),
        vm((PR, D), F32),
        vm((PR, D), F32),
        vm((LAG * SEG, D), U32),
        vm((LAG * SEG, F), U32),
        vm((NSEG, SEG, D), BF16),
        vm((L2, L2), jnp.int32),
        vm((L2, L2), F32),
        pltpu.SemaphoreType.DMA((14 + (NKS + 1) * NS,)),
        pltpu.SemaphoreType.DMA((NCH,)),
        pltpu.SemaphoreType.DMA(()),
    ]
    out = pl.pallas_call(
        _kernel,
        out_shape=jax.ShapeDtypeStruct((NSEG, SEG, D), BF16),
        in_specs=[pl.BlockSpec(memory_space=pl.ANY)] * 11,
        out_specs=pl.BlockSpec(memory_space=pl.ANY),
        scratch_shapes=scratch,
        compiler_params=pltpu.CompilerParams(vmem_limit_bytes=120 * 1024 * 1024,
                                             disable_bounds_checks=True,
                                             disable_semaphore_checks=True),
    )(
        A_x.reshape(NSEG, SEG, D),
        A_mem0.reshape(MEM, D),
        A_Wq.reshape(D // 2, 2 * H, DH),
        A_Wk.reshape(D // 2, 2 * H, DH),
        A_Wv.reshape(D // 2, 2 * H, DH),
        A_Wo.reshape(HD, D),
        B_w1, B_w3, B_w2, c, w_mod,
    )
    return out.reshape(1, S, D)
```

```python
import functools
import math

import jax
import jax.numpy as jnp
from jax import lax
import jax.experimental.pallas as pl
import jax.experimental.pallas.tpu as pltpu

S, D, H, DH, MEM, SEG, F = 2048, 1024, 32, 128, 8, 32, 3584
NSEG = S // SEG
NP = H // 2
HD = H * DH
EARLY = 8
NEARLY = NSEG * EARLY
L2 = 2 * (MEM + SEG)
CH = 8
NCH = 3 * H // CH
SL = (0, 256, 512, 768, D)
NS = len(SL) - 1
NKS = 3
XS = 8
NDEF = 1
NPAIR = NSEG // 2
PR = 2 * SEG
LAG = 2
EPS = 1e-5
SCALE = DH ** -0.5
MASK_FILL = -1000000000.0

BF16, F32, U32 = jnp.bfloat16, jnp.float32, jnp.uint32


def _bf(x_u32):
    return pltpu.bitcast(x_u32, BF16)


def _pk(x_f32):
    return pltpu.bitcast(x_f32.astype(BF16), U32)


def _dot(a, b):
    return jnp.dot(a, b, preferred_element_type=F32)


def _affine(x, scale8, shift8=None):
    y = x.reshape(-1, 8, x.shape[-1]) * scale8[None]
    if shift8 is not None:
        y = y + shift8[None]
    return y.reshape(x.shape)


def _norm(x):
    m = jnp.mean(x, axis=-1, keepdims=True)
    xc = x - m
    v = jnp.mean(xc * xc, axis=-1, keepdims=True)
    return xc * lax.rsqrt(v + EPS)


def _attn_mask():
    def meta(i):
        head = jnp.where(i < 2 * SEG, i // SEG, (i - 2 * SEG) // EARLY)
        j = i % SEG
        pos = jnp.where(i < 2 * SEG, jnp.where(j < MEM, j, j + EARLY), MEM + (i - 2 * SEG) % EARLY)
        return head, pos
    r = lax.broadcasted_iota(jnp.int32, (L2, L2), 0)
    c = lax.broadcasted_iota(jnp.int32, (L2, L2), 1)
    rh, rp = meta(r)
    chd, cp = meta(c)
    same = rh == chd
    keep = same & ((rp < MEM) | (rp >= cp))
    fill = jnp.where(same, MASK_FILL / SCALE, -jnp.inf).astype(F32)
    return keep, fill


def _kernel(x_hbm, m0_hbm, wq_hbm, wk_hbm, wv_hbm, wo_hbm, w1_hbm, w3_hbm, w2_hbm, c_hbm, wm_hbm,
            out_hbm,
            wqkv, wo, w1, w3, w2, wm, xb, xe, cb, m0, mod, nrm, p32, part, pre, l32, ob, oda, abuf,
            x1n, x1c, h2, act, ost, keep_s, fill_s, sem, wsem, osem):
    w_hbm = [r.bitcast(U32) for r in (wq_hbm, wk_hbm, wv_hbm)]
    wm_u = wm_hbm.bitcast(U32)

    def pair_copies(m, j, dsem, r0=0, r1=D // 2):
        return [pltpu.make_async_copy(w_hbm[m].at[r0:r1, par * NP + j, :],
                                      wqkv.at[m * H + 2 * j + par, r0:r1, :], dsem) for par in range(2)]

    def chunk_copies(t):
        m, c0 = divmod(t, H // CH)
        return [cp for jj in range(CH // 2)
                for cp in pair_copies(m, c0 * (CH // 2) + jj, wsem.at[t])]

    def wait_chunk(t):
        blk = wqkv.at[pl.ds(t * CH, CH)]
        pltpu.make_async_copy(blk, blk, wsem.at[t]).wait()

    def unzip(slot, r0=0, r1=D // 2):
        for r in range(r0, r1, 32):
            e, o = wqkv[slot, r:r + 32, :], wqkv[slot + 1, r:r + 32, :]
            wqkv[slot, r:r + 32, :] = (e & 0xFFFF) | (o << 16)
            wqkv[slot + 1, r:r + 32, :] = (e >> 16) | (o & jnp.uint32(0xFFFF0000))

    def start_all(cps):
        for cp in cps:
            cp.start()

    def wait_all(cps):
        for cp in cps:
            cp.wait()

    cp_c = pltpu.make_async_copy(c_hbm, cb, sem.at[0])
    x_u = x_hbm.bitcast(U32)
    cp_xe = pltpu.make_async_copy(x_hbm.at[:, 0:EARLY, :], xe, sem.at[1])
    cp_x0 = pltpu.make_async_copy(x_u.at[0], xb.at[0], sem.at[2])
    cp_m0 = pltpu.make_async_copy(m0_hbm, m0, sem.at[3])
    cp_xr = pltpu.make_async_copy(x_u.at[1:XS], xb.at[1:XS], sem.at[4])
    cp_wo = pltpu.make_async_copy(wo_hbm.bitcast(U32), wo, sem.at[5])
    cp_w1 = pltpu.make_async_copy(w1_hbm.bitcast(U32), w1, sem.at[6])
    cp_w3 = pltpu.make_async_copy(w3_hbm.bitcast(U32), w3, sem.at[7])
    cp_w2 = pltpu.make_async_copy(w2_hbm.bitcast(U32), w2, sem.at[8])
    cp_wm = [pltpu.make_async_copy(wm_u.at[:, k * D:(k + 1) * D], wm.at[k], sem.at[7 + k])
             for k in range(2, 6)]
    cp_xl = pltpu.make_async_copy(x_u.at[XS:NSEG], xb.at[XS:NSEG], sem.at[13])
    cp_wa = [[pltpu.make_async_copy(wm_u.at[:, k * D + SL[q]:k * D + SL[q + 1]],
                                    wm.at[k, :, SL[q]:SL[q + 1]], sem.at[14 + (NKS + 1) * q])
              for k in range(2)] for q in range(NS)]
    cp_ks = [[[cp for j in range(4 * t, 4 * t + 4)
               for cp in pair_copies(0, j, sem.at[15 + (NKS + 1) * q + t], SL[q] // 2, SL[q + 1] // 2)]
              for t in range(NKS)] for q in range(NS)]

    start_all([cp_xe, cp_c, cp_x0, cp_m0] + cp_wa[0])
    keep, fill = _attn_mask()
    keep_s[...] = keep.astype(jnp.int32)
    fill_s[...] = fill
    abuf[...] = jnp.zeros((PR, D), F32)
    x1n[...] = jnp.zeros((PR, D), F32)
    mod[2:6] = jnp.zeros((4, 8, D), F32)
    wait_all([cp_xe, cp_c, cp_x0, cp_m0])
    start_all([cp for t in range(NKS) for cp in cp_ks[0][t]])
    cf = cb[...].astype(F32)
    sc16 = jnp.broadcast_to(cf * jax.nn.sigmoid(cf), (16, D)).astype(BF16)
    for g in range(NSEG // 8):
        nrm[64 * g:64 * g + 64, :] = _norm(xe[8 * g:8 * g + 8].astype(F32).reshape(8 * EARLY, D))

    def mod_unit(k, c0, c1):
        mod[k, :, c0:c1] = _dot(sc16, _bf(wm[k, :, c0:c1]))[0:8]

    def ln1_mod(n, c0=0, c1=D):
        return _affine(n, 1.0 + mod[1, :, c0:c1], mod[0, :, c0:c1])

    def next_lhs(mem_f32, s):
        hx = ln1_mod(_norm(_bf(xb[s]).astype(F32)[EARLY:SEG]))
        l32[...] = _pk(jnp.concatenate([mem_f32, hx], axis=0))

    def early_dot(head, c, c0=0, c1=D):
        return _dot(_bf(p32[64 * c:64 * c + 64, c0:c1]), _bf(wqkv[head, c0 // 2:c1 // 2, :]))

    def early_store(slot, c, ab):
        pre[slot // 2, 16 * c:16 * c + 16] = _pk(
            jnp.concatenate([v.reshape(16, EARLY, DH) for v in ab], axis=1))

    def early_pair(slot, c0=0, c1=D, blocks=range(NEARLY // 128), between=()):
        between = list(between)
        for c in blocks:
            ab = [early_dot(slot + hh, c, c0, c1) for hh in range(2)]
            if between:
                between.pop(0)()
            rows = slice(128 * c, 128 * c + 128)
            if c0 > 0:
                ab = [ab[hh] + part[slot + hh, rows, :] for hh in range(2)]
            if c1 < D:
                for hh in range(2):
                    part[slot + hh, rows, :] = ab[hh]
            else:
                early_store(slot, c, ab)

    def early_run(slot0, npairs, blocks=range(NEARLY // 128)):
        unzip(slot0)
        for slot in range(0, 2 * npairs, 2):
            if slot + 2 < 2 * npairs:
                unzip(slot0 + slot + 2)
            early_pair(slot0 + slot, blocks=blocks)

    def ln1_early(q):
        for n in range(SL[q], SL[q + 1], 128):
            for g in range(NEARLY // 128):
                p32[64 * g:64 * g + 64, n:n + 128] = _pk(
                    ln1_mod(nrm[128 * g:128 * g + 128, n:n + 128], n, n + 128))

    def ks(q, *ts):
        return [cp for t in ts for cp in cp_ks[q][t]]

    def ch(*ts):
        return [cp for t in ts for cp in chunk_copies(t)]

    jobs = [(q, 2 * g) for q in range(NS) for g in range(NKS * CH // 2)]
    sync = {3: (ks(0, 1), [], None),
            7: (ks(0, 2), cp_wa[2] + ks(2, 0), None),
            11: (cp_wa[1] + ks(1, 0), ks(2, 1, 2), 1),
            15: (ks(1, 1, 2), cp_wa[3] + ks(3, 0, 1, 2), None),
            22: (cp_wa[2] + ks(2, 0), ch(3, 4), 2),
            27: (ks(2, 1, 2), [], None),
            34: (cp_wa[3] + ks(3, 0, 1, 2), ch(5, 6, 7, 8), 3)}
    wait_all(cp_wa[0])
    for k in range(2):
        mod_unit(k, 0, SL[1])
    ln1_early(0)
    start_all(cp_wa[1] + ks(1, 0, 1, 2))
    wait_all(ks(0, 0))
    unzip(0, 0, SL[1] // 2)
    for i, (q, slot) in enumerate(jobs):
        waits, issue, done = sync.get(i, ([], [], None))
        start_all(issue)
        wait_all(waits)
        if i + 1 < len(jobs):
            qn, slotn = jobs[i + 1]
            unzip(slotn, SL[qn] // 2, SL[qn + 1] // 2)
        if done is None:
            early_pair(slot, SL[q], SL[q + 1])
        else:
            early_pair(slot, SL[q], SL[q + 1], between=[
                functools.partial(mod_unit, k, n, n + 128)
                for n in range(SL[done], SL[done + 1], 128) for k in range(2)])
            ln1_early(done)
    next_lhs(m0[...].astype(F32), 0)

    def prologue(r, carry):
        wait_chunk(2 * r + 1)
        wait_chunk(2 * r + 2)

        @pl.when(r == 1)
        def _():
            start_all(ch(*range(9, NCH)))

        @pl.when(r == 2)
        def _():
            start_all([cp_xr, cp_wo] + cp_wm + [cp_w1, cp_w3, cp_w2, cp_xl])

        early_run((2 * r + 1) * CH, CH)
        return carry

    lax.fori_loop(1, (NCH - NDEF - 1) // 2, prologue, 0)

    for t in range(NCH - NDEF, NCH):
        wait_chunk(t)
    wait_all([cp_xr, cp_wo])
    early_run((NCH - NDEF) * CH, NDEF * CH // 2, blocks=(0,))

    def resid1(p, dst):
        for n in range(0, D, 256):
            xf = _bf(xb[pl.ds(2 * p, 2), :, n:n + 256]).astype(F32).reshape(PR, 256)
            dst[:, n:n + 256] = xf + _affine(abuf[:, n:n + 256], mod[2, :, n:n + 256])

    def advance(p):
        x1c[...] = x1n[...]
        resid1(p, x1n)

    def ln2(src, q):
        h2[q * SEG:(q + 1) * SEG, :] = _pk(_affine(_norm(src[...]), 1.0 + mod[4], mod[3]))

    def gate_up_units(q0, q1, chunks):
        r0, r1 = q0 * SEG, q1 * SEG
        half = {}

        def gate(f0):
            half[f0] = 0.5 * _dot(_bf(h2[r0:r1, :]), _bf(w1[:, f0:f0 + 128]))

        def up(f0):
            t = half.pop(f0)
            u = _dot(_bf(h2[r0:r1, :]), _bf(w3[:, f0:f0 + 128]))
            act[r0:r1, f0:f0 + 128] = _pk((t + t * jnp.tanh(t)) * u)

        return [functools.partial(fn, 128 * ck) for ck in chunks for fn in (gate, up)]

    def down_units(p, q, x1, nsplit):
        kq = F // nsplit
        acc = {}

        def down(n0, k):
            y = _dot(_bf(act[q * SEG:(q + 1) * SEG, k * kq:(k + 1) * kq]),
                     _bf(w2[k * kq // 2:(k + 1) * kq // 2, n0:n0 + 128]))
            if k > 0:
                y = y + acc.pop(n0)
            if k + 1 < nsplit:
                acc[n0] = y
                return
            res = x1[:, n0:n0 + 128] + _affine(y, mod[5, :, n0:n0 + 128])
            ost[pl.ds(2 * p, 2), :, n0:n0 + 128] = res.astype(BF16).reshape(2, SEG, 128)

        return [functools.partial(down, n0, k) for n0 in range(0, D, 128) for k in range(nsplit)]

    def out_copy(p, npairs):
        rows = pl.ds(2 * p, 2 * npairs)
        return pltpu.make_async_copy(ost.at[rows], out_hbm.at[rows], osem)

    c_exp = SCALE * math.log2(math.e)
    nb = 256

    def step(s, second, fill):
        rows = SEG + 2 * EARLY if second else SEG
        lhs = _bf(l32[...])
        qkv, prob = {}, {}

        def project(j):
            out = []
            for m in range(3):
                a = _dot(lhs, _bf(wqkv[m * H + 2 * j])).astype(BF16)
                b = _dot(lhs, _bf(wqkv[m * H + 2 * j + 1])).astype(BF16)
                out.append(jnp.concatenate([a, b, _bf(pre[m * NP + j, s])], axis=0))
                fill(3 * j + m)
            qkv[j] = out

        def scores(j):
            q, k, _ = qkv[j]
            sc_ = lax.dot_general(q, k, (((1,), (1,)), ((), ())), preferred_element_type=F32)
            sc_ = jnp.where(keep_s[...] != 0, sc_, fill_s[...])
            e = jnp.exp2((sc_ - jnp.max(sc_, axis=1, keepdims=True)) * c_exp)
            den = jnp.sum(e, axis=1, keepdims=True)
            r = pl.reciprocal(den, approx=True)
            r = r * (2.0 - den * r)
            prob[j] = (e * r).astype(BF16)

        def values(j):
            o = _dot(prob.pop(j), qkv.pop(j)[2])
            for hh in range(2):
                c0 = (2 * j + hh) * DH
                main = o[hh * SEG:(hh + 1) * SEG]
                early = o[2 * SEG + hh * EARLY:2 * SEG + (hh + 1) * EARLY]
                if second:
                    ob[:, c0:c0 + DH] = _pk(jnp.concatenate([main, oda[:, c0:c0 + DH], early], axis=0))
                else:
                    ob[0:SEG // 2, c0:c0 + DH] = _pk(main)
                    oda[:, c0:c0 + DH] = early

        def wo_part(n, j0, j1):
            k0, k1 = j0 * 2 * DH, j1 * 2 * DH
            return _dot(_bf(ob[0:rows // 2, k0:k1]), _bf(wo[k0 // 2:k1 // 2, n * nb:(n + 1) * nb]))

        for j in range(NP):
            project(j)
            if j >= 1:
                scores(j - 1)
            if j >= 3:
                values(j - 3)
        y0 = wo_part(0, 0, 6)
        scores(NP - 1)
        values(NP - 3)
        y0 = y0 + wo_part(0, 6, 12)
        values(NP - 2)
        fill('mid')
        y1 = wo_part(1, 0, 8)
        values(NP - 1)
        y1 = y1 + wo_part(1, 8, 13)
        y2 = wo_part(2, 0, 14)
        y0 = y0 + wo_part(0, 12, NP)
        y1 = y1 + wo_part(1, 13, NP)
        y2 = y2 + wo_part(2, 14, NP)
        y = jnp.concatenate([y0, y1, y2, wo_part(3, 0, NP)], axis=1)
        next_lhs(y[0:MEM], jnp.minimum(s + 1, NSEG - 1))
        fill('end')
        return y

    def pair(i, units, counts):
        units = list(units)

        def filler(second):
            def fill(point):
                for _ in range(counts.get((second, point), 0)):
                    units.pop(0)()
            return fill

        advance(jnp.maximum(i - 1, 0))
        ya = step(2 * i, False, filler(False))
        abuf[EARLY:SEG, :] = ya[MEM:SEG]
        yb = step(2 * i + 1, True, filler(True))
        abuf[0:EARLY, :] = yb[SEG:SEG + EARLY]
        abuf[SEG:SEG + EARLY, :] = yb[SEG + EARLY:SEG + 2 * EARLY]
        abuf[SEG + EARLY:PR, :] = yb[MEM:SEG]
        assert not units

    def head_pairs(i, carry):
        for kk in range(2):
            k = 2 + 2 * i + kk
            pltpu.make_async_copy(wm.at[k], wm.at[k], sem.at[7 + k]).wait()
        mods = [functools.partial(mod_unit, 2 + 2 * i + kk, n0, n0 + 128)
                for kk in range(2) for n0 in range(0, D, 128)]
        npr = NDEF * CH // 2 // LAG
        slot0 = (NCH - NDEF) * CH + 2 * npr * i
        held = {}

        def piece(slot, c, hh, hf):
            v = early_dot(slot + hh, c, hf * D // 2, (hf + 1) * D // 2)
            held[hh] = v if hf == 0 else v + held[hh]
            if hh == 1 and hf == 1:
                early_store(slot, c, [held.pop(0), held.pop(1)])

        pieces = [functools.partial(piece, slot0 + 2 * g, c, hh, hf)
                  for g in range(npr) for c in range(1, 4) for hh in range(2) for hf in range(2)]
        units, counts = [], {}
        tail = {(False, 'mid'): 1, (False, 'end'): 3, (True, 'mid'): 1, (True, 'end'): 2}
        inner = len(pieces) - sum(tail.values())
        for second in (False, True):
            for pt in list(range(3 * NP)) + ['mid', 'end']:
                if pt in ('mid', 'end'):
                    n = tail[(second, pt)]
                else:
                    k = second * 3 * NP + pt
                    n = (k + 1) * inner // (6 * NP) - k * inner // (6 * NP)
                here = []
                for _ in range(n):
                    here.append(pieces.pop(0))
                    if mods:
                        here.append(mods.pop(0))
                if second and pt == 'mid':
                    assert not mods
                    here.append(functools.partial(ln2, x1n, 0))
                units += here
                counts[(second, pt)] = len(here)
        pair(i, units, counts)
        return carry

    lax.fori_loop(0, LAG, head_pairs, 0)
    wait_all([cp_w1, cp_w3, cp_w2])

    nf = F // 128
    counts = {(False, 'mid'): 2, (False, 'end'): 4, (True, 'mid'): 2, (True, 'end'): 5}
    n_inner = 2 * nf + 1 + 32 - sum(counts.values())
    for k in range(6 * NP):
        counts[(k >= 3 * NP, k % (3 * NP))] = (k + 1) * n_inner // (6 * NP) - k * n_inner // (6 * NP)

    def main_pairs(p, carry):
        @pl.when(p == 1)
        def _():
            cp_xl.wait()

        @pl.when(p >= 1)
        def _():
            out_copy(p - 1, 1).start()

        units = gate_up_units(0, 1, range(nf))
        units.append(functools.partial(ln2, x1n, 0))
        units += down_units(p, 0, x1c, 4)
        pair(p + LAG, units, counts)
        return carry

    lax.fori_loop(0, NPAIR - LAG, main_pairs, 0)

    p0 = NPAIR - LAG
    out_copy(p0 - 1, 1).start()
    resid1(p0 + 1, x1c)
    ln2(x1c, 1)
    units = gate_up_units(0, 1, range(2)) + gate_up_units(1, 2, range(2)) + gate_up_units(0, 2, range(2, nf))
    for q in range(LAG):
        units += down_units(p0 + q, q, (x1n, x1c)[q], 1) + [out_copy(p0 + q, 1).start]
    for unit in units:
        unit()
    out_copy(0, NPAIR).wait()


@jax.jit
def pallas_adaLN_cond__memory_aug_recurrent_mem_tr__glu_gated_swiglu__prompt_kernel(
    A_x, A_mem0, A_Wq, A_Wk, A_Wv, A_Wo, A_seg_len, B_x, B_w1, B_w3, B_w2, c, w_mod,
):
    assert A_x.shape == (1, S, D) and A_mem0.shape == (1, MEM, D)
    del A_seg_len
    del B_x
    vm = pltpu.VMEM
    scratch = [
        vm((3 * H, D // 2, DH), U32),
        vm((HD // 2, D), U32),
        vm((D // 2, F), U32),
        vm((D // 2, F), U32),
        vm((F // 2, D), U32),
        vm((6, D // 2, D), U32),
        vm((NSEG, SEG // 2, D), U32),
        vm((NSEG, EARLY, D), BF16),
        vm((1, D), BF16),
        vm((MEM, D), BF16),
        vm((6, 8, D), F32),
        vm((NEARLY, D), F32),
        vm((NEARLY // 2, D), U32),
        vm((NKS * CH, NEARLY, DH), F32),
        vm((3 * NP, NSEG, EARLY, DH), U32),
        vm((SEG // 2, D), U32),
        vm((SEG // 2 + EARLY, HD), U32),
        vm((EARLY, HD), F32),
        vm((PR, D), F32),
        vm((PR, D), F32),
        vm((PR, D), F32),
        vm((LAG * SEG, D), U32),
        vm((LAG * SEG, F), U32),
        vm((NSEG, SEG, D), BF16),
        vm((L2, L2), jnp.int32),
        vm((L2, L2), F32),
        pltpu.SemaphoreType.DMA((14 + (NKS + 1) * NS,)),
        pltpu.SemaphoreType.DMA((NCH,)),
        pltpu.SemaphoreType.DMA(()),
    ]
    out = pl.pallas_call(
        _kernel,
        out_shape=jax.ShapeDtypeStruct((NSEG, SEG, D), BF16),
        in_specs=[pl.BlockSpec(memory_space=pl.ANY)] * 11,
        out_specs=pl.BlockSpec(memory_space=pl.ANY),
        scratch_shapes=scratch,
        compiler_params=pltpu.CompilerParams(vmem_limit_bytes=120 * 1024 * 1024,
                                             disable_bounds_checks=True,
                                             disable_semaphore_checks=True),
    )(
        A_x.reshape(NSEG, SEG, D),
        A_mem0.reshape(MEM, D),
        A_Wq.reshape(D // 2, 2 * H, DH),
        A_Wk.reshape(D // 2, 2 * H, DH),
        A_Wv.reshape(D // 2, 2 * H, DH),
        A_Wo.reshape(HD, D),
        B_w1, B_w3, B_w2, c, w_mod,
    )
    return out.reshape(1, S, D)
```

```python
import functools
import math

import jax
import jax.numpy as jnp
from jax import lax
import jax.experimental.pallas as pl
import jax.experimental.pallas.tpu as pltpu

S, D, H, DH, MEM, SEG, F = 2048, 1024, 32, 128, 8, 32, 3584
NSEG = S // SEG
NP = H // 2
HD = H * DH
EARLY = 8
NEARLY = NSEG * EARLY
L2 = 2 * (MEM + SEG)
CH = 8
NCH = 3 * H // CH
SL = (0, 256, 512, 768, D)
NS = len(SL) - 1
NKS = 3
XS = 8
NDEF = 1
NPAIR = NSEG // 2
PR = 2 * SEG
LAG = 2
EPS = 1e-5
SCALE = DH ** -0.5
MASK_FILL = -1000000000.0

BF16, F32, U32 = jnp.bfloat16, jnp.float32, jnp.uint32


def _bf(x_u32):
    return pltpu.bitcast(x_u32, BF16)


def _pk(x_f32):
    return pltpu.bitcast(x_f32.astype(BF16), U32)


def _dot(a, b):
    return jnp.dot(a, b, preferred_element_type=F32)


def _affine(x, scale8, shift8=None):
    y = x.reshape(-1, 8, x.shape[-1]) * scale8[None]
    if shift8 is not None:
        y = y + shift8[None]
    return y.reshape(x.shape)


def _norm(x):
    m = jnp.mean(x, axis=-1, keepdims=True)
    xc = x - m
    v = jnp.mean(xc * xc, axis=-1, keepdims=True)
    return xc * lax.rsqrt(v + EPS)


WO_POINTS = tuple('w%d' % w for w in range(7))
FILL_POINTS = tuple(range(3 * NP)) + ('mid',) + WO_POINTS + ('end',)


def spread(n, fixed):
    counts = dict(fixed)
    n -= sum(fixed.values())
    for k in range(6 * NP):
        counts[(k >= 3 * NP, k % (3 * NP))] = (k + 1) * n // (6 * NP) - k * n // (6 * NP)
    return counts


def _attn_mask():
    def meta(i):
        head = jnp.where(i < 2 * SEG, i // SEG, (i - 2 * SEG) // EARLY)
        j = i % SEG
        pos = jnp.where(i < 2 * SEG, jnp.where(j < MEM, j, j + EARLY), MEM + (i - 2 * SEG) % EARLY)
        return head, pos
    r = lax.broadcasted_iota(jnp.int32, (L2, L2), 0)
    c = lax.broadcasted_iota(jnp.int32, (L2, L2), 1)
    rh, rp = meta(r)
    chd, cp = meta(c)
    same = rh == chd
    keep = same & ((rp < MEM) | (rp >= cp))
    fill = jnp.where(same, MASK_FILL / SCALE, -jnp.inf).astype(F32)
    return keep, fill


def _kernel(x_hbm, m0_hbm, wq_hbm, wk_hbm, wv_hbm, wo_hbm, w1_hbm, w3_hbm, w2_hbm, c_hbm, wm_hbm,
            out_hbm,
            wqkv, wo, w1, w3, w2, wm, xb, xe, cb, m0, mod, nrm, p32, part, pre, l32, ob, oda, abuf,
            x1n, x1c, h2, act, ost, keep_s, fill_s, sem, wsem, osem):
    w_hbm = [r.bitcast(U32) for r in (wq_hbm, wk_hbm, wv_hbm)]
    wm_u = wm_hbm.bitcast(U32)

    def pair_copies(m, j, dsem, r0=0, r1=D // 2):
        return [pltpu.make_async_copy(w_hbm[m].at[r0:r1, par * NP + j, :],
                                      wqkv.at[m * H + 2 * j + par, r0:r1, :], dsem) for par in range(2)]

    def chunk_copies(t):
        m, c0 = divmod(t, H // CH)
        return [cp for jj in range(CH // 2)
                for cp in pair_copies(m, c0 * (CH // 2) + jj, wsem.at[t])]

    def wait_chunk(t):
        blk = wqkv.at[pl.ds(t * CH, CH)]
        pltpu.make_async_copy(blk, blk, wsem.at[t]).wait()

    def unzip(slot, r0=0, r1=D // 2):
        for r in range(r0, r1, 32):
            e, o = wqkv[slot, r:r + 32, :], wqkv[slot + 1, r:r + 32, :]
            wqkv[slot, r:r + 32, :] = (e & 0xFFFF) | (o << 16)
            wqkv[slot + 1, r:r + 32, :] = (e >> 16) | (o & jnp.uint32(0xFFFF0000))

    def start_all(cps):
        for cp in cps:
            cp.start()

    def wait_all(cps):
        for cp in cps:
            cp.wait()

    cp_c = pltpu.make_async_copy(c_hbm, cb, sem.at[0])
    x_u = x_hbm.bitcast(U32)
    cp_xe = pltpu.make_async_copy(x_hbm.at[:, 0:EARLY, :], xe, sem.at[1])
    cp_x0 = pltpu.make_async_copy(x_u.at[0], xb.at[0], sem.at[2])
    cp_m0 = pltpu.make_async_copy(m0_hbm, m0, sem.at[3])
    cp_xr = pltpu.make_async_copy(x_u.at[1:XS], xb.at[1:XS], sem.at[4])
    cp_wo = pltpu.make_async_copy(wo_hbm.bitcast(U32), wo, sem.at[5])
    cp_w1 = pltpu.make_async_copy(w1_hbm.bitcast(U32), w1, sem.at[6])
    cp_w3 = pltpu.make_async_copy(w3_hbm.bitcast(U32), w3, sem.at[7])
    cp_w2 = pltpu.make_async_copy(w2_hbm.bitcast(U32), w2, sem.at[8])
    cp_wm = [pltpu.make_async_copy(wm_u.at[:, k * D:(k + 1) * D], wm.at[k], sem.at[7 + k])
             for k in range(2, 6)]
    cp_xl = pltpu.make_async_copy(x_u.at[XS:NSEG], xb.at[XS:NSEG], sem.at[13])
    cp_wa = [[pltpu.make_async_copy(wm_u.at[:, k * D + SL[q]:k * D + SL[q + 1]],
                                    wm.at[k, :, SL[q]:SL[q + 1]], sem.at[14 + (NKS + 1) * q])
              for k in range(2)] for q in range(NS)]
    cp_ks = [[[cp for j in range(4 * t, 4 * t + 4)
               for cp in pair_copies(0, j, sem.at[15 + (NKS + 1) * q + t], SL[q] // 2, SL[q + 1] // 2)]
              for t in range(NKS)] for q in range(NS)]

    start_all([cp_xe, cp_c, cp_x0, cp_m0] + cp_wa[0])
    keep, fill = _attn_mask()
    keep_s[...] = keep.astype(jnp.int32)
    fill_s[...] = fill
    abuf[...] = jnp.zeros((PR, D), F32)
    x1n[...] = jnp.zeros((PR, D), F32)
    mod[2:6] = jnp.zeros((4, 8, D), F32)
    wait_all([cp_xe, cp_c, cp_x0, cp_m0])
    start_all([cp for t in range(NKS) for cp in cp_ks[0][t]])
    cf = cb[...].astype(F32)
    sc16 = jnp.broadcast_to(cf * jax.nn.sigmoid(cf), (16, D)).astype(BF16)
    for g in range(NSEG // 8):
        nrm[64 * g:64 * g + 64, :] = _norm(xe[8 * g:8 * g + 8].astype(F32).reshape(8 * EARLY, D))

    def mod_unit(k, c0, c1):
        mod[k, :, c0:c1] = _dot(sc16, _bf(wm[k, :, c0:c1]))[0:8]

    def ln1_mod(n, c0=0, c1=D):
        return _affine(n, 1.0 + mod[1, :, c0:c1], mod[0, :, c0:c1])

    def next_lhs(mem_f32, s):
        hx = ln1_mod(_norm(_bf(xb[s]).astype(F32)[EARLY:SEG]))
        l32[...] = _pk(jnp.concatenate([mem_f32, hx], axis=0))

    def early_dot(head, c, c0=0, c1=D):
        return _dot(_bf(p32[64 * c:64 * c + 64, c0:c1]), _bf(wqkv[head, c0 // 2:c1 // 2, :]))

    def early_store(slot, c, ab):
        pre[slot // 2, 16 * c:16 * c + 16] = _pk(
            jnp.concatenate([v.reshape(16, EARLY, DH) for v in ab], axis=1))

    def early_pair(slot, c0=0, c1=D, blocks=range(NEARLY // 128), between=()):
        between = list(between)
        for c in blocks:
            ab = [early_dot(slot + hh, c, c0, c1) for hh in range(2)]
            if between:
                between.pop(0)()
            rows = slice(128 * c, 128 * c + 128)
            if c0 > 0:
                ab = [ab[hh] + part[slot + hh, rows, :] for hh in range(2)]
            if c1 < D:
                for hh in range(2):
                    part[slot + hh, rows, :] = ab[hh]
            else:
                early_store(slot, c, ab)

    def early_run(slot0, npairs, blocks=range(NEARLY // 128)):
        unzip(slot0)
        for slot in range(0, 2 * npairs, 2):
            if slot + 2 < 2 * npairs:
                unzip(slot0 + slot + 2)
            early_pair(slot0 + slot, blocks=blocks)

    def ln1_early(q):
        for n in range(SL[q], SL[q + 1], 128):
            for g in range(NEARLY // 128):
                p32[64 * g:64 * g + 64, n:n + 128] = _pk(
                    ln1_mod(nrm[128 * g:128 * g + 128, n:n + 128], n, n + 128))

    def ks(q, *ts):
        return [cp for t in ts for cp in cp_ks[q][t]]

    def ch(*ts):
        return [cp for t in ts for cp in chunk_copies(t)]

    jobs = [(q, 2 * g) for q in range(NS) for g in range(NKS * CH // 2)]
    sync = {3: (ks(0, 1), [], None),
            7: (ks(0, 2), cp_wa[2] + ks(2, 0), None),
            11: (cp_wa[1] + ks(1, 0), ks(2, 1, 2), 1),
            15: (ks(1, 1, 2), cp_wa[3] + ks(3, 0, 1, 2), None),
            22: (cp_wa[2] + ks(2, 0), ch(3, 4), 2),
            27: (ks(2, 1, 2), [], None),
            34: (cp_wa[3] + ks(3, 0, 1, 2), ch(5, 6, 7, 8), 3)}
    wait_all(cp_wa[0])
    for k in range(2):
        mod_unit(k, 0, SL[1])
    ln1_early(0)
    start_all(cp_wa[1] + ks(1, 0, 1, 2))
    wait_all(ks(0, 0))
    unzip(0, 0, SL[1] // 2)
    for i, (q, slot) in enumerate(jobs):
        waits, issue, done = sync.get(i, ([], [], None))
        start_all(issue)
        wait_all(waits)
        if i + 1 < len(jobs):
            qn, slotn = jobs[i + 1]
            unzip(slotn, SL[qn] // 2, SL[qn + 1] // 2)
        if done is None:
            early_pair(slot, SL[q], SL[q + 1])
        else:
            early_pair(slot, SL[q], SL[q + 1], between=[
                functools.partial(mod_unit, k, n, n + 128)
                for n in range(SL[done], SL[done + 1], 128) for k in range(2)])
            ln1_early(done)
    next_lhs(m0[...].astype(F32), 0)

    def prologue(r, carry):
        wait_chunk(2 * r + 1)
        wait_chunk(2 * r + 2)

        @pl.when(r == 1)
        def _():
            start_all(ch(*range(9, NCH)))

        @pl.when(r == 2)
        def _():
            start_all([cp_xr, cp_wo] + cp_wm + [cp_w1, cp_w3, cp_w2, cp_xl])

        early_run((2 * r + 1) * CH, CH)
        return carry

    lax.fori_loop(1, (NCH - NDEF - 1) // 2, prologue, 0)

    for t in range(NCH - NDEF, NCH):
        wait_chunk(t)
    wait_all([cp_xr, cp_wo])
    early_run((NCH - NDEF) * CH, NDEF * CH // 2, blocks=(0,))

    def resid1(p, dst):
        for n in range(0, D, 256):
            xf = _bf(xb[pl.ds(2 * p, 2), :, n:n + 256]).astype(F32).reshape(PR, 256)
            dst[:, n:n + 256] = xf + _affine(abuf[:, n:n + 256], mod[2, :, n:n + 256])

    def advance(p):
        x1c[...] = x1n[...]
        resid1(p, x1n)

    def ln2(src, q):
        h2[q * SEG:(q + 1) * SEG, :] = _pk(_affine(_norm(src[...]), 1.0 + mod[4], mod[3]))

    def gate_up_units(q0, q1, chunks):
        r0, r1 = q0 * SEG, q1 * SEG
        half = {}

        def gate(f0):
            half[f0] = 0.5 * _dot(_bf(h2[r0:r1, :]), _bf(w1[:, f0:f0 + 128]))

        def up(f0):
            t = half.pop(f0)
            u = _dot(_bf(h2[r0:r1, :]), _bf(w3[:, f0:f0 + 128]))
            act[r0:r1, f0:f0 + 128] = _pk((t + t * jnp.tanh(t)) * u)

        return [functools.partial(fn, 128 * ck) for ck in chunks for fn in (gate, up)]

    def down_units(p, q, x1, nsplit):
        kq = F // nsplit
        acc = {}

        def down(n0, k):
            y = _dot(_bf(act[q * SEG:(q + 1) * SEG, k * kq:(k + 1) * kq]),
                     _bf(w2[k * kq // 2:(k + 1) * kq // 2, n0:n0 + 128]))
            if k > 0:
                y = y + acc.pop(n0)
            if k + 1 < nsplit:
                acc[n0] = y
                return
            res = x1[:, n0:n0 + 128] + _affine(y, mod[5, :, n0:n0 + 128])
            ost[pl.ds(2 * p, 2), :, n0:n0 + 128] = res.astype(BF16).reshape(2, SEG, 128)

        return [functools.partial(down, n0, k) for n0 in range(0, D, 128) for k in range(nsplit)]

    def out_copy(p, npairs):
        rows = pl.ds(2 * p, 2 * npairs)
        return pltpu.make_async_copy(ost.at[rows], out_hbm.at[rows], osem)

    c_exp = SCALE * math.log2(math.e)
    nb = 256

    def step(s, second, fill):
        rows = SEG + 2 * EARLY if second else SEG
        lhs = _bf(l32[...])
        qkv, prob = {}, {}

        def project(j):
            out = []
            for m in range(3):
                a = _dot(lhs, _bf(wqkv[m * H + 2 * j])).astype(BF16)
                b = _dot(lhs, _bf(wqkv[m * H + 2 * j + 1])).astype(BF16)
                out.append(jnp.concatenate([a, b, _bf(pre[m * NP + j, s])], axis=0))
                fill(3 * j + m)
            qkv[j] = out

        def scores(j):
            q, k, _ = qkv[j]
            sc_ = lax.dot_general(q, k, (((1,), (1,)), ((), ())), preferred_element_type=F32)
            sc_ = jnp.where(keep_s[...] != 0, sc_, fill_s[...])
            e = jnp.exp2((sc_ - jnp.max(sc_, axis=1, keepdims=True)) * c_exp)
            den = jnp.sum(e, axis=1, keepdims=True)
            r = pl.reciprocal(den, approx=True)
            r = r * (2.0 - den * r)
            prob[j] = (e * r).astype(BF16)

        def values(j):
            o = _dot(prob.pop(j), qkv.pop(j)[2])
            for hh in range(2):
                c0 = (2 * j + hh) * DH
                main = o[hh * SEG:(hh + 1) * SEG]
                early = o[2 * SEG + hh * EARLY:2 * SEG + (hh + 1) * EARLY]
                if second:
                    ob[:, c0:c0 + DH] = _pk(jnp.concatenate([main, oda[:, c0:c0 + DH], early], axis=0))
                else:
                    ob[0:SEG // 2, c0:c0 + DH] = _pk(main)
                    oda[:, c0:c0 + DH] = early

        def wo_part(n, j0, j1):
            k0, k1 = j0 * 2 * DH, j1 * 2 * DH
            return _dot(_bf(ob[0:rows // 2, k0:k1]), _bf(wo[k0 // 2:k1 // 2, n * nb:(n + 1) * nb]))

        for j in range(NP):
            project(j)
            if j >= 1:
                scores(j - 1)
            if j >= 3:
                values(j - 3)
        y0 = wo_part(0, 0, 6)
        scores(NP - 1)
        values(NP - 3)
        y0 = y0 + wo_part(0, 6, 12)
        values(NP - 2)
        fill('mid')
        y1 = wo_part(1, 0, 8)
        values(NP - 1)
        y1 = y1 + wo_part(1, 8, 13)
        fill('w0')
        y2 = wo_part(2, 0, 7)
        fill('w1')
        y2 = y2 + wo_part(2, 7, 14)
        fill('w2')
        y0 = y0 + wo_part(0, 12, NP)
        fill('w3')
        y1 = y1 + wo_part(1, 13, NP)
        y2 = y2 + wo_part(2, 14, NP)
        fill('w4')
        y3 = wo_part(3, 0, 5)
        fill('w5')
        y3 = y3 + wo_part(3, 5, 10)
        fill('w6')
        y3 = y3 + wo_part(3, 10, NP)
        y = jnp.concatenate([y0, y1, y2, y3], axis=1)
        next_lhs(y[0:MEM], jnp.minimum(s + 1, NSEG - 1))
        fill('end')
        return y

    def pair(i, units, counts):
        units = list(units)

        def filler(second):
            def fill(point):
                for _ in range(counts.get((second, point), 0)):
                    units.pop(0)()
            return fill

        advance(jnp.maximum(i - 1, 0))
        ya = step(2 * i, False, filler(False))
        abuf[EARLY:SEG, :] = ya[MEM:SEG]
        yb = step(2 * i + 1, True, filler(True))
        abuf[0:EARLY, :] = yb[SEG:SEG + EARLY]
        abuf[SEG:SEG + EARLY, :] = yb[SEG + EARLY:SEG + 2 * EARLY]
        abuf[SEG + EARLY:PR, :] = yb[MEM:SEG]
        assert not units

    def head_pairs(i, carry):
        for kk in range(2):
            k = 2 + 2 * i + kk
            pltpu.make_async_copy(wm.at[k], wm.at[k], sem.at[7 + k]).wait()
        mods = [functools.partial(mod_unit, 2 + 2 * i + kk, n0, n0 + 128)
                for kk in range(2) for n0 in range(0, D, 128)]
        npr = NDEF * CH // 2 // LAG
        slot0 = (NCH - NDEF) * CH + 2 * npr * i
        held = {}

        def piece(slot, c, hh, hf):
            v = early_dot(slot + hh, c, hf * D // 2, (hf + 1) * D // 2)
            held[hh] = v if hf == 0 else v + held[hh]
            if hh == 1 and hf == 1:
                early_store(slot, c, [held.pop(0), held.pop(1)])

        pieces = [functools.partial(piece, slot0 + 2 * g, c, hh, hf)
                  for g in range(npr) for c in range(1, 4) for hh in range(2) for hf in range(2)]
        npieces = spread(len(pieces), {(False, 'mid'): 1, (False, 'end'): 3, (True, 'mid'): 1, (True, 'end'): 2})
        units, counts = [], {}
        for second in (False, True):
            for pt in FILL_POINTS:
                here = []
                for _ in range(npieces.get((second, pt), 0)):
                    here.append(pieces.pop(0))
                    if len(mods) > len(WO_POINTS) and len(pieces) % 2 == 0:
                        here.append(mods.pop(0))
                if second and pt == 'mid':
                    assert len(mods) == len(WO_POINTS)
                    here.append(functools.partial(ln2, x1n, 0))
                if second and pt in WO_POINTS:
                    here.append(mods.pop(0))
                units += here
                counts[(second, pt)] = len(here)
        pair(i, units, counts)
        return carry

    lax.fori_loop(0, LAG, head_pairs, 0)
    wait_all([cp_w1, cp_w3, cp_w2])

    nf = F // 128
    counts = spread(2 * nf + 1 + 32, {(False, 'mid'): 2, (False, 'end'): 4, (True, 'mid'): 2, (True, 'end'): 5})

    def main_pairs(p, carry):
        @pl.when(p == 1)
        def _():
            cp_xl.wait()

        @pl.when(p >= 1)
        def _():
            out_copy(p - 1, 1).start()

        units = gate_up_units(0, 1, range(nf))
        units.append(functools.partial(ln2, x1n, 0))
        units += down_units(p, 0, x1c, 4)
        pair(p + LAG, units, counts)
        return carry

    lax.fori_loop(0, NPAIR - LAG, main_pairs, 0)

    p0 = NPAIR - LAG
    out_copy(p0 - 1, 1).start()
    resid1(p0 + 1, x1c)
    ln2(x1c, 1)
    units = gate_up_units(0, 1, range(2)) + gate_up_units(1, 2, range(2)) + gate_up_units(0, 2, range(2, nf))
    for q in range(LAG):
        units += down_units(p0 + q, q, (x1n, x1c)[q], 1) + [out_copy(p0 + q, 1).start]
    for unit in units:
        unit()
    out_copy(0, NPAIR).wait()


@jax.jit
def pallas_adaLN_cond__memory_aug_recurrent_mem_tr__glu_gated_swiglu__prompt_kernel(
    A_x, A_mem0, A_Wq, A_Wk, A_Wv, A_Wo, A_seg_len, B_x, B_w1, B_w3, B_w2, c, w_mod,
):
    assert A_x.shape == (1, S, D) and A_mem0.shape == (1, MEM, D)
    del A_seg_len
    del B_x
    vm = pltpu.VMEM
    scratch = [
        vm((3 * H, D // 2, DH), U32),
        vm((HD // 2, D), U32),
        vm((D // 2, F), U32),
        vm((D // 2, F), U32),
        vm((F // 2, D), U32),
        vm((6, D // 2, D), U32),
        vm((NSEG, SEG // 2, D), U32),
        vm((NSEG, EARLY, D), BF16),
        vm((1, D), BF16),
        vm((MEM, D), BF16),
        vm((6, 8, D), F32),
        vm((NEARLY, D), F32),
        vm((NEARLY // 2, D), U32),
        vm((NKS * CH, NEARLY, DH), F32),
        vm((3 * NP, NSEG, EARLY, DH), U32),
        vm((SEG // 2, D), U32),
        vm((SEG // 2 + EARLY, HD), U32),
        vm((EARLY, HD), F32),
        vm((PR, D), F32),
        vm((PR, D), F32),
        vm((PR, D), F32),
        vm((LAG * SEG, D), U32),
        vm((LAG * SEG, F), U32),
        vm((NSEG, SEG, D), BF16),
        vm((L2, L2), jnp.int32),
        vm((L2, L2), F32),
        pltpu.SemaphoreType.DMA((14 + (NKS + 1) * NS,)),
        pltpu.SemaphoreType.DMA((NCH,)),
        pltpu.SemaphoreType.DMA(()),
    ]
    out = pl.pallas_call(
        _kernel,
        out_shape=jax.ShapeDtypeStruct((NSEG, SEG, D), BF16),
        in_specs=[pl.BlockSpec(memory_space=pl.ANY)] * 11,
        out_specs=pl.BlockSpec(memory_space=pl.ANY),
        scratch_shapes=scratch,
        compiler_params=pltpu.CompilerParams(vmem_limit_bytes=120 * 1024 * 1024,
                                             disable_bounds_checks=True,
                                             disable_semaphore_checks=True),
    )(
        A_x.reshape(NSEG, SEG, D),
        A_mem0.reshape(MEM, D),
        A_Wq.reshape(D // 2, 2 * H, DH),
        A_Wk.reshape(D // 2, 2 * H, DH),
        A_Wv.reshape(D // 2, 2 * H, DH),
        A_Wo.reshape(HD, D),
        B_w1, B_w3, B_w2, c, w_mod,
    )
    return out.reshape(1, S, D)
```

```python
import functools
import math

import jax
import jax.numpy as jnp
from jax import lax
import jax.experimental.pallas as pl
import jax.experimental.pallas.tpu as pltpu

S, D, H, DH, MEM, SEG, F = 2048, 1024, 32, 128, 8, 32, 3584
NSEG = S // SEG
NP = H // 2
HD = H * DH
EARLY = 8
NEARLY = NSEG * EARLY
L2 = 2 * (MEM + SEG)
CH = 8
NCH = 3 * H // CH
SL = (0, 256, 512, 768, D)
NS = len(SL) - 1
NKS = 3
XS = 8
NDEF = 3
NPAIR = NSEG // 2
PR = 2 * SEG
LAG = 2
FH = F // 2
NCOMB = 2
NBLK = 8 // NCOMB
EPS = 1e-5
SCALE = DH ** -0.5
MASK_FILL = -1000000000.0

BF16, F32, U32 = jnp.bfloat16, jnp.float32, jnp.uint32


def _bf(x_u32):
    return pltpu.bitcast(x_u32, BF16)


def _pk(x_f32):
    return pltpu.bitcast(x_f32.astype(BF16), U32)


def _dot(a, b):
    return jnp.dot(a, b, preferred_element_type=F32)


def _affine(x, scale8, shift8=None):
    y = x.reshape(-1, 8, x.shape[-1]) * scale8[None]
    if shift8 is not None:
        y = y + shift8[None]
    return y.reshape(x.shape)


def _lhs7(a11, a12, a21, a22):
    return [a11 + a22, a21 + a22, a11, a22, a11 + a12, a21 - a11, a12 - a22]


def _out4(m):
    return m[0] + m[3] - m[4] + m[6], m[2] + m[4], m[1] + m[3], m[0] - m[1] + m[2] + m[5]


RHS7 = (('s', 0), ('r', 0), ('s', 1), ('s', 2), ('r', 1), ('s', 3), ('s', 4))


def _norm(x):
    m = jnp.mean(x, axis=-1, keepdims=True)
    xc = x - m
    v = jnp.mean(xc * xc, axis=-1, keepdims=True)
    return xc * lax.rsqrt(v + EPS)


WO_POINTS = tuple('w%d' % w for w in range(7))
FILL_POINTS = tuple(range(3 * NP)) + ('m0', 'mid') + WO_POINTS + ('end',)


def spread(n, fixed):
    counts = dict(fixed)
    n -= sum(fixed.values())
    for k in range(6 * NP):
        counts[(k >= 3 * NP, k % (3 * NP))] = (k + 1) * n // (6 * NP) - k * n // (6 * NP)
    return counts


def _attn_mask():
    def meta(i):
        head = jnp.where(i < 2 * SEG, i // SEG, (i - 2 * SEG) // EARLY)
        j = i % SEG
        pos = jnp.where(i < 2 * SEG, jnp.where(j < MEM, j, j + EARLY), MEM + (i - 2 * SEG) % EARLY)
        return head, pos
    r = lax.broadcasted_iota(jnp.int32, (L2, L2), 0)
    c = lax.broadcasted_iota(jnp.int32, (L2, L2), 1)
    rh, rp = meta(r)
    chd, cp = meta(c)
    same = rh == chd
    keep = same & ((rp < MEM) | (rp >= cp))
    fill = jnp.where(same, MASK_FILL / SCALE, -jnp.inf).astype(F32)
    return keep, fill


def _kernel(x_hbm, m0_hbm, wq_hbm, wk_hbm, wv_hbm, wo_hbm, w1_hbm, w3_hbm, w2_hbm, c_hbm, wm_hbm,
            out_hbm,
            wqkv, wo, w1r, w1s, w3r, w3s, w2r, w2s, wm, xb, xe, cb, m0, mod, nrm, p32, part, pre, l32, ob, oda, abuf,
            x1n, x1c, h2, act, ost, keep_s, fill_s, sem, wsem, osem):
    w_hbm = [r.bitcast(U32) for r in (wq_hbm, wk_hbm, wv_hbm)]
    wm_u = wm_hbm.bitcast(U32)

    def pair_copies(m, j, dsem, r0=0, r1=D // 2):
        return [pltpu.make_async_copy(w_hbm[m].at[r0:r1, par * NP + j, :],
                                      wqkv.at[m * H + 2 * j + par, r0:r1, :], dsem) for par in range(2)]

    def chunk_copies(t):
        m, c0 = divmod(t, H // CH)
        return [cp for jj in range(CH // 2)
                for cp in pair_copies(m, c0 * (CH // 2) + jj, wsem.at[t])]

    def wait_chunk(t):
        blk = wqkv.at[pl.ds(t * CH, CH)]
        pltpu.make_async_copy(blk, blk, wsem.at[t]).wait()

    def unzip(slot, r0=0, r1=D // 2):
        for r in range(r0, r1, 32):
            e, o = wqkv[slot, r:r + 32, :], wqkv[slot + 1, r:r + 32, :]
            wqkv[slot, r:r + 32, :] = (e & 0xFFFF) | (o << 16)
            wqkv[slot + 1, r:r + 32, :] = (e >> 16) | (o & jnp.uint32(0xFFFF0000))

    def start_all(cps):
        for cp in cps:
            cp.start()

    def wait_all(cps):
        for cp in cps:
            cp.wait()

    cp_c = pltpu.make_async_copy(c_hbm, cb, sem.at[0])
    x_u = x_hbm.bitcast(U32)
    cp_xe = pltpu.make_async_copy(x_hbm.at[:, 0:EARLY, :], xe, sem.at[1])
    cp_x0 = pltpu.make_async_copy(x_u.at[0], xb.at[0], sem.at[2])
    cp_m0 = pltpu.make_async_copy(m0_hbm, m0, sem.at[3])
    cp_xr = pltpu.make_async_copy(x_u.at[1:XS], xb.at[1:XS], sem.at[4])
    cp_wo = pltpu.make_async_copy(wo_hbm.bitcast(U32), wo, sem.at[5])
    def quadrant_copies(src, w, dsem):
        r, c = w[1].shape[1:]
        src_u = src.bitcast(U32)
        return [pltpu.make_async_copy(src_u.at[0:r // 2, 0:c], w[0].at[0], dsem),
                pltpu.make_async_copy(src.at[0:r, c:2 * c], w[1].at[1], dsem),
                pltpu.make_async_copy(src.at[r:2 * r, 0:c], w[1].at[2], dsem),
                pltpu.make_async_copy(src_u.at[r // 2:r, c:2 * c], w[0].at[1], dsem)]

    w1, w3, w2 = (w1r, w1s), (w3r, w3s), (w2r, w2s)
    cp_ffn = [cp for src, w, k in ((w1_hbm, w1, 6), (w3_hbm, w3, 7), (w2_hbm, w2, 8))
              for cp in quadrant_copies(src, w, sem.at[k])]

    def rhs(w, t, n):
        kind, k = RHS7[t]
        return _bf(w[0][k, :, n:n + 128]) if kind == 'r' else w[1][k, :, n:n + 128]

    cp_wm = [pltpu.make_async_copy(wm_u.at[:, k * D:(k + 1) * D], wm.at[k], sem.at[7 + k])
             for k in range(2, 6)]
    cp_xl = pltpu.make_async_copy(x_u.at[XS:NSEG], xb.at[XS:NSEG], sem.at[13])
    cp_wa = [[pltpu.make_async_copy(wm_u.at[:, k * D + SL[q]:k * D + SL[q + 1]],
                                    wm.at[k, :, SL[q]:SL[q + 1]], sem.at[14 + (NKS + 1) * q])
              for k in range(2)] for q in range(NS)]
    cp_ks = [[[cp for j in range(4 * t, 4 * t + 4)
               for cp in pair_copies(0, j, sem.at[15 + (NKS + 1) * q + t], SL[q] // 2, SL[q + 1] // 2)]
              for t in range(NKS)] for q in range(NS)]

    start_all([cp_xe, cp_c, cp_x0, cp_m0] + cp_wa[0])
    keep, fill = _attn_mask()
    keep_s[...] = keep.astype(jnp.int32)
    fill_s[...] = fill
    abuf[...] = jnp.zeros((PR, D), F32)
    x1n[...] = jnp.zeros((PR, D), F32)
    mod[2:6] = jnp.zeros((4, 8, D), F32)
    wait_all([cp_xe, cp_c, cp_x0, cp_m0])
    start_all([cp for t in range(NKS) for cp in cp_ks[0][t]])
    cf = cb[...].astype(F32)
    sc16 = jnp.broadcast_to(cf * jax.nn.sigmoid(cf), (16, D)).astype(BF16)
    for g in range(NSEG // 8):
        nrm[64 * g:64 * g + 64, :] = _norm(xe[8 * g:8 * g + 8].astype(F32).reshape(8 * EARLY, D))

    def mod_unit(k, c0, c1):
        mod[k, :, c0:c1] = _dot(sc16, _bf(wm[k, :, c0:c1]))[0:8]

    def ln1_mod(n, c0=0, c1=D):
        return _affine(n, 1.0 + mod[1, :, c0:c1], mod[0, :, c0:c1])

    def next_lhs(mem_f32, s):
        hx = ln1_mod(_norm(_bf(xb[s]).astype(F32)[EARLY:SEG]))
        l32[...] = _pk(jnp.concatenate([mem_f32, hx], axis=0))

    def early_dot(head, c, c0=0, c1=D):
        rows = slice(64 * c, 64 * c + 64) if isinstance(c, int) else pl.ds(pl.multiple_of(64 * c, 64), 64)
        return _dot(_bf(p32[rows, c0:c1]), _bf(wqkv[head, c0 // 2:c1 // 2, :]))

    def early_store(slot, c, ab):
        pre[slot // 2, pl.ds(16 * c, 16)] = _pk(
            jnp.concatenate([v.reshape(16, EARLY, DH) for v in ab], axis=1))

    def early_pair(slot, c0=0, c1=D, blocks=range(NEARLY // 128), between=()):
        between = list(between)
        for c in blocks:
            ab = [early_dot(slot + hh, c, c0, c1) for hh in range(2)]
            if between:
                between.pop(0)()
            rows = slice(128 * c, 128 * c + 128) if c1 - c0 < D else None
            if c0 > 0:
                ab = [ab[hh] + part[slot + hh, rows, :] for hh in range(2)]
            if c1 < D:
                for hh in range(2):
                    part[slot + hh, rows, :] = ab[hh]
            else:
                early_store(slot, c, ab)

    def early_run(slot0, npairs, blocks=range(NEARLY // 128)):
        unzip(slot0)
        for slot in range(0, 2 * npairs, 2):
            if slot + 2 < 2 * npairs:
                unzip(slot0 + slot + 2)
            early_pair(slot0 + slot, blocks=blocks)

    def ln1_early(q):
        for n in range(SL[q], SL[q + 1], 128):
            for g in range(NEARLY // 128):
                p32[64 * g:64 * g + 64, n:n + 128] = _pk(
                    ln1_mod(nrm[128 * g:128 * g + 128, n:n + 128], n, n + 128))

    def ks(q, *ts):
        return [cp for t in ts for cp in cp_ks[q][t]]

    def ch(*ts):
        return [cp for t in ts for cp in chunk_copies(t)]

    jobs = [(q, 2 * g) for q in range(NS) for g in range(NKS * CH // 2)]
    sync = {3: (ks(0, 1), [], None),
            7: (ks(0, 2), cp_wa[2] + ks(2, 0), None),
            11: (cp_wa[1] + ks(1, 0), ks(2, 1, 2), 1),
            15: (ks(1, 1, 2), cp_wa[3] + ks(3, 0, 1, 2), None),
            22: (cp_wa[2] + ks(2, 0), ch(3, 4), 2),
            27: (ks(2, 1, 2), [], None),
            34: (cp_wa[3] + ks(3, 0, 1, 2), ch(5, 6, 7, 8), 3)}
    wait_all(cp_wa[0])
    for k in range(2):
        mod_unit(k, 0, SL[1])
    ln1_early(0)
    start_all(cp_wa[1] + ks(1, 0, 1, 2))
    wait_all(ks(0, 0))
    unzip(0, 0, SL[1] // 2)
    for i, (q, slot) in enumerate(jobs):
        waits, issue, done = sync.get(i, ([], [], None))
        start_all(issue)
        wait_all(waits)
        if i + 1 < len(jobs):
            qn, slotn = jobs[i + 1]
            unzip(slotn, SL[qn] // 2, SL[qn + 1] // 2)
        if done is None:
            early_pair(slot, SL[q], SL[q + 1])
        else:
            early_pair(slot, SL[q], SL[q + 1], between=[
                functools.partial(mod_unit, k, n, n + 128)
                for n in range(SL[done], SL[done + 1], 128) for k in range(2)])
            ln1_early(done)
    next_lhs(m0[...].astype(F32), 0)

    def prologue(r, carry):
        wait_chunk(2 * r + 1)
        wait_chunk(2 * r + 2)

        @pl.when(r == 1)
        def _():
            start_all(ch(*range(9, NCH)))

        @pl.when(r == 2)
        def _():
            start_all([cp_xr, cp_wo] + cp_wm + cp_ffn + [cp_xl])

        early_run((2 * r + 1) * CH, CH)
        return carry

    lax.fori_loop(1, (NCH - NDEF - 1) // 2, prologue, 0)

    def last_chunks(t, carry):
        wait_chunk(t)
        early_run(t * CH, CH // 2, blocks=(0,))
        return carry

    lax.fori_loop(NCH - NDEF, NCH, last_chunks, 0)
    wait_all([cp_xr, cp_wo])

    def resid1(p, dst):
        for n in range(0, D, 256):
            xf = _bf(xb[pl.ds(2 * p, 2), :, n:n + 256]).astype(F32).reshape(PR, 256)
            dst[:, n:n + 256] = xf + _affine(abuf[:, n:n + 256], mod[2, :, n:n + 256])

    def advance(p):
        x1c[...] = x1n[...]
        resid1(p, x1n)

    def ln2(src, q):
        h = _affine(_norm(src[...]), 1.0 + mod[4], mod[3])
        quads = [h[a * SEG:(a + 1) * SEG, b * (D // 2):(b + 1) * (D // 2)] for a in range(2) for b in range(2)]
        for t, v in enumerate(_lhs7(*quads)):
            h2[q, t] = _pk(v)

    def combine(w, block0):
        rb = w[1].shape[1] // NCOMB

        def body(i, carry):
            for k in range(NBLK):
                b = block0 + NBLK * i + k
                early_pair((NCH - NDEF) * CH + 2 * (b // 3), blocks=(1 + b % 3,))
            for n0 in range(0, w[1].shape[2], 512):
                for r in range(0, rb, 16):
                    r0 = pl.multiple_of(i * rb + r, 16)
                    for n in range(n0, min(n0 + 512, w[1].shape[2]), 256):
                        b11, b22 = [_bf(w[0][k, pl.ds(pl.multiple_of(r0 // 2, 8), 8), n:n + 256]).astype(F32)
                                    for k in range(2)]
                        b12, b21 = [w[1][k, pl.ds(r0, 16), n:n + 256].astype(F32) for k in (1, 2)]
                        for k, v in enumerate((b11 + b22, b12 - b22, b21 - b11, b11 + b12, b21 + b22)):
                            w[1][k, pl.ds(r0, 16), n:n + 256] = v.astype(BF16)
            return carry
        lax.fori_loop(0, NCOMB, body, 0)

    def gate_up_units(q):
        held = {}

        def unit(f0, w, t0, t1):
            m = held.setdefault('m', [])
            m += [_dot(_bf(h2[q, t]), rhs(w, t, f0)) for t in range(t0, t1)]
            if t1 < 7:
                return
            c = _out4(held.pop('m'))
            if w is w1:
                held['g'] = c
                return
            a = [(0.5 * g) * (1.0 + jnp.tanh(0.5 * g)) * u for g, u in zip(held.pop('g'), c)]
            for t, v in enumerate(_lhs7(*a)):
                act[q, t, :, f0:f0 + 128] = _pk(v)

        return [functools.partial(unit, f0, w, t0, t1)
                for f0 in range(0, FH, 128) for w in (w1, w3) for t0, t1 in ((0, 4), (4, 7))]

    def down_units(p, q, x1):
        m = {}

        def unit(n0, t):
            m[t] = _dot(_bf(act[q, t]), rhs(w2, t, n0))
            if len(m) < 7:
                return
            c = _out4(m)
            m.clear()
            for b in range(2):
                cols = slice(b * (D // 2) + n0, b * (D // 2) + n0 + 128)
                res = x1[:, cols] + _affine(jnp.concatenate([c[b], c[2 + b]], axis=0), mod[5, :, cols])
                ost[pl.ds(2 * p, 2), :, cols] = res.astype(BF16).reshape(2, SEG, 128)

        return [functools.partial(unit, n0, t) for n0 in range(0, D // 2, 128) for t in (0, 2, 3, 5, 6, 1, 4)]

    def out_copy(p, npairs):
        rows = pl.ds(2 * p, 2 * npairs)
        return pltpu.make_async_copy(ost.at[rows], out_hbm.at[rows], osem)

    c_exp = SCALE * math.log2(math.e)
    nb = 256

    def step(s, second, fill, eager_wo):
        rows = SEG + 2 * EARLY if second else SEG
        lhs = _bf(l32[...])
        qkv, prob = {}, {}

        def project(j):
            out = []
            for m in range(3):
                a = _dot(lhs, _bf(wqkv[m * H + 2 * j])).astype(BF16)
                b = _dot(lhs, _bf(wqkv[m * H + 2 * j + 1])).astype(BF16)
                out.append(jnp.concatenate([a, b, _bf(pre[m * NP + j, s])], axis=0))
                fill(3 * j + m)
            qkv[j] = out

        def scores(j):
            q, k, _ = qkv[j]
            sc_ = lax.dot_general(q, k, (((1,), (1,)), ((), ())), preferred_element_type=F32)
            sc_ = jnp.where(keep_s[...] != 0, sc_, fill_s[...])
            e = jnp.exp2((sc_ - jnp.max(sc_, axis=1, keepdims=True)) * c_exp)
            den = jnp.sum(e, axis=1, keepdims=True)
            r = pl.reciprocal(den, approx=True)
            r = r * (2.0 - den * r)
            prob[j] = (e * r).astype(BF16)

        def values(j):
            o = _dot(prob.pop(j), qkv.pop(j)[2])
            for hh in range(2):
                c0 = (2 * j + hh) * DH
                main = o[hh * SEG:(hh + 1) * SEG]
                early = o[2 * SEG + hh * EARLY:2 * SEG + (hh + 1) * EARLY]
                if second:
                    ob[:, c0:c0 + DH] = _pk(jnp.concatenate([main, oda[:, c0:c0 + DH], early], axis=0))
                else:
                    ob[0:SEG // 2, c0:c0 + DH] = _pk(main)
                    oda[:, c0:c0 + DH] = early

        def wo_part(n, j0, j1):
            k0, k1 = j0 * 2 * DH, j1 * 2 * DH
            return _dot(_bf(ob[0:rows // 2, k0:k1]), _bf(wo[k0 // 2:k1 // 2, n * nb:(n + 1) * nb]))

        ys = [None] * (D // nb)

        def wo_acc(n, j0, j1):
            v = wo_part(n, j0, j1)
            ys[n] = v if ys[n] is None else ys[n] + v

        for j in range(NP):
            project(j)
            if j >= 1:
                scores(j - 1)
            if j >= 3:
                values(j - 3)
            if eager_wo and j in (5, 7, 9, 11, 13):
                for n in range(D // nb):
                    wo_acc(n, j - 5, j - 3)
        d0 = 10 if eager_wo else 0
        if d0 == 0:
            wo_acc(0, 0, 6)
        else:
            fill('m0')
        scores(NP - 1)
        values(NP - 3)
        wo_acc(0, max(6, d0), 12)
        if d0:
            wo_acc(1, d0, 12)
        values(NP - 2)
        fill('mid')
        if d0 == 0:
            wo_acc(1, 0, 8)
        values(NP - 1)
        if d0 == 0:
            wo_acc(1, 8, 12)
        fill('w0')
        if d0 == 0:
            wo_acc(2, 0, 7)
        fill('w1')
        wo_acc(2, max(7, d0), 14)
        fill('w2')
        if d0:
            wo_acc(3, d0, 14)
        wo_acc(0, 12, NP)
        fill('w3')
        wo_acc(1, 12, NP)
        wo_acc(2, 14, NP)
        fill('w4')
        if d0 == 0:
            wo_acc(3, 0, 5)
        fill('w5')
        if d0 == 0:
            wo_acc(3, 5, 10)
        fill('w6')
        wo_acc(3, 14 if d0 else 10, NP)
        y = jnp.concatenate(ys, axis=1)
        next_lhs(y[0:MEM], jnp.minimum(s + 1, NSEG - 1))
        fill('end')
        return y

    def pair(i, units, counts, eager_wo=False):
        units = list(units)

        def filler(second):
            def fill(point):
                for _ in range(counts.get((second, point), 0)):
                    units.pop(0)()
            return fill

        advance(jnp.maximum(i - 1, 0))
        ya = step(2 * i, False, filler(False), False)
        abuf[EARLY:SEG, :] = ya[MEM:SEG]
        yb = step(2 * i + 1, True, filler(True), eager_wo)
        abuf[0:EARLY, :] = yb[SEG:SEG + EARLY]
        abuf[SEG:SEG + EARLY, :] = yb[SEG + EARLY:SEG + 2 * EARLY]
        abuf[SEG + EARLY:PR, :] = yb[MEM:SEG]
        assert not units

    def head_pairs(i, carry):
        for kk in range(2):
            k = 2 + 2 * i + kk
            pltpu.make_async_copy(wm.at[k], wm.at[k], sem.at[7 + k]).wait()
        mods = [functools.partial(mod_unit, 2 + 2 * i + kk, n0, n0 + 128)
                for kk in range(2) for n0 in range(0, D, 128)]
        npr = CH // 2 // LAG
        slot0 = (NCH - 1) * CH + 2 * npr * i
        held = {}

        def piece(slot, c, hh, hf):
            v = early_dot(slot + hh, c, hf * D // 2, (hf + 1) * D // 2)
            held[hh] = v if hf == 0 else v + held[hh]
            if hh == 1 and hf == 1:
                early_store(slot, c, [held.pop(0), held.pop(1)])

        pieces = [functools.partial(piece, slot0 + 2 * g, c, hh, hf)
                  for g in range(npr) for c in range(1, 4) for hh in range(2) for hf in range(2)]
        npieces = spread(len(pieces), {(False, 'mid'): 1, (False, 'end'): 3, (True, 'mid'): 1, (True, 'end'): 2})
        units, counts = [], {}
        for second in (False, True):
            for pt in FILL_POINTS:
                here = []
                for _ in range(npieces.get((second, pt), 0)):
                    here.append(pieces.pop(0))
                    if len(mods) > len(WO_POINTS) and len(pieces) % 2 == 0:
                        here.append(mods.pop(0))
                if second and pt == 'mid':
                    assert len(mods) == len(WO_POINTS)
                    here.append(functools.partial(ln2, x1n, 0))
                if second and pt in WO_POINTS:
                    here.append(mods.pop(0))
                units += here
                counts[(second, pt)] = len(here)
        pair(i, units, counts)
        return carry

    lax.fori_loop(0, LAG, head_pairs, 0)
    for k, w in enumerate((w1, w3, w2)):
        wait_all(cp_ffn[4 * k:4 * k + 4])
        combine(w, 8 * k)

    counts = spread(4 * (FH // 128) + 28,
                    {(False, 'mid'): 2, (False, 'end'): 4,
                     (True, 'm0'): 2, (True, 'mid'): 3, (True, 'w0'): 2, (True, 'end'): 6})

    def main_pairs(p, carry):
        @pl.when(p == 1)
        def _():
            cp_xl.wait()

        @pl.when(p >= 1)
        def _():
            out_copy(p - 1, 1).start()

        units = gate_up_units(0) + down_units(p, 0, x1c)
        last = units[4 * (FH // 128) + 1]
        units[4 * (FH // 128) + 1] = lambda: (last(), ln2(x1n, 0))
        pair(p + LAG, units, counts, eager_wo=True)
        return carry

    lax.fori_loop(0, NPAIR - LAG, main_pairs, 0)

    p0 = NPAIR - LAG
    out_copy(p0 - 1, 1).start()
    resid1(p0 + 1, x1c)
    ln2(x1c, 1)
    units = gate_up_units(0) + gate_up_units(1)
    for q in range(LAG):
        units += down_units(p0 + q, q, (x1n, x1c)[q]) + [out_copy(p0 + q, 1).start]
    for unit in units:
        unit()
    out_copy(0, NPAIR).wait()


@jax.jit
def pallas_adaLN_cond__memory_aug_recurrent_mem_tr__glu_gated_swiglu__prompt_kernel(
    A_x, A_mem0, A_Wq, A_Wk, A_Wv, A_Wo, A_seg_len, B_x, B_w1, B_w3, B_w2, c, w_mod,
):
    assert A_x.shape == (1, S, D) and A_mem0.shape == (1, MEM, D)
    del A_seg_len
    del B_x
    vm = pltpu.VMEM
    scratch = [
        vm((3 * H, D // 2, DH), U32),
        vm((HD // 2, D), U32),
        vm((2, D // 4, F // 2), U32),
        vm((5, D // 2, F // 2), BF16),
        vm((2, D // 4, F // 2), U32),
        vm((5, D // 2, F // 2), BF16),
        vm((2, F // 4, D // 2), U32),
        vm((5, F // 2, D // 2), BF16),
        vm((6, D // 2, D), U32),
        vm((NSEG, SEG // 2, D), U32),
        vm((NSEG, EARLY, D), BF16),
        vm((1, D), BF16),
        vm((MEM, D), BF16),
        vm((6, 8, D), F32),
        vm((NEARLY, D), F32),
        vm((NEARLY // 2, D), U32),
        vm((NKS * CH, NEARLY, DH), F32),
        vm((3 * NP, NSEG, EARLY, DH), U32),
        vm((SEG // 2, D), U32),
        vm((SEG // 2 + EARLY, HD), U32),
        vm((EARLY, HD), F32),
        vm((PR, D), F32),
        vm((PR, D), F32),
        vm((PR, D), F32),
        vm((LAG, 7, SEG // 2, D // 2), U32),
        vm((LAG, 7, SEG // 2, F // 2), U32),
        vm((NSEG, SEG, D), BF16),
        vm((L2, L2), jnp.int32),
        vm((L2, L2), F32),
        pltpu.SemaphoreType.DMA((14 + (NKS + 1) * NS,)),
        pltpu.SemaphoreType.DMA((NCH,)),
        pltpu.SemaphoreType.DMA(()),
    ]
    out = pl.pallas_call(
        _kernel,
        out_shape=jax.ShapeDtypeStruct((NSEG, SEG, D), BF16),
        in_specs=[pl.BlockSpec(memory_space=pl.ANY)] * 11,
        out_specs=pl.BlockSpec(memory_space=pl.ANY),
        scratch_shapes=scratch,
        compiler_params=pltpu.CompilerParams(vmem_limit_bytes=124 * 1024 * 1024,
                                             disable_bounds_checks=True,
                                             disable_semaphore_checks=True),
    )(
        A_x.reshape(NSEG, SEG, D),
        A_mem0.reshape(MEM, D),
        A_Wq.reshape(D // 2, 2 * H, DH),
        A_Wk.reshape(D // 2, 2 * H, DH),
        A_Wv.reshape(D // 2, 2 * H, DH),
        A_Wo.reshape(HD, D),
        B_w1, B_w3, B_w2, c, w_mod,
    )
    return out.reshape(1, S, D)
```

```python
import functools
import math

import jax
import jax.numpy as jnp
from jax import lax
import jax.experimental.pallas as pl
import jax.experimental.pallas.tpu as pltpu

S, D, H, DH, MEM, SEG, F = 2048, 1024, 32, 128, 8, 32, 3584
NSEG = S // SEG
NP = H // 2
HD = H * DH
EARLY = 8
NEARLY = NSEG * EARLY
L2 = 2 * (MEM + SEG)
CH = 8
NCH = 3 * H // CH
SL = (0, 256, 512, 768, D)
NS = len(SL) - 1
NKS = 3
XS = 8
NDEF = 3
NPAIR = NSEG // 2
PR = 2 * SEG
LAG = 2
FH = F // 2
NCOMB = 2
NBLK = 8 // NCOMB
EPS = 1e-5
SCALE = DH ** -0.5
MASK_FILL = -1000000000.0

BF16, F32, U32 = jnp.bfloat16, jnp.float32, jnp.uint32


def _bf(x_u32):
    return pltpu.bitcast(x_u32, BF16)


def _pk(x_f32):
    return pltpu.bitcast(x_f32.astype(BF16), U32)


def _dot(a, b):
    return jnp.dot(a, b, preferred_element_type=F32)


def _affine(x, scale8, shift8=None):
    y = x.reshape(-1, 8, x.shape[-1]) * scale8[None]
    if shift8 is not None:
        y = y + shift8[None]
    return y.reshape(x.shape)


def _lhs7(a11, a12, a21, a22):
    return [a11 + a22, a21 + a22, a11, a22, a11 + a12, a21 - a11, a12 - a22]


TERMS7 = ((1, 0, 3), (1, 0), (-1, 1, 3), (-1, 2, 0), (1, 3), (1, 0, 1), (1, 2, 3))
RHS7 = (('s', 0), ('r', 0), ('s', 1), ('s', 2), ('r', 1), ('s', 3), ('s', 4))


def _out4(m):
    return m[0] + m[3] - m[4] + m[6], m[2] + m[4], m[1] + m[3], m[0] - m[1] + m[2] + m[5]


def _norm(x):
    m = jnp.mean(x, axis=-1, keepdims=True)
    xc = x - m
    v = jnp.mean(xc * xc, axis=-1, keepdims=True)
    return xc * lax.rsqrt(v + EPS)


WO_POINTS = tuple('w%d' % w for w in range(7))
FILL_POINTS = tuple(range(3 * NP)) + ('m0', 'mid') + WO_POINTS + ('end',)


def spread(n, fixed):
    counts = dict(fixed)
    n -= sum(fixed.values())
    for k in range(6 * NP):
        counts[(k >= 3 * NP, k % (3 * NP))] = (k + 1) * n // (6 * NP) - k * n // (6 * NP)
    return counts


def _attn_mask():
    def meta(i):
        head = jnp.where(i < 2 * SEG, i // SEG, (i - 2 * SEG) // EARLY)
        j = i % SEG
        pos = jnp.where(i < 2 * SEG, jnp.where(j < MEM, j, j + EARLY), MEM + (i - 2 * SEG) % EARLY)
        return head, pos
    r = lax.broadcasted_iota(jnp.int32, (L2, L2), 0)
    c = lax.broadcasted_iota(jnp.int32, (L2, L2), 1)
    rh, rp = meta(r)
    chd, cp = meta(c)
    same = rh == chd
    keep = same & ((rp < MEM) | (rp >= cp))
    fill = jnp.where(same, MASK_FILL / SCALE, -jnp.inf).astype(F32)
    return keep, fill


def _kernel(x_hbm, m0_hbm, wq_hbm, wk_hbm, wv_hbm, wo_hbm, w1_hbm, w3_hbm, w2_hbm, c_hbm, wm_hbm,
            out_hbm,
            wqkv, wo, w1r, w1s, w3r, w3s, w2r, w2s, wm, xb, xe, cb, m0, mod, nrm, p32, p7, part, pre, l32, ob, oda, abuf,
            x1n, x1c, h2, act, ost, keep_s, fill_s, sem, wsem, osem):
    w_hbm = [r.bitcast(U32) for r in (wq_hbm, wk_hbm, wv_hbm)]
    wm_u = wm_hbm.bitcast(U32)

    def pair_copies(m, j, dsem, r0=0, r1=D // 2):
        return [pltpu.make_async_copy(w_hbm[m].at[r0:r1, par * NP + j, :],
                                      wqkv.at[m * H + 2 * j + par, r0:r1, :], dsem) for par in range(2)]

    def chunk_copies(t):
        m, c0 = divmod(t, H // CH)
        return [cp for jj in range(CH // 2)
                for cp in pair_copies(m, c0 * (CH // 2) + jj, wsem.at[t])]

    def wait_chunk(t):
        blk = wqkv.at[pl.ds(t * CH, CH)]
        pltpu.make_async_copy(blk, blk, wsem.at[t]).wait()

    def unzip(slot, r0=0, r1=D // 2):
        for r in range(r0, r1, 32):
            e, o = wqkv[slot, r:r + 32, :], wqkv[slot + 1, r:r + 32, :]
            wqkv[slot, r:r + 32, :] = (e & 0xFFFF) | (o << 16)
            wqkv[slot + 1, r:r + 32, :] = (e >> 16) | (o & jnp.uint32(0xFFFF0000))

    def start_all(cps):
        for cp in cps:
            cp.start()

    def wait_all(cps):
        for cp in cps:
            cp.wait()

    cp_c = pltpu.make_async_copy(c_hbm, cb, sem.at[0])
    x_u = x_hbm.bitcast(U32)
    cp_xe = pltpu.make_async_copy(x_hbm.at[:, 0:EARLY, :], xe, sem.at[1])
    cp_x0 = pltpu.make_async_copy(x_u.at[0], xb.at[0], sem.at[2])
    cp_m0 = pltpu.make_async_copy(m0_hbm, m0, sem.at[3])
    cp_xr = pltpu.make_async_copy(x_u.at[1:XS], xb.at[1:XS], sem.at[4])
    cp_wo = pltpu.make_async_copy(wo_hbm.bitcast(U32), wo, sem.at[5])
    def quadrant_copies(src, w, dsem):
        r, c = w[1].shape[1:]
        src_u = src.bitcast(U32)
        return [pltpu.make_async_copy(src_u.at[0:r // 2, 0:c], w[0].at[0], dsem),
                pltpu.make_async_copy(src.at[0:r, c:2 * c], w[1].at[1], dsem),
                pltpu.make_async_copy(src.at[r:2 * r, 0:c], w[1].at[2], dsem),
                pltpu.make_async_copy(src_u.at[r // 2:r, c:2 * c], w[0].at[1], dsem)]

    w1, w3, w2 = (w1r, w1s), (w3r, w3s), (w2r, w2s)
    cp_ffn = [cp for src, w, k in ((w1_hbm, w1, 6), (w3_hbm, w3, 7), (w2_hbm, w2, 8))
              for cp in quadrant_copies(src, w, sem.at[k])]

    def rhs(w, t, n):
        kind, k = RHS7[t]
        return _bf(w[0][k, :, n:n + 128]) if kind == 'r' else w[1][k, :, n:n + 128]

    cp_wm = [pltpu.make_async_copy(wm_u.at[:, k * D:(k + 1) * D], wm.at[k], sem.at[7 + k])
             for k in range(2, 6)]
    cp_xl = pltpu.make_async_copy(x_u.at[XS:NSEG], xb.at[XS:NSEG], sem.at[13])
    cp_wa = [[pltpu.make_async_copy(wm_u.at[:, k * D + SL[q]:k * D + SL[q + 1]],
                                    wm.at[k, :, SL[q]:SL[q + 1]], sem.at[14 + (NKS + 1) * q])
              for k in range(2)] for q in range(NS)]
    cp_ks = [[[cp for j in range(4 * t, 4 * t + 4)
               for cp in pair_copies(0, j, sem.at[15 + (NKS + 1) * q + t], SL[q] // 2, SL[q + 1] // 2)]
              for t in range(NKS)] for q in range(NS)]

    start_all([cp_xe, cp_c, cp_x0, cp_m0] + cp_wa[0])
    keep, fill = _attn_mask()
    keep_s[...] = keep.astype(jnp.int32)
    fill_s[...] = fill
    abuf[...] = jnp.zeros((PR, D), F32)
    x1n[...] = jnp.zeros((PR, D), F32)
    mod[2:6] = jnp.zeros((4, 8, D), F32)
    wait_all([cp_xe, cp_c, cp_x0, cp_m0])
    start_all([cp for t in range(NKS) for cp in cp_ks[0][t]])
    cf = cb[...].astype(F32)
    sc16 = jnp.broadcast_to(cf * jax.nn.sigmoid(cf), (16, D)).astype(BF16)
    for g in range(NSEG // 8):
        nrm[64 * g:64 * g + 64, :] = _norm(xe[8 * g:8 * g + 8].astype(F32).reshape(8 * EARLY, D))

    def mod_unit(k, c0, c1):
        mod[k, :, c0:c1] = _dot(sc16, _bf(wm[k, :, c0:c1]))[0:8]

    def ln1_mod(n, c0=0, c1=D):
        return _affine(n, 1.0 + mod[1, :, c0:c1], mod[0, :, c0:c1])

    def next_lhs(mem_f32, s):
        hx = ln1_mod(_norm(_bf(xb[s]).astype(F32)[EARLY:SEG]))
        l32[...] = _pk(jnp.concatenate([mem_f32, hx], axis=0))

    def early_dot(head, c, c0=0, c1=D):
        rows = slice(64 * c, 64 * c + 64) if isinstance(c, int) else pl.ds(pl.multiple_of(64 * c, 64), 64)
        return _dot(_bf(p32[rows, c0:c1]), _bf(wqkv[head, c0 // 2:c1 // 2, :]))

    def early_store(slot, c, ab):
        pre[slot // 2, pl.ds(16 * c, 16)] = _pk(
            jnp.concatenate([v.reshape(16, EARLY, DH) for v in ab], axis=1))

    def early_pair(slot, c0=0, c1=D, blocks=range(NEARLY // 128), between=()):
        between = list(between)
        for c in blocks:
            ab = [early_dot(slot + hh, c, c0, c1) for hh in range(2)]
            if between:
                between.pop(0)()
            rows = slice(128 * c, 128 * c + 128) if c1 - c0 < D else None
            if c0 > 0:
                ab = [ab[hh] + part[slot + hh, rows, :] for hh in range(2)]
            if c1 < D:
                for hh in range(2):
                    part[slot + hh, rows, :] = ab[hh]
            else:
                early_store(slot, c, ab)

    def early_run(slot0, npairs, halves=(0, 1)):
        unzip(slot0)
        for slot in range(0, 2 * npairs, 2):
            if slot + 2 < 2 * npairs:
                unzip(slot0 + slot + 2)
            for u in halves:
                m = {}
                for t in (1, 4, 0, 2, 3, 5, 6):
                    q = [_bf(wqkv[slot0 + slot + ab % 2, (ab // 2) * (D // 4):(ab // 2 + 1) * (D // 4), :])
                         for ab in TERMS7[t][1:]]
                    if len(q) == 2:
                        a_, b_ = q[0].astype(F32), q[1].astype(F32)
                        q = [(a_ + b_ if TERMS7[t][0] > 0 else a_ - b_).astype(BF16)]
                    m[t] = _dot(p7[u, t], q[0])
                c = _out4(m)
                for a in range(2):
                    early_store(slot0 + slot, 2 * u + a, c[2 * a:2 * a + 2])

    def ln1_early7(n):
        for u in range(2):
            for r in range(0, 128, 32):
                quads = [ln1_mod(nrm[128 * (2 * u + a) + r:128 * (2 * u + a) + r + 32, c:c + 256], c, c + 256)
                         for a in range(2) for c in (n, D // 2 + n)]
                for t, v in enumerate(_lhs7(*quads)):
                    p7[u, t, r:r + 32, n:n + 256] = v.astype(BF16)

    def ln1_early(q):
        for n in range(SL[q], SL[q + 1], 128):
            for g in range(NEARLY // 128):
                p32[64 * g:64 * g + 64, n:n + 128] = _pk(
                    ln1_mod(nrm[128 * g:128 * g + 128, n:n + 128], n, n + 128))

    def ks(q, *ts):
        return [cp for t in ts for cp in cp_ks[q][t]]

    def ch(*ts):
        return [cp for t in ts for cp in chunk_copies(t)]

    jobs = [(q, 2 * g) for q in range(NS) for g in range(NKS * CH // 2)]
    sync = {3: (ks(0, 1), [], None),
            7: (ks(0, 2), cp_wa[2] + ks(2, 0), None),
            11: (cp_wa[1] + ks(1, 0), ks(2, 1, 2), 1),
            15: (ks(1, 1, 2), cp_wa[3] + ks(3, 0, 1, 2), None),
            22: (cp_wa[2] + ks(2, 0), ch(3, 4), 2),
            27: (ks(2, 1, 2), [], None),
            34: (cp_wa[3] + ks(3, 0, 1, 2), ch(5, 6, 7, 8), 3)}
    wait_all(cp_wa[0])
    for k in range(2):
        mod_unit(k, 0, SL[1])
    ln1_early(0)
    start_all(cp_wa[1] + ks(1, 0, 1, 2))
    wait_all(ks(0, 0))
    unzip(0, 0, SL[1] // 2)
    for i, (q, slot) in enumerate(jobs):
        waits, issue, done = sync.get(i, ([], [], None))
        start_all(issue)
        wait_all(waits)
        if i + 1 < len(jobs):
            qn, slotn = jobs[i + 1]
            unzip(slotn, SL[qn] // 2, SL[qn + 1] // 2)
        if done is None:
            early_pair(slot, SL[q], SL[q + 1])
        else:
            early_pair(slot, SL[q], SL[q + 1], between=[
                functools.partial(mod_unit, k, n, n + 128)
                for n in range(SL[done], SL[done + 1], 128) for k in range(2)])
            ln1_early(done)
            if done >= 2:
                ln1_early7(SL[done] - D // 2)
    next_lhs(m0[...].astype(F32), 0)

    def prologue(r, carry):
        wait_chunk(2 * r + 1)
        wait_chunk(2 * r + 2)

        @pl.when(r == 1)
        def _():
            start_all(ch(*range(9, NCH)))

        @pl.when(r == 2)
        def _():
            start_all([cp_xr, cp_wo] + cp_wm[:3] + cp_ffn + [cp_wm[3], cp_xl])

        early_run((2 * r + 1) * CH, CH)
        return carry

    lax.fori_loop(1, (NCH - NDEF - 1) // 2, prologue, 0)

    def last_chunks(t, carry):
        wait_chunk(t)
        early_run(t * CH, CH // 2, halves=(0,))
        return carry

    lax.fori_loop(NCH - NDEF, NCH, last_chunks, 0)
    wait_all([cp_xr, cp_wo])

    def resid1(p, dst):
        for n in range(0, D, 256):
            xf = _bf(xb[pl.ds(2 * p, 2), :, n:n + 256]).astype(F32).reshape(PR, 256)
            dst[:, n:n + 256] = xf + _affine(abuf[:, n:n + 256], mod[2, :, n:n + 256])

    def advance(p):
        x1c[...] = x1n[...]
        resid1(p, x1n)

    def ln2(src, q):
        h = _affine(_norm(src[...]), 1.0 + mod[4], mod[3])
        quads = [h[a * SEG:(a + 1) * SEG, b * (D // 2):(b + 1) * (D // 2)] for a in range(2) for b in range(2)]
        for t, v in enumerate(_lhs7(*quads)):
            h2[q, t] = _pk(v)

    def combine(w, block0):
        rb = w[1].shape[1] // NCOMB

        def body(i, carry):
            for k in range(NBLK):
                b = block0 + NBLK * i + k
                early_pair((NCH - NDEF) * CH + 2 * (b // 2), blocks=(2 + b % 2,))
            for n0 in range(0, w[1].shape[2], 512):
                for r in range(0, rb, 16):
                    r0 = pl.multiple_of(i * rb + r, 16)
                    for n in range(n0, min(n0 + 512, w[1].shape[2]), 256):
                        b11, b22 = [_bf(w[0][k, pl.ds(pl.multiple_of(r0 // 2, 8), 8), n:n + 256]).astype(F32)
                                    for k in range(2)]
                        b12, b21 = [w[1][k, pl.ds(r0, 16), n:n + 256].astype(F32) for k in (1, 2)]
                        for k, v in enumerate((b11 + b22, b12 - b22, b21 - b11, b11 + b12, b21 + b22)):
                            w[1][k, pl.ds(r0, 16), n:n + 256] = v.astype(BF16)
            return carry
        lax.fori_loop(0, NCOMB, body, 0)

    def gate_up_units(q):
        held = {}

        def unit(f0, w, t0, t1):
            m = held.setdefault('m', [])
            m += [_dot(_bf(h2[q, t]), rhs(w, t, f0)) for t in range(t0, t1)]
            if t1 < 7:
                return
            c = _out4(held.pop('m'))
            if w is w1:
                held['g'] = c
                return
            a = [(0.5 * g) * (1.0 + jnp.tanh(0.5 * g)) * u for g, u in zip(held.pop('g'), c)]
            for t, v in enumerate(_lhs7(*a)):
                act[q, t, :, f0:f0 + 128] = _pk(v)

        return [functools.partial(unit, f0, w, t0, t1)
                for f0 in range(0, FH, 128) for w in (w1, w3) for t0, t1 in ((0, 4), (4, 7))]

    def down_units(p, q, x1):
        m = {}

        def unit(n0, t):
            m[t] = _dot(_bf(act[q, t]), rhs(w2, t, n0))
            if len(m) < 7:
                return
            c = _out4(m)
            m.clear()
            for b in range(2):
                cols = slice(b * (D // 2) + n0, b * (D // 2) + n0 + 128)
                res = x1[:, cols] + _affine(jnp.concatenate([c[b], c[2 + b]], axis=0), mod[5, :, cols])
                ost[pl.ds(2 * p, 2), :, cols] = res.astype(BF16).reshape(2, SEG, 128)

        return [functools.partial(unit, n0, t) for n0 in range(0, D // 2, 128) for t in (0, 2, 3, 5, 6, 1, 4)]

    def out_copy(p, npairs):
        rows = pl.ds(2 * p, 2 * npairs)
        return pltpu.make_async_copy(ost.at[rows], out_hbm.at[rows], osem)

    c_exp = SCALE * math.log2(math.e)
    nb = 256

    def step(s, second, fill, eager_wo):
        rows = SEG + 2 * EARLY if second else SEG
        lhs = _bf(l32[...])
        qkv, prob = {}, {}

        def project(j):
            out = []
            for m in range(3):
                a = _dot(lhs, _bf(wqkv[m * H + 2 * j])).astype(BF16)
                b = _dot(lhs, _bf(wqkv[m * H + 2 * j + 1])).astype(BF16)
                out.append(jnp.concatenate([a, b, _bf(pre[m * NP + j, s])], axis=0))
                fill(3 * j + m)
            qkv[j] = out

        def scores(j):
            q, k, _ = qkv[j]
            sc_ = lax.dot_general(q, k, (((1,), (1,)), ((), ())), preferred_element_type=F32)
            sc_ = jnp.where(keep_s[...] != 0, sc_, fill_s[...])
            e = jnp.exp2((sc_ - jnp.max(sc_, axis=1, keepdims=True)) * c_exp)
            den = jnp.sum(e, axis=1, keepdims=True)
            r = pl.reciprocal(den, approx=True)
            r = r * (2.0 - den * r)
            prob[j] = (e * r).astype(BF16)

        def values(j):
            o = _dot(prob.pop(j), qkv.pop(j)[2])
            for hh in range(2):
                c0 = (2 * j + hh) * DH
                main = o[hh * SEG:(hh + 1) * SEG]
                early = o[2 * SEG + hh * EARLY:2 * SEG + (hh + 1) * EARLY]
                if second:
                    ob[:, c0:c0 + DH] = _pk(jnp.concatenate([main, oda[:, c0:c0 + DH], early], axis=0))
                else:
                    ob[0:SEG // 2, c0:c0 + DH] = _pk(main)
                    oda[:, c0:c0 + DH] = early

        def wo_part(n, j0, j1):
            k0, k1 = j0 * 2 * DH, j1 * 2 * DH
            return _dot(_bf(ob[0:rows // 2, k0:k1]), _bf(wo[k0 // 2:k1 // 2, n * nb:(n + 1) * nb]))

        ys = [None] * (D // nb)

        def wo_acc(n, j0, j1):
            v = wo_part(n, j0, j1)
            ys[n] = v if ys[n] is None else ys[n] + v

        for j in range(NP):
            project(j)
            if j >= 1:
                scores(j - 1)
            if j >= 3:
                values(j - 3)
            if eager_wo and j in (5, 7, 9, 11, 13):
                for n in range(D // nb):
                    wo_acc(n, j - 5, j - 3)
        d0 = 10 if eager_wo else 0
        if d0 == 0:
            wo_acc(0, 0, 6)
        fill('m0')
        scores(NP - 1)
        values(NP - 3)
        wo_acc(0, max(6, d0), 12)
        if d0:
            wo_acc(1, d0, 12)
        values(NP - 2)
        fill('mid')
        if d0 == 0:
            wo_acc(1, 0, 8)
        values(NP - 1)
        if d0 == 0:
            wo_acc(1, 8, 12)
        fill('w0')
        if d0 == 0:
            wo_acc(2, 0, 7)
        fill('w1')
        wo_acc(2, max(7, d0), 14)
        fill('w2')
        if d0:
            wo_acc(3, d0, 14)
        wo_acc(0, 12, NP)
        fill('w3')
        wo_acc(1, 12, NP)
        wo_acc(2, 14, NP)
        fill('w4')
        if d0 == 0:
            wo_acc(3, 0, 5)
        fill('w5')
        if d0 == 0:
            wo_acc(3, 5, 10)
        fill('w6')
        wo_acc(3, 14 if d0 else 10, NP)
        y = jnp.concatenate(ys, axis=1)
        next_lhs(y[0:MEM], jnp.minimum(s + 1, NSEG - 1))
        fill('end')
        return y

    def pair(i, units, counts, eager_wo=False):
        units = list(units)

        def filler(second):
            def fill(point):
                for _ in range(counts.get((second, point), 0)):
                    units.pop(0)()
            return fill

        advance(jnp.maximum(i - 1, 0))
        ya = step(2 * i, False, filler(False), False)
        abuf[EARLY:SEG, :] = ya[MEM:SEG]
        yb = step(2 * i + 1, True, filler(True), eager_wo)
        abuf[0:EARLY, :] = yb[SEG:SEG + EARLY]
        abuf[SEG:SEG + EARLY, :] = yb[SEG + EARLY:SEG + 2 * EARLY]
        abuf[SEG + EARLY:PR, :] = yb[MEM:SEG]
        assert not units

    def head_pairs(i, carry):
        @pl.when(i == 0)
        def _():
            cp_wm[1].wait()

        k = 2 + 2 * i
        pltpu.make_async_copy(wm.at[k], wm.at[k], sem.at[7 + k]).wait()
        units = [functools.partial(mod_unit, k, n0, n0 + 128) for n0 in range(0, D, 128)]
        units.append(functools.partial(ln2, x1n, 0))
        units += [functools.partial(mod_unit, 3, n0, n0 + 128) for n0 in range(0, D, 128)]
        counts = {(False, 'mid'): 2, (False, 'end'): 4, (True, 'm0'): 2, (True, 'mid'): 2}
        counts.update({(True, pt): 1 for pt in WO_POINTS})
        pair(i, units, counts)
        return carry

    lax.fori_loop(0, LAG, head_pairs, 0)
    for k, w in enumerate((w1, w3, w2)):
        wait_all(cp_ffn[4 * k:4 * k + 4])
        combine(w, 8 * k)
    cp_wm[3].wait()
    mod_unit(5, 0, D)

    counts = spread(4 * (FH // 128) + 28,
                    {(False, 'mid'): 2, (False, 'end'): 4,
                     (True, 'm0'): 2, (True, 'mid'): 3, (True, 'w0'): 2, (True, 'end'): 6})

    def main_pairs(p, carry):
        @pl.when(p == 1)
        def _():
            cp_xl.wait()

        @pl.when(p >= 1)
        def _():
            out_copy(p - 1, 1).start()

        units = gate_up_units(0) + down_units(p, 0, x1c)
        last = units[4 * (FH // 128) + 1]
        units[4 * (FH // 128) + 1] = lambda: (last(), ln2(x1n, 0))
        pair(p + LAG, units, counts, eager_wo=True)
        return carry

    lax.fori_loop(0, NPAIR - LAG, main_pairs, 0)

    p0 = NPAIR - LAG
    out_copy(p0 - 1, 1).start()
    resid1(p0 + 1, x1c)
    ln2(x1c, 1)
    units = gate_up_units(0) + gate_up_units(1)
    for q in range(LAG):
        units += down_units(p0 + q, q, (x1n, x1c)[q]) + [out_copy(p0 + q, 1).start]
    for unit in units:
        unit()
    out_copy(0, NPAIR).wait()


@jax.jit
def pallas_adaLN_cond__memory_aug_recurrent_mem_tr__glu_gated_swiglu__prompt_kernel(
    A_x, A_mem0, A_Wq, A_Wk, A_Wv, A_Wo, A_seg_len, B_x, B_w1, B_w3, B_w2, c, w_mod,
):
    assert A_x.shape == (1, S, D) and A_mem0.shape == (1, MEM, D)
    del A_seg_len
    del B_x
    vm = pltpu.VMEM
    scratch = [
        vm((3 * H, D // 2, DH), U32),
        vm((HD // 2, D), U32),
        vm((2, D // 4, F // 2), U32),
        vm((5, D // 2, F // 2), BF16),
        vm((2, D // 4, F // 2), U32),
        vm((5, D // 2, F // 2), BF16),
        vm((2, F // 4, D // 2), U32),
        vm((5, F // 2, D // 2), BF16),
        vm((6, D // 2, D), U32),
        vm((NSEG, SEG // 2, D), U32),
        vm((NSEG, EARLY, D), BF16),
        vm((1, D), BF16),
        vm((MEM, D), BF16),
        vm((6, 8, D), F32),
        vm((NEARLY, D), F32),
        vm((NEARLY // 2, D), U32),
        vm((2, 7, 128, D // 2), BF16),
        vm((NKS * CH, NEARLY, DH), F32),
        vm((3 * NP, NSEG, EARLY, DH), U32),
        vm((SEG // 2, D), U32),
        vm((SEG // 2 + EARLY, HD), U32),
        vm((EARLY, HD), F32),
        vm((PR, D), F32),
        vm((PR, D), F32),
        vm((PR, D), F32),
        vm((LAG, 7, SEG // 2, D // 2), U32),
        vm((LAG, 7, SEG // 2, F // 2), U32),
        vm((NSEG, SEG, D), BF16),
        vm((L2, L2), jnp.int32),
        vm((L2, L2), F32),
        pltpu.SemaphoreType.DMA((14 + (NKS + 1) * NS,)),
        pltpu.SemaphoreType.DMA((NCH,)),
        pltpu.SemaphoreType.DMA(()),
    ]
    out = pl.pallas_call(
        _kernel,
        out_shape=jax.ShapeDtypeStruct((NSEG, SEG, D), BF16),
        in_specs=[pl.BlockSpec(memory_space=pl.ANY)] * 11,
        out_specs=pl.BlockSpec(memory_space=pl.ANY),
        scratch_shapes=scratch,
        compiler_params=pltpu.CompilerParams(vmem_limit_bytes=124 * 1024 * 1024,
                                             disable_bounds_checks=True,
                                             disable_semaphore_checks=True),
    )(
        A_x.reshape(NSEG, SEG, D),
        A_mem0.reshape(MEM, D),
        A_Wq.reshape(D // 2, 2 * H, DH),
        A_Wk.reshape(D // 2, 2 * H, DH),
        A_Wv.reshape(D // 2, 2 * H, DH),
        A_Wo.reshape(HD, D),
        B_w1, B_w3, B_w2, c, w_mod,
    )
    return out.reshape(1, S, D)
```

```python
import functools
import math

import jax
import jax.numpy as jnp
from jax import lax
import jax.experimental.pallas as pl
import jax.experimental.pallas.tpu as pltpu

S, D, H, DH, MEM, SEG, F = 2048, 1024, 32, 128, 8, 32, 3584
NSEG = S // SEG
NP = H // 2
HD = H * DH
EARLY = 8
NEARLY = NSEG * EARLY
L2 = 2 * (MEM + SEG)
CH = 8
NCH = 3 * H // CH
SL = (0, 256, 512, 768, D)
NS = len(SL) - 1
NKS = 3
XS = 8
NDEF = 5
NPAIR = NSEG // 2
PR = 2 * SEG
LAG = 2
NCOMB = 2
NBLK = 6
NHB = 2
GSPL = (0, 5, 10, 14, 18, 22, 26)
NGU = 7 * (len(GSPL) - 1)
EPS = 1e-5
SCALE = DH ** -0.5
MASK_FILL = -1000000000.0

BF16, F32, U32 = jnp.bfloat16, jnp.float32, jnp.uint32


def _bf(x_u32):
    return pltpu.bitcast(x_u32, BF16)


def _pk(x_f32):
    return pltpu.bitcast(x_f32.astype(BF16), U32)


def _dot(a, b):
    return jnp.dot(a, b, preferred_element_type=F32)


def _affine(x, scale8, shift8=None):
    y = x.reshape(-1, 8, x.shape[-1]) * scale8[None]
    if shift8 is not None:
        y = y + shift8[None]
    return y.reshape(x.shape)


def _lhs7(a11, a12, a21, a22):
    return [a11 + a22, a21 + a22, a11, a22, a11 + a12, a21 - a11, a12 - a22]


TERMS7 = ((1, 0, 3), (1, 0), (-1, 1, 3), (-1, 2, 0), (1, 3), (1, 0, 1), (1, 2, 3))

FAST = [[[(i, 1 if ch == '+' else -1) for i, ch in enumerate(part) if ch != '.'] for part in row.split()]
        for row in (
    '....++.+ ...+........-... +.+--.-+',
    '...+++.+ ............+... +.+-...+',
    '....+.+. .+.............. +-..-+..',
    '+...++.+ ...+............ -.-++...',
    '+...+.+. .+......+....... -+..+...',
    '+.+.+.+. ........+....... +-......',
    '....++.. ..++........-... ....+.+.',
    '+....-.. ..++-........... ..+.+...',
    '+....... ++.+-........... +...-...',
    '++...... ....+........... +.+.....',
    '+...+... -.++....+....... ....-...',
    '......++ .............+.. .-.+.+.-',
    '.+-..... .....+.......... .++..--.',
    '.+-..+.. .....+....+..... ..-..++.',
    '...+..++ ...........+.+.. .+.-...+',
    '.+-..+-. ..........+..... .....--.',
    '..++..++ ...........+.... .-.+....',
    '......+. .+.......-+..+.. .....-..',
    '..+..... .....+..++.+.... .+......',
    '.....+.. ..++.+-.....-.+. ..+...-.',
    '...+.-.. .......+....-.+. ..+....-',
    '.....+.+ ...+........-.+. ......+-',
    '.+.+.... .......+........ ..-+....',
    '.+...+.. ....-.++..+..... ..+.....',
    '...+.... .......-....++.+ ...+...-',
    '...+...+ ...........++.-- .......-',
)]
NF = len(FAST)
assert all(sum(sa * sb * sc for f in FAST for i, sa in f[0] for j, sb in f[1] for k, sc in f[2]
               if (i, j, k) == (a, b, c)) == (a % 4 == b // 4 and c == a // 4 * 4 + b % 4)
           for a in range(8) for b in range(16) for c in range(8))
RAWB = [f[1][0][0] for f in FAST if len(f[1]) == 1]
SUMB = [f[1] for f in FAST if len(f[1]) > 1]
CGRP = ((15, 14), (13, 4, 5), (10, 2, 3), (8, 7), (0, 11, 12), (6, 1, 9))
LAND = {0: 13, 2: 10, 6: 2, 9: 6, 14: 0, 15: 15}
assert all(max(g for g, grp in enumerate(CGRP) for k in grp if b in dict(SUMB[k]))
           <= [slot in grp for grp in CGRP].index(True) for b, slot in LAND.items())


def _signed_sum(terms):
    terms = sorted(terms, key=lambda t: -t[1])
    acc = terms[0][0] if terms[0][1] > 0 else -terms[0][0]
    for v, sg in terms[1:]:
        acc = acc + v if sg > 0 else acc - v
    return acc


def _fast_lhs(blocks):
    return [_signed_sum([(blocks[i], sg) for i, sg in f[0]]) for f in FAST]


def _fast_acc(acc, t, v):
    for o, sg in FAST[t][2]:
        if o not in acc:
            acc[o] = (v, sg)
        else:
            a, sa = acc[o]
            acc[o] = (a + v, sa) if sa == sg else ((a - v, 1) if sa > 0 else (v - a, 1))


def _fast_out(acc):
    return [acc[o][0] if acc[o][1] > 0 else -acc[o][0] for o in range(8)]


def _out4(m):
    return m[0] + m[3] - m[4] + m[6], m[2] + m[4], m[1] + m[3], m[0] - m[1] + m[2] + m[5]


def _norm(x):
    m = jnp.mean(x, axis=-1, keepdims=True)
    xc = x - m
    v = jnp.mean(xc * xc, axis=-1, keepdims=True)
    return xc * lax.rsqrt(v + EPS)


WO_POINTS = tuple('w%d' % w for w in range(7))
FILL_POINTS = tuple(range(3 * NP)) + ('m0', 'mid') + WO_POINTS + ('end',)


def spread(n, fixed):
    counts = dict(fixed)
    n -= sum(fixed.values())
    for k in range(6 * NP):
        counts[(k >= 3 * NP, k % (3 * NP))] = (k + 1) * n // (6 * NP) - k * n // (6 * NP)
    return counts


def _attn_mask():
    def meta(i):
        head = jnp.where(i < 2 * SEG, i // SEG, (i - 2 * SEG) // EARLY)
        j = i % SEG
        pos = jnp.where(i < 2 * SEG, jnp.where(j < MEM, j, j + EARLY), MEM + (i - 2 * SEG) % EARLY)
        return head, pos
    r = lax.broadcasted_iota(jnp.int32, (L2, L2), 0)
    c = lax.broadcasted_iota(jnp.int32, (L2, L2), 1)
    rh, rp = meta(r)
    chd, cp = meta(c)
    same = rh == chd
    keep = same & ((rp < MEM) | (rp >= cp))
    fill = jnp.where(same, MASK_FILL / SCALE, -jnp.inf).astype(F32)
    return keep, fill


def _kernel(x_hbm, m0_hbm, wq_hbm, wk_hbm, wv_hbm, wo_hbm, w1_hbm, w3_hbm, w2_hbm, c_hbm, wm_hbm,
            out_hbm,
            wqkv, wo, w1r, w1s, w3r, w3s, w2r, w2s, wm, xb, xe, cb, m0, mod, nrm, p32, p7, part, pre, l32, ob, oda, abuf,
            x1n, x1c, h2, act, ost, keep_s, fill_s, sem, wsem, osem):
    w_hbm = [r.bitcast(U32) for r in (wq_hbm, wk_hbm, wv_hbm)]
    wm_u = wm_hbm.bitcast(U32)

    def pair_copies(m, j, dsem, r0=0, r1=D // 2):
        return [pltpu.make_async_copy(w_hbm[m].at[r0:r1, par * NP + j, :],
                                      wqkv.at[m * H + 2 * j + par, r0:r1, :], dsem) for par in range(2)]

    def chunk_copies(t):
        m, c0 = divmod(t, H // CH)
        return [cp for jj in range(CH // 2)
                for cp in pair_copies(m, c0 * (CH // 2) + jj, wsem.at[t])]

    def wait_chunk(t):
        blk = wqkv.at[pl.ds(t * CH, CH)]
        pltpu.make_async_copy(blk, blk, wsem.at[t]).wait()

    def unzip(slot, r0=0, r1=D // 2):
        for r in range(r0, r1, 32):
            e, o = wqkv[slot, r:r + 32, :], wqkv[slot + 1, r:r + 32, :]
            wqkv[slot, r:r + 32, :] = (e & 0xFFFF) | (o << 16)
            wqkv[slot + 1, r:r + 32, :] = (e >> 16) | (o & jnp.uint32(0xFFFF0000))

    def start_all(cps):
        for cp in cps:
            cp.start()

    def wait_all(cps):
        for cp in cps:
            cp.wait()

    cp_c = pltpu.make_async_copy(c_hbm, cb, sem.at[0])
    x_u = x_hbm.bitcast(U32)
    cp_xe = pltpu.make_async_copy(x_hbm.at[:, 0:EARLY, :], xe, sem.at[1])
    cp_x0 = pltpu.make_async_copy(x_u.at[0], xb.at[0], sem.at[2])
    cp_m0 = pltpu.make_async_copy(m0_hbm, m0, sem.at[3])
    cp_xr = pltpu.make_async_copy(x_u.at[1:XS], xb.at[1:XS], sem.at[4])
    cp_wo = pltpu.make_async_copy(wo_hbm.bitcast(U32), wo, sem.at[5])
    def block_copies(src, w, dsem, part=0, nparts=1):
        r, c = w[1].shape[1:]
        r0, r1 = part * r // nparts, (part + 1) * r // nparts
        src_u = src.bitcast(U32)
        cps = []
        for b in range(16):
            k, n = divmod(b, 4)
            if b in RAWB:
                cps.append(pltpu.make_async_copy(src_u.at[(k * r + r0) // 2:(k * r + r1) // 2, n * c:(n + 1) * c],
                                                 w[0].at[RAWB.index(b), r0 // 2:r1 // 2], dsem))
            else:
                cps.append(pltpu.make_async_copy(src.at[k * r + r0:k * r + r1, n * c:(n + 1) * c],
                                                 w[1].at[LAND[b], r0:r1], dsem))
        return cps

    w1, w3, w2 = (w1r, w1s), (w3r, w3s), (w2r, w2s)
    cp_w1, cp_w3 = block_copies(w1_hbm, w1, sem.at[6]), block_copies(w3_hbm, w3, sem.at[7])
    cp_w2 = [block_copies(w2_hbm, w2, wsem.at[i], i, NCOMB) for i in range(NCOMB)]

    def rhs(w, t, n):
        f = FAST[t][1]
        return _bf(w[0][RAWB.index(f[0][0]), :, n:n + 128]) if len(f) == 1 else w[1][SUMB.index(f), :, n:n + 128]

    cp_wm = [pltpu.make_async_copy(wm_u.at[:, k * D:(k + 1) * D], wm.at[k], sem.at[7 + k])
             for k in range(2, 6)]
    cp_xl = pltpu.make_async_copy(x_u.at[XS:NSEG], xb.at[XS:NSEG], sem.at[13])
    cp_wa = [[pltpu.make_async_copy(wm_u.at[:, k * D + SL[q]:k * D + SL[q + 1]],
                                    wm.at[k, :, SL[q]:SL[q + 1]], sem.at[14 + (NKS + 1) * q])
              for k in range(2)] for q in range(NS)]
    cp_ks = [[[cp for j in range(4 * t, 4 * t + 4)
               for cp in pair_copies(0, j, sem.at[15 + (NKS + 1) * q + t], SL[q] // 2, SL[q + 1] // 2)]
              for t in range(NKS)] for q in range(NS)]

    start_all([cp_xe, cp_c, cp_x0, cp_m0] + cp_wa[0])
    keep, fill = _attn_mask()
    keep_s[...] = keep.astype(jnp.int32)
    fill_s[...] = fill
    abuf[...] = jnp.zeros((PR, D), F32)
    wait_all([cp_xe, cp_c, cp_x0, cp_m0])
    start_all([cp for t in range(NKS) for cp in cp_ks[0][t]])
    cf = cb[...].astype(F32)
    sc16 = jnp.broadcast_to(cf * jax.nn.sigmoid(cf), (16, D)).astype(BF16)
    for g in range(NSEG // 8):
        nrm[64 * g:64 * g + 64, :] = _norm(xe[8 * g:8 * g + 8].astype(F32).reshape(8 * EARLY, D))

    def mod_unit(k, c0, c1):
        mod[k, :, c0:c1] = _dot(sc16, _bf(wm[k, :, c0:c1]))[0:8]

    def ln1_mod(n, c0=0, c1=D):
        return _affine(n, 1.0 + mod[1, :, c0:c1], mod[0, :, c0:c1])

    def next_lhs(mem_f32, s):
        hx = ln1_mod(_norm(_bf(xb[s]).astype(F32)[EARLY:SEG]))
        l32[...] = _pk(jnp.concatenate([mem_f32, hx], axis=0))

    def early_dot(head, c, c0=0, c1=D):
        rows = slice(64 * c, 64 * c + 64) if isinstance(c, int) else pl.ds(pl.multiple_of(64 * c, 64), 64)
        return _dot(_bf(p32[rows, c0:c1]), _bf(wqkv[head, c0 // 2:c1 // 2, :]))

    def early_store(slot, c, ab):
        pre[slot // 2, pl.ds(16 * c, 16)] = _pk(
            jnp.concatenate([v.reshape(16, EARLY, DH) for v in ab], axis=1))

    def early_pair(slot, c0=0, c1=D, blocks=range(NEARLY // 128), between=()):
        between = list(between)
        for c in blocks:
            ab = []
            for hh in range(2):
                ab.append(early_dot(slot + hh, c, c0, c1))
                if between and (hh == 1 or c1 - c0 == D):
                    between.pop(0)()
            rows = slice(128 * c, 128 * c + 128) if c1 - c0 < D else None
            if c0 > 0:
                ab = [ab[hh] + part[slot + hh, rows, :] for hh in range(2)]
            if c1 < D:
                for hh in range(2):
                    part[slot + hh, rows, :] = ab[hh]
            else:
                early_store(slot, c, ab)

    def early_run(slot0, npairs, halves=(0, 1)):
        unzip(slot0)
        for slot in range(0, 2 * npairs, 2):
            if slot + 2 < 2 * npairs:
                unzip(slot0 + slot + 2)
            for u in halves:
                m = {}
                for t in (1, 4, 0, 2, 3, 5, 6):
                    q = [_bf(wqkv[slot0 + slot + ab % 2, (ab // 2) * (D // 4):(ab // 2 + 1) * (D // 4), :])
                         for ab in TERMS7[t][1:]]
                    if len(q) == 2:
                        a_, b_ = q[0].astype(F32), q[1].astype(F32)
                        q = [(a_ + b_ if TERMS7[t][0] > 0 else a_ - b_).astype(BF16)]
                    m[t] = _dot(p7[u, t], q[0])
                c = _out4(m)
                for a in range(2):
                    early_store(slot0 + slot, 2 * u + a, c[2 * a:2 * a + 2])

    def ln1_early7(n):
        for u in range(2):
            for r in range(0, 128, 32):
                quads = [ln1_mod(nrm[128 * (2 * u + a) + r:128 * (2 * u + a) + r + 32, c:c + 256], c, c + 256)
                         for a in range(2) for c in (n, D // 2 + n)]
                for t, v in enumerate(_lhs7(*quads)):
                    p7[u, t, r:r + 32, n:n + 256] = v.astype(BF16)

    def ln1_early(q):
        for n in range(SL[q], SL[q + 1], 128):
            for g in range(NEARLY // 128):
                p32[64 * g:64 * g + 64, n:n + 128] = _pk(
                    ln1_mod(nrm[128 * g:128 * g + 128, n:n + 128], n, n + 128))

    def ks(q, *ts):
        return [cp for t in ts for cp in cp_ks[q][t]]

    def ch(*ts):
        return [cp for t in ts for cp in chunk_copies(t)]

    jobs = [(q, 2 * g) for q in range(NS) for g in range(NKS * CH // 2)]
    sync = {3: (ks(0, 1), [], None),
            7: (ks(0, 2), cp_wa[2] + ks(2, 0), None),
            11: (cp_wa[1] + ks(1, 0), ks(2, 1, 2), 1),
            15: (ks(1, 1, 2), cp_wa[3] + ks(3, 0, 1, 2), None),
            22: (cp_wa[2] + ks(2, 0), ch(3, 4), 2),
            27: (ks(2, 1, 2), [], None),
            34: (cp_wa[3] + ks(3, 0, 1, 2), ch(5, 6, 7, 8), 3)}
    wait_all(cp_wa[0])
    for k in range(2):
        mod_unit(k, 0, SL[1])
    ln1_early(0)
    start_all(cp_wa[1] + ks(1, 0, 1, 2))
    wait_all(ks(0, 0))
    unzip(0, 0, SL[1] // 2)
    for i, (q, slot) in enumerate(jobs):
        waits, issue, done = sync.get(i, ([], [], None))
        start_all(issue)
        wait_all(waits)
        if i + 1 < len(jobs):
            qn, slotn = jobs[i + 1]
            unzip(slotn, SL[qn] // 2, SL[qn + 1] // 2)
        if done is None:
            early_pair(slot, SL[q], SL[q + 1])
        else:
            early_pair(slot, SL[q], SL[q + 1], between=[
                functools.partial(mod_unit, k, n, n + 128)
                for n in range(SL[done], SL[done + 1], 128) for k in range(2)])
            ln1_early(done)
            if done >= 2:
                ln1_early7(SL[done] - D // 2)
    next_lhs(m0[...].astype(F32), 0)

    def prologue(r, carry):
        wait_chunk(2 * r + 1)
        wait_chunk(2 * r + 2)

        @pl.when(r == 1)
        def _():
            start_all(ch(*range(9, NCH)))

        @pl.when(r == 2)
        def _():
            start_all([cp_xr, cp_wo] + cp_w1 + cp_wm[0:2])

        early_run((2 * r + 1) * CH, CH)
        return carry

    lax.fori_loop(1, (NCH - NDEF - 1) // 2, prologue, 0)

    def last_chunks(t, carry):
        wait_chunk(t)

        @pl.when(t == NCH - 3)
        def _():
            start_all(cp_w3 + [cp_wm[2]] + cp_w2[0] + cp_w2[1] + [cp_wm[3], cp_xl])

        early_run(t * CH, CH // 2, halves=(0,))
        return carry

    lax.fori_loop(NCH - NDEF, NCH, last_chunks, 0)
    wait_all([cp_xr, cp_wo])

    def resid1(p, dst, attn=abuf):
        for n in range(0, D, 256):
            xf = _bf(xb[pl.ds(2 * p, 2), :, n:n + 256]).astype(F32).reshape(PR, 256)
            dst[:, n:n + 256] = xf + _affine(attn[:, n:n + 256], mod[2, :, n:n + 256])

    def advance(p):
        x1c[...] = x1n[...]
        resid1(p, x1n)

    def ln2(src, q):
        h = _affine(_norm(src[...]), 1.0 + mod[4], mod[3])
        blocks = [h[a * SEG:(a + 1) * SEG, k * (D // 4):(k + 1) * (D // 4)] for a in range(2) for k in range(4)]
        for t, v in enumerate(_fast_lhs(blocks)):
            h2[q, t] = v.astype(BF16)

    def deferred(b, between=()):
        early_pair((NCH - NDEF) * CH + 2 * (b // 2), blocks=(2 + b % 2,), between=between)

    def combine(w, block0, kmod, waits=lambda i: ()):
        rb = w[1].shape[1] // NCOMB

        def body(i, carry):
            wait_all(waits(i))
            for k in range(NBLK):
                mods = [functools.partial(mod_unit, kmod(i), n, n + 128) for n in (256 * k, 256 * k + 128)
                        if kmod and k < 4]
                deferred(block0 + NBLK * i + k, mods)
            for n in range(0, w[1].shape[2], 256):
                cols = slice(n, min(n + 256, w[1].shape[2]))
                for grp in CGRP:
                    for r in range(0, rb, 16):
                        r0 = pl.multiple_of(i * rb + r, 16)
                        raw = {}
                        for b in sorted({b for k in grp for b, _ in SUMB[k]}):
                            if b in RAWB:
                                raw[b] = _bf(w[0][RAWB.index(b), pl.ds(pl.multiple_of(r0 // 2, 8), 8), cols]).astype(F32)
                            else:
                                raw[b] = w[1][LAND[b], pl.ds(r0, 16), cols].astype(F32)
                        for k in grp:
                            w[1][k, pl.ds(r0, 16), cols] = _signed_sum([(raw[b], sg) for b, sg in SUMB[k]]).astype(BF16)
            return carry
        lax.fori_loop(0, NCOMB, body, 0)

    def gate_up_units(q):
        held = {}

        def unit(f0, t0, t1):
            m = held.setdefault('m', {})
            for t in range(t0, t1):
                _fast_acc(m, t, _dot(h2[q, t],
                                     jnp.concatenate([rhs(w1, t, f0), rhs(w3, t, f0)], axis=1)))
            if t1 < NF:
                return
            a = [(0.5 * c[:, :128]) * (1.0 + jnp.tanh(0.5 * c[:, :128])) * c[:, 128:] for c in _fast_out(held.pop('m'))]
            for t, v in enumerate(_fast_lhs(a)):
                act[q, t, :, f0:f0 + 128] = _pk(v)

        return [functools.partial(unit, f0, t0, t1) for f0 in range(0, F // 4, 128) for t0, t1 in zip(GSPL, GSPL[1:])]

    def down_units(p, q, x1):
        m = {}

        def unit(n0, t0, t1):
            for t in range(t0, t1):
                _fast_acc(m, t, _dot(_bf(act[q, t]), rhs(w2, t, n0)))
            if t1 < NF:
                return
            c = _fast_out(m)
            m.clear()
            for b in range(4):
                cols = slice(b * (D // 4) + n0, b * (D // 4) + n0 + 128)
                res = x1[:, cols] + _affine(jnp.concatenate([c[b], c[4 + b]], axis=0), mod[5, :, cols])
                ost[pl.ds(2 * p, 2), :, cols] = res.astype(BF16).reshape(2, SEG, 128)

        return [functools.partial(unit, n0, t, t + 2) for n0 in range(0, D // 4, 128) for t in range(0, NF, 2)]

    def out_copy(p, npairs):
        rows = pl.ds(2 * p, 2 * npairs)
        return pltpu.make_async_copy(ost.at[rows], out_hbm.at[rows], osem)

    c_exp = SCALE * math.log2(math.e)
    nb = 256

    def step(s, second, fill, eager_wo):
        rows = SEG + 2 * EARLY if second else SEG
        lhs = _bf(l32[...])
        qkv, prob = {}, {}

        def project(j):
            out = []
            for m in range(3):
                a = _dot(lhs, _bf(wqkv[m * H + 2 * j])).astype(BF16)
                b = _dot(lhs, _bf(wqkv[m * H + 2 * j + 1])).astype(BF16)
                out.append(jnp.concatenate([a, b, _bf(pre[m * NP + j, s])], axis=0))
                fill(3 * j + m)
            qkv[j] = out

        def scores(j):
            q, k, _ = qkv[j]
            sc_ = lax.dot_general(q, k, (((1,), (1,)), ((), ())), preferred_element_type=F32)
            sc_ = jnp.where(keep_s[...] != 0, sc_, fill_s[...])
            e = jnp.exp2((sc_ - jnp.max(sc_, axis=1, keepdims=True)) * c_exp)
            den = jnp.sum(e, axis=1, keepdims=True)
            r = pl.reciprocal(den, approx=True)
            r = r * (2.0 - den * r)
            prob[j] = (e * r).astype(BF16)

        def values(j):
            o = _dot(prob.pop(j), qkv.pop(j)[2])
            for hh in range(2):
                c0 = (2 * j + hh) * DH
                main = o[hh * SEG:(hh + 1) * SEG]
                early = o[2 * SEG + hh * EARLY:2 * SEG + (hh + 1) * EARLY]
                if second:
                    ob[:, c0:c0 + DH] = _pk(jnp.concatenate([main, oda[:, c0:c0 + DH], early], axis=0))
                else:
                    ob[0:SEG // 2, c0:c0 + DH] = _pk(main)
                    oda[:, c0:c0 + DH] = early

        def wo_part(n, j0, j1):
            k0, k1 = j0 * 2 * DH, j1 * 2 * DH
            return _dot(_bf(ob[0:rows // 2, k0:k1]), _bf(wo[k0 // 2:k1 // 2, n * nb:(n + 1) * nb]))

        ys = [None] * (D // nb)

        def wo_acc(n, j0, j1):
            v = wo_part(n, j0, j1)
            ys[n] = v if ys[n] is None else ys[n] + v

        for j in range(NP):
            project(j)
            if j >= 1:
                scores(j - 1)
            if j >= 3:
                values(j - 3)
            if eager_wo and j in (5, 7, 9, 11, 13):
                for n in range(D // nb):
                    wo_acc(n, j - 5, j - 3)
        d0 = 10 if eager_wo else 0
        if d0 == 0:
            wo_acc(0, 0, 6)
        fill('m0')
        scores(NP - 1)
        values(NP - 3)
        wo_acc(0, max(6, d0), 12)
        if d0:
            wo_acc(1, d0, 12)
        values(NP - 2)
        fill('mid')
        if d0 == 0:
            wo_acc(1, 0, 8)
        values(NP - 1)
        if d0 == 0:
            wo_acc(1, 8, 12)
        fill('w0')
        if d0 == 0:
            wo_acc(2, 0, 7)
        fill('w1')
        wo_acc(2, max(7, d0), 14)
        fill('w2')
        if d0:
            wo_acc(3, d0, 14)
        wo_acc(0, 12, NP)
        fill('w3')
        wo_acc(1, 12, NP)
        wo_acc(2, 14, NP)
        fill('w4')
        if d0 == 0:
            wo_acc(3, 0, 5)
        fill('w5')
        if d0 == 0:
            wo_acc(3, 5, 10)
        fill('w6')
        wo_acc(3, 14 if d0 else 10, NP)
        y = jnp.concatenate(ys, axis=1)
        next_lhs(y[0:MEM], jnp.minimum(s + 1, NSEG - 1))
        fill('end')
        return y

    def pair(i, units, counts, first=False):
        units = list(units)

        def filler(second):
            def fill(point):
                for _ in range(counts.get((second, point), 0)):
                    units.pop(0)()
            return fill

        if first:
            x1n[...] = abuf[...]
        else:
            advance(i - 1)
        ya = step(2 * i, False, filler(False), False)
        abuf[EARLY:SEG, :] = ya[MEM:SEG]
        yb = step(2 * i + 1, True, filler(True), not first)
        abuf[0:EARLY, :] = yb[SEG:SEG + EARLY]
        abuf[SEG:SEG + EARLY, :] = yb[SEG + EARLY:SEG + 2 * EARLY]
        abuf[SEG + EARLY:PR, :] = yb[MEM:SEG]
        assert not units

    def head_pairs(i, carry):
        units = [functools.partial(deferred, NHB * i + k) for k in range(NHB)]
        pair(i, units, {(False, 'end'): 1, (True, 'end'): 1}, first=True)
        return carry

    lax.fori_loop(0, LAG, head_pairs, 0)
    wait_all(cp_w1 + cp_wm[0:2])
    combine(w1, NHB * LAG, lambda i: 2 + i)
    wait_all(cp_w3 + [cp_wm[2]])
    combine(w3, NHB * LAG + NBLK * NCOMB, lambda i: 4)
    combine(w2, NHB * LAG + 2 * NBLK * NCOMB, None, lambda i: block_copies(w2_hbm, w2, wsem.at[i], 0, NCOMB))
    cp_wm[3].wait()
    mod_unit(5, 0, D)
    resid1(0, x1n, x1n)
    ln2(x1n, 0)

    counts = spread(NGU + NF,
                    {(False, 'mid'): 2, (False, 'end'): 3,
                     (True, 'm0'): 2, (True, 'mid'): 3, (True, 'w0'): 2, (True, 'end'): 6})

    def main_pairs(p, carry):
        @pl.when(p == 1)
        def _():
            cp_xl.wait()

        @pl.when(p >= 1)
        def _():
            out_copy(p - 1, 1).start()

        units = gate_up_units(0) + down_units(p, 0, x1c)
        last = units[NGU + 1]
        units[NGU + 1] = lambda: (last(), ln2(x1n, 0))
        pair(p + LAG, units, counts)
        return carry

    lax.fori_loop(0, NPAIR - LAG, main_pairs, 0)

    p0 = NPAIR - LAG
    out_copy(p0 - 1, 1).start()
    resid1(p0 + 1, x1c)
    ln2(x1c, 1)
    units = gate_up_units(0) + gate_up_units(1)
    for q in range(LAG):
        units += down_units(p0 + q, q, (x1n, x1c)[q]) + [out_copy(p0 + q, 1).start]
    for unit in units:
        unit()
    out_copy(0, NPAIR).wait()


@jax.jit
def pallas_adaLN_cond__memory_aug_recurrent_mem_tr__glu_gated_swiglu__prompt_kernel(
    A_x, A_mem0, A_Wq, A_Wk, A_Wv, A_Wo, A_seg_len, B_x, B_w1, B_w3, B_w2, c, w_mod,
):
    assert A_x.shape == (1, S, D) and A_mem0.shape == (1, MEM, D)
    del A_seg_len
    del B_x
    vm = pltpu.VMEM
    scratch = [
        vm((3 * H, D // 2, DH), U32),
        vm((HD // 2, D), U32),
        vm((len(RAWB), D // 8, F // 4), U32),
        vm((len(SUMB), D // 4, F // 4), BF16),
        vm((len(RAWB), D // 8, F // 4), U32),
        vm((len(SUMB), D // 4, F // 4), BF16),
        vm((len(RAWB), F // 8, D // 4), U32),
        vm((len(SUMB), F // 4, D // 4), BF16),
        vm((6, D // 2, D), U32),
        vm((NSEG, SEG // 2, D), U32),
        vm((NSEG, EARLY, D), BF16),
        vm((1, D), BF16),
        vm((MEM, D), BF16),
        vm((6, 8, D), F32),
        vm((NEARLY, D), F32),
        vm((NEARLY // 2, D), U32),
        vm((2, 7, 128, D // 2), BF16),
        vm((NKS * CH, NEARLY, DH), F32),
        vm((3 * NP, NSEG, EARLY, DH), U32),
        vm((SEG // 2, D), U32),
        vm((SEG // 2 + EARLY, HD), U32),
        vm((EARLY, HD), F32),
        vm((PR, D), F32),
        vm((PR, D), F32),
        vm((PR, D), F32),
        vm((LAG, NF, SEG, D // 4), BF16),
        vm((LAG, NF, SEG // 2, F // 4), U32),
        vm((NSEG, SEG, D), BF16),
        vm((L2, L2), jnp.int32),
        vm((L2, L2), F32),
        pltpu.SemaphoreType.DMA((14 + (NKS + 1) * NS,)),
        pltpu.SemaphoreType.DMA((NCH,)),
        pltpu.SemaphoreType.DMA(()),
    ]
    out = pl.pallas_call(
        _kernel,
        out_shape=jax.ShapeDtypeStruct((NSEG, SEG, D), BF16),
        in_specs=[pl.BlockSpec(memory_space=pl.ANY)] * 11,
        out_specs=pl.BlockSpec(memory_space=pl.ANY),
        scratch_shapes=scratch,
        compiler_params=pltpu.CompilerParams(vmem_limit_bytes=124 * 1024 * 1024,
                                             disable_bounds_checks=True,
                                             disable_semaphore_checks=True),
    )(
        A_x.reshape(NSEG, SEG, D),
        A_mem0.reshape(MEM, D),
        A_Wq.reshape(D // 2, 2 * H, DH),
        A_Wk.reshape(D // 2, 2 * H, DH),
        A_Wv.reshape(D // 2, 2 * H, DH),
        A_Wo.reshape(HD, D),
        B_w1, B_w3, B_w2, c, w_mod,
    )
    return out.reshape(1, S, D)
```

```python
import functools
import math

import jax
import jax.numpy as jnp
from jax import lax
import jax.experimental.pallas as pl
import jax.experimental.pallas.tpu as pltpu

S, D, H, DH, MEM, SEG, F = 2048, 1024, 32, 128, 8, 32, 3584
NSEG = S // SEG
NP = H // 2
HD = H * DH
EARLY = 8
NEARLY = NSEG * EARLY
L2 = 2 * (MEM + SEG)
CH = 8
NCH = 3 * H // CH
SL = (0, 256, 512, 768, D)
NS = len(SL) - 1
NKS = 3
XS = 8
NDEF = 5
NPAIR = NSEG // 2
PR = 2 * SEG
LAG = 2
NCOMB = 2
NBLK = 6
NHB = 2
GSPL = (0, 5, 10, 14, 18, 22, 26)
NGU = 7 * (len(GSPL) - 1)
EPS = 1e-5
SCALE = DH ** -0.5
MASK_FILL = -1000000000.0

BF16, F32, U32 = jnp.bfloat16, jnp.float32, jnp.uint32


def _bf(x_u32):
    return pltpu.bitcast(x_u32, BF16)


def _pk(x_f32):
    return pltpu.bitcast(x_f32.astype(BF16), U32)


def _dot(a, b):
    return jnp.dot(a, b, preferred_element_type=F32)


def _affine(x, scale8, shift8=None):
    y = x.reshape(-1, 8, x.shape[-1]) * scale8[None]
    if shift8 is not None:
        y = y + shift8[None]
    return y.reshape(x.shape)


def _lhs7(a11, a12, a21, a22):
    return [a11 + a22, a21 + a22, a11, a22, a11 + a12, a21 - a11, a12 - a22]


TERMS7 = ((1, 0, 3), (1, 0), (-1, 1, 3), (-1, 2, 0), (1, 3), (1, 0, 1), (1, 2, 3))

FAST = [[[(i, 1 if ch == '+' else -1) for i, ch in enumerate(part) if ch != '.'] for part in row.split()]
        for row in (
    '....++.+ ...+........-... +.+--.-+',
    '...+++.+ ............+... +.+-...+',
    '....+.+. .+.............. +-..-+..',
    '+...++.+ ...+............ -.-++...',
    '+...+.+. .+......+....... -+..+...',
    '+.+.+.+. ........+....... +-......',
    '....++.. ..++........-... ....+.+.',
    '+....-.. ..++-........... ..+.+...',
    '+....... ++.+-........... +...-...',
    '++...... ....+........... +.+.....',
    '+...+... -.++....+....... ....-...',
    '......++ .............+.. .-.+.+.-',
    '.+-..... .....+.......... .++..--.',
    '.+-..+.. .....+....+..... ..-..++.',
    '...+..++ ...........+.+.. .+.-...+',
    '.+-..+-. ..........+..... .....--.',
    '..++..++ ...........+.... .-.+....',
    '......+. .+.......-+..+.. .....-..',
    '..+..... .....+..++.+.... .+......',
    '.....+.. ..++.+-.....-.+. ..+...-.',
    '...+.-.. .......+....-.+. ..+....-',
    '.....+.+ ...+........-.+. ......+-',
    '.+.+.... .......+........ ..-+....',
    '.+...+.. ....-.++..+..... ..+.....',
    '...+.... .......-....++.+ ...+...-',
    '...+...+ ...........++.-- .......-',
)]
NF = len(FAST)
assert all(sum(sa * sb * sc for f in FAST for i, sa in f[0] for j, sb in f[1] for k, sc in f[2]
               if (i, j, k) == (a, b, c)) == (a % 4 == b // 4 and c == a // 4 * 4 + b % 4)
           for a in range(8) for b in range(16) for c in range(8))
RAWB = [f[1][0][0] for f in FAST if len(f[1]) == 1]
SUMB = [f[1] for f in FAST if len(f[1]) > 1]
CGRP = ((15, 14), (13, 4, 5), (10, 2, 3), (8, 7), (0, 11, 12), (6, 1, 9))
LAND = {0: 13, 2: 10, 6: 2, 9: 6, 14: 0, 15: 15}
assert all(max(g for g, grp in enumerate(CGRP) for k in grp if b in dict(SUMB[k]))
           <= [slot in grp for grp in CGRP].index(True) for b, slot in LAND.items())


def _signed_sum(terms):
    terms = sorted(terms, key=lambda t: -t[1])
    acc = terms[0][0] if terms[0][1] > 0 else -terms[0][0]
    for v, sg in terms[1:]:
        acc = acc + v if sg > 0 else acc - v
    return acc


def _fast_lhs(blocks):
    return [_signed_sum([(blocks[i], sg) for i, sg in f[0]]) for f in FAST]


def _fast_acc(acc, t, v):
    for o, sg in FAST[t][2]:
        if o not in acc:
            acc[o] = (v, sg)
        else:
            a, sa = acc[o]
            acc[o] = (a + v, sa) if sa == sg else ((a - v, 1) if sa > 0 else (v - a, 1))


def _fast_out(acc):
    return [acc[o][0] if acc[o][1] > 0 else -acc[o][0] for o in range(8)]


def _out4(m):
    return m[0] + m[3] - m[4] + m[6], m[2] + m[4], m[1] + m[3], m[0] - m[1] + m[2] + m[5]


def _norm(x):
    m = jnp.mean(x, axis=-1, keepdims=True)
    xc = x - m
    v = jnp.mean(xc * xc, axis=-1, keepdims=True)
    return xc * lax.rsqrt(v + EPS)


WO_POINTS = tuple('w%d' % w for w in range(7))
FILL_POINTS = tuple(range(3 * NP)) + ('m0', 'mid') + WO_POINTS + ('end',)


def spread(n, fixed):
    counts = dict(fixed)
    n -= sum(fixed.values())
    for k in range(6 * NP):
        counts[(k >= 3 * NP, k % (3 * NP))] = (k + 1) * n // (6 * NP) - k * n // (6 * NP)
    return counts


def _attn_mask():
    def meta(i):
        head = jnp.where(i < 2 * SEG, i // SEG, (i - 2 * SEG) // EARLY)
        j = i % SEG
        pos = jnp.where(i < 2 * SEG, jnp.where(j < MEM, j, j + EARLY), MEM + (i - 2 * SEG) % EARLY)
        return head, pos
    r = lax.broadcasted_iota(jnp.int32, (L2, L2), 0)
    c = lax.broadcasted_iota(jnp.int32, (L2, L2), 1)
    rh, rp = meta(r)
    chd, cp = meta(c)
    same = rh == chd
    keep = same & ((rp < MEM) | (rp >= cp))
    fill = jnp.where(same, MASK_FILL / SCALE, -jnp.inf).astype(F32)
    return keep, fill


def _kernel(x_hbm, m0_hbm, wq_hbm, wk_hbm, wv_hbm, wo_hbm, w1_hbm, w3_hbm, w2_hbm, c_hbm, wm_hbm,
            out_hbm,
            wqkv, wo, w1r, w1s, w3r, w3s, w2r, w2s, wm, xb, xe, cb, m0, mod, nrm, p32, p7, part, pre, l32, ob, oda, abuf,
            x1n, x1c, h2, act, ost, keep_s, fill_s, sem, wsem, osem):
    w_hbm = [r.bitcast(U32) for r in (wq_hbm, wk_hbm, wv_hbm)]
    wm_u = wm_hbm.bitcast(U32)

    def pair_copies(m, j, dsem, r0=0, r1=D // 2):
        return [pltpu.make_async_copy(w_hbm[m].at[r0:r1, par * NP + j, :],
                                      wqkv.at[m * H + 2 * j + par, r0:r1, :], dsem) for par in range(2)]

    def chunk_copies(t):
        m, c0 = divmod(t, H // CH)
        return [cp for jj in range(CH // 2)
                for cp in pair_copies(m, c0 * (CH // 2) + jj, wsem.at[t])]

    def wait_chunk(t):
        blk = wqkv.at[pl.ds(t * CH, CH)]
        pltpu.make_async_copy(blk, blk, wsem.at[t]).wait()

    def unzip(slot, r0=0, r1=D // 2):
        for r in range(r0, r1, 32):
            e, o = wqkv[slot, r:r + 32, :], wqkv[slot + 1, r:r + 32, :]
            wqkv[slot, r:r + 32, :] = (e & 0xFFFF) | (o << 16)
            wqkv[slot + 1, r:r + 32, :] = (e >> 16) | (o & jnp.uint32(0xFFFF0000))

    def start_all(cps):
        for cp in cps:
            cp.start()

    def wait_all(cps):
        for cp in cps:
            cp.wait()

    cp_c = pltpu.make_async_copy(c_hbm, cb, sem.at[0])
    x_u = x_hbm.bitcast(U32)
    cp_xe = pltpu.make_async_copy(x_hbm.at[:, 0:EARLY, :], xe, sem.at[1])
    cp_x0 = pltpu.make_async_copy(x_u.at[0], xb.at[0], sem.at[2])
    cp_m0 = pltpu.make_async_copy(m0_hbm, m0, sem.at[3])
    cp_xr = pltpu.make_async_copy(x_u.at[1:XS], xb.at[1:XS], sem.at[4])
    cp_wo = pltpu.make_async_copy(wo_hbm.bitcast(U32), wo, sem.at[5])
    def block_copies(src, w, dsem, part=0, nparts=1):
        r, c = w[1].shape[1:]
        nr = r // nparts
        src_u = src.bitcast(U32)

        def rows(start, size):
            return pl.ds(start if isinstance(start, int) else pl.multiple_of(start, 8), size)

        cps = []
        for b in range(16):
            k, n = divmod(b, 4)
            if b in RAWB:
                cps.append(pltpu.make_async_copy(
                    src_u.at[rows(k * r // 2 + part * (nr // 2), nr // 2), n * c:(n + 1) * c],
                    w[0].at[RAWB.index(b), rows(part * (nr // 2), nr // 2)], dsem))
            else:
                cps.append(pltpu.make_async_copy(src.at[rows(k * r + part * nr, nr), n * c:(n + 1) * c],
                                                 w[1].at[LAND[b], rows(part * nr, nr)], dsem))
        return cps

    w1, w3, w2 = (w1r, w1s), (w3r, w3s), (w2r, w2s)
    cp_w1, cp_w3 = block_copies(w1_hbm, w1, sem.at[6]), block_copies(w3_hbm, w3, sem.at[7])
    cp_w2 = [block_copies(w2_hbm, w2, wsem.at[i], i, NCOMB) for i in range(NCOMB)]

    def rhs(w, t, n):
        f = FAST[t][1]
        return _bf(w[0][RAWB.index(f[0][0]), :, n:n + 128]) if len(f) == 1 else w[1][SUMB.index(f), :, n:n + 128]

    cp_wm = [pltpu.make_async_copy(wm_u.at[:, k * D:(k + 1) * D], wm.at[k], sem.at[7 + k])
             for k in range(2, 6)]
    cp_xl = pltpu.make_async_copy(x_u.at[XS:NSEG], xb.at[XS:NSEG], sem.at[13])
    cp_wa = [[pltpu.make_async_copy(wm_u.at[:, k * D + SL[q]:k * D + SL[q + 1]],
                                    wm.at[k, :, SL[q]:SL[q + 1]], sem.at[14 + (NKS + 1) * q])
              for k in range(2)] for q in range(NS)]
    cp_ks = [[[cp for j in range(4 * t, 4 * t + 4)
               for cp in pair_copies(0, j, sem.at[15 + (NKS + 1) * q + t], SL[q] // 2, SL[q + 1] // 2)]
              for t in range(NKS)] for q in range(NS)]

    start_all([cp_xe, cp_c, cp_x0, cp_m0] + cp_wa[0])
    keep, fill = _attn_mask()
    keep_s[...] = keep.astype(jnp.int32)
    fill_s[...] = fill
    abuf[...] = jnp.zeros((PR, D), F32)
    wait_all([cp_xe, cp_c, cp_x0, cp_m0])
    start_all([cp for t in range(NKS) for cp in cp_ks[0][t]])
    cf = cb[...].astype(F32)
    sc16 = jnp.broadcast_to(cf * jax.nn.sigmoid(cf), (16, D)).astype(BF16)
    for g in range(NSEG // 8):
        nrm[64 * g:64 * g + 64, :] = _norm(xe[8 * g:8 * g + 8].astype(F32).reshape(8 * EARLY, D))

    def mod_unit(k, c0, c1):
        mod[k, :, c0:c1] = _dot(sc16, _bf(wm[k, :, c0:c1]))[0:8]

    def ln1_mod(n, c0=0, c1=D):
        return _affine(n, 1.0 + mod[1, :, c0:c1], mod[0, :, c0:c1])

    def next_lhs(mem_f32, s):
        hx = ln1_mod(_norm(_bf(xb[s]).astype(F32)[EARLY:SEG]))
        l32[...] = _pk(jnp.concatenate([mem_f32, hx], axis=0))

    def early_dot(head, c, c0=0, c1=D):
        rows = slice(64 * c, 64 * c + 64) if isinstance(c, int) else pl.ds(pl.multiple_of(64 * c, 64), 64)
        return _dot(_bf(p32[rows, c0:c1]), _bf(wqkv[head, c0 // 2:c1 // 2, :]))

    def early_store(slot, c, ab):
        pre[slot // 2, pl.ds(16 * c, 16)] = _pk(
            jnp.concatenate([v.reshape(16, EARLY, DH) for v in ab], axis=1))

    def early_pair(slot, c0=0, c1=D, blocks=range(NEARLY // 128), between=()):
        between = list(between)
        for c in blocks:
            ab = []
            for hh in range(2):
                ab.append(early_dot(slot + hh, c, c0, c1))
                if between and (hh == 1 or c1 - c0 == D):
                    between.pop(0)()
            rows = slice(128 * c, 128 * c + 128) if c1 - c0 < D else None
            if c0 > 0:
                ab = [ab[hh] + part[slot + hh, rows, :] for hh in range(2)]
            if c1 < D:
                for hh in range(2):
                    part[slot + hh, rows, :] = ab[hh]
            else:
                early_store(slot, c, ab)

    def early_run(slot0, npairs, halves=(0, 1)):
        unzip(slot0)
        for slot in range(0, 2 * npairs, 2):
            if slot + 2 < 2 * npairs:
                unzip(slot0 + slot + 2)
            for u in halves:
                m = {}
                for t in (1, 4, 0, 2, 3, 5, 6):
                    q = [_bf(wqkv[slot0 + slot + ab % 2, (ab // 2) * (D // 4):(ab // 2 + 1) * (D // 4), :])
                         for ab in TERMS7[t][1:]]
                    if len(q) == 2:
                        a_, b_ = q[0].astype(F32), q[1].astype(F32)
                        q = [(a_ + b_ if TERMS7[t][0] > 0 else a_ - b_).astype(BF16)]
                    m[t] = _dot(p7[u, t], q[0])
                c = _out4(m)
                for a in range(2):
                    early_store(slot0 + slot, 2 * u + a, c[2 * a:2 * a + 2])

    def ln1_early7(n):
        for u in range(2):
            for r in range(0, 128, 32):
                quads = [ln1_mod(nrm[128 * (2 * u + a) + r:128 * (2 * u + a) + r + 32, c:c + 256], c, c + 256)
                         for a in range(2) for c in (n, D // 2 + n)]
                for t, v in enumerate(_lhs7(*quads)):
                    p7[u, t, r:r + 32, n:n + 256] = v.astype(BF16)

    def ln1_early(q):
        for n in range(SL[q], SL[q + 1], 128):
            for g in range(NEARLY // 128):
                p32[64 * g:64 * g + 64, n:n + 128] = _pk(
                    ln1_mod(nrm[128 * g:128 * g + 128, n:n + 128], n, n + 128))

    def ks(q, *ts):
        return [cp for t in ts for cp in cp_ks[q][t]]

    def ch(*ts):
        return [cp for t in ts for cp in chunk_copies(t)]

    jobs = [(q, 2 * g) for q in range(NS) for g in range(NKS * CH // 2)]
    sync = {3: (ks(0, 1), [], None),
            7: (ks(0, 2), cp_wa[2] + ks(2, 0), None),
            11: (cp_wa[1] + ks(1, 0), ks(2, 1, 2), 1),
            15: (ks(1, 1, 2), cp_wa[3] + ks(3, 0, 1, 2), None),
            22: (cp_wa[2] + ks(2, 0), ch(3, 4), 2),
            27: (ks(2, 1, 2), [], None),
            34: (cp_wa[3] + ks(3, 0, 1, 2), ch(5, 6, 7, 8), 3)}
    wait_all(cp_wa[0])
    for k in range(2):
        mod_unit(k, 0, SL[1])
    ln1_early(0)
    start_all(cp_wa[1] + ks(1, 0, 1, 2))
    wait_all(ks(0, 0))
    unzip(0, 0, SL[1] // 2)
    for i, (q, slot) in enumerate(jobs):
        waits, issue, done = sync.get(i, ([], [], None))
        start_all(issue)
        wait_all(waits)
        if i + 1 < len(jobs):
            qn, slotn = jobs[i + 1]
            unzip(slotn, SL[qn] // 2, SL[qn + 1] // 2)
        if done is None:
            early_pair(slot, SL[q], SL[q + 1])
        else:
            early_pair(slot, SL[q], SL[q + 1], between=[
                functools.partial(mod_unit, k, n, n + 128)
                for n in range(SL[done], SL[done + 1], 128) for k in range(2)])
            ln1_early(done)
            if done >= 2:
                ln1_early7(SL[done] - D // 2)
    next_lhs(m0[...].astype(F32), 0)

    def prologue(r, carry):
        wait_chunk(2 * r + 1)
        wait_chunk(2 * r + 2)

        @pl.when(r == 1)
        def _():
            start_all(ch(*range(9, NCH)))

        @pl.when(r == 2)
        def _():
            start_all([cp_xr, cp_wo] + cp_w1 + cp_wm[0:2])

        early_run((2 * r + 1) * CH, CH)
        return carry

    lax.fori_loop(1, (NCH - NDEF - 1) // 2, prologue, 0)

    def last_chunks(t, carry):
        wait_chunk(t)

        @pl.when(t == NCH - 3)
        def _():
            start_all(cp_w3 + [cp_wm[2]] + cp_w2[0] + cp_w2[1] + [cp_wm[3], cp_xl])

        early_run(t * CH, CH // 2, halves=(0,))
        return carry

    lax.fori_loop(NCH - NDEF, NCH, last_chunks, 0)
    wait_all([cp_xr, cp_wo])

    def resid1(p, dst, attn=abuf):
        for n in range(0, D, 256):
            xf = _bf(xb[pl.ds(2 * p, 2), :, n:n + 256]).astype(F32).reshape(PR, 256)
            dst[:, n:n + 256] = xf + _affine(attn[:, n:n + 256], mod[2, :, n:n + 256])

    def advance(p):
        x1c[...] = x1n[...]
        resid1(p, x1n)

    def ln2(src, q):
        h = _affine(_norm(src[...]), 1.0 + mod[4], mod[3])
        blocks = [h[a * SEG:(a + 1) * SEG, k * (D // 4):(k + 1) * (D // 4)] for a in range(2) for k in range(4)]
        for t, v in enumerate(_fast_lhs(blocks)):
            h2[q, t] = v.astype(BF16)

    def deferred(b, between=()):
        early_pair((NCH - NDEF) * CH + 2 * (b // 2), blocks=(2 + b % 2,), between=between)

    def combine(w, block0, kmod, waits=lambda i: ()):
        rb = w[1].shape[1] // NCOMB

        def body(i, carry):
            wait_all(waits(i))
            for k in range(NBLK):
                mods = [functools.partial(mod_unit, kmod(i), n, n + 128) for n in (256 * k, 256 * k + 128)
                        if kmod and k < 4]
                deferred(block0 + NBLK * i + k, mods)
            for n in range(0, w[1].shape[2], 256):
                cols = slice(n, min(n + 256, w[1].shape[2]))
                for grp in CGRP:
                    for r in range(0, rb, 16):
                        r0 = pl.multiple_of(i * rb + r, 16)
                        raw = {}
                        for b in sorted({b for k in grp for b, _ in SUMB[k]}):
                            if b in RAWB:
                                raw[b] = _bf(w[0][RAWB.index(b), pl.ds(pl.multiple_of(r0 // 2, 8), 8), cols]).astype(F32)
                            else:
                                raw[b] = w[1][LAND[b], pl.ds(r0, 16), cols].astype(F32)
                        for k in grp:
                            w[1][k, pl.ds(r0, 16), cols] = _signed_sum([(raw[b], sg) for b, sg in SUMB[k]]).astype(BF16)
            return carry
        lax.fori_loop(0, NCOMB, body, 0)

    def gate_up_units(q):
        held = {}

        def unit(f0, t0, t1):
            m = held.setdefault('m', {})
            for t in range(t0, t1):
                _fast_acc(m, t, _dot(h2[q, t],
                                     jnp.concatenate([rhs(w1, t, f0), rhs(w3, t, f0)], axis=1)))
            if t1 < NF:
                return
            a = [(0.5 * c[:, :128]) * (1.0 + jnp.tanh(0.5 * c[:, :128])) * c[:, 128:] for c in _fast_out(held.pop('m'))]
            for t, v in enumerate(_fast_lhs(a)):
                act[q, t, :, f0:f0 + 128] = _pk(v)

        return [functools.partial(unit, f0, t0, t1) for f0 in range(0, F // 4, 128) for t0, t1 in zip(GSPL, GSPL[1:])]

    def down_units(p, q, x1):
        m = {}

        plain = [t for t in range(NF) if len(FAST[t][1]) == 1][-4:]
        order = {0: list(range(NF)), 128: [t for t in range(NF) if t not in plain] + plain}

        def unit(n0, t0, t1):
            for t in order[n0][t0:t1]:
                _fast_acc(m, t, _dot(_bf(act[q, t]), rhs(w2, t, n0)))
            if t1 < NF:
                return
            c = _fast_out(m)
            m.clear()
            for b in range(4):
                cols = slice(b * (D // 4) + n0, b * (D // 4) + n0 + 128)
                res = x1[:, cols] + _affine(jnp.concatenate([c[b], c[4 + b]], axis=0), mod[5, :, cols])
                ost[pl.ds(2 * p, 2), :, cols] = res.astype(BF16).reshape(2, SEG, 128)

        return [functools.partial(unit, n0, t, t + 2) for n0 in range(0, D // 4, 128) for t in range(0, NF, 2)]

    def out_copy(p, npairs):
        rows = pl.ds(2 * p, 2 * npairs)
        return pltpu.make_async_copy(ost.at[rows], out_hbm.at[rows], osem)

    c_exp = SCALE * math.log2(math.e)
    nb = 256

    def step(s, second, fill, eager_wo):
        rows = SEG + 2 * EARLY if second else SEG
        lhs = _bf(l32[...])
        qkv, prob = {}, {}

        def project(j):
            out = []
            for m in range(3):
                a = _dot(lhs, _bf(wqkv[m * H + 2 * j])).astype(BF16)
                b = _dot(lhs, _bf(wqkv[m * H + 2 * j + 1])).astype(BF16)
                out.append(jnp.concatenate([a, b, _bf(pre[m * NP + j, s])], axis=0))
                fill(3 * j + m)
            qkv[j] = out

        def scores(j):
            q, k, _ = qkv[j]
            sc_ = lax.dot_general(q, k, (((1,), (1,)), ((), ())), preferred_element_type=F32)
            sc_ = jnp.where(keep_s[...] != 0, sc_, fill_s[...])
            e = jnp.exp2((sc_ - jnp.max(sc_, axis=1, keepdims=True)) * c_exp)
            den = jnp.sum(e, axis=1, keepdims=True)
            r = pl.reciprocal(den, approx=True)
            r = r * (2.0 - den * r)
            prob[j] = (e * r).astype(BF16)

        def values(j):
            o = _dot(prob.pop(j), qkv.pop(j)[2])
            for hh in range(2):
                c0 = (2 * j + hh) * DH
                main = o[hh * SEG:(hh + 1) * SEG]
                early = o[2 * SEG + hh * EARLY:2 * SEG + (hh + 1) * EARLY]
                if second:
                    ob[:, c0:c0 + DH] = _pk(jnp.concatenate([main, oda[:, c0:c0 + DH], early], axis=0))
                else:
                    ob[0:SEG // 2, c0:c0 + DH] = _pk(main)
                    oda[:, c0:c0 + DH] = early

        def wo_part(n, j0, j1):
            k0, k1 = j0 * 2 * DH, j1 * 2 * DH
            return _dot(_bf(ob[0:rows // 2, k0:k1]), _bf(wo[k0 // 2:k1 // 2, n * nb:(n + 1) * nb]))

        ys = [None] * (D // nb)

        def wo_acc(n, j0, j1):
            v = wo_part(n, j0, j1)
            ys[n] = v if ys[n] is None else ys[n] + v

        for j in range(NP):
            project(j)
            if j >= 1:
                scores(j - 1)
            if j >= 3:
                values(j - 3)
            if eager_wo and j in (5, 7, 9, 11, 13):
                for n in range(D // nb):
                    wo_acc(n, j - 5, j - 3)
        d0 = 10 if eager_wo else 0
        if d0 == 0:
            wo_acc(0, 0, 6)
        fill('m0')
        scores(NP - 1)
        values(NP - 3)
        wo_acc(0, max(6, d0), 12)
        if d0:
            wo_acc(1, d0, 12)
        values(NP - 2)
        fill('mid')
        if d0 == 0:
            wo_acc(1, 0, 8)
        values(NP - 1)
        if d0 == 0:
            wo_acc(1, 8, 12)
        fill('w0')
        if d0 == 0:
            wo_acc(2, 0, 7)
        fill('w1')
        wo_acc(2, max(7, d0), 14)
        fill('w2')
        if d0:
            wo_acc(3, d0, 14)
        wo_acc(0, 12, NP)
        fill('w3')
        wo_acc(1, 12, NP)
        wo_acc(2, 14, NP)
        fill('w4')
        if d0 == 0:
            wo_acc(3, 0, 5)
        fill('w5')
        if d0 == 0:
            wo_acc(3, 5, 10)
        fill('w6')
        wo_acc(3, 14 if d0 else 10, NP)
        y = jnp.concatenate(ys, axis=1)
        next_lhs(y[0:MEM], jnp.minimum(s + 1, NSEG - 1))
        fill('end')
        return y

    def pair(i, units, counts, first=False):
        units = list(units)

        def filler(second):
            def fill(point):
                for _ in range(counts.get((second, point), 0)):
                    units.pop(0)()
            return fill

        if first:
            x1n[...] = abuf[...]
        else:
            advance(i - 1)
        ya = step(2 * i, False, filler(False), False)
        abuf[EARLY:SEG, :] = ya[MEM:SEG]
        yb = step(2 * i + 1, True, filler(True), not first)
        abuf[0:EARLY, :] = yb[SEG:SEG + EARLY]
        abuf[SEG:SEG + EARLY, :] = yb[SEG + EARLY:SEG + 2 * EARLY]
        abuf[SEG + EARLY:PR, :] = yb[MEM:SEG]
        assert not units

    def head_pairs(i, carry):
        units = [functools.partial(deferred, NHB * i + k) for k in range(NHB)]
        pair(i, units, {(False, 'end'): 1, (True, 'end'): 1}, first=True)
        return carry

    lax.fori_loop(0, LAG, head_pairs, 0)
    wait_all(cp_w1 + cp_wm[0:2])
    combine(w1, NHB * LAG, lambda i: 2 + i)
    wait_all(cp_w3 + [cp_wm[2]])
    combine(w3, NHB * LAG + NBLK * NCOMB, lambda i: 4)
    combine(w2, NHB * LAG + 2 * NBLK * NCOMB, None, lambda i: block_copies(w2_hbm, w2, wsem.at[i], i, NCOMB))
    cp_wm[3].wait()
    mod_unit(5, 0, D)
    resid1(0, x1n, x1n)
    ln2(x1n, 0)

    counts = spread(NGU + NF,
                    {(False, 'mid'): 2, (False, 'end'): 3,
                     (True, 'm0'): 2, (True, 'mid'): 3, (True, 'w0'): 2, (True, 'end'): 6})

    def main_pairs(p, carry):
        @pl.when(p == 1)
        def _():
            cp_xl.wait()

        @pl.when(p >= 1)
        def _():
            out_copy(p - 1, 1).start()

        units = gate_up_units(0) + down_units(p, 0, x1c)
        last = units[NGU + 1]
        units[NGU + 1] = lambda: (last(), ln2(x1n, 0))
        pair(p + LAG, units, counts)
        return carry

    lax.fori_loop(0, NPAIR - LAG, main_pairs, 0)

    p0 = NPAIR - LAG
    out_copy(p0 - 1, 1).start()
    resid1(p0 + 1, x1c)
    ln2(x1c, 1)
    units = gate_up_units(0) + gate_up_units(1)
    for q in range(LAG):
        units += down_units(p0 + q, q, (x1n, x1c)[q]) + [out_copy(p0 + q, 1).start]
    for unit in units:
        unit()
    out_copy(0, NPAIR).wait()


@jax.jit
def pallas_adaLN_cond__memory_aug_recurrent_mem_tr__glu_gated_swiglu__prompt_kernel(
    A_x, A_mem0, A_Wq, A_Wk, A_Wv, A_Wo, A_seg_len, B_x, B_w1, B_w3, B_w2, c, w_mod,
):
    assert A_x.shape == (1, S, D) and A_mem0.shape == (1, MEM, D)
    del A_seg_len
    del B_x
    vm = pltpu.VMEM
    scratch = [
        vm((3 * H, D // 2, DH), U32),
        vm((HD // 2, D), U32),
        vm((len(RAWB), D // 8, F // 4), U32),
        vm((len(SUMB), D // 4, F // 4), BF16),
        vm((len(RAWB), D // 8, F // 4), U32),
        vm((len(SUMB), D // 4, F // 4), BF16),
        vm((len(RAWB), F // 8, D // 4), U32),
        vm((len(SUMB), F // 4, D // 4), BF16),
        vm((6, D // 2, D), U32),
        vm((NSEG, SEG // 2, D), U32),
        vm((NSEG, EARLY, D), BF16),
        vm((1, D), BF16),
        vm((MEM, D), BF16),
        vm((6, 8, D), F32),
        vm((NEARLY, D), F32),
        vm((NEARLY // 2, D), U32),
        vm((2, 7, 128, D // 2), BF16),
        vm((NKS * CH, NEARLY, DH), F32),
        vm((3 * NP, NSEG, EARLY, DH), U32),
        vm((SEG // 2, D), U32),
        vm((SEG // 2 + EARLY, HD), U32),
        vm((EARLY, HD), F32),
        vm((PR, D), F32),
        vm((PR, D), F32),
        vm((PR, D), F32),
        vm((LAG, NF, SEG, D // 4), BF16),
        vm((LAG, NF, SEG // 2, F // 4), U32),
        vm((NSEG, SEG, D), BF16),
        vm((L2, L2), jnp.int32),
        vm((L2, L2), F32),
        pltpu.SemaphoreType.DMA((14 + (NKS + 1) * NS,)),
        pltpu.SemaphoreType.DMA((NCH,)),
        pltpu.SemaphoreType.DMA(()),
    ]
    out = pl.pallas_call(
        _kernel,
        out_shape=jax.ShapeDtypeStruct((NSEG, SEG, D), BF16),
        in_specs=[pl.BlockSpec(memory_space=pl.ANY)] * 11,
        out_specs=pl.BlockSpec(memory_space=pl.ANY),
        scratch_shapes=scratch,
        compiler_params=pltpu.CompilerParams(vmem_limit_bytes=124 * 1024 * 1024,
                                             disable_bounds_checks=True,
                                             disable_semaphore_checks=True),
    )(
        A_x.reshape(NSEG, SEG, D),
        A_mem0.reshape(MEM, D),
        A_Wq.reshape(D // 2, 2 * H, DH),
        A_Wk.reshape(D // 2, 2 * H, DH),
        A_Wv.reshape(D // 2, 2 * H, DH),
        A_Wo.reshape(HD, D),
        B_w1, B_w3, B_w2, c, w_mod,
    )
    return out.reshape(1, S, D)
```

```python
import functools
import math

import jax
import jax.numpy as jnp
from jax import lax
import jax.experimental.pallas as pl
import jax.experimental.pallas.tpu as pltpu

S, D, H, DH, MEM, SEG, F = 2048, 1024, 32, 128, 8, 32, 3584
NSEG = S // SEG
NP = H // 2
HD = H * DH
EARLY = 8
NEARLY = NSEG * EARLY
L2 = 2 * (MEM + SEG)
CH = 8
NCH = 3 * H // CH
SL = (0, 256, 512, 768, D)
NS = len(SL) - 1
NKS = 3
XS = 8
NDEF = 5
NPAIR = NSEG // 2
PR = 2 * SEG
LAG = 2
NCOMB = 2
NBLK = (7, 7, 6)
GSPL = (0, 5, 10, 14, 18, 22, 26)
NGU = 7 * (len(GSPL) - 1)
EPS = 1e-5
SCALE = DH ** -0.5
MASK_FILL = -1000000000.0

BF16, F32, U32 = jnp.bfloat16, jnp.float32, jnp.uint32


def _bf(x_u32):
    return pltpu.bitcast(x_u32, BF16)


def _pk(x_f32):
    return pltpu.bitcast(x_f32.astype(BF16), U32)


def _dot(a, b):
    return jnp.dot(a, b, preferred_element_type=F32)


def _affine(x, scale8, shift8=None):
    y = x.reshape(-1, 8, x.shape[-1]) * scale8[None]
    if shift8 is not None:
        y = y + shift8[None]
    return y.reshape(x.shape)


def _lhs7(a11, a12, a21, a22):
    return [a11 + a22, a21 + a22, a11, a22, a11 + a12, a21 - a11, a12 - a22]


TERMS7 = ((1, 0, 3), (1, 0), (-1, 1, 3), (-1, 2, 0), (1, 3), (1, 0, 1), (1, 2, 3))

FAST = [[[(i, 1 if ch == '+' else -1) for i, ch in enumerate(part) if ch != '.'] for part in row.split()]
        for row in (
    '....++.+ ...+........-... +.+--.-+',
    '...+++.+ ............+... +.+-...+',
    '....+.+. .+.............. +-..-+..',
    '+...++.+ ...+............ -.-++...',
    '+...+.+. .+......+....... -+..+...',
    '+.+.+.+. ........+....... +-......',
    '....++.. ..++........-... ....+.+.',
    '+....-.. ..++-........... ..+.+...',
    '+....... ++.+-........... +...-...',
    '++...... ....+........... +.+.....',
    '+...+... -.++....+....... ....-...',
    '......++ .............+.. .-.+.+.-',
    '.+-..... .....+.......... .++..--.',
    '.+-..+.. .....+....+..... ..-..++.',
    '...+..++ ...........+.+.. .+.-...+',
    '.+-..+-. ..........+..... .....--.',
    '..++..++ ...........+.... .-.+....',
    '......+. .+.......-+..+.. .....-..',
    '..+..... .....+..++.+.... .+......',
    '.....+.. ..++.+-.....-.+. ..+...-.',
    '...+.-.. .......+....-.+. ..+....-',
    '.....+.+ ...+........-.+. ......+-',
    '.+.+.... .......+........ ..-+....',
    '.+...+.. ....-.++..+..... ..+.....',
    '...+.... .......-....++.+ ...+...-',
    '...+...+ ...........++.-- .......-',
)]
NF = len(FAST)
assert all(sum(sa * sb * sc for f in FAST for i, sa in f[0] for j, sb in f[1] for k, sc in f[2]
               if (i, j, k) == (a, b, c)) == (a % 4 == b // 4 and c == a // 4 * 4 + b % 4)
           for a in range(8) for b in range(16) for c in range(8))
RAWB = [f[1][0][0] for f in FAST if len(f[1]) == 1]
SUMB = [f[1] for f in FAST if len(f[1]) > 1]
CGRP = ((15, 14), (13, 4, 5), (10, 2, 3), (8, 7), (0, 11, 12), (6, 1, 9))
LAND = {0: 13, 2: 10, 6: 2, 9: 6, 14: 0, 15: 15}
assert all(max(g for g, grp in enumerate(CGRP) for k in grp if b in dict(SUMB[k]))
           <= [slot in grp for grp in CGRP].index(True) for b, slot in LAND.items())


def _signed_sum(terms):
    terms = sorted(terms, key=lambda t: -t[1])
    acc = terms[0][0] if terms[0][1] > 0 else -terms[0][0]
    for v, sg in terms[1:]:
        acc = acc + v if sg > 0 else acc - v
    return acc


def _fast_lhs(blocks):
    return [_signed_sum([(blocks[i], sg) for i, sg in f[0]]) for f in FAST]


def _fast_acc(acc, t, v):
    for o, sg in FAST[t][2]:
        if o not in acc:
            acc[o] = (v, sg)
        else:
            a, sa = acc[o]
            acc[o] = (a + v, sa) if sa == sg else ((a - v, 1) if sa > 0 else (v - a, 1))


def _fast_out(acc):
    return [acc[o][0] if acc[o][1] > 0 else -acc[o][0] for o in range(8)]


def _out4(m):
    return m[0] + m[3] - m[4] + m[6], m[2] + m[4], m[1] + m[3], m[0] - m[1] + m[2] + m[5]


def _norm(x):
    m = jnp.mean(x, axis=-1, keepdims=True)
    xc = x - m
    v = jnp.mean(xc * xc, axis=-1, keepdims=True)
    return xc * lax.rsqrt(v + EPS)


WO_POINTS = tuple('w%d' % w for w in range(7))
FILL_POINTS = tuple(range(3 * NP)) + ('m0', 'mid') + WO_POINTS + ('end',)


def spread(n, fixed):
    counts = dict(fixed)
    n -= sum(fixed.values())
    for k in range(6 * NP):
        counts[(k >= 3 * NP, k % (3 * NP))] = (k + 1) * n // (6 * NP) - k * n // (6 * NP)
    return counts


def _attn_mask():
    def meta(i):
        head = jnp.where(i < 2 * SEG, i // SEG, (i - 2 * SEG) // EARLY)
        j = i % SEG
        pos = jnp.where(i < 2 * SEG, jnp.where(j < MEM, j, j + EARLY), MEM + (i - 2 * SEG) % EARLY)
        return head, pos
    r = lax.broadcasted_iota(jnp.int32, (L2, L2), 0)
    c = lax.broadcasted_iota(jnp.int32, (L2, L2), 1)
    rh, rp = meta(r)
    chd, cp = meta(c)
    same = rh == chd
    keep = same & ((rp < MEM) | (rp >= cp))
    fill = jnp.where(same, MASK_FILL / SCALE, -jnp.inf).astype(F32)
    return keep, fill


def _kernel(x_hbm, m0_hbm, wq_hbm, wk_hbm, wv_hbm, wo_hbm, w1_hbm, w3_hbm, w2_hbm, c_hbm, wm_hbm,
            out_hbm,
            wqkv, wo, w1r, w1s, w3r, w3s, w2r, w2s, wm, xb, xe, cb, m0, mod, nrm, p32, p7, part, pre,
            l32, ob, oda, abuf, x1n, x1c, h2, act, ost, keep_s, fill_s, sem, wsem, osem):
    w_hbm = [r.bitcast(U32) for r in (wq_hbm, wk_hbm, wv_hbm)]
    wm_u = wm_hbm.bitcast(U32)

    def pair_copies(m, j, dsem, r0=0, r1=D // 2):
        return [pltpu.make_async_copy(w_hbm[m].at[r0:r1, par * NP + j, :],
                                      wqkv.at[m * H + 2 * j + par, r0:r1, :], dsem) for par in range(2)]

    def chunk_copies(t):
        m, c0 = divmod(t, H // CH)
        return [cp for jj in range(CH // 2)
                for cp in pair_copies(m, c0 * (CH // 2) + jj, wsem.at[t])]

    def wait_chunk(t):
        blk = wqkv.at[pl.ds(t * CH, CH)]
        pltpu.make_async_copy(blk, blk, wsem.at[t]).wait()

    def unzip(slot, r0=0, r1=D // 2):
        for r in range(r0, r1, 32):
            e, o = wqkv[slot, r:r + 32, :], wqkv[slot + 1, r:r + 32, :]
            wqkv[slot, r:r + 32, :] = (e & 0xFFFF) | (o << 16)
            wqkv[slot + 1, r:r + 32, :] = (e >> 16) | (o & jnp.uint32(0xFFFF0000))

    def start_all(cps):
        for cp in cps:
            cp.start()

    def wait_all(cps):
        for cp in cps:
            cp.wait()

    cp_c = pltpu.make_async_copy(c_hbm, cb, sem.at[0])
    x_u = x_hbm.bitcast(U32)
    cp_xe = pltpu.make_async_copy(x_hbm.at[:, 0:EARLY, :], xe, sem.at[1])
    cp_x0 = pltpu.make_async_copy(x_u.at[0], xb.at[0], sem.at[2])
    cp_m0 = pltpu.make_async_copy(m0_hbm, m0, sem.at[3])
    cp_xr = pltpu.make_async_copy(x_u.at[1:XS], xb.at[1:XS], sem.at[4])
    cp_wo = pltpu.make_async_copy(wo_hbm.bitcast(U32), wo, sem.at[5])

    def block_copies(src, w, dsem, part=0, nparts=1):
        r, c = w[1].shape[1:]
        nr = r // nparts
        src_u = src.bitcast(U32)

        def rows(start, size):
            return pl.ds(start if isinstance(start, int) else pl.multiple_of(start, 8), size)

        cps = []
        for b in range(16):
            k, n = divmod(b, 4)
            if b in RAWB:
                cps.append(pltpu.make_async_copy(
                    src_u.at[rows(k * r // 2 + part * (nr // 2), nr // 2), n * c:(n + 1) * c],
                    w[0].at[RAWB.index(b), rows(part * (nr // 2), nr // 2)], dsem))
            else:
                cps.append(pltpu.make_async_copy(src.at[rows(k * r + part * nr, nr), n * c:(n + 1) * c],
                                                 w[1].at[LAND[b], rows(part * nr, nr)], dsem))
        return cps

    w1, w3, w2 = (w1r, w1s), (w3r, w3s), (w2r, w2s)
    cp_w1, cp_w3 = block_copies(w1_hbm, w1, sem.at[6]), block_copies(w3_hbm, w3, sem.at[7])
    cp_w2 = [block_copies(w2_hbm, w2, wsem.at[i], i, NCOMB) for i in range(NCOMB)]

    def rhs(w, t, n):
        f = FAST[t][1]
        return _bf(w[0][RAWB.index(f[0][0]), :, n:n + 128]) if len(f) == 1 else w[1][SUMB.index(f), :, n:n + 128]

    cp_wm = [pltpu.make_async_copy(wm_u.at[:, k * D:(k + 1) * D], wm.at[k], sem.at[7 + k])
             for k in range(2, 6)]
    cp_xl = pltpu.make_async_copy(x_u.at[XS:NSEG], xb.at[XS:NSEG], sem.at[13])
    cp_wa = [[pltpu.make_async_copy(wm_u.at[:, k * D + SL[q]:k * D + SL[q + 1]],
                                    wm.at[k, :, SL[q]:SL[q + 1]], sem.at[14 + (NKS + 1) * q])
              for k in range(2)] for q in range(NS)]
    cp_ks = [[[cp for j in range(4 * t, 4 * t + 4)
               for cp in pair_copies(0, j, sem.at[15 + (NKS + 1) * q + t], SL[q] // 2, SL[q + 1] // 2)]
              for t in range(NKS)] for q in range(NS)]

    start_all([cp_xe, cp_c, cp_x0, cp_m0] + cp_wa[0])
    keep, fill = _attn_mask()
    keep_s[...] = keep.astype(jnp.int32)
    fill_s[...] = fill
    abuf[...] = jnp.zeros((PR, D), F32)
    wait_all([cp_xe, cp_c, cp_x0, cp_m0])
    start_all([cp for t in range(NKS) for cp in cp_ks[0][t]])
    cf = cb[...].astype(F32)
    sc16 = jnp.broadcast_to(cf * jax.nn.sigmoid(cf), (16, D)).astype(BF16)
    for g in range(NSEG // 8):
        nrm[64 * g:64 * g + 64, :] = _norm(xe[8 * g:8 * g + 8].astype(F32).reshape(8 * EARLY, D))

    def mod_unit(k, c0, c1):
        mod[k, :, c0:c1] = _dot(sc16, _bf(wm[k, :, c0:c1]))[0:8]

    def ln1_mod(n, c0=0, c1=D):
        return _affine(n, 1.0 + mod[1, :, c0:c1], mod[0, :, c0:c1])

    def next_lhs(mem_f32, s):
        hx = ln1_mod(_norm(_bf(xb[s]).astype(F32)[EARLY:SEG]))
        l32[...] = _pk(jnp.concatenate([mem_f32, hx], axis=0))

    def early_dot(head, c, c0=0, c1=D):
        rows = slice(64 * c, 64 * c + 64) if isinstance(c, int) else pl.ds(pl.multiple_of(64 * c, 64), 64)
        return _dot(_bf(p32[rows, c0:c1]), _bf(wqkv[head, c0 // 2:c1 // 2, :]))

    def early_store(slot, c, ab):
        pre[slot // 2, pl.ds(16 * c, 16)] = _pk(
            jnp.concatenate([v.reshape(16, EARLY, DH) for v in ab], axis=1))

    def early_pair(slot, c0=0, c1=D, blocks=range(NEARLY // 128), between=()):
        between = list(between)
        for c in blocks:
            ab = []
            for hh in range(2):
                ab.append(early_dot(slot + hh, c, c0, c1))
                if between and (hh == 1 or c1 - c0 == D):
                    between.pop(0)()
            rows = slice(128 * c, 128 * c + 128) if c1 - c0 < D else None
            if c0 > 0:
                ab = [ab[hh] + part[slot + hh, rows, :] for hh in range(2)]
            if c1 < D:
                for hh in range(2):
                    part[slot + hh, rows, :] = ab[hh]
            else:
                early_store(slot, c, ab)

    def early_run(slot0, npairs, halves=(0, 1)):
        unzip(slot0)
        for slot in range(0, 2 * npairs, 2):
            if slot + 2 < 2 * npairs:
                unzip(slot0 + slot + 2)
            for u in halves:
                m = {}
                for t in (1, 4, 0, 2, 3, 5, 6):
                    q = [_bf(wqkv[slot0 + slot + ab % 2, (ab // 2) * (D // 4):(ab // 2 + 1) * (D // 4), :])
                         for ab in TERMS7[t][1:]]
                    if len(q) == 2:
                        a_, b_ = q[0].astype(F32), q[1].astype(F32)
                        q = [(a_ + b_ if TERMS7[t][0] > 0 else a_ - b_).astype(BF16)]
                    m[t] = _dot(p7[u, t], q[0])
                c = _out4(m)
                for a in range(2):
                    early_store(slot0 + slot, 2 * u + a, c[2 * a:2 * a + 2])

    def ln1_early7(n):
        for u in range(2):
            for r in range(0, 128, 32):
                quads = [ln1_mod(nrm[128 * (2 * u + a) + r:128 * (2 * u + a) + r + 32, c:c + 256], c, c + 256)
                         for a in range(2) for c in (n, D // 2 + n)]
                for t, v in enumerate(_lhs7(*quads)):
                    p7[u, t, r:r + 32, n:n + 256] = v.astype(BF16)

    def ln1_early(q):
        for n in range(SL[q], SL[q + 1], 128):
            for g in range(NEARLY // 128):
                p32[64 * g:64 * g + 64, n:n + 128] = _pk(
                    ln1_mod(nrm[128 * g:128 * g + 128, n:n + 128], n, n + 128))

    def ks(q, *ts):
        return [cp for t in ts for cp in cp_ks[q][t]]

    def ch(*ts):
        return [cp for t in ts for cp in chunk_copies(t)]

    jobs = [(q, 2 * g) for q in range(NS) for g in range(NKS * CH // 2)]
    sync = {3: (ks(0, 1), [], None),
            7: (ks(0, 2), cp_wa[2] + ks(2, 0), None),
            11: (cp_wa[1] + ks(1, 0), ks(2, 1, 2), 1),
            15: (ks(1, 1, 2), cp_wa[3] + ks(3, 0, 1, 2), None),
            22: (cp_wa[2] + ks(2, 0), ch(3, 4), 2),
            27: (ks(2, 1, 2), [], None),
            34: (cp_wa[3] + ks(3, 0, 1, 2), ch(5, 6, 7, 8), 3)}
    wait_all(cp_wa[0])
    for k in range(2):
        mod_unit(k, 0, SL[1])
    ln1_early(0)
    start_all(cp_wa[1] + ks(1, 0, 1, 2))
    wait_all(ks(0, 0))
    unzip(0, 0, SL[1] // 2)
    for i, (q, slot) in enumerate(jobs):
        waits, issue, done = sync.get(i, ([], [], None))
        start_all(issue)
        wait_all(waits)
        if i + 1 < len(jobs):
            qn, slotn = jobs[i + 1]
            unzip(slotn, SL[qn] // 2, SL[qn + 1] // 2)
        if done is None:
            early_pair(slot, SL[q], SL[q + 1])
        else:
            early_pair(slot, SL[q], SL[q + 1], between=[
                functools.partial(mod_unit, k, n, n + 128)
                for n in range(SL[done], SL[done + 1], 128) for k in range(2)])
            ln1_early(done)
            if done >= 2:
                ln1_early7(SL[done] - D // 2)
    next_lhs(m0[...].astype(F32), 0)

    def prologue(r, carry):
        wait_chunk(2 * r + 1)
        wait_chunk(2 * r + 2)

        @pl.when(r == 1)
        def _():
            start_all(ch(*range(9, NCH)))

        @pl.when(r == 2)
        def _():
            start_all([cp_xr, cp_wo] + cp_w1 + cp_wm[0:2])

        early_run((2 * r + 1) * CH, CH)
        return carry

    lax.fori_loop(1, (NCH - NDEF - 1) // 2, prologue, 0)

    def last_chunks(t, carry):
        wait_chunk(t)

        @pl.when(t == NCH - 3)
        def _():
            start_all(cp_w3 + [cp_wm[2]] + cp_w2[0] + cp_w2[1] + [cp_wm[3], cp_xl])

        early_run(t * CH, CH // 2, halves=(0,))
        return carry

    lax.fori_loop(NCH - NDEF, NCH, last_chunks, 0)
    wait_all([cp_xr, cp_wo])

    def resid1(p, dst, attn=abuf):
        for n in range(0, D, 256):
            xf = _bf(xb[pl.ds(2 * p, 2), :, n:n + 256]).astype(F32).reshape(PR, 256)
            dst[:, n:n + 256] = xf + _affine(attn[:, n:n + 256], mod[2, :, n:n + 256])

    def advance(p):
        x1c[...] = x1n[...]
        resid1(p, x1n)

    def ln2(src, q):
        h = _affine(_norm(src[...]), 1.0 + mod[4], mod[3])
        blocks = [h[a * SEG:(a + 1) * SEG, k * (D // 4):(k + 1) * (D // 4)] for a in range(2) for k in range(4)]
        for t, v in enumerate(_fast_lhs(blocks)):
            h2[q, t] = v.astype(BF16)

    def combine(w, m, kmod, waits=lambda i: ()):
        rb = w[1].shape[1] // NCOMB

        def body(i, carry):
            wait_all(waits(i))
            for k in range(NBLK[m]):
                b = NCOMB * sum(NBLK[:m]) + NBLK[m] * i + k
                mods = [functools.partial(mod_unit, kmod(i), n, n + 128) for n in (256 * k, 256 * k + 128)
                        if kmod and k < 4]
                early_pair((NCH - NDEF) * CH + 2 * (b // 2), blocks=(2 + b % 2,), between=mods)
            for n in range(0, w[1].shape[2], 256):
                cols = slice(n, min(n + 256, w[1].shape[2]))
                for grp in CGRP:
                    for r in range(0, rb, 16):
                        r0 = pl.multiple_of(i * rb + r, 16)
                        raw = {}
                        for b in sorted({b for k in grp for b, _ in SUMB[k]}):
                            if b in RAWB:
                                raw[b] = _bf(w[0][RAWB.index(b), pl.ds(pl.multiple_of(r0 // 2, 8), 8), cols]).astype(F32)
                            else:
                                raw[b] = w[1][LAND[b], pl.ds(r0, 16), cols].astype(F32)
                        for k in grp:
                            w[1][k, pl.ds(r0, 16), cols] = _signed_sum([(raw[b], sg) for b, sg in SUMB[k]]).astype(BF16)
            return carry
        lax.fori_loop(0, NCOMB, body, 0)

    def gate_up_units(q):
        held = {}

        def unit(f0, t0, t1):
            m = held.setdefault('m', {})
            for t in range(t0, t1):
                _fast_acc(m, t, _dot(h2[q, t],
                                     jnp.concatenate([rhs(w1, t, f0), rhs(w3, t, f0)], axis=1)))
            if t1 < NF:
                return
            a = [(0.5 * c[:, :128]) * (1.0 + jnp.tanh(0.5 * c[:, :128])) * c[:, 128:] for c in _fast_out(held.pop('m'))]
            for t, v in enumerate(_fast_lhs(a)):
                act[q, t, :, f0:f0 + 128] = _pk(v)

        return [functools.partial(unit, f0, t0, t1) for f0 in range(0, F // 4, 128) for t0, t1 in zip(GSPL, GSPL[1:])]

    def down_units(p, q, x1):
        m = {}

        plain = [t for t in range(NF) if len(FAST[t][1]) == 1][-4:]
        order = {0: list(range(NF)), 128: [t for t in range(NF) if t not in plain] + plain}

        def unit(n0, t0, t1):
            for t in order[n0][t0:t1]:
                _fast_acc(m, t, _dot(_bf(act[q, t]), rhs(w2, t, n0)))
            if t1 < NF:
                return
            c = _fast_out(m)
            m.clear()
            for b in range(4):
                cols = slice(b * (D // 4) + n0, b * (D // 4) + n0 + 128)
                res = x1[:, cols] + _affine(jnp.concatenate([c[b], c[4 + b]], axis=0), mod[5, :, cols])
                ost[pl.ds(2 * p, 2), :, cols] = res.astype(BF16).reshape(2, SEG, 128)

        return [functools.partial(unit, n0, t, t + 2) for n0 in range(0, D // 4, 128) for t in range(0, NF, 2)]

    def out_copy(p, npairs):
        rows = pl.ds(2 * p, 2 * npairs)
        return pltpu.make_async_copy(ost.at[rows], out_hbm.at[rows], osem)

    c_exp = SCALE * math.log2(math.e)
    nb = 256

    def step(s, second, fill, eager_wo):
        rows = SEG + 2 * EARLY if second else SEG
        lhs = _bf(l32[...])
        qkv, prob = {}, {}

        def project(j):
            out = []
            for m in range(3):
                a = _dot(lhs, _bf(wqkv[m * H + 2 * j])).astype(BF16)
                b = _dot(lhs, _bf(wqkv[m * H + 2 * j + 1])).astype(BF16)
                out.append(jnp.concatenate([a, b, _bf(pre[m * NP + j, s])], axis=0))
                fill(3 * j + m)
            qkv[j] = out

        def scores(j):
            q, k, _ = qkv[j]
            sc_ = lax.dot_general(q, k, (((1,), (1,)), ((), ())), preferred_element_type=F32)
            sc_ = jnp.where(keep_s[...] != 0, sc_, fill_s[...])
            e = jnp.exp2((sc_ - jnp.max(sc_, axis=1, keepdims=True)) * c_exp)
            den = jnp.sum(e, axis=1, keepdims=True)
            r = pl.reciprocal(den, approx=True)
            r = r * (2.0 - den * r)
            prob[j] = (e * r).astype(BF16)

        def values(j):
            o = _dot(prob.pop(j), qkv.pop(j)[2])
            for hh in range(2):
                c0 = (2 * j + hh) * DH
                main = o[hh * SEG:(hh + 1) * SEG]
                early = o[2 * SEG + hh * EARLY:2 * SEG + (hh + 1) * EARLY]
                if second:
                    ob[:, c0:c0 + DH] = _pk(jnp.concatenate([main, oda[:, c0:c0 + DH], early], axis=0))
                else:
                    ob[0:SEG // 2, c0:c0 + DH] = _pk(main)
                    oda[:, c0:c0 + DH] = early

        def wo_part(n, j0, j1):
            k0, k1 = j0 * 2 * DH, j1 * 2 * DH
            return _dot(_bf(ob[0:rows // 2, k0:k1]), _bf(wo[k0 // 2:k1 // 2, n * nb:(n + 1) * nb]))

        ys = [None] * (D // nb)

        def wo_acc(n, j0, j1):
            v = wo_part(n, j0, j1)
            ys[n] = v if ys[n] is None else ys[n] + v

        for j in range(NP):
            project(j)
            if j >= 1:
                scores(j - 1)
            if j >= 3:
                values(j - 3)
            if eager_wo and j in (5, 7, 9, 11, 13):
                for n in range(D // nb):
                    wo_acc(n, j - 5, j - 3)
        d0 = 10 if eager_wo else 0
        if d0 == 0:
            wo_acc(0, 0, 6)
        fill('m0')
        scores(NP - 1)
        values(NP - 3)
        wo_acc(0, max(6, d0), 12)
        if d0:
            wo_acc(1, d0, 12)
        values(NP - 2)
        fill('mid')
        if d0 == 0:
            wo_acc(1, 0, 8)
        values(NP - 1)
        if d0 == 0:
            wo_acc(1, 8, 12)
        fill('w0')
        if d0 == 0:
            wo_acc(2, 0, 7)
        fill('w1')
        wo_acc(2, max(7, d0), 14)
        fill('w2')
        if d0:
            wo_acc(3, d0, 14)
        wo_acc(0, 12, NP)
        fill('w3')
        wo_acc(1, 12, NP)
        wo_acc(2, 14, NP)
        fill('w4')
        if d0 == 0:
            wo_acc(3, 0, 5)
        fill('w5')
        if d0 == 0:
            wo_acc(3, 5, 10)
        fill('w6')
        wo_acc(3, 14 if d0 else 10, NP)
        y = jnp.concatenate(ys, axis=1)
        next_lhs(y[0:MEM], jnp.minimum(s + 1, NSEG - 1))
        fill('end')
        return y

    def pair(i, units, counts, first=False):
        units = list(units)

        def filler(second):
            def fill(point):
                for _ in range(counts.get((second, point), 0)):
                    units.pop(0)()
            return fill

        if first:
            x1n[...] = abuf[...]
        else:
            advance(i - 1)
        ya = step(2 * i, False, filler(False), False)
        abuf[EARLY:SEG, :] = ya[MEM:SEG]
        yb = step(2 * i + 1, True, filler(True), not first)
        abuf[0:EARLY, :] = yb[SEG:SEG + EARLY]
        abuf[SEG:SEG + EARLY, :] = yb[SEG + EARLY:SEG + 2 * EARLY]
        abuf[SEG + EARLY:PR, :] = yb[MEM:SEG]
        assert not units

    def head_pairs(i, carry):
        pair(i, [], {}, first=True)
        return carry

    lax.fori_loop(0, LAG, head_pairs, 0)
    assert NCOMB * sum(NBLK) == NDEF * CH
    wait_all(cp_w1 + cp_wm[0:2])
    combine(w1, 0, lambda i: 2 + i)
    wait_all(cp_w3 + [cp_wm[2]])
    combine(w3, 1, lambda i: 4)
    combine(w2, 2, None, lambda i: block_copies(w2_hbm, w2, wsem.at[i], i, NCOMB))
    cp_wm[3].wait()
    mod_unit(5, 0, D)
    resid1(0, x1n, x1n)
    ln2(x1n, 0)

    counts = spread(NGU + NF,
                    {(False, 'mid'): 2, (False, 'end'): 3,
                     (True, 'm0'): 2, (True, 'mid'): 3, (True, 'w0'): 2, (True, 'end'): 6})

    def main_pairs(p, carry):
        @pl.when(p == 1)
        def _():
            cp_xl.wait()

        @pl.when(p >= 1)
        def _():
            out_copy(p - 1, 1).start()

        units = gate_up_units(0) + down_units(p, 0, x1c)
        last = units[NGU + 1]
        units[NGU + 1] = lambda: (last(), ln2(x1n, 0))
        pair(p + LAG, units, counts)
        return carry

    lax.fori_loop(0, NPAIR - LAG, main_pairs, 0)

    p0 = NPAIR - LAG
    out_copy(p0 - 1, 1).start()
    resid1(p0 + 1, x1c)
    ln2(x1c, 1)
    units = gate_up_units(0) + gate_up_units(1)
    for q in range(LAG):
        units += down_units(p0 + q, q, (x1n, x1c)[q]) + [out_copy(p0 + q, 1).start]
    for unit in units:
        unit()
    out_copy(0, NPAIR).wait()


@jax.jit
def pallas_adaLN_cond__memory_aug_recurrent_mem_tr__glu_gated_swiglu__prompt_kernel(
    A_x, A_mem0, A_Wq, A_Wk, A_Wv, A_Wo, A_seg_len, B_x, B_w1, B_w3, B_w2, c, w_mod,
):
    assert A_x.shape == (1, S, D) and A_mem0.shape == (1, MEM, D)
    del A_seg_len
    del B_x
    vm = pltpu.VMEM
    scratch = [
        vm((3 * H, D // 2, DH), U32),
        vm((HD // 2, D), U32),
        vm((len(RAWB), D // 8, F // 4), U32),
        vm((len(SUMB), D // 4, F // 4), BF16),
        vm((len(RAWB), D // 8, F // 4), U32),
        vm((len(SUMB), D // 4, F // 4), BF16),
        vm((len(RAWB), F // 8, D // 4), U32),
        vm((len(SUMB), F // 4, D // 4), BF16),
        vm((6, D // 2, D), U32),
        vm((NSEG, SEG // 2, D), U32),
        vm((NSEG, EARLY, D), BF16),
        vm((1, D), BF16),
        vm((MEM, D), BF16),
        vm((6, 8, D), F32),
        vm((NEARLY, D), F32),
        vm((NEARLY // 2, D), U32),
        vm((2, 7, 128, D // 2), BF16),
        vm((NKS * CH, NEARLY, DH), F32),
        vm((3 * NP, NSEG, EARLY, DH), U32),
        vm((SEG // 2, D), U32),
        vm((SEG // 2 + EARLY, HD), U32),
        vm((EARLY, HD), F32),
        vm((PR, D), F32),
        vm((PR, D), F32),
        vm((PR, D), F32),
        vm((LAG, NF, SEG, D // 4), BF16),
        vm((LAG, NF, SEG // 2, F // 4), U32),
        vm((NSEG, SEG, D), BF16),
        vm((L2, L2), jnp.int32),
        vm((L2, L2), F32),
        pltpu.SemaphoreType.DMA((14 + (NKS + 1) * NS,)),
        pltpu.SemaphoreType.DMA((NCH,)),
        pltpu.SemaphoreType.DMA(()),
    ]
    out = pl.pallas_call(
        _kernel,
        out_shape=jax.ShapeDtypeStruct((NSEG, SEG, D), BF16),
        in_specs=[pl.BlockSpec(memory_space=pl.ANY)] * 11,
        out_specs=pl.BlockSpec(memory_space=pl.ANY),
        scratch_shapes=scratch,
        compiler_params=pltpu.CompilerParams(vmem_limit_bytes=124 * 1024 * 1024,
                                             disable_bounds_checks=True,
                                             disable_semaphore_checks=True),
    )(
        A_x.reshape(NSEG, SEG, D),
        A_mem0.reshape(MEM, D),
        A_Wq.reshape(D // 2, 2 * H, DH),
        A_Wk.reshape(D // 2, 2 * H, DH),
        A_Wv.reshape(D // 2, 2 * H, DH),
        A_Wo.reshape(HD, D),
        B_w1, B_w3, B_w2, c, w_mod,
    )
    return out.reshape(1, S, D)
```
